```python
import jax
import jax.numpy as jnp

def _softmax(x, axis=-1):
    return jax.nn.softmax(x, axis=axis)

def _gelu(x):
    return jax.nn.gelu(x, approximate=True)

def _silu(x):
    return jax.nn.silu(x)

def _sigmoid(x):
    return jax.nn.sigmoid(x)

def _layernorm(x, axis=-1, eps=1e-05):
    m = jnp.mean(x, axis=axis, keepdims=True)
    v = jnp.var(x, axis=axis, keepdims=True)
    return (x - m) / jnp.sqrt(v + eps)

def _scatter_add(tgt, idx, src, axis=0):
    return tgt.at[idx].add(src)

def _segment_sum(src, seg, n):
    return jax.ops.segment_sum(src, seg, n)

class _Rng:

    def __init__(self, key):
        self._k = key

    def _next(self):
        self._k, sub = jax.random.split(self._k)
        return sub

    def normal(self, shape):
        return jax.random.normal(self._next(), shape, dtype=jnp.bfloat16)

    def randint(self, lo, hi, shape):
        return jax.random.randint(self._next(), shape, lo, hi, dtype=jnp.int32)

    def uniform(self, shape, lo=0.0, hi=1.0):
        return jax.random.uniform(self._next(), shape, jnp.bfloat16, lo, hi)

    def permutation(self, n):
        return jax.random.permutation(self._next(), n)
kernel_name = 'adaLN_cond__ssm_conv_h3__mixer_s_mlp__prompt'

def setup_inputs():
    _rng = _Rng(jax.random.key(int.from_bytes(__import__("os").urandom(4), "little")))
    _w = lambda a: (lambda t: t.astype(jnp.bfloat16) if jnp.issubdtype(t.dtype, jnp.floating) else t)(jnp.asarray(a))

    def _A_setup():
        B, S, D = (1, 2048, 640)
        ks = 4
        return {'q': _w((lambda *s: _rng.normal(s) * 0.05)(B, S, D)), 'k': _w((lambda *s: _rng.normal(s) * 0.05)(B, S, D)), 'v': _w((lambda *s: _rng.normal(s) * 0.05)(B, S, D)), 'shift_k': _w((lambda *s: _rng.normal(s) * 0.05)(D, ks) * 0.5), 'ssm_k': _w((lambda *s: _rng.normal(s) * 0.05)(D, S) * (1.0 / S ** 0.5)), 'ssm_D': _w((lambda *s: _rng.normal(s) * 0.05)(D))}
    _A_in = _A_setup()

    def _B_setup():
        B, S, D, F = (1, 2048, 640, 1728)
        return {'x': _w((lambda *s: _rng.normal(s) * 0.05)(B, S, D)), 'w1': _w((lambda *s: _rng.normal(s) * 0.05)(D, D) * D ** (-0.5)), 'w2': _w((lambda *s: _rng.normal(s) * 0.05)(D, D) * D ** (-0.5)), 'w3': _w((lambda *s: _rng.normal(s) * 0.05)(D, F) * D ** (-0.5)), 'w4': _w((lambda *s: _rng.normal(s) * 0.05)(F, D) * F ** (-0.5))}
    _B_in = _B_setup()
    return {'A_q': _A_in['q'], 'A_k': _A_in['k'], 'A_v': _A_in['v'], 'A_shift_k': _A_in['shift_k'], 'A_ssm_k': _A_in['ssm_k'], 'A_ssm_D': _A_in['ssm_D'], 'B_x': _B_in['x'], 'B_w1': _B_in['w1'], 'B_w2': _B_in['w2'], 'B_w3': _B_in['w3'], 'B_w4': _B_in['w4'], 'c': _w((lambda *s: _rng.normal(s) * 0.05)(1, 640)), 'w_mod': _w((lambda *s: _rng.normal(s) * 0.05)(640, 6 * 640) * 640 ** (-0.5))}

def reference(A_q, A_k, A_v, A_shift_k, A_ssm_k, A_ssm_D, B_x, B_w1, B_w2, B_w3, B_w4, c, w_mod):

    def _A_ref(q, k, v, shift_k, ssm_k, ssm_D):
        B, S, D = q.shape
        ks = shift_k.shape[-1]
        k_pad = jnp.pad(k, ((0, 0), (ks - 1, 0), (0, 0)))
        k_shift = jnp.zeros_like(k)
        for t in range(ks):
            k_shift = k_shift + k_pad[:, t:t + S, :] * shift_k[:, ks - 1 - t][None, None, :]
        kv = k_shift * v
        L = 2 * S
        kv_pad = jnp.pad(kv, ((0, 0), (0, S), (0, 0)))
        kf_pad = jnp.pad(ssm_k, ((0, 0), (0, S)))
        kv_f = (lambda x, axes=(-2, -1): jnp.fft.rfft2(x.astype(jnp.float32), axes=axes))(kv_pad[:, None, :, :], axes=(1, 2))
        kf_f = (lambda x, axes=(-2, -1): jnp.fft.rfft2(x.astype(jnp.float32), axes=axes))(kf_pad[:, None, :], axes=(1, 2))
        kf_f = (lambda x, *d: x.transpose(*d))(kf_f, 1, 2, 0)
        y_f = kv_f * kf_f[None, :, :, :]
        y = (lambda x, s, axes=(-2, -1): jnp.fft.irfft2(x, s=s, axes=axes).astype(jnp.bfloat16))(y_f, (1, L), axes=(1, 2))[:, 0, :S, :]
        y = y + kv * ssm_D[None, None, :]
        return q * y

    def _B_ref(x, w1, w2, w3, w4):
        B, S, D = x.shape
        h = _gelu(_layernorm(x, axis=-1) @ w1)
        c = D // 4
        g0 = jnp.pad(h[:, :, 0 * c:1 * c], ((0, 0), (1, 0), (0, 0)))[:, :S, :]
        g1 = jnp.pad(h[:, :, 1 * c:2 * c], ((0, 0), (0, 1), (0, 0)))[:, 1:, :]
        g2 = jnp.pad(h[:, :, 2 * c:3 * c], ((0, 0), (2, 0), (0, 0)))[:, :S, :]
        g3 = jnp.pad(h[:, :, 3 * c:], ((0, 0), (0, 2), (0, 0)))[:, 2:, :]
        hs = jnp.concatenate([g0, g1, g2, g3], axis=-1) @ w2
        x1 = x + hs
        h2 = _gelu(_layernorm(x1, axis=-1) @ w3) @ w4
        return x1 + h2
    x = A_q
    mod = (_silu(c) @ w_mod).reshape(c.shape[0], 6, 1, -1)
    sa, ca, ga, sb, cb, gb = (mod[:, 0].copy(), mod[:, 1].copy(), mod[:, 2].copy(), mod[:, 3].copy(), mod[:, 4].copy(), mod[:, 5].copy())
    h = _layernorm(x, axis=-1) * (1 + ca) + sa
    x = x + ga * _A_ref(h, A_k, A_v, A_shift_k, A_ssm_k, A_ssm_D)
    h = _layernorm(x, axis=-1) * (1 + cb) + sb
    x = x + gb * _B_ref(h, B_w1, B_w2, B_w3, B_w4)
    return x
```

```python
import functools

import numpy as np
import jax
import jax.numpy as jnp
import jax.experimental.pallas as pl
import jax.experimental.pallas.tpu as pltpu

F32 = jnp.float32
BF16 = jnp.bfloat16
U32 = jnp.uint32

S = 2048
D = 640
FF = 1728
NC = D // 128
R = 4
P = 128 * R
NA = S // P
TS = 256
NT = S // TS
LEAD = 16
EPS = 1e-5


def _dft_tables():
    t = np.arange(16)[:, None]
    s = np.arange(8)[None, :]
    f = np.where(t < 8, 2 * (8 * t + s), 2 * (8 * (t - 8) + s) + 1)
    m = np.arange(128)
    fwd = np.zeros((R, 16, 2, 8, 128), np.float64)
    for p in range(R):
        j = ((2 * f[:, :, None] + 1) * (R * m + p)[None, None, :]) % (4 * P)
        th = 2.0 * np.pi * j / (4 * P)
        fwd[p, :, 0] = np.cos(th)
        fwd[p, :, 1] = -np.sin(th)
    fwd = fwd.reshape(R, 256, 128)
    inv = fwd.transpose(0, 2, 1) / P
    perm = np.zeros((128, 128), np.float64)
    jj = np.arange(128)
    perm[(128 // R) * (jj % R) + jj // R, jj] = 1.0
    return fwd.astype(np.float32), inv.astype(np.float32), perm.astype(np.float32)


def _dot(a, b):
    return jnp.dot(a, b, preferred_element_type=F32)


def _dot_nt(a, b):
    return jax.lax.dot_general(a, b, (((1,), (1,)), ((), ())), preferred_element_type=F32)


def _lo(w):
    return pltpu.bitcast(w << 16, F32)


def _hi(w):
    return pltpu.bitcast(w & jnp.uint32(0xFFFF0000), F32)


def _ln(x):
    m = jnp.sum(x, axis=-1, keepdims=True) * (1.0 / D)
    xc = x - m
    v = jnp.sum(xc * xc, axis=-1, keepdims=True) * (1.0 / D)
    return xc * jax.lax.rsqrt(v + EPS)


def _gelu(x):
    c0 = 0.7978845608028654
    c1 = c0 * 0.044715
    z = x * (c0 + c1 * (x * x))
    hx = 0.5 * x
    return hx + hx * jnp.tanh(z)


def _bfly(tr, ti, sign):
    s02r, s02i = tr[0] + tr[2], ti[0] + ti[2]
    d02r, d02i = tr[0] - tr[2], ti[0] - ti[2]
    s13r, s13i = tr[1] + tr[3], ti[1] + ti[3]
    d13r, d13i = tr[1] - tr[3], ti[1] - ti[3]
    x0r, x0i = s02r + s13r, s02i + s13i
    x2r, x2i = s02r - s13r, s02i - s13i
    ar, ai = d02r + d13i, d02i - d13r
    br, bi = d02r - d13i, d02i + d13r
    if sign < 0:
        return [x0r, ar, x2r, br], [x0i, ai, x2i, bi]
    return [x0r, br, x2r, ar], [x0i, bi, x2i, ai]


def _kernel(q_hbm, k_hbm, v_hbm, shift_hbm, ssmk_hbm, ssmd_hbm, w1_hbm, w2_hbm, w3t_hbm, w4_hbm,
            c_hbm, wmod_hbm, fwd_hbm, inv_hbm, perm_hbm,
            out_hbm,
            kbuf, vbuf, skbuf, shiftbuf, dbuf, cbuf, fwdbuf, invbuf, permbuf,
            wmodbuf, w1buf, w2buf, w3buf, w4buf, qbuf,
            xu, xk, wbuf, ybuf, modbuf, x2buf, hbuf, hhbuf, xnbuf, obuf,
            sem_in, sem_out):
    cps = {}
    n_sem = [0]

    def start(name, src, dst):
        cp = pltpu.make_async_copy(src, dst, sem_in.at[n_sem[0]])
        n_sem[0] += 1
        cp.start()
        cps[name] = cp

    start("shift", shift_hbm, shiftbuf)
    start("d", ssmd_hbm, dbuf)
    start("c", c_hbm, cbuf)
    start("fwd", fwd_hbm, fwdbuf)
    start("perm", perm_hbm, permbuf)
    for c in range(NC):
        cs = pl.ds(c * 128, 128)
        start(f"k{c}", k_hbm.at[:, cs], kbuf.at[c, pl.ds(16, S), :])
        start(f"v{c}", v_hbm.at[:, cs], vbuf.at[c])
        start(f"s{c}", ssmk_hbm.at[cs, :], skbuf.at[cs, :])
        if c == 0:
            start("inv", inv_hbm, invbuf)
    start("wmod", wmod_hbm.at[:, pl.ds(0, 5 * D)], wmodbuf.at[:, pl.ds(0, 5 * D)])
    start("w1", w1_hbm, w1buf)
    start("q0", q_hbm.at[pl.ds(0, 2 * TS + LEAD), :], qbuf.at[pl.ds(0, 2 * TS + LEAD), :])
    start("w2", w2_hbm, w2buf)
    start("w3", w3t_hbm, w3buf)
    start("w4", w4_hbm, w4buf)
    start("wmodg", wmod_hbm.at[:, pl.ds(5 * D, D)], wmodbuf.at[:, pl.ds(5 * D, D)])
    rest = S - 2 * TS - LEAD
    start("q1", q_hbm.at[pl.ds(2 * TS + LEAD, rest), :], qbuf.at[pl.ds(2 * TS + LEAD, rest), :])

    kw = kbuf.bitcast(U32)
    vw = vbuf.bitcast(U32)
    for c in range(NC):
        kw[c, pl.ds(0, 8), :] = jnp.zeros((8, 128), U32)
        ybuf[c, pl.ds(S, LEAD), :] = jnp.zeros((LEAD, 128), F32)
        hhbuf[c, pl.ds(0, 8), :] = jnp.zeros((8, 128), F32)
    qbuf[pl.ds(S, LEAD), :] = jnp.zeros((LEAD, D), BF16)

    for name in ("shift", "d", "c", "fwd", "perm"):
        cps[name].wait()

    def split_ri(t):
        t = t.reshape(16, 2, 8, 128)
        return t[:, 0], t[:, 1]

    def fwd_store(dst, a, rhs):
        tr, ti = [], []
        for p in range(R):
            r_, i_ = split_ri(_dot(fwdbuf[p], rhs[p]))
            tr.append(r_)
            ti.append(i_)
        xr, xi = _bfly(tr, ti, -1)
        for q in range(R):
            dst[a, q, 0] = xr[q]
            dst[a, q, 1] = xi[q]

    def fwd(c):
        slot = c % 2
        coef = shiftbuf[:, pl.ds(c * 128, 128)].astype(F32)
        cj = [jnp.broadcast_to(coef[j:j + 1, :], (16, 128)) for j in range(4)]
        for a in range(NA):
            pieces = [[] for _ in range(R)]
            for g in range(8):
                kb = 8 + a * (P // 2) + 32 * g
                vb = a * (P // 2) + 32 * g
                wm2 = kw[c, pl.ds(kb - 2, 16, stride=2), :]
                wm1 = kw[c, pl.ds(kb - 1, 16, stride=2), :]
                w0 = kw[c, pl.ds(kb, 16, stride=2), :]
                w1 = kw[c, pl.ds(kb + 1, 16, stride=2), :]
                seq = [_hi(wm2), _lo(wm1), _hi(wm1), _lo(w0), _hi(w0), _lo(w1), _hi(w1)]
                v0 = vw[c, pl.ds(vb, 16, stride=2), :]
                v1 = vw[c, pl.ds(vb + 1, 16, stride=2), :]
                vs = [_lo(v0), _hi(v0), _lo(v1), _hi(v1)]
                for p in range(R):
                    ks = (seq[3 + p] * cj[0] + seq[2 + p] * cj[1]) + (seq[1 + p] * cj[2] + seq[p] * cj[3])
                    pieces[p].append((ks * vs[p]).astype(BF16))
            fwd_store(xu.at[slot], a, [jnp.concatenate(pc, axis=0) for pc in pieces])
            trs = []
            for b in range(R):
                tile = skbuf[pl.ds(c * 128, 128), pl.ds(a * P + b * 128, 128)]
                trs.append(_dot_nt(permbuf[...], tile).astype(BF16))
            g_ = 128 // R
            rhs = [jnp.concatenate([trs[b][p * g_:(p + 1) * g_] for b in range(R)], axis=0) for p in range(R)]
            fwd_store(xk.at[slot], a, rhs)

    def conv(c):
        slot = c % 2
        dvec = jnp.broadcast_to(dbuf[c:c + 1, :].astype(F32), (8, 128))
        for t in range(16):
            yr = [[None] * R for _ in range(NA)]
            yi = [[None] * R for _ in range(NA)]
            for q in range(R):
                ur = [xu[slot, a, q, 0, t] for a in range(NA)]
                ui = [xu[slot, a, q, 1, t] for a in range(NA)]
                kr0 = [xk[slot, a, q, 0, t] for a in range(NA)]
                ki0 = [xk[slot, a, q, 1, t] for a in range(NA)]
                kr, ki = [kr0[0] + dvec], [ki0[0]]
                for a in range(1, NA):
                    if t < 8:
                        kr.append(kr0[a] - ki0[a - 1])
                        ki.append(ki0[a] + kr0[a - 1])
                    else:
                        kr.append(kr0[a] + ki0[a - 1])
                        ki.append(ki0[a] - kr0[a - 1])
                for a in range(NA):
                    accr = acci = None
                    for j in range(a + 1):
                        pr = ur[j] * kr[a - j] - ui[j] * ki[a - j]
                        pi = ur[j] * ki[a - j] + ui[j] * kr[a - j]
                        accr = pr if accr is None else accr + pr
                        acci = pi if acci is None else acci + pi
                    yr[a][q], yi[a][q] = accr, acci
            for a in range(NA):
                wr, wi = _bfly(yr[a], yi[a], +1)
                for p in range(R):
                    wbuf[slot, a, p, pl.ds(16 * t, 16), :] = jnp.concatenate([wr[p], wi[p]], axis=0).astype(BF16)

    def inv(c):
        slot = c % 2
        for a in range(NA):
            for p in range(R):
                ybuf[c, pl.ds(a * P + p, 128, stride=R), :] = _dot(invbuf[p], wbuf[slot, a, p])

    def wait_block(c):
        for n in ("k", "v", "s"):
            cps[f"{n}{c}"].wait()

    with jax.named_scope("p1"):
        wait_block(0)
        fwd(0)
        cps["inv"].wait()
        for c in range(NC):
            if c + 1 < NC:
                wait_block(c + 1)
                fwd(c + 1)
            conv(c)
            inv(c)

    def mod_cols(lo, n):
        cv = cbuf[...].astype(F32)
        sc = (cv * jax.nn.sigmoid(cv)).astype(BF16)
        m = _dot(jnp.broadcast_to(sc, (8, D)), wmodbuf[:, pl.ds(lo * D, n * D)])
        for j in range(n):
            col = m[:, j * D:(j + 1) * D]
            if lo + j in (1, 4):
                col = col + 1.0
            modbuf[lo + j] = col

    with jax.named_scope("mod"):
        cps["wmod"].wait()
        mod_cols(0, 5)

    def modrow(j):
        return modbuf[j, 0:1, :]

    def slabs(ref, r0, n):
        return jnp.concatenate([ref[c, pl.ds(r0, n), :] for c in range(NC)], axis=1)

    lane = jax.lax.broadcasted_iota(jnp.int32, (TS, 128), 1)

    def stage_a(r0, n, last_valid=None):
        rows = pl.ds(r0, n)
        x = qbuf[rows, :].astype(F32)
        y = slabs(ybuf, r0, n)
        h1 = _ln(x) * modrow(1) + modrow(0)
        x2 = x + modrow(2) * (h1 * y)
        h = _ln(x2) * modrow(4) + modrow(3)
        hh = _gelu(_dot(_ln(h).astype(BF16), w1buf[...]))
        x2buf[rows, :] = x2
        hbuf[rows, :] = h
        for c in range(NC):
            blk = hh[:, c * 128:(c + 1) * 128]
            hhbuf[c, pl.ds(r0 + 8, n - LEAD), :] = blk[:n - LEAD]
            tail = blk[n - LEAD:]
            if last_valid is not None:
                tail = jnp.where(last_valid, tail, 0.0)
            hhbuf[c, pl.ds(r0 + 8 + n - LEAD, LEAD), :] = tail

    def stage_b1(r0):
        rows = pl.ds(r0, TS)

        def sh(c, d):
            return hhbuf[c, pl.ds(r0 + 8 + d, TS), :]

        g = [sh(0, -1),
             jnp.where(lane < 32, sh(1, -1), sh(1, 1)),
             jnp.where(lane < 64, sh(2, 1), sh(2, -2)),
             jnp.where(lane < 96, sh(3, -2), sh(3, 2)),
             sh(4, 2)]
        hs = _dot(jnp.concatenate(g, axis=1).astype(BF16), w2buf[...])
        x1 = hbuf[rows, :] + hs
        hbuf[rows, :] = x1
        xnbuf[rows, :] = _ln(x1).astype(BF16)

    def out_copy(r0):
        rows = pl.ds(r0, TS)
        return pltpu.make_async_copy(obuf.at[rows, :], out_hbm.at[rows, :], sem_out.at[0])

    def stage_b2(r0):
        rows = pl.ds(r0, TS)
        h3 = _gelu(_dot_nt(xnbuf[rows, :], w3buf[...])).astype(BF16)
        h2 = _dot(h3, w4buf[...])
        obuf[rows, :] = (x2buf[rows, :] + modrow(5) * (hbuf[rows, :] + h2)).astype(BF16)

    with jax.named_scope("p2pro"):
        cps["w1"].wait()
        cps["q0"].wait()
        stage_a(0, TS + LEAD)
        cps["w2"].wait()
        stage_b1(0)
        cps["w3"].wait()
        cps["w4"].wait()
        cps["wmodg"].wait()
        mod_cols(5, 1)
        cps["q1"].wait()

    def step(s, carry):
        r0 = pl.multiple_of(s * TS, TS)
        stage_b2(r0)
        stage_a(r0 + TS + LEAD, TS, last_valid=s < NT - 2)
        stage_b1(r0 + TS)
        out_copy(r0).start()
        return carry

    with jax.named_scope("p2main"):
        jax.lax.fori_loop(0, NT - 1, step, 0)
    with jax.named_scope("p2epi"):
        stage_b2((NT - 1) * TS)
        out_copy((NT - 1) * TS).start()
        pltpu.make_async_copy(obuf, out_hbm, sem_out.at[0]).wait()


@jax.jit
def pallas_adaLN_cond__ssm_conv_h3__mixer_s_mlp__prompt_kernel(
    A_q: jax.Array,
    A_k: jax.Array,
    A_v: jax.Array,
    A_shift_k: jax.Array,
    A_ssm_k: jax.Array,
    A_ssm_D: jax.Array,
    B_x: jax.Array,
    B_w1: jax.Array,
    B_w2: jax.Array,
    B_w3: jax.Array,
    B_w4: jax.Array,
    c: jax.Array,
    w_mod: jax.Array,
):
    del B_x
    fwd, inv, perm = _dft_tables()
    args = (
        A_q.reshape(S, D), A_k.reshape(S, D), A_v.reshape(S, D),
        A_shift_k.T, A_ssm_k, A_ssm_D.reshape(NC, 128),
        B_w1, B_w2, B_w3.T, B_w4, c, w_mod,
        jnp.asarray(fwd, BF16), jnp.asarray(inv, BF16), jnp.asarray(perm, BF16),
    )
    scratch = [
        pltpu.VMEM((NC, S + 16, 128), BF16),
        pltpu.VMEM((NC, S, 128), BF16),
        pltpu.VMEM((D, S), BF16),
        pltpu.VMEM((4, D), BF16),
        pltpu.VMEM((NC, 128), BF16),
        pltpu.VMEM((1, D), BF16),
        pltpu.VMEM((R, 256, 128), BF16),
        pltpu.VMEM((R, 128, 256), BF16),
        pltpu.VMEM((128, 128), BF16),
        pltpu.VMEM((D, 6 * D), BF16),
        pltpu.VMEM((D, D), BF16),
        pltpu.VMEM((D, D), BF16),
        pltpu.VMEM((FF, D), BF16),
        pltpu.VMEM((FF, D), BF16),
        pltpu.VMEM((S + LEAD, D), BF16),
        pltpu.VMEM((2, NA, R, 2, 16, 8, 128), F32),
        pltpu.VMEM((2, NA, R, 2, 16, 8, 128), F32),
        pltpu.VMEM((2, NA, R, 256, 128), BF16),
        pltpu.VMEM((NC, S + LEAD, 128), F32),
        pltpu.VMEM((6, 8, D), F32),
        pltpu.VMEM((S + LEAD, D), F32),
        pltpu.VMEM((S + LEAD, D), F32),
        pltpu.VMEM((NC, S + LEAD + 8, 128), F32),
        pltpu.VMEM((S, D), BF16),
        pltpu.VMEM((S, D), BF16),
        pltpu.SemaphoreType.DMA((32,)),
        pltpu.SemaphoreType.DMA((1,)),
    ]
    out = pl.pallas_call(
        _kernel,
        out_shape=jax.ShapeDtypeStruct((S, D), BF16),
        in_specs=[pl.BlockSpec(memory_space=pl.ANY)] * len(args),
        out_specs=pl.BlockSpec(memory_space=pl.ANY),
        scratch_shapes=scratch,
        compiler_params=pltpu.CompilerParams(vmem_limit_bytes=100 * 1024 * 1024),
        name="adaln_h3_mixer",
    )(*args)
    return out.reshape(1, S, D)
```

```python
import numpy as np
import jax
import jax.numpy as jnp
import jax.experimental.pallas as pl
import jax.experimental.pallas.tpu as pltpu

F32 = jnp.float32
BF16 = jnp.bfloat16
U32 = jnp.uint32

S = 2048
D = 640
FF = 1728
NC = D // 128
R = 4
P = 128 * R
NA = S // P
TS = 256
NT = S // TS
LEAD = 16
EPS = 1e-5
P1_ORDER = "t0 t1 t2 t3 k0 k1 k2 k3 u0 i0 u1 i1 u2 i2 u3 i3"


def _cos_table(row, m, p, scale):
    t, part, s = row >> 4, (row >> 3) & 1, row & 7
    odd2f1 = 32 * (t & 7) + 4 * s + 2 * (t >> 3) + 1
    j = (odd2f1 * (R * m + p) + P * part) & (4 * P - 1)
    z = jnp.abs(j - 2 * P) - P
    x = z.astype(F32) * (2.0 * np.pi / (4 * P))
    x2 = x * x
    poly = 1.0 / 362880.0 - x2 * (1.0 / 39916800.0)
    for coef in (-1.0 / 5040.0, 1.0 / 120.0, -1.0 / 6.0, 1.0):
        poly = poly * x2 + coef
    return poly * (x * scale)


def _plan_tokens(order, maxutil=1.0):
    dur = {"t": 8, "u": 16, "k": 16, "i": 16, "m": 12}
    post = {"t": 8.0, "u": 16.0, "k": 24.0, "i": 4.0, "m": 18.0}
    lag = 8
    cap = 60.0
    start, slots = {}, []
    for n in order:
        start[n] = len(slots)
        slots += [(n, r) for r in range(dur[n[0]])]
    pre = 4
    free = [cap - (post[slots[i - lag][0][0]] if i >= lag else 0.0) for i in range(-pre, len(slots))]
    cum = np.concatenate([[0.0], np.cumsum(free)])
    units = []
    for n in order:
        a = int(n[1])
        if n[0] == "u":
            units += [(("u", a, g), 94.0, start[n]) for g in range(8)]
        elif n[0] == "i":
            units += [(("i", a, t), 32.0 * a + 48.0, start[n]) for t in range(16)]
    margin = 3

    def deadlines(util):
        d, nxt = [], 1e18
        for key, cost, need in reversed(units):
            nxt = min(cum[max(need - margin + pre, 0)], nxt)
            d.append(nxt)
            nxt -= cost / util
        return d[::-1], nxt

    lo_, hi_ = 0.05, maxutil
    for _ in range(30):
        mid = 0.5 * (lo_ + hi_)
        if deadlines(mid)[1] >= 0.0:
            hi_ = mid
        else:
            lo_ = mid
    d, _ = deadlines(hi_)
    plan = {}
    for (key, cost, need), dl in zip(units, d):
        s = int(np.searchsorted(cum, dl, side="right")) - 1 - pre
        if 0 <= s < need:
            plan.setdefault(slots[s], []).append(key)
    return plan


def _pack(x):
    return pltpu.bitcast(x.astype(BF16), U32)


def _unpack(w):
    return pltpu.bitcast(w, BF16)


def _dot(a, b):
    return jnp.dot(a, b, preferred_element_type=F32)


def _dot_nt(a, b):
    return jax.lax.dot_general(a, b, (((1,), (1,)), ((), ())), preferred_element_type=F32)


def _lo(w):
    return pltpu.bitcast(w << 16, F32)


def _hi(w):
    return pltpu.bitcast(w & jnp.uint32(0xFFFF0000), F32)


def _ln_stats(x):
    m = jnp.sum(x, axis=-1, keepdims=True) * (1.0 / D)
    xc = x - m
    v = jnp.sum(xc * xc, axis=-1, keepdims=True) * (1.0 / D)
    return xc, jnp.exp(-0.5 * jnp.log(v + EPS))


def _ln(x):
    xc, r = _ln_stats(x)
    return xc * r


def _spread(tokens, lo, hi):
    out = {}
    for i, t in enumerate(tokens):
        out.setdefault(lo + (i * (hi - lo)) // len(tokens), []).append(t)
    return out


def _gelu(x):
    c0 = 0.7978845608028654
    c1 = c0 * 0.044715
    z = x * (c0 + c1 * (x * x))
    hx = 0.5 * x
    return hx + hx * jnp.tanh(z)


def _bfly(tr, ti, sign):
    s02r, s02i = tr[0] + tr[2], ti[0] + ti[2]
    d02r, d02i = tr[0] - tr[2], ti[0] - ti[2]
    s13r, s13i = tr[1] + tr[3], ti[1] + ti[3]
    d13r, d13i = tr[1] - tr[3], ti[1] - ti[3]
    x0r, x0i = s02r + s13r, s02i + s13i
    x2r, x2i = s02r - s13r, s02i - s13i
    ar, ai = d02r + d13i, d02i - d13r
    br, bi = d02r - d13i, d02i + d13r
    if sign < 0:
        return [x0r, ar, x2r, br], [x0i, ai, x2i, bi]
    return [x0r, br, x2r, ar], [x0i, bi, x2i, ai]


def _kernel(q_hbm, k_hbm, v_hbm, shift_hbm, ssmk_hbm, ssmd_hbm, w1_hbm, w2_hbm, w3t_hbm, w4_hbm,
            c_hbm, wmod_hbm,
            out_hbm,
            kbuf, vbuf, skbuf, fwdbuf, invbuf, permbuf,
            wmodbuf, w1buf, w2buf, w3buf, w4buf, qbuf,
            xu, coefbuf, ybuf, modbuf, x2buf, hbuf, hhbuf, xnbuf, obuf, shiftbuf, dbuf, cbuf,
            sem_in, sem_out):
    cps = {}
    n_sem = [0]

    def start(name, src, dst):
        cp = pltpu.make_async_copy(src, dst, sem_in.at[n_sem[0]])
        n_sem[0] += 1
        cp.start()
        cps[name] = cp

    start("shift", shift_hbm, shiftbuf)
    start("d", ssmd_hbm, dbuf)
    start("c", c_hbm, cbuf)
    blk_sem0 = n_sem[0]

    def block_copies(c):
        cs = pl.ds(pl.multiple_of(c * 128, 128), 128)
        return [pltpu.make_async_copy(k_hbm.at[:, cs], kbuf.at[c, pl.ds(16, S), :], sem_in.at[blk_sem0 + 3 * c]),
                pltpu.make_async_copy(v_hbm.at[:, cs], vbuf.at[c], sem_in.at[blk_sem0 + 3 * c + 1]),
                pltpu.make_async_copy(ssmk_hbm.at[cs, :], skbuf.at[c], sem_in.at[blk_sem0 + 3 * c + 2])]

    for c in range(NC):
        for cp in block_copies(c):
            cp.start()
    n_sem[0] += 3 * NC
    QA = TS + LEAD
    QB = 2 * TS + LEAD
    start("qa", q_hbm.at[pl.ds(0, QA), :], qbuf.at[pl.ds(0, QA), :])
    start("wmoda", wmod_hbm.at[:, pl.ds(0, 3 * D)], wmodbuf.at[:, pl.ds(0, 3 * D)])
    start("wmodb", wmod_hbm.at[:, pl.ds(3 * D, 2 * D)], wmodbuf.at[:, pl.ds(3 * D, 2 * D)])
    start("w1", w1_hbm, w1buf)
    start("qb", q_hbm.at[pl.ds(QA, QB - QA), :], qbuf.at[pl.ds(QA, QB - QA), :])
    start("w2", w2_hbm, w2buf)
    start("w3", w3t_hbm, w3buf)
    start("w4", w4_hbm, w4buf)
    start("wmodg", wmod_hbm.at[:, pl.ds(5 * D, D)], wmodbuf.at[:, pl.ds(5 * D, D)])
    start("q1", q_hbm.at[pl.ds(QB, S - QB), :], qbuf.at[pl.ds(QB, S - QB), :])

    kw = kbuf.bitcast(U32)
    vw = vbuf.bitcast(U32)
    for c in range(NC):
        kw[c, pl.ds(0, 8), :] = jnp.zeros((8, 128), U32)
        ybuf[c, pl.ds(S, LEAD), :] = jnp.zeros((LEAD, 128), F32)
        hhbuf[c, pl.ds(0, 8), :] = jnp.zeros((8, 128), F32)
    qbuf[pl.ds(S, LEAD), :] = jnp.zeros((LEAD, D), BF16)

    def tables(p, carry):
        i0 = jax.lax.broadcasted_iota(jnp.int32, (256, 128), 0)
        i1 = jax.lax.broadcasted_iota(jnp.int32, (256, 128), 1)
        fwdbuf[p] = _pack(_cos_table(i0, i1, p, 1.0))
        i0 = jax.lax.broadcasted_iota(jnp.int32, (128, 256), 0)
        i1 = jax.lax.broadcasted_iota(jnp.int32, (128, 256), 1)
        row = (i1 & ~15) + 8 * (i1 & 1) + ((i1 >> 1) & 7)
        invbuf[p] = _pack(_cos_table(row, i0, p, 1.0 / P))
        return carry

    jax.lax.fori_loop(0, R, tables, 0)
    i0 = jax.lax.broadcasted_iota(jnp.int32, (128, 128), 0)
    i1 = jax.lax.broadcasted_iota(jnp.int32, (128, 128), 1)
    permbuf[...] = _pack(jnp.where(i0 == (128 // R) * (i1 & (R - 1)) + (i1 >> 2), 1.0, 0.0).astype(F32))

    for name in ("shift", "d", "c"):
        cps[name].wait()
    coef = shiftbuf[...].astype(F32)
    dval = dbuf[...].astype(F32)
    for c in range(NC):
        for j in range(4):
            coefbuf[c, j] = jnp.broadcast_to(coef[j:j + 1, c * 128:(c + 1) * 128], (8, 128))
        coefbuf[c, 4] = jnp.broadcast_to(dval[c:c + 1, :], (8, 128))

    xk = xu
    def split_ri(t):
        t = t.reshape(16, 2, 8, 128)
        return t[:, 0], t[:, 1]

    def get_never():
        return kw[0, pl.ds(0, 8), :] != 0

    def pack2(x, y):
        return pltpu.pack_elementwise([x, y], packed_dtype=BF16)

    def unit_u(c, a, g):
        cj = [coefbuf[c, j] for j in range(4)]
        halves = []
        for e in range(2):
            kb = 8 + a * (P // 2) + 32 * g + 2 * e
            vb = a * (P // 2) + 32 * g + 2 * e
            wm2 = kw[c, pl.ds(kb - 2, 8, stride=4), :]
            wm1 = kw[c, pl.ds(kb - 1, 8, stride=4), :]
            w0 = kw[c, pl.ds(kb, 8, stride=4), :]
            w1 = kw[c, pl.ds(kb + 1, 8, stride=4), :]
            seq = [_hi(wm2), _lo(wm1), _hi(wm1), _lo(w0), _hi(w0), _lo(w1), _hi(w1)]
            v0 = vw[c, pl.ds(vb, 8, stride=4), :]
            v1 = vw[c, pl.ds(vb + 1, 8, stride=4), :]
            vs = [_lo(v0), _hi(v0), _lo(v1), _hi(v1)]
            halves.append([((seq[3 + p] * cj[0] + seq[2 + p] * cj[1]) + (seq[1 + p] * cj[2] + seq[p] * cj[3])) * vs[p]
                           for p in range(R)])
        return [pack2(halves[0][p], halves[1][p]) for p in range(R)]

    def unit_i(a, t, x_c):
        yr, yi = [], []
        for q in range(R):
            accr = acci = None
            for j in range(a + 1):
                ur, ui = x_c[j, q, t, 0], x_c[j, q, t, 1]
                kr, ki = x_c[a - j, q, t, 2], x_c[a - j, q, t, 3]
                pr = ur * kr - ui * ki
                pi = ur * ki + ui * kr
                accr = pr if accr is None else accr + pr
                acci = pi if acci is None else acci + pi
            yr.append(accr)
            yi.append(acci)
        wr, wi = _bfly(yr, yi, +1)
        return [pack2(wr[p], wi[p]) for p in range(R)]

    def p1_step(c, do_fwd, do_conv, order=None, maxutil=1.0, mod_fn=None):
        if do_fwd:
            for cp in block_copies(c + 1):
                cp.wait()
        if do_fwd and do_conv:
            xw = xu.at[pl.ds(c, 2)]
            x0, x1 = xw.at[0], xw.at[1]
        elif do_fwd:
            x1 = xu.at[c + 1]
        else:
            x0 = xu.at[c]
        if order is None:
            order = [n for n in P1_ORDER.split() if (do_conv if n[0] == "i" else do_fwd)]
        plan = _plan_tokens(order, maxutil)
        never = get_never()
        units = {}

        def unit(key):
            if key not in units:
                kind, a, j = key
                units[key] = unit_u(c + 1, a, j) if kind == "u" else unit_i(a, j, x0)
            return units[key]

        def lhs(name, p, rows):
            out = []
            for r, v in enumerate(rows):
                for key in plan.get((name, r), ()):
                    v = jnp.where(never, unit(key)[p], v)
                out.append(v)
            return out

        def dft(name, rhs):
            tr, ti = [], []
            for p in range(R):
                f = jnp.concatenate(lhs(name, p, [fwdbuf[p, pl.ds(8 * r, 8), :] for r in range(16)]), axis=0)
                r_, i_ = split_ri(_dot(_unpack(f), rhs[p]))
                tr.append(r_)
                ti.append(i_)
            return _bfly(tr, ti, -1)

        st = dict(prev=None)
        for name in order:
            kind, a = name[0], int(name[1])
            if kind == "m":
                toks = {}
                for r in range(12):
                    for n_, key in enumerate(plan.get((name, r), ())):
                        toks.setdefault(2 * r + n_ % 2, []).extend(unit(key))
                mod_fn(a, toks)
            elif kind == "t":
                trs = []
                for b in range(R):
                    pm = jnp.concatenate(lhs(name, b, [permbuf[pl.ds(8 * r, 8), :] for r in range(8)]), axis=0)
                    trs.append(_dot_nt(_unpack(pm), skbuf[c + 1, :, pl.ds(a * P + b * 128, 128)]))
                g_ = 128 // R
                st[a] = [jnp.concatenate([trs[b][p * g_:(p + 1) * g_] for b in range(R)], axis=0).astype(BF16)
                         for p in range(R)]
            elif kind == "u":
                rhs = [_unpack(jnp.concatenate([unit(("u", a, g))[p] for g in range(8)], axis=0)) for p in range(R)]
                xr, xi = dft(name, rhs)
                for q in range(R):
                    x1[a, q, :, 0] = xr[q]
                    x1[a, q, :, 1] = xi[q]
            elif kind == "k":
                xr, xi = dft(name, st[a])
                prev = st["prev"]
                for q in range(R):
                    if prev is None:
                        x1[a, q, :, 2] = xr[q] + coefbuf[c + 1, 4]
                        x1[a, q, :, 3] = xi[q]
                    else:
                        pr, pi = prev[0][q], prev[1][q]
                        x1[a, q, pl.ds(0, 8), 2] = xr[q][:8] - pi[:8]
                        x1[a, q, pl.ds(0, 8), 3] = xi[q][:8] + pr[:8]
                        x1[a, q, pl.ds(8, 8), 2] = xr[q][8:] + pi[8:]
                        x1[a, q, pl.ds(8, 8), 3] = xi[q][8:] - pr[8:]
                st["prev"] = (xr, xi)
            else:
                for p in range(R):
                    wave = 8 * (p // 2)
                    cols = []
                    for kt in range(2):
                        rows = [None] * wave + [invbuf[p, pl.ds(8 * r, 8), pl.ds(128 * kt, 128)] for r in range(8)]
                        sub = {k_: v_ for k_, v_ in plan.items() if k_[0] == name and wave <= k_[1] < wave + 8}
                        vs = []
                        for r in range(wave, wave + 8):
                            v = rows[r]
                            for key in sub.get((name, r), ()):
                                v = jnp.where(never, unit(key)[2 * (p % 2) + kt], v)
                            vs.append(v)
                        cols.append(jnp.concatenate(vs, axis=0))
                    g = _unpack(jnp.concatenate(cols, axis=1))
                    wp = _unpack(jnp.concatenate([unit(("i", a, t))[p] for t in range(16)], axis=0))
                    ybuf[c, pl.ds(a * P + p, 128, stride=R), :] = _dot(g, wp)

    def once(lo, fn):
        def body(c, carry):
            fn(c)
            return carry
        jax.lax.fori_loop(lo, lo + one, body, 0)

    one = jnp.minimum(pl.program_id(0) + 1, 1)
    with jax.named_scope("p1"):
        once(-1, lambda c: p1_step(c, True, False))
        def p1s(c, carry):
            with jax.named_scope("p1step"):
                p1_step(c, True, True)
            return carry
        jax.lax.fori_loop(0, NC - 1, p1s, 0)

    def mod_cols(lo, n, toks=None):
        cv = cbuf[...].astype(F32)
        sc = (cv * jax.nn.sigmoid(cv)).astype(BF16)
        m = _dot(jnp.broadcast_to(sc, (8, D)), weights(wmodbuf, toks, lo * NC, (lo + n) * NC))
        return [m[:, j * D:(j + 1) * D] for j in range(n)]

    def mul_mod(x, j, cols=None):
        m = modbuf[j] if cols is None else modbuf[j, :, cols]
        return (x.reshape(-1, 8, x.shape[-1]) * m[None]).reshape(x.shape)

    def add_mod(x, j):
        return (x.reshape(-1, 8, x.shape[-1]) + modbuf[j][None]).reshape(x.shape)

    def slabs(ref, r0, n):
        return jnp.concatenate([ref[c, pl.ds(r0, n), :] for c in range(NC)], axis=1)

    def window(base, n):
        rows = pl.ds(base, n)
        return dict(q=qbuf.at[rows, :], y=ybuf.at[:, rows, :], x2=x2buf.at[rows, :], h=hbuf.at[rows, :],
                    hh=hhbuf.at[:, pl.ds(base, n + 8), :], xn=xnbuf.at[pl.ds(base, n - LEAD), :],
                    o=obuf.at[pl.ds(base, n - LEAD), :])

    def weights(ref, toks, c0=0, c1=None, nt=False):
        nrow = ref.shape[0]
        c1 = ref.shape[1] // 128 if c1 is None else c1
        if not toks:
            return ref[:, pl.ds(c0 * 128, (c1 - c0) * 128)]
        never = get_never()
        rt = -(-nrow // 128)
        cols = []
        for j in range(c0, c1):
            wu = pltpu.bitcast(ref[:, pl.ds(j * 128, 128)], U32)
            parts, last = [], 0
            for i in range(rt):
                pos = i * (c1 - c0) + (j - c0) if nt else (j - c0) * rt + i
                for n_, t in enumerate(toks.get(pos, ())):
                    r = 64 * i + 8 * n_
                    if r > last:
                        parts.append(wu[last:r])
                    parts.append(jnp.where(never, t, wu[r:r + 8]))
                    last = r + 8
            parts.append(wu[last:])
            cols.append(pltpu.bitcast(jnp.concatenate(parts, axis=0), BF16))
        return jnp.concatenate(cols, axis=1)

    def row_tokens(r):
        return [pltpu.bitcast(jnp.broadcast_to(r[i:i + 8], (8, 128)), U32) for i in range(0, r.shape[0], 8)]

    def stage_a0(w, r0, n):
        rows = pl.ds(r0, n)
        x = w["q"][rows, :].astype(F32)
        y = slabs(w["y"], r0, n)
        x2 = x + add_mod(mul_mod(_ln(x), 1), 0) * y
        w["x2"][rows, :] = x2
        return _ln(x2)

    def stage_a1(w, r0, n, n2=None):
        if n2 is None:
            n2 = stage_a0(w, r0, n)
        h = add_mod(mul_mod(n2, 4), 3)
        w["h"][pl.ds(r0, n), :] = h
        hc, r = _ln_stats(h)
        return (hc * r).astype(BF16), row_tokens(r)

    def stage_a2(w, n3, r0, n, last_valid=None, toks=None):
        hh = _gelu(_dot(n3, weights(w1buf, toks)))
        for c in range(NC):
            blk = hh[:, c * 128:(c + 1) * 128]
            w["hh"][c, pl.ds(r0 + 8, n - LEAD), :] = blk[:n - LEAD]
            tail = blk[n - LEAD:]
            if last_valid is not None:
                tail = jnp.where(last_valid, tail, 0.0)
            w["hh"][c, pl.ds(r0 + 8 + n - LEAD, LEAD), :] = tail

    def stage_b1a(w, r0, n, toks=None):
        rows = pl.ds(r0, n)
        lane = jax.lax.broadcasted_iota(jnp.int32, (n, 128), 1)

        def sh(c, d):
            return w["hh"][c, pl.ds(r0 + 8 + d, n), :]

        g = [sh(0, -1),
             jnp.where(lane < 32, sh(1, -1), sh(1, 1)),
             jnp.where(lane < 64, sh(2, 1), sh(2, -2)),
             jnp.where(lane < 96, sh(3, -2), sh(3, 2)),
             sh(4, 2)]
        hs = _dot(jnp.concatenate(g, axis=1).astype(BF16), weights(w2buf, toks))
        x1 = w["h"][rows, :] + hs
        w["h"][rows, :] = x1
        return x1

    def stage_b1b(w, x1, r0, n):
        w["xn"][pl.ds(r0, n), :] = _ln(x1).astype(BF16)

    def stage_b1(w, r0, n, toks=None):
        stage_b1b(w, stage_b1a(w, r0, n, toks), r0, n)

    def out_copy(r0):
        rows = pl.ds(r0, TS)
        return pltpu.make_async_copy(obuf.at[rows, :], out_hbm.at[rows, :], sem_out.at[0])

    def stage_b2a(w, r0, toks=None):
        rows = pl.ds(r0, TS)
        return _gelu(_dot_nt(w["xn"][rows, :], weights(w3buf, toks, nt=True))).astype(BF16)

    def stage_b2b(w, h3, r0, c0, c1, toks=None):
        rows = pl.ds(r0, TS)
        cols = pl.ds(c0 * 128, (c1 - c0) * 128)
        h2 = _dot(h3, weights(w4buf, toks, c0, c1))
        w["o"][rows, cols] = (w["x2"][rows, cols] + mul_mod(w["h"][rows, cols] + h2, 5, cols)).astype(BF16)

    w = window(0, 2 * TS + LEAD)
    H = TS // 2
    with jax.named_scope("t0a"):
        cps["qa"].wait()
        cps["wmoda"].wait()

        mv = {}

        def mod_fn(j, toks):
            mv[j] = mod_cols(j, 1, toks)[0]
            if len(mv) == 3:
                modbuf[0] = mv[2] * mv[0]
                modbuf[1] = mv[2] * (1.0 + mv[1])

        p1_step(NC - 1, False, True, order="m0 i0 m1 i1 m2 i2 i3".split(),
                maxutil=1.5, mod_fn=mod_fn)
        w["h"][pl.ds(0, QA), :] = stage_a0(w, 0, QA)
    with jax.named_scope("t0b"):
        cps["wmodb"].wait()
        sb, cb = mod_cols(3, 2)
        modbuf[3] = sb
        modbuf[4] = 1.0 + cb
        n3, _ = stage_a1(w, 0, QA, n2=w["h"][pl.ds(0, QA), :])
    with jax.named_scope("t1"):
        cps["w1"].wait()
        stage_a2(w, n3, 0, QA)
    with jax.named_scope("t2"):
        cps["qb"].wait()
        cps["w2"].wait()
        n3a, _ = stage_a1(w, QA, H)
        n3b, _ = stage_a1(w, QA + H, H)
        stage_b1(w, 0, TS)
        stage_a2(w, n3a, QA, H)
        stage_a2(w, n3b, QA + H, H)
        stage_b1(w, TS, H)
        stage_b1a(w, TS + H, H)
    with jax.named_scope("t3"):
        cps["w3"].wait()
        stage_b1b(w, w["h"][pl.ds(TS + H, H), :], TS + H, H)
        h3 = stage_b2a(w, 0)
    with jax.named_scope("t4"):
        cps["w4"].wait()
        cps["wmodg"].wait()
        modbuf[5] = mod_cols(5, 1)[0]
        stage_b2b(w, h3, 0, 0, 5)
        out_copy(0).start()
        cps["q1"].wait()

    NSUB = 4

    def step(s, carry):
        r0 = pl.multiple_of(s * TS, TS)
        w = window(r0, 2 * TS + LEAD)
        h3 = stage_b2a(w, 0)
        sub = TS // NSUB
        for j in range(NSUB):
            if j > 0:
                stage_b2b(w, h3, 0, j - 1, j)
            ra = TS + LEAD + j * sub
            stage_a2(w, stage_a1(w, ra, sub)[0], ra, sub, last_valid=(s < NT - 2) if j == NSUB - 1 else None)
        stage_b2b(w, h3, 0, 3, 4)
        stage_b1(w, TS, TS)
        stage_b2b(w, h3, 0, 4, 5)
        out_copy(r0).start()
        return carry

    with jax.named_scope("p2main"):
        jax.lax.fori_loop(1, NT - 1, step, 0)
    with jax.named_scope("p2epi"):
        w = window((NT - 2) * TS, 2 * TS + LEAD)
        stage_b2b(w, stage_b2a(w, TS), TS, 0, 5)
        out_copy((NT - 1) * TS).start()
        pltpu.make_async_copy(obuf, out_hbm, sem_out.at[0]).wait()


@jax.jit
def pallas_adaLN_cond__ssm_conv_h3__mixer_s_mlp__prompt_kernel(
    A_q: jax.Array,
    A_k: jax.Array,
    A_v: jax.Array,
    A_shift_k: jax.Array,
    A_ssm_k: jax.Array,
    A_ssm_D: jax.Array,
    B_x: jax.Array,
    B_w1: jax.Array,
    B_w2: jax.Array,
    B_w3: jax.Array,
    B_w4: jax.Array,
    c: jax.Array,
    w_mod: jax.Array,
):
    del B_x
    args = (
        A_q.reshape(S, D), A_k.reshape(S, D), A_v.reshape(S, D),
        A_shift_k.T, A_ssm_k, A_ssm_D.reshape(NC, 128),
        B_w1, B_w2, B_w3.T, B_w4, c, w_mod,
    )
    scratch = [
        pltpu.VMEM((NC, S + 64, 128), BF16),
        pltpu.VMEM((NC, S, 128), BF16),
        pltpu.VMEM((NC, 128, S), BF16),
        pltpu.VMEM((R, 128, 128), U32),
        pltpu.VMEM((R, 64, 256), U32),
        pltpu.VMEM((64, 128), U32),
        pltpu.VMEM((D, 6 * D), BF16),
        pltpu.VMEM((D, D), BF16),
        pltpu.VMEM((D, D), BF16),
        pltpu.VMEM((FF, D), BF16),
        pltpu.VMEM((FF, D), BF16),
        pltpu.VMEM((S + 64, D), BF16),
        pltpu.VMEM((NC, NA, R, 16, 4, 8, 128), F32),
        pltpu.VMEM((NC, 8, 8, 128), F32),
        pltpu.VMEM((NC, S + 32, 128), F32),
        pltpu.VMEM((8, 8, D), F32),
        pltpu.VMEM((S + 32, D), F32),
        pltpu.VMEM((S + 32, D), F32),
        pltpu.VMEM((NC, S + 32, 128), F32),
        pltpu.VMEM((S, D), BF16),
        pltpu.VMEM((S, D), BF16),
        pltpu.VMEM((4, D), BF16),
        pltpu.VMEM((NC, 128), BF16),
        pltpu.VMEM((1, D), BF16),
        pltpu.SemaphoreType.DMA((32,)),
        pltpu.SemaphoreType.DMA((1,)),
    ]
    out = pl.pallas_call(
        _kernel,
        out_shape=jax.ShapeDtypeStruct((S, D), BF16),
        in_specs=[pl.BlockSpec(memory_space=pl.ANY)] * len(args),
        out_specs=pl.BlockSpec(memory_space=pl.ANY),
        scratch_shapes=scratch,
        grid=(1,),
        compiler_params=pltpu.CompilerParams(vmem_limit_bytes=100 * 1024 * 1024),
        name="adaln_h3_mixer",
    )(*args)
    return out.reshape(1, S, D)
```

```python
import numpy as np
import jax
import jax.numpy as jnp
import jax.experimental.pallas as pl
import jax.experimental.pallas.tpu as pltpu

F32 = jnp.float32
BF16 = jnp.bfloat16
U32 = jnp.uint32

S = 2048
D = 640
FF = 1728
NC = D // 128
R = 4
P = 128 * R
NA = S // P
TS = 256
NT = S // TS
LEAD = 16
EPS = 1e-5
P1_ORDER = "t0 t1 t2 t3 k0 k1 k2 k3 u0 i0 u1 i1 u2 i2 u3 i3"


def _cos_table(row, m, p, scale):
    t, part, s = row >> 4, (row >> 3) & 1, row & 7
    odd2f1 = 32 * (t & 7) + 4 * s + 2 * (t >> 3) + 1
    j = (odd2f1 * (R * m + p) + P * part) & (4 * P - 1)
    z = jnp.abs(j - 2 * P) - P
    x = z.astype(F32) * (2.0 * np.pi / (4 * P))
    x2 = x * x
    poly = 1.0 / 362880.0 - x2 * (1.0 / 39916800.0)
    for coef in (-1.0 / 5040.0, 1.0 / 120.0, -1.0 / 6.0, 1.0):
        poly = poly * x2 + coef
    return poly * (x * scale)


def _plan_tokens(order, maxutil=1.0):
    dur = {"t": 8, "u": 16, "k": 16, "i": 16, "m": 12}
    post = {"t": 8.0, "u": 16.0, "k": 24.0, "i": 4.0, "m": 18.0}
    lag = 8
    cap = 60.0
    start, slots = {}, []
    for n in order:
        start[n] = len(slots)
        slots += [(n, r) for r in range(dur[n[0]])]
    pre = 4
    free = [cap - (post[slots[i - lag][0][0]] if i >= lag else 0.0) for i in range(-pre, len(slots))]
    cum = np.concatenate([[0.0], np.cumsum(free)])
    units = []
    for n in order:
        a = int(n[1])
        if n[0] == "u":
            units += [(("u", a, g), 94.0, start[n]) for g in range(8)]
        elif n[0] == "i":
            units += [(("i", a, t), 32.0 * a + 48.0, start[n]) for t in range(16)]
    margin = 3

    def deadlines(util):
        d, nxt = [], 1e18
        for key, cost, need in reversed(units):
            nxt = min(cum[max(need - margin + pre, 0)], nxt)
            d.append(nxt)
            nxt -= cost / util
        return d[::-1], nxt

    lo_, hi_ = 0.05, maxutil
    for _ in range(30):
        mid = 0.5 * (lo_ + hi_)
        if deadlines(mid)[1] >= 0.0:
            hi_ = mid
        else:
            lo_ = mid
    d, _ = deadlines(hi_)
    plan = {}
    for (key, cost, need), dl in zip(units, d):
        s = int(np.searchsorted(cum, dl, side="right")) - 1 - pre
        if 0 <= s < need:
            plan.setdefault(slots[s], []).append(key)
    return plan


def _pack(x):
    return pltpu.bitcast(x.astype(BF16), U32)


def _unpack(w):
    return pltpu.bitcast(w, BF16)


def _dot(a, b):
    return jnp.dot(a, b, preferred_element_type=F32)


def _dot_nt(a, b):
    return jax.lax.dot_general(a, b, (((1,), (1,)), ((), ())), preferred_element_type=F32)


def _lo(w):
    return pltpu.bitcast(w << 16, F32)


def _hi(w):
    return pltpu.bitcast(w & jnp.uint32(0xFFFF0000), F32)


def _ln_stats(x):
    m = jnp.sum(x, axis=-1, keepdims=True) * (1.0 / D)
    xc = x - m
    v = jnp.sum(xc * xc, axis=-1, keepdims=True) * (1.0 / D)
    return xc, jnp.exp(-0.5 * jnp.log(v + EPS))


def _ln(x):
    xc, r = _ln_stats(x)
    return xc * r


def _spread(tokens, lo, hi):
    out = {}
    for i, t in enumerate(tokens):
        out.setdefault(lo + (i * (hi - lo)) // len(tokens), []).append(t)
    return out


def _gelu(x):
    c0 = 0.7978845608028654
    c1 = c0 * 0.044715
    z = x * (c0 + c1 * (x * x))
    hx = 0.5 * x
    return hx + hx * jnp.tanh(z)


def _bfly(tr, ti, sign):
    s02r, s02i = tr[0] + tr[2], ti[0] + ti[2]
    d02r, d02i = tr[0] - tr[2], ti[0] - ti[2]
    s13r, s13i = tr[1] + tr[3], ti[1] + ti[3]
    d13r, d13i = tr[1] - tr[3], ti[1] - ti[3]
    x0r, x0i = s02r + s13r, s02i + s13i
    x2r, x2i = s02r - s13r, s02i - s13i
    ar, ai = d02r + d13i, d02i - d13r
    br, bi = d02r - d13i, d02i + d13r
    if sign < 0:
        return [x0r, ar, x2r, br], [x0i, ai, x2i, bi]
    return [x0r, br, x2r, ar], [x0i, bi, x2i, ai]


def _kernel(q_hbm, k_hbm, v_hbm, shift_hbm, ssmk_hbm, ssmd_hbm, w1_hbm, w2_hbm, w3t_hbm, w4_hbm,
            c_hbm, wmod_hbm,
            out_hbm,
            kbuf, vbuf, skbuf, fwdbuf, invbuf, permbuf,
            wmodbuf, w1buf, w2buf, w3buf, w4buf, qbuf,
            xu, coefbuf, ybuf, modbuf, x2buf, hbuf, hhbuf, xnbuf, obuf, shiftbuf, dbuf, cbuf,
            sem_in, sem_out):
    cps = {}
    n_sem = [0]

    def start(name, src, dst):
        cp = pltpu.make_async_copy(src, dst, sem_in.at[n_sem[0]])
        n_sem[0] += 1
        cp.start()
        cps[name] = cp

    blk_sem0 = 0
    n_sem[0] = 3 * NC

    def block_copies(c):
        cs = pl.ds(pl.multiple_of(c * 128, 128), 128)
        return [pltpu.make_async_copy(k_hbm.at[:, cs], kbuf.at[c, pl.ds(16, S), :], sem_in.at[blk_sem0 + 3 * c]),
                pltpu.make_async_copy(v_hbm.at[:, cs], vbuf.at[c, pl.ds(0, S), :], sem_in.at[blk_sem0 + 3 * c + 1]),
                pltpu.make_async_copy(ssmk_hbm.at[cs, :], skbuf.at[c], sem_in.at[blk_sem0 + 3 * c + 2])]

    for c in range(NC):
        for i, cp in enumerate(block_copies(c)):
            cp.start()
            if c == 0 and i == 1:
                start("shift", shift_hbm, shiftbuf)
                start("d", ssmd_hbm, dbuf)
                start("c", c_hbm, cbuf)
    QA = TS + LEAD
    QB = 2 * TS + LEAD
    start("qa", q_hbm.at[pl.ds(0, QA), :], qbuf.at[pl.ds(0, QA), :])
    start("wmoda", wmod_hbm.at[:, pl.ds(0, 3 * D)], wmodbuf.at[:, pl.ds(0, 3 * D)])
    start("wmodb", wmod_hbm.at[:, pl.ds(3 * D, 2 * D)], wmodbuf.at[:, pl.ds(3 * D, 2 * D)])
    start("w1", w1_hbm, w1buf)
    start("qb", q_hbm.at[pl.ds(QA, QB - QA), :], qbuf.at[pl.ds(QA, QB - QA), :])
    start("w2", w2_hbm, w2buf)
    start("w3", w3t_hbm, w3buf)
    start("w4", w4_hbm, w4buf)
    start("wmodg", wmod_hbm.at[:, pl.ds(5 * D, D)], wmodbuf.at[:, pl.ds(5 * D, D)])
    start("q1", q_hbm.at[pl.ds(QB, S - QB), :], qbuf.at[pl.ds(QB, S - QB), :])

    kw = kbuf.bitcast(U32)
    vw = vbuf.bitcast(U32)
    for c in range(NC):
        kw[c, pl.ds(0, 8), :] = jnp.zeros((8, 128), U32)
        ybuf[c, pl.ds(S, LEAD), :] = jnp.zeros((LEAD, 128), F32)
        hhbuf[c, pl.ds(0, 8), :] = jnp.zeros((8, 128), F32)
    qbuf[pl.ds(S, LEAD), :] = jnp.zeros((LEAD, D), BF16)

    def tables(p, carry):
        i0 = jax.lax.broadcasted_iota(jnp.int32, (256, 128), 0)
        i1 = jax.lax.broadcasted_iota(jnp.int32, (256, 128), 1)
        fwdbuf[p] = _pack(_cos_table(i0, i1, p, 1.0))
        i0 = jax.lax.broadcasted_iota(jnp.int32, (128, 256), 0)
        i1 = jax.lax.broadcasted_iota(jnp.int32, (128, 256), 1)
        row = (i1 & ~15) + 8 * (i1 & 1) + ((i1 >> 1) & 7)
        invbuf[p] = _pack(_cos_table(row, i0, p, 1.0 / P))
        return carry

    jax.lax.fori_loop(0, R, tables, 0)
    i0 = jax.lax.broadcasted_iota(jnp.int32, (128, 128), 0)
    i1 = jax.lax.broadcasted_iota(jnp.int32, (128, 128), 1)
    permbuf[...] = _pack(jnp.where(i0 == (128 // R) * (i1 & (R - 1)) + (i1 >> 2), 1.0, 0.0).astype(F32))

    for name in ("shift", "d", "c"):
        cps[name].wait()
    coef = shiftbuf[...].astype(F32)
    dval = dbuf[...].astype(F32)
    for c in range(NC):
        for j in range(4):
            coefbuf[c, j] = jnp.broadcast_to(coef[j:j + 1, c * 128:(c + 1) * 128], (8, 128))
        coefbuf[c, 4] = jnp.broadcast_to(dval[c:c + 1, :], (8, 128))

    xk = xu
    def split_ri(t):
        t = t.reshape(16, 2, 8, 128)
        return t[:, 0], t[:, 1]

    def get_never():
        return kw[0, pl.ds(0, 8), :] != 0

    def pack2(x, y):
        return pltpu.pack_elementwise([x, y], packed_dtype=BF16)

    def unit_u(c, a, g):
        cj = [coefbuf[c, j] for j in range(4)]
        halves = []
        for e in range(2):
            kb = 8 + a * (P // 2) + 32 * g + 2 * e
            vb = a * (P // 2) + 32 * g + 2 * e
            wm2 = kw[c, pl.ds(kb - 2, 8, stride=4), :]
            wm1 = kw[c, pl.ds(kb - 1, 8, stride=4), :]
            w0 = kw[c, pl.ds(kb, 8, stride=4), :]
            w1 = kw[c, pl.ds(kb + 1, 8, stride=4), :]
            seq = [_hi(wm2), _lo(wm1), _hi(wm1), _lo(w0), _hi(w0), _lo(w1), _hi(w1)]
            v0 = vw[c, pl.ds(vb, 8, stride=4), :]
            v1 = vw[c, pl.ds(vb + 1, 8, stride=4), :]
            vs = [_lo(v0), _hi(v0), _lo(v1), _hi(v1)]
            halves.append([((seq[3 + p] * cj[0] + seq[2 + p] * cj[1]) + (seq[1 + p] * cj[2] + seq[p] * cj[3])) * vs[p]
                           for p in range(R)])
        return [pack2(halves[0][p], halves[1][p]) for p in range(R)]

    def unit_i(a, t, x_c):
        yr, yi = [], []
        for q in range(R):
            accr = acci = None
            for j in range(a + 1):
                ur, ui = x_c[j, q, t, 0], x_c[j, q, t, 1]
                kr, ki = x_c[a - j, q, t, 2], x_c[a - j, q, t, 3]
                pr = ur * kr - ui * ki
                pi = ur * ki + ui * kr
                accr = pr if accr is None else accr + pr
                acci = pi if acci is None else acci + pi
            yr.append(accr)
            yi.append(acci)
        wr, wi = _bfly(yr, yi, +1)
        return [pack2(wr[p], wi[p]) for p in range(R)]

    def p1_step(c, do_fwd, do_conv, order=None, maxutil=1.0, mod_fn=None):
        if do_fwd:
            for cp in block_copies(c + 1):
                cp.wait()
        if do_fwd and do_conv:
            xw = xu.at[pl.ds(c, 2)]
            x0, x1 = xw.at[0], xw.at[1]
        elif do_fwd:
            x1 = xu.at[c + 1]
        else:
            x0 = xu.at[c]
        if order is None:
            order = [n for n in P1_ORDER.split() if (do_conv if n[0] == "i" else do_fwd)]
        plan = _plan_tokens(order, maxutil)
        never = get_never()
        units = {}

        def unit(key):
            if key not in units:
                kind, a, j = key
                units[key] = unit_u(c + 1, a, j) if kind == "u" else unit_i(a, j, x0)
            return units[key]

        def lhs(name, p, rows):
            out = []
            for r, v in enumerate(rows):
                for key in plan.get((name, r), ()):
                    v = jnp.where(never, unit(key)[p], v)
                out.append(v)
            return out

        def dft(name, rhs):
            tr, ti = [], []
            for p in range(R):
                f = jnp.concatenate(lhs(name, p, [fwdbuf[p, pl.ds(8 * r, 8), :] for r in range(16)]), axis=0)
                r_, i_ = split_ri(_dot(_unpack(f), rhs[p]))
                tr.append(r_)
                ti.append(i_)
            return _bfly(tr, ti, -1)

        st = dict(prev=None)
        for name in order:
            kind, a = name[0], int(name[1])
            if kind == "m":
                toks = {}
                for r in range(12):
                    for n_, key in enumerate(plan.get((name, r), ())):
                        toks.setdefault(2 * r + n_ % 2, []).extend(unit(key))
                mod_fn(a, toks)
            elif kind == "t":
                trs = []
                for b in range(R):
                    pm = jnp.concatenate(lhs(name, b, [permbuf[pl.ds(8 * r, 8), :] for r in range(8)]), axis=0)
                    trs.append(_dot_nt(_unpack(pm), skbuf[c + 1, :, pl.ds(a * P + b * 128, 128)]))
                g_ = 128 // R
                st[a] = [jnp.concatenate([trs[b][p * g_:(p + 1) * g_] for b in range(R)], axis=0).astype(BF16)
                         for p in range(R)]
            elif kind == "u":
                rhs = [_unpack(jnp.concatenate([unit(("u", a, g))[p] for g in range(8)], axis=0)) for p in range(R)]
                xr, xi = dft(name, rhs)
                for q in range(R):
                    x1[a, q, :, 0] = xr[q]
                    x1[a, q, :, 1] = xi[q]
            elif kind == "k":
                xr, xi = dft(name, st[a])
                prev = st["prev"]
                for q in range(R):
                    if prev is None:
                        x1[a, q, :, 2] = xr[q] + coefbuf[c + 1, 4]
                        x1[a, q, :, 3] = xi[q]
                    else:
                        pr, pi = prev[0][q], prev[1][q]
                        x1[a, q, pl.ds(0, 8), 2] = xr[q][:8] - pi[:8]
                        x1[a, q, pl.ds(0, 8), 3] = xi[q][:8] + pr[:8]
                        x1[a, q, pl.ds(8, 8), 2] = xr[q][8:] + pi[8:]
                        x1[a, q, pl.ds(8, 8), 3] = xi[q][8:] - pr[8:]
                st["prev"] = (xr, xi)
            else:
                for p in range(R):
                    wave = 8 * (p // 2)
                    cols = []
                    for kt in range(2):
                        rows = [None] * wave + [invbuf[p, pl.ds(8 * r, 8), pl.ds(128 * kt, 128)] for r in range(8)]
                        sub = {k_: v_ for k_, v_ in plan.items() if k_[0] == name and wave <= k_[1] < wave + 8}
                        vs = []
                        for r in range(wave, wave + 8):
                            v = rows[r]
                            for key in sub.get((name, r), ()):
                                v = jnp.where(never, unit(key)[2 * (p % 2) + kt], v)
                            vs.append(v)
                        cols.append(jnp.concatenate(vs, axis=0))
                    g = _unpack(jnp.concatenate(cols, axis=1))
                    wp = _unpack(jnp.concatenate([unit(("i", a, t))[p] for t in range(16)], axis=0))
                    ybuf[c, pl.ds(a * P + p, 128, stride=R), :] = _dot(g, wp)

    def once(lo, fn):
        def body(c, carry):
            fn(c)
            return carry
        jax.lax.fori_loop(lo, lo + one, body, 0)

    one = jnp.minimum(pl.program_id(0) + 1, 1)
    with jax.named_scope("p1"):
        once(-1, lambda c: p1_step(c, True, False))
        def p1s(c, carry):
            with jax.named_scope("p1step"):
                p1_step(c, True, True)
            return carry
        jax.lax.fori_loop(0, NC - 1, p1s, 0)

    def mod_cols(lo, n, toks=None):
        cv = cbuf[...].astype(F32)
        sc = (cv * jax.nn.sigmoid(cv)).astype(BF16)
        m = _dot(jnp.broadcast_to(sc, (8, D)), weights(wmodbuf, toks, lo * NC, (lo + n) * NC))
        return [m[:, j * D:(j + 1) * D] for j in range(n)]

    def mul_mod(x, j, cols=None):
        m = modbuf[j] if cols is None else modbuf[j, :, cols]
        return (x.reshape(-1, 8, x.shape[-1]) * m[None]).reshape(x.shape)

    def add_mod(x, j):
        return (x.reshape(-1, 8, x.shape[-1]) + modbuf[j][None]).reshape(x.shape)

    def slabs(ref, r0, n):
        return jnp.concatenate([ref[c, pl.ds(r0, n), :] for c in range(NC)], axis=1)

    def window(base, n):
        rows = pl.ds(base, n)
        return dict(q=qbuf.at[rows, :], y=ybuf.at[:, rows, :], x2=x2buf.at[rows, :], h=hbuf.at[rows, :],
                    hh=hhbuf.at[:, pl.ds(base, n + 8), :], xn=xnbuf.at[pl.ds(base, n - LEAD), :],
                    o=obuf.at[pl.ds(base, n - LEAD), :])

    def weights(ref, toks, c0=0, c1=None, nt=False):
        nrow = ref.shape[0]
        c1 = ref.shape[1] // 128 if c1 is None else c1
        if not toks:
            return ref[:, pl.ds(c0 * 128, (c1 - c0) * 128)]
        never = get_never()
        rt = -(-nrow // 128)
        cols = []
        for j in range(c0, c1):
            wu = pltpu.bitcast(ref[:, pl.ds(j * 128, 128)], U32)
            parts, last = [], 0
            for i in range(rt):
                pos = i * (c1 - c0) + (j - c0) if nt else (j - c0) * rt + i
                for n_, t in enumerate(toks.get(pos, ())):
                    r = 64 * i + 8 * n_
                    if r > last:
                        parts.append(wu[last:r])
                    parts.append(jnp.where(never, t, wu[r:r + 8]))
                    last = r + 8
            parts.append(wu[last:])
            cols.append(pltpu.bitcast(jnp.concatenate(parts, axis=0), BF16))
        return jnp.concatenate(cols, axis=1)

    def row_tokens(r):
        return [pltpu.bitcast(jnp.broadcast_to(r[i:i + 8], (8, 128)), U32) for i in range(0, r.shape[0], 8)]

    def stage_a0(w, r0, n):
        rows = pl.ds(r0, n)
        x = w["q"][rows, :].astype(F32)
        y = slabs(w["y"], r0, n)
        x2 = x + add_mod(mul_mod(_ln(x), 1), 0) * y
        w["x2"][rows, :] = x2
        return _ln(x2)

    def stage_a1(w, r0, n, n2=None):
        if n2 is None:
            n2 = stage_a0(w, r0, n)
        h = add_mod(mul_mod(n2, 4), 3)
        w["h"][pl.ds(r0, n), :] = h
        hc, r = _ln_stats(h)
        return (hc * r).astype(BF16), row_tokens(r)

    def stage_a2(w, n3, r0, n, last_valid=None, toks=None):
        hh = _gelu(_dot(n3, weights(w1buf, toks)))
        for c in range(NC):
            blk = hh[:, c * 128:(c + 1) * 128]
            w["hh"][c, pl.ds(r0 + 8, n - LEAD), :] = blk[:n - LEAD]
            tail = blk[n - LEAD:]
            if last_valid is not None:
                tail = jnp.where(last_valid, tail, 0.0)
            w["hh"][c, pl.ds(r0 + 8 + n - LEAD, LEAD), :] = tail

    def stage_b1a(w, r0, n, toks=None):
        rows = pl.ds(r0, n)
        lane = jax.lax.broadcasted_iota(jnp.int32, (n, 128), 1)

        def sh(c, d):
            return w["hh"][c, pl.ds(r0 + 8 + d, n), :]

        g = [sh(0, -1),
             jnp.where(lane < 32, sh(1, -1), sh(1, 1)),
             jnp.where(lane < 64, sh(2, 1), sh(2, -2)),
             jnp.where(lane < 96, sh(3, -2), sh(3, 2)),
             sh(4, 2)]
        hs = _dot(jnp.concatenate(g, axis=1).astype(BF16), weights(w2buf, toks))
        x1 = w["h"][rows, :] + hs
        w["h"][rows, :] = x1
        return x1

    def stage_b1b(w, x1, r0, n):
        w["xn"][pl.ds(r0, n), :] = _ln(x1).astype(BF16)

    def stage_b1(w, r0, n, toks=None):
        stage_b1b(w, stage_b1a(w, r0, n, toks), r0, n)

    def out_copy(r0):
        rows = pl.ds(r0, TS)
        return pltpu.make_async_copy(obuf.at[rows, :], out_hbm.at[rows, :], sem_out.at[0])

    FM = (FF // 128) * 128
    FR = FF - FM

    def stage_b2a(w, r0, n=TS):
        xn = w["xn"][pl.ds(r0, n), :]
        ht = _gelu(_dot_nt(w3buf[pl.ds(FM, FR), :], xn))
        h3 = _gelu(_dot_nt(xn, w3buf[pl.ds(0, FM), :])).astype(BF16)
        hl = jnp.concatenate([ht[:, j * 128:(j + 1) * 128] for j in range(n // 128)], axis=0)
        hl = [hl[j * 128:(j + 1) * 128].T.astype(BF16) for j in range(n // 256)]
        return h3, hl

    def stage_b2b(w, hh3, r0, c0, c1, n=TS):
        h3, hl = hh3
        rows = pl.ds(r0, n)
        cols = pl.ds(c0 * 128, (c1 - c0) * 128)
        wl = w4buf[pl.ds(FM, FR), cols]
        z = jnp.zeros_like(wl)
        wlo, whi = jnp.concatenate([wl, z], axis=0), jnp.concatenate([z, wl], axis=0)
        rest = jnp.concatenate([_dot(h, wz) for h in hl for wz in (wlo, whi)], axis=0)
        h2 = _dot(h3, w4buf[pl.ds(0, FM), cols]) + rest
        w["o"][rows, cols] = (w["x2"][rows, cols] + mul_mod(w["h"][rows, cols] + h2, 5, cols)).astype(BF16)

    w = window(0, 2 * TS + LEAD)
    H = TS // 2
    with jax.named_scope("t0a"):
        cps["qa"].wait()
        cps["wmoda"].wait()

        mv = {}

        def mod_fn(j, toks):
            mv[j] = mod_cols(j, 1, toks)[0]
            if len(mv) == 3:
                modbuf[0] = mv[2] * mv[0]
                modbuf[1] = mv[2] * (1.0 + mv[1])

        p1_step(NC - 1, False, True, order="m0 i0 m1 i1 m2 i2 i3".split(),
                maxutil=1.5, mod_fn=mod_fn)
        w["h"][pl.ds(0, QA), :] = stage_a0(w, 0, QA)
    with jax.named_scope("t0b"):
        cps["wmodb"].wait()
        sb, cb = mod_cols(3, 2)
        modbuf[3] = sb
        modbuf[4] = 1.0 + cb
        n3, _ = stage_a1(w, 0, QA, n2=w["h"][pl.ds(0, QA), :])
    with jax.named_scope("t1"):
        cps["w1"].wait()
        stage_a2(w, n3, 0, QA)
    with jax.named_scope("t2"):
        cps["qb"].wait()
        cps["w2"].wait()
        n3a, _ = stage_a1(w, QA, H)
        n3b, _ = stage_a1(w, QA + H, H)
        stage_b1(w, 0, TS)
        stage_a2(w, n3a, QA, H)
        stage_a2(w, n3b, QA + H, H)
        stage_b1(w, TS, H)
        stage_b1a(w, TS + H, H)
    with jax.named_scope("t3"):
        cps["w3"].wait()
        stage_b1b(w, w["h"][pl.ds(TS + H, H), :], TS + H, H)
        h3 = stage_b2a(w, 0)
    with jax.named_scope("t4"):
        cps["w4"].wait()
        cps["wmodg"].wait()
        modbuf[5] = mod_cols(5, 1)[0]
        stage_b2b(w, h3, 0, 0, 5)
        out_copy(0).start()
        cps["q1"].wait()

    NSUB = 4

    def step(s, carry):
        r0 = pl.multiple_of(s * TS, TS)
        w = window(r0, 2 * TS + LEAD)
        h3 = stage_b2a(w, 0)
        sub = TS // NSUB
        for j in range(NSUB):
            if j > 0:
                stage_b2b(w, h3, 0, j - 1, j)
            ra = TS + LEAD + j * sub
            stage_a2(w, stage_a1(w, ra, sub)[0], ra, sub, last_valid=(s < NT - 2) if j == NSUB - 1 else None)
        stage_b2b(w, h3, 0, 3, 4)
        stage_b1(w, TS, TS)
        stage_b2b(w, h3, 0, 4, 5)
        out_copy(r0).start()
        return carry

    with jax.named_scope("p2main"):
        jax.lax.fori_loop(1, NT - 1, step, 0)
    with jax.named_scope("p2epi"):
        w = window((NT - 2) * TS, 2 * TS + LEAD)
        h3 = stage_b2a(w, TS)
        rows = pl.ds((NT - 1) * TS, TS)
        for c0, c1 in ((0, 2), (2, 4), (4, 5)):
            stage_b2b(w, h3, TS, c0, c1)
            cols = pl.ds(c0 * 128, (c1 - c0) * 128)
            pltpu.make_async_copy(obuf.at[rows, cols], out_hbm.at[rows, cols], sem_out.at[0]).start()
        pltpu.make_async_copy(obuf, out_hbm, sem_out.at[0]).wait()


@jax.jit
def pallas_adaLN_cond__ssm_conv_h3__mixer_s_mlp__prompt_kernel(
    A_q: jax.Array,
    A_k: jax.Array,
    A_v: jax.Array,
    A_shift_k: jax.Array,
    A_ssm_k: jax.Array,
    A_ssm_D: jax.Array,
    B_x: jax.Array,
    B_w1: jax.Array,
    B_w2: jax.Array,
    B_w3: jax.Array,
    B_w4: jax.Array,
    c: jax.Array,
    w_mod: jax.Array,
):
    del B_x
    args = (
        A_q.reshape(S, D), A_k.reshape(S, D), A_v.reshape(S, D),
        A_shift_k.T, A_ssm_k, A_ssm_D.reshape(NC, 128),
        B_w1, B_w2, B_w3.T, B_w4, c, w_mod,
    )
    scratch = [
        pltpu.VMEM((NC, S + 64, 128), BF16),
        pltpu.VMEM((NC, S + 64, 128), BF16),
        pltpu.VMEM((NC, 128, S), BF16),
        pltpu.VMEM((R, 128, 128), U32),
        pltpu.VMEM((R, 64, 256), U32),
        pltpu.VMEM((64, 128), U32),
        pltpu.VMEM((D, 6 * D), BF16),
        pltpu.VMEM((D, D), BF16),
        pltpu.VMEM((D, D), BF16),
        pltpu.VMEM((FF, D), BF16),
        pltpu.VMEM((FF, D), BF16),
        pltpu.VMEM((S + 64, D), BF16),
        pltpu.VMEM((NC, NA, R, 16, 4, 8, 128), F32),
        pltpu.VMEM((NC, 8, 8, 128), F32),
        pltpu.VMEM((NC, S + 32, 128), F32),
        pltpu.VMEM((8, 8, D), F32),
        pltpu.VMEM((S + 32, D), F32),
        pltpu.VMEM((S + 32, D), F32),
        pltpu.VMEM((NC, S + 32, 128), F32),
        pltpu.VMEM((S, D), BF16),
        pltpu.VMEM((S, D), BF16),
        pltpu.VMEM((4, D), BF16),
        pltpu.VMEM((NC, 128), BF16),
        pltpu.VMEM((1, D), BF16),
        pltpu.SemaphoreType.DMA((32,)),
        pltpu.SemaphoreType.DMA((1,)),
    ]
    out = pl.pallas_call(
        _kernel,
        out_shape=jax.ShapeDtypeStruct((S, D), BF16),
        in_specs=[pl.BlockSpec(memory_space=pl.ANY)] * len(args),
        out_specs=pl.BlockSpec(memory_space=pl.ANY),
        scratch_shapes=scratch,
        grid=(1,),
        compiler_params=pltpu.CompilerParams(vmem_limit_bytes=100 * 1024 * 1024, disable_semaphore_checks=True,
                                             disable_bounds_checks=True),
        name="adaln_h3_mixer",
    )(*args)
    return out.reshape(1, S, D)
```

```python
import numpy as np
import jax
import jax.numpy as jnp
import jax.experimental.pallas as pl
import jax.experimental.pallas.tpu as pltpu

F32 = jnp.float32
BF16 = jnp.bfloat16
U32 = jnp.uint32

S = 2048
D = 640
FF = 1728
NC = D // 128
R = 4
P = 128 * R
NA = S // P
TS = 256
NT = S // TS
LEAD = 16
EPS = 1e-5
P1_ORDER = "t0 t1 t2 t3 k0 k1 k2 k3 u0 i0 u1 i1 u2 i2 u3 i3"


def _freq(row):
    t, part, s = row >> 4, (row >> 3) & 1, row & 7
    return 32 * (t & 7) + 4 * s + 2 * (t >> 3) + 1, P * part


def _cos(j, scale):
    jf = (j & (4 * P - 1)).astype(F32)
    u = 2.0 * np.pi / (4 * P)
    x = jnp.abs(jf * u - np.pi) - 0.5 * np.pi
    x2 = x * x
    poly = scale / 362880.0 - x2 * (scale / 39916800.0)
    for coef in (-1.0 / 5040.0, 1.0 / 120.0, -1.0 / 6.0, 1.0):
        poly = poly * x2 + coef * scale
    return poly * x


_DUR = {"t": 8, "u": 16, "k": 16, "i": 16, "m": 12, "g": 0, "c": 0, "j": 16}
_POST = {"t": 8.0, "u": 16.0, "k": 24.0, "i": 4.0, "j": 4.0, "m": 18.0}


def _plan_tokens(order, maxutil):
    lag, cap, pre, margin = 8, 60, 4, 3
    start, slots = {}, []
    for n in order:
        start[n] = len(slots)
        slots += [(n, r) for r in range(_DUR[n[0]])]
    nslot = len(slots) + lag
    free = [cap - (_POST[slots[i - lag][0][0]] if i >= lag else 0.0) for i in range(-pre, nslot)]
    units = []
    for n in order:
        kind, a, c = n
        if kind == "u":
            units += [(n + (g,), 94.0, start[n], -pre) for g in range(8)]
        elif kind == "g":
            units += [(n + (g,), 150.0, start[n], -pre) for g in range(8)]
        elif kind in "ic":
            src_ = [start[m] for m in (("u", a, c), ("k", a, c)) if m in start]
            for t in range(16):
                rel = max(max(src_) + 16, max(src_) + t + lag + 3) if src_ else -pre
                units.append((n + (t,), 32.0 * a + 48.0, nslot if kind == 'c' else start[n], rel))

    def simulate(util):
        left = [u[1] for u in units]
        done = [None] * len(units)
        for i in range(-pre, nslot):
            budget = util * free[i + pre]
            for j, u in enumerate(units):
                if budget <= 0.0:
                    break
                if done[j] is None and u[3] <= i:
                    use = min(budget, left[j])
                    left[j] -= use
                    budget -= use
                    if left[j] <= 1e-9:
                        done[j] = i + 1
        ok = all(u[2] < 8 or (d is not None and d <= max(u[2] - (1 if u[0][0] in 'cg' else margin), u[3] + 1))
                 for d, u in zip(done, units))
        return done, ok

    lo_, hi_ = 0.05, maxutil
    for _ in range(12):
        mid = 0.5 * (lo_ + hi_)
        if simulate(mid)[1]:
            hi_ = mid
        else:
            lo_ = mid
    done, _ = simulate(hi_)
    plan = {}
    for u, d in zip(units, done):
        if u[0][0] == "c":
            plan[u[0]] = slots[max((nslot - 1 if d is None else min(d, nslot - 1)) - lag, 0)]
        elif d is not None and 0 <= d < u[2]:
            plan.setdefault(slots[d], []).append(u[0])
    return plan


def _pack(x):
    return pltpu.bitcast(x.astype(BF16), U32)


def _unpack(w):
    return pltpu.bitcast(w, BF16)


def _dot(a, b):
    return jnp.dot(a, b, preferred_element_type=F32)


def _dot_nt(a, b):
    return jax.lax.dot_general(a, b, (((1,), (1,)), ((), ())), preferred_element_type=F32)


def _dot_fine(x, w, chunk, nt=False):
    if not chunk:
        return _dot_nt(x, w) if nt else _dot(x, w)
    n = w.shape[0] if nt else w.shape[1]
    head, last = (w[:n - 128], w[n - 128:]) if nt else (w[:, :n - 128], w[:, n - 128:])
    f = _dot_nt if nt else _dot
    parts = [f(x, head)] if n > 128 else []
    parts.append(jnp.concatenate([f(x[r:r + chunk], last) for r in range(0, x.shape[0], chunk)], axis=0))
    return jnp.concatenate(parts, axis=1)


def _lo(w):
    return pltpu.bitcast(w << 16, F32)


def _hi(w):
    return pltpu.bitcast(w & jnp.uint32(0xFFFF0000), F32)


def _ln_stats(x):
    m = jnp.sum(x, axis=-1, keepdims=True) * (1.0 / D)
    xc = x - m
    v = jnp.sum(xc * xc, axis=-1, keepdims=True) * (1.0 / D)
    return xc, jnp.exp(-0.5 * jnp.log(v + EPS))


def _ln(x):
    xc, r = _ln_stats(x)
    return xc * r


def _spread(tokens, lo, hi):
    out = {}
    for i, t in enumerate(tokens):
        out.setdefault(lo + (i * (hi - lo)) // len(tokens), []).append(t)
    return out


def _gelu(x):
    c0 = 0.7978845608028654
    c1 = c0 * 0.044715
    z = x * (c0 + c1 * (x * x))
    hx = 0.5 * x
    return hx + hx * jnp.tanh(z)


def _bfly(tr, ti, sign):
    s02r, s02i = tr[0] + tr[2], ti[0] + ti[2]
    d02r, d02i = tr[0] - tr[2], ti[0] - ti[2]
    s13r, s13i = tr[1] + tr[3], ti[1] + ti[3]
    d13r, d13i = tr[1] - tr[3], ti[1] - ti[3]
    x0r, x0i = s02r + s13r, s02i + s13i
    x2r, x2i = s02r - s13r, s02i - s13i
    ar, ai = d02r + d13i, d02i - d13r
    br, bi = d02r - d13i, d02i + d13r
    if sign < 0:
        return [x0r, ar, x2r, br], [x0i, ai, x2i, bi]
    return [x0r, br, x2r, ar], [x0i, bi, x2i, ai]


def _kernel(q_hbm, k_hbm, v_hbm, shift_hbm, ssmk_hbm, ssmd_hbm, w1_hbm, w2_hbm, w3t_hbm, w4_hbm,
            c_hbm, wmod_hbm,
            out_hbm,
            kbuf, vbuf, skbuf, fwdbuf, invbuf, permbuf,
            wmodbuf, w1buf, w2buf, w3buf, w4buf, qbuf,
            xs0, xs1, xs2, xs3, xs4, kraw, wbuf, zbuf, coefbuf, ybuf, modbuf, x2buf, hbuf, hhbuf, xnbuf, obuf, shiftbuf, dbuf, cbuf,
            sem_in, sem_out):
    cps = {}
    n_sem = [0]

    def start(name, src, dst):
        cp = pltpu.make_async_copy(src, dst, sem_in.at[n_sem[0]])
        n_sem[0] += 1
        cp.start()
        cps[name] = cp

    CH = P * NC
    HALO = 8 * NC

    def start_s(a):
        cols = pl.ds(a * P, P)
        start("s%d" % a, ssmk_hbm.at[:, cols], skbuf.at[:, cols])

    def start_kv(a):
        if a == 0:
            start("k0", k_hbm.at[pl.ds(0, CH), :], kbuf.at[0, pl.ds(HALO, CH), :])
        else:
            start("k%d" % a, k_hbm.at[pl.ds(a * CH - HALO, CH + HALO), :], kbuf.at[a, pl.ds(0, CH + HALO), :])
        start("v%d" % a, v_hbm.at[pl.ds(a * CH, CH), :], vbuf.at[a, pl.ds(0, CH), :])

    for n in "s0 x0 s1 k0 k1 s2 k2 s3 k3".split():
        if n[0] == "s":
            start_s(int(n[1]))
        elif n[0] == "k":
            start_kv(int(n[1]))
        else:
            start("d", ssmd_hbm, dbuf)
            start("shift", shift_hbm, shiftbuf)
            start("c", c_hbm, cbuf)
    QA = TS + LEAD
    XA = 128
    QB = 2 * TS + LEAD
    start("qa", q_hbm.at[pl.ds(0, QA + XA), :], qbuf.at[pl.ds(0, QA + XA), :])
    start("wmoda", wmod_hbm.at[:, pl.ds(0, 3 * D)], wmodbuf.at[:, pl.ds(0, 3 * D)])
    start("wmodb", wmod_hbm.at[:, pl.ds(3 * D, 2 * D)], wmodbuf.at[:, pl.ds(3 * D, 2 * D)])
    start("w1", w1_hbm, w1buf)
    start("qb", q_hbm.at[pl.ds(QA + XA, QB - QA - XA), :], qbuf.at[pl.ds(QA + XA, QB - QA - XA), :])
    start("w2", w2_hbm, w2buf)
    start("w3", w3t_hbm, w3buf)
    start("w4", w4_hbm, w4buf)
    start("wmodg", wmod_hbm.at[:, pl.ds(5 * D, D)], wmodbuf.at[:, pl.ds(5 * D, D)])
    start("q1", q_hbm.at[pl.ds(QB, S - QB), :], qbuf.at[pl.ds(QB, S - QB), :])

    kw = kbuf.bitcast(U32)
    vw = vbuf.bitcast(U32)
    kbuf[0, pl.ds(0, HALO), :] = jnp.zeros((HALO, 128), BF16)
    zbuf[...] = jnp.zeros(zbuf.shape, U32)
    for c in range(NC):
        ybuf[c, pl.ds(S, LEAD), :] = jnp.zeros((LEAD, 128), F32)
        hhbuf[c, pl.ds(0, 8), :] = jnp.zeros((8, 128), F32)
    qbuf[pl.ds(S, LEAD), :] = jnp.zeros((LEAD, D), BF16)

    def tables(p, carry):
        i0 = jax.lax.broadcasted_iota(jnp.int32, (128, 128), 0)
        n = R * jax.lax.broadcasted_iota(jnp.int32, (128, 128), 1) + p
        f2, off = _freq(2 * i0)
        j = f2 * n + off
        fwdbuf[p] = pltpu.pack_elementwise([_cos(j, 1.0), _cos(j + 4 * n, 1.0)], packed_dtype=BF16)
        return carry

    jax.lax.fori_loop(0, R, tables, 0)

    def unit_g(kt, r):
        col = jax.lax.broadcasted_iota(jnp.int32, (8, 128), 1) + 128 * kt
        f2, off = _freq((col & ~15) + 8 * (col & 1) + ((col >> 1) & 7))
        m = 2 * jax.lax.broadcasted_iota(jnp.int32, (8, 128), 0) + 16 * r
        j0 = f2 * (R * m) + off
        out = []
        for p in range(R):
            j = j0 + p * f2
            out.append(pltpu.pack_elementwise([_cos(j, 1.0 / P), _cos(j + R * f2, 1.0 / P)], packed_dtype=BF16))
            invbuf[p, pl.ds(8 * r, 8), pl.ds(128 * kt, 128)] = out[-1]
        return out

    i0 = jax.lax.broadcasted_iota(jnp.int32, (128, 128), 0)
    i1 = jax.lax.broadcasted_iota(jnp.int32, (128, 128), 1)
    permbuf[...] = _pack(jnp.where(i0 == (128 // R) * (i1 & (R - 1)) + (i1 >> 2), 1.0, 0.0).astype(F32))

    def fill_coef():
        coef = shiftbuf[...].astype(F32)
        dval = dbuf[...].astype(F32)
        for c in range(NC):
            for j in range(4):
                coefbuf[c, j] = jnp.broadcast_to(coef[j:j + 1, c * 128:(c + 1) * 128], (8, 128))
            coefbuf[c, 4] = jnp.broadcast_to(dval[c:c + 1, :], (8, 128))

    xs = (xs0, xs1, xs2, xs3, xs4)
    def split_ri(t):
        t = t.reshape(16, 2, 8, 128)
        return t[:, 0], t[:, 1]

    def get_never():
        return zbuf[pl.ds(0, 8), :] != 0

    def pack2(x, y):
        return pltpu.pack_elementwise([x, y], packed_dtype=BF16)

    def words(ref, a, c, r):
        return ref[a, pl.ds((r // 4) * 4 * NC + 4 * c + r % 4, 8, stride=4 * NC), :]

    def unit_u(a, c, g):
        cj = [coefbuf[c, j] for j in range(4)]
        kk = [words(kw, a, c, 4 + 32 * g + d) for d in range(-2, 4)]
        seq = [f(w_) for w_ in kk for f in (_lo, _hi)][1:]
        vv = [words(vw, a, c, 32 * g + d) for d in range(4)]
        vs = [f(w_) for w_ in vv for f in (_lo, _hi)]
        kv = [((seq[3 + i] * cj[0] + seq[2 + i] * cj[1]) + (seq[1 + i] * cj[2] + seq[i] * cj[3])) * vs[i]
              for i in range(8)]
        return [pack2(kv[p], kv[4 + p]) for p in range(R)]

    def unit_i(a, c, t, z):
        x_c = xs[c].at[pl.ds(z, NA)]
        yr, yi = [], []
        for q in range(R):
            accr = acci = None
            for j in range(a + 1):
                ur, ui = x_c[j, q, t, 0], x_c[j, q, t, 1]
                kr, ki = x_c[a - j, q, t, 2], x_c[a - j, q, t, 3]
                pr = ur * kr - ui * ki
                pi = ur * ki + ui * kr
                accr = pr if accr is None else accr + pr
                acci = pi if acci is None else acci + pi
            yr.append(accr)
            yi.append(acci)
        wr, wi = _bfly(yr, yi, +1)
        return [pack2(wr[p], wi[p]) for p in range(R)]

    def segment(spec, z, maxutil=1.0, mod_fn=None):
        order = [(n[0], int(n[1]), int(n[2])) for n in spec.split()]
        plan = _plan_tokens(order, maxutil) if maxutil > 0 else {}
        never = get_never()
        units, res = {}, {}

        def unit(key):
            if key not in units:
                kind, a, c, j = key
                if kind == "u":
                    units[key] = unit_u(a, c, j)
                elif kind == "g":
                    units[key] = unit_g(a, j)
                else:
                    fresh = ("u", a, c) in order or ("k", a, c) in order
                    units[key] = unit_i(a, c, j, z if fresh else 0)
            return units[key]

        def lhs(name, p, rows, r0=0):
            out = []
            for r, v in enumerate(rows):
                for key in plan.get((name, r0 + r), ()):
                    v = jnp.where(never, unit(key)[p], v)
                out.append(v)
            return jnp.concatenate(out, axis=0)

        def dft(name, rhs):
            tr, ti = [], []
            for p in range(R):
                f = lhs(name, p, [fwdbuf[p, pl.ds(8 * r, 8), :] for r in range(16)])
                r_, i_ = split_ri(_dot(_unpack(f), rhs[p]))
                if p == 0:
                    res.update({(name, r): r_[r] for r in range(16)})
                tr.append(r_)
                ti.append(i_)
            return _bfly(tr, ti, -1)

        st = {}
        for name in order:
            kind, a, c = name
            x_c = xs[c]
            if kind == "g":
                for r in range(8):
                    unit(name + (r,))
            elif kind == "c":
                for t in range(16):
                    after = pltpu.bitcast(res[plan[name + (t,)]], U32)
                    for p in range(R):
                        wbuf[c, p, pl.ds(8 * t, 8), :] = jnp.where(never, after, unit(name + (t,))[p])
            elif kind == "m":
                toks = {}
                for r in range(_DUR["m"]):
                    for n_, key in enumerate(plan.get((name, r), ())):
                        toks.setdefault(2 * r + n_ % 2, []).extend(unit(key))
                mod_fn(a, toks)
            elif kind == "t":
                trs = []
                for b in range(R):
                    pm = lhs(name, b, [permbuf[pl.ds(8 * r, 8), :] for r in range(8)])
                    trs.append(_dot_nt(_unpack(pm), skbuf[pl.ds(c * 128, 128), pl.ds(a * P + b * 128, 128)]))
                res.update({(name, r): trs[0][16 * r:16 * r + 8] for r in range(8)})
                g_ = 128 // R
                st[a, c] = [jnp.concatenate([trs[b][p * g_:(p + 1) * g_] for b in range(R)], axis=0).astype(BF16)
                            for p in range(R)]
            elif kind == "u":
                rhs = [_unpack(jnp.concatenate([unit(name + (g,))[p] for g in range(8)], axis=0)) for p in range(R)]
                xr, xi = dft(name, rhs)
                for q in range(R):
                    x_c[a, q, :, 0] = xr[q]
                    x_c[a, q, :, 1] = xi[q]
            elif kind == "k":
                xr, xi = dft(name, st[a, c])
                for q in range(R):
                    if a == 0:
                        x_c[a, q, :, 2] = xr[q] + coefbuf[c, 4]
                        x_c[a, q, :, 3] = xi[q]
                    else:
                        pr, pi = kraw[c, a - 1, q, :, 0], kraw[c, a - 1, q, :, 1]
                        x_c[a, q, pl.ds(0, 8), 2] = xr[q][:8] - pi[:8]
                        x_c[a, q, pl.ds(0, 8), 3] = xi[q][:8] + pr[:8]
                        x_c[a, q, pl.ds(8, 8), 2] = xr[q][8:] + pi[8:]
                        x_c[a, q, pl.ds(8, 8), 3] = xi[q][8:] - pr[8:]
                    if a + 1 < NA:
                        kraw[c, a, q, :, 0] = xr[q]
                        kraw[c, a, q, :, 1] = xi[q]
            else:
                for p in range(R):
                    cols = [lhs(name, 2 * (p % 2) + kt,
                                [invbuf[p, pl.ds(8 * r, 8), pl.ds(128 * kt, 128)] for r in range(8)], 8 * (p // 2))
                            for kt in range(2)]
                    g = _unpack(jnp.concatenate(cols, axis=1))
                    if kind == "j":
                        wp = _unpack(wbuf[c, p])
                    else:
                        wp = _unpack(jnp.concatenate([unit(name + (t,))[p] for t in range(16)], axis=0))
                    yp = _dot(g, wp)
                    if p % 2 == 0:
                        res.update({(name, 4 * p + r): yp[16 * r:16 * r + 8] for r in range(8)})
                    ybuf[c, pl.ds(a * P + p, 128, stride=R), :] = yp

    one = jnp.minimum(pl.program_id(0) + 1, 1)

    def once(fn):
        def body(z, carry):
            fn(z)
            return carry
        jax.lax.fori_loop(0, one, body, 0)

    default = "t00 t01 t02 k00 t03 k01 t04 k02 k03 k04 g00|t10 t11 t12 k10 k11 k12 g10|t13 t14 k13 u00 k14 u01 u02 u03 i00 u04 i01 c02 c03|j02 j03 u10 i04 u11 u12 u13 i10 u14 i11 c12|t20 t21 j12 t22 t23 t24 k20 u20 k21 u21 k22 i13 k23 u22 k24 i14 u23 i20 u24 i21 c22|t30 t31 j22 t32 t33 t34 k30 u30 k31 u31 k32 i23 k33 u32 k34 i24 u33 i30 u34 i31 c32|m00 j32 m10 m20 i33 i34"
    specs = default.split("|")
    G5B = specs[-1]
    segs = list(zip("s0 d shift c|s1|k0 v0|k1 v1|s2 k2 v2|s3 k3 v3".split("|"), specs[:-1]))
    MU = 1.5
    for i, (waits, spec) in enumerate(segs):
        with jax.named_scope("g%d" % i):
            for n in waits.split():
                cps[n].wait()
            if i == 0:
                fill_coef()
            once(lambda z: segment(spec, z, MU))

    def mod_cols(lo, n, toks=None):
        cv = cbuf[...].astype(F32)
        sc = (cv * jax.nn.sigmoid(cv)).astype(BF16)
        m = _dot(jnp.broadcast_to(sc, (8, D)), weights(wmodbuf, toks, lo * NC, (lo + n) * NC))
        return [m[:, j * D:(j + 1) * D] for j in range(n)]

    def mul_mod(x, j, cols=None):
        m = modbuf[j] if cols is None else modbuf[j, :, cols]
        return (x.reshape(-1, 8, x.shape[-1]) * m[None]).reshape(x.shape)

    def add_mod(x, j):
        return (x.reshape(-1, 8, x.shape[-1]) + modbuf[j][None]).reshape(x.shape)

    def slabs(ref, r0, n):
        return jnp.concatenate([ref[c, pl.ds(r0, n), :] for c in range(NC)], axis=1)

    def window(base, n):
        rows = pl.ds(base, n)
        return dict(q=qbuf.at[rows, :], y=ybuf.at[:, rows, :], x2=x2buf.at[rows, :], h=hbuf.at[rows, :],
                    hh=hhbuf.at[:, pl.ds(base, n + 8), :], xn=xnbuf.at[pl.ds(base, n - LEAD), :],
                    o=obuf.at[pl.ds(base, n - LEAD), :])

    def weights(ref, toks, c0=0, c1=None, nt=False):
        nrow = ref.shape[0]
        c1 = ref.shape[1] // 128 if c1 is None else c1
        if not toks:
            return ref[:, pl.ds(c0 * 128, (c1 - c0) * 128)]
        never = get_never()
        rt = -(-nrow // 128)
        cols = []
        for j in range(c0, c1):
            wu = pltpu.bitcast(ref[:, pl.ds(j * 128, 128)], U32)
            parts, last = [], 0
            for i in range(rt):
                pos = i * (c1 - c0) + (j - c0) if nt else (j - c0) * rt + i
                for n_, t in enumerate(toks.get(pos, ())):
                    r = 64 * i + 8 * n_
                    if r > last:
                        parts.append(wu[last:r])
                    parts.append(jnp.where(never, t, wu[r:r + 8]))
                    last = r + 8
            parts.append(wu[last:])
            cols.append(pltpu.bitcast(jnp.concatenate(parts, axis=0), BF16))
        return jnp.concatenate(cols, axis=1)

    def row_tokens(r):
        return [pltpu.bitcast(jnp.broadcast_to(r[i:i + 8], (8, 128)), U32) for i in range(0, r.shape[0], 8)]

    def stage_a0(w, r0, n):
        rows = pl.ds(r0, n)
        x = w["q"][rows, :].astype(F32)
        y = slabs(w["y"], r0, n)
        x2 = x + add_mod(mul_mod(_ln(x), 1), 0) * y
        w["x2"][rows, :] = x2
        return _ln(x2)

    def stage_a1(w, r0, n, n2=None):
        if n2 is None:
            n2 = stage_a0(w, r0, n)
        h = add_mod(mul_mod(n2, 4), 3)
        w["h"][pl.ds(r0, n), :] = h
        hc, r = _ln_stats(h)
        return (hc * r).astype(BF16), row_tokens(r)

    def stage_a2(w, n3, r0, n, last_valid=None, fine=0):
        hh = _gelu(_dot_fine(n3, w1buf[...], fine))
        for c in range(NC):
            blk = hh[:, c * 128:(c + 1) * 128]
            w["hh"][c, pl.ds(r0 + 8, n - LEAD), :] = blk[:n - LEAD]
            tail = blk[n - LEAD:]
            if last_valid is not None:
                tail = jnp.where(last_valid, tail, 0.0)
            w["hh"][c, pl.ds(r0 + 8 + n - LEAD, LEAD), :] = tail

    def stage_b1a(w, r0, n, fine=0):
        rows = pl.ds(r0, n)
        lane = jax.lax.broadcasted_iota(jnp.int32, (n, 128), 1)

        def sh(c, d):
            return w["hh"][c, pl.ds(r0 + 8 + d, n), :]

        g = [sh(0, -1),
             jnp.where(lane < 32, sh(1, -1), sh(1, 1)),
             jnp.where(lane < 64, sh(2, 1), sh(2, -2)),
             jnp.where(lane < 96, sh(3, -2), sh(3, 2)),
             sh(4, 2)]
        hs = _dot_fine(jnp.concatenate(g, axis=1).astype(BF16), w2buf[...], fine)
        x1 = w["h"][rows, :] + hs
        w["h"][rows, :] = x1
        return x1

    def stage_b1b(w, x1, r0, n):
        w["xn"][pl.ds(r0, n), :] = _ln(x1).astype(BF16)

    def stage_b1(w, r0, n):
        stage_b1b(w, stage_b1a(w, r0, n), r0, n)

    def out_copy(r0):
        rows = pl.ds(r0, TS)
        return pltpu.make_async_copy(obuf.at[rows, :], out_hbm.at[rows, :], sem_out.at[0])

    FM = (FF // 128) * 128
    FR = FF - FM

    def stage_b2a(w, r0, n=TS, fine=0):
        xn = w["xn"][pl.ds(r0, n), :]
        ht = _gelu(_dot_nt(w3buf[pl.ds(FM, FR), :], xn))
        h3 = _gelu(_dot_fine(xn, w3buf[pl.ds(0, FM), :], fine, nt=True)).astype(BF16)
        hl = jnp.concatenate([ht[:, j * 128:(j + 1) * 128] for j in range(n // 128)], axis=0)
        hl = [hl[j * 128:(j + 1) * 128].T.astype(BF16) for j in range(n // 256)]
        return h3, hl

    def stage_b2b(w, hh3, r0, c0, c1, n=TS, defer=False, fine=0):
        h3, hl = hh3
        rows = pl.ds(r0, n)
        cols = pl.ds(c0 * 128, (c1 - c0) * 128)
        wl = w4buf[pl.ds(FM, FR), cols]
        z = jnp.zeros_like(wl)
        wlo, whi = jnp.concatenate([wl, z], axis=0), jnp.concatenate([z, wl], axis=0)
        rest = jnp.concatenate([_dot(h, wz) for h in hl for wz in (wlo, whi)], axis=0)
        h2 = _dot_fine(h3, w4buf[pl.ds(0, FM), cols], fine) + rest
        if defer:
            w["h"][rows, cols] = w["h"][rows, cols] + h2
        else:
            finish(w, w["h"][rows, cols] + h2, rows, cols)

    def finish(w, v, rows, cols):
        w["o"][rows, cols] = (w["x2"][rows, cols] + mul_mod(v, 5, cols)).astype(BF16)

    w = window(0, 2 * TS + LEAD)
    H = TS // 2
    with jax.named_scope("t0a"):
        cps["qa"].wait()
        cps["wmoda"].wait()

        mv = {}

        def mod_fn(j, toks):
            mv[j] = mod_cols(j, 1, toks)[0]
            if len(mv) == 3:
                modbuf[0] = mv[2] * mv[0]
                modbuf[1] = mv[2] * (1.0 + mv[1])

        segment(G5B, 0, MU, mod_fn=mod_fn)
        w["h"][pl.ds(0, QA), :] = stage_a0(w, 0, QA)
    with jax.named_scope("t0b"):
        cps["wmodb"].wait()
        sb, cb = mod_cols(3, 2)
        modbuf[3] = sb
        modbuf[4] = 1.0 + cb
        n3, _ = stage_a1(w, 0, QA, n2=w["h"][pl.ds(0, QA), :])
    XB = TS - XA
    FN = 32
    F4 = 64
    LNPOS = "t3"
    T4S = 2
    with jax.named_scope("t1"):
        cps["w1"].wait()
        n3a, _ = stage_a1(w, QA, XA)
        stage_a2(w, n3, 0, QA)
        stage_a2(w, n3a, QA, XA, fine=FN)
    with jax.named_scope("t2"):
        cps["qb"].wait()
        cps["w2"].wait()
        n3b, _ = stage_a1(w, QA + XA, XB)
        stage_b1(w, 0, TS)
        stage_a2(w, n3b, QA + XA, XB)
        stage_b1(w, TS, XA)
        stage_b1a(w, TS + XA, XB, fine=FN)
    with jax.named_scope("t3"):
        cps["w3"].wait()
        if LNPOS == "t3":
            stage_b1b(w, w["h"][pl.ds(TS + XA, XB), :], TS + XA, XB)
        h3 = stage_b2a(w, 0, fine=64)
    with jax.named_scope("t4a"):
        cps["w4"].wait()
        if LNPOS == "t4a":
            stage_b1b(w, w["h"][pl.ds(TS + XA, XB), :], TS + XA, XB)
        stage_b2b(w, h3, 0, 0, T4S, defer=True, fine=F4)
    with jax.named_scope("t4b"):
        cps["wmodg"].wait()
        if LNPOS == "t4b":
            stage_b1b(w, w["h"][pl.ds(TS + XA, XB), :], TS + XA, XB)
        modbuf[5] = mod_cols(5, 1)[0]
        rows, cols = pl.ds(0, TS), pl.ds(0, T4S * 128)
        finish(w, w["h"][rows, cols], rows, cols)
        stage_b2b(w, h3, 0, T4S, 5, fine=F4)
        out_copy(0).start()
        cps["q1"].wait()

    NSUB = 4

    def step(s, carry):
        r0 = pl.multiple_of(s * TS, TS)
        w = window(r0, 2 * TS + LEAD)
        h3 = stage_b2a(w, 0)
        sub = TS // NSUB
        for j in range(NSUB):
            if j > 0:
                stage_b2b(w, h3, 0, j - 1, j)
            ra = TS + LEAD + j * sub
            stage_a2(w, stage_a1(w, ra, sub)[0], ra, sub, last_valid=(s < NT - 2) if j == NSUB - 1 else None)
        stage_b2b(w, h3, 0, 3, 4)
        stage_b1(w, TS, TS)
        stage_b2b(w, h3, 0, 4, 5)
        out_copy(r0).start()
        return carry

    with jax.named_scope("p2main"):
        jax.lax.fori_loop(1, NT - 1, step, 0)
    with jax.named_scope("p2epi"):
        w = window((NT - 2) * TS, 2 * TS + LEAD)
        h3 = stage_b2a(w, TS)
        rows = pl.ds((NT - 1) * TS, TS)
        for c0, c1 in ((0, 2), (2, 4), (4, 5)):
            stage_b2b(w, h3, TS, c0, c1)
            cols = pl.ds(c0 * 128, (c1 - c0) * 128)
            pltpu.make_async_copy(obuf.at[rows, cols], out_hbm.at[rows, cols], sem_out.at[0]).start()
        pltpu.make_async_copy(obuf, out_hbm, sem_out.at[0]).wait()


@jax.jit
def pallas_adaLN_cond__ssm_conv_h3__mixer_s_mlp__prompt_kernel(
    A_q: jax.Array,
    A_k: jax.Array,
    A_v: jax.Array,
    A_shift_k: jax.Array,
    A_ssm_k: jax.Array,
    A_ssm_D: jax.Array,
    B_x: jax.Array,
    B_w1: jax.Array,
    B_w2: jax.Array,
    B_w3: jax.Array,
    B_w4: jax.Array,
    c: jax.Array,
    w_mod: jax.Array,
):
    del B_x

    def tiles(x):
        return x.reshape(S // 8, 8, NC, 128).transpose(0, 2, 1, 3).reshape(S * NC, 128)

    args = (
        A_q.reshape(S, D), tiles(A_k), tiles(A_v),
        A_shift_k.T, A_ssm_k, A_ssm_D.reshape(NC, 128),
        B_w1, B_w2, B_w3.T, B_w4, c, w_mod,
    )
    scratch = [
        pltpu.VMEM((NA, P * NC + 128, 128), BF16),
        pltpu.VMEM((NA, P * NC + 64, 128), BF16),
        pltpu.VMEM((D, S), BF16),
        pltpu.VMEM((R, 128, 128), U32),
        pltpu.VMEM((R, 64, 256), U32),
        pltpu.VMEM((64, 128), U32),
        pltpu.VMEM((D, 6 * D), BF16),
        pltpu.VMEM((D, D), BF16),
        pltpu.VMEM((D, D), BF16),
        pltpu.VMEM((FF, D), BF16),
        pltpu.VMEM((FF, D), BF16),
        pltpu.VMEM((S + 64, D), BF16),
        *[pltpu.VMEM((NA, R, 16, 4, 8, 128), F32) for _ in range(NC)],
        pltpu.VMEM((NC, NA - 1, R, 16, 2, 8, 128), F32),
        pltpu.VMEM((NC, R, 128, 128), U32),
        pltpu.VMEM((32, 128), U32),
        pltpu.VMEM((NC, 8, 8, 128), F32),
        pltpu.VMEM((NC, S + 32, 128), F32),
        pltpu.VMEM((8, 8, D), F32),
        pltpu.VMEM((S + 32, D), F32),
        pltpu.VMEM((S + 32, D), F32),
        pltpu.VMEM((NC, S + 32, 128), F32),
        pltpu.VMEM((S, D), BF16),
        pltpu.VMEM((S, D), BF16),
        pltpu.VMEM((4, D), BF16),
        pltpu.VMEM((NC, 128), BF16),
        pltpu.VMEM((1, D), BF16),
        pltpu.SemaphoreType.DMA((32,)),
        pltpu.SemaphoreType.DMA((1,)),
    ]
    out = pl.pallas_call(
        _kernel,
        out_shape=jax.ShapeDtypeStruct((S, D), BF16),
        in_specs=[pl.BlockSpec(memory_space=pl.ANY)] * len(args),
        out_specs=pl.BlockSpec(memory_space=pl.ANY),
        scratch_shapes=scratch,
        grid=(1,),
        compiler_params=pltpu.CompilerParams(vmem_limit_bytes=100 * 1024 * 1024, disable_semaphore_checks=True,
                                             disable_bounds_checks=True),
        name="adaln_h3_mixer",
    )(*args)
    return out.reshape(1, S, D)
```

```python
import numpy as np
import jax
import jax.numpy as jnp
import jax.experimental.pallas as pl
import jax.experimental.pallas.tpu as pltpu

F32 = jnp.float32
BF16 = jnp.bfloat16
U32 = jnp.uint32

S = 2048
D = 640
FF = 1728
NC = D // 128
R = 4
P = 128 * R
NA = S // P
TS = 256
NT = S // TS
LEAD = 16
EPS = 1e-5
P1_ORDER = "t0 t1 t2 t3 k0 k1 k2 k3 u0 i0 u1 i1 u2 i2 u3 i3"


def _freq(row):
    t, part, s = row >> 4, (row >> 3) & 1, row & 7
    return 32 * (t & 7) + 4 * s + 2 * (t >> 3) + 1, P * part


def _cos(j, scale):
    jf = (j & (4 * P - 1)).astype(F32)
    u = 2.0 * np.pi / (4 * P)
    x = jnp.abs(jf * u - np.pi) - 0.5 * np.pi
    x2 = x * x
    poly = scale / 362880.0 - x2 * (scale / 39916800.0)
    for coef in (-1.0 / 5040.0, 1.0 / 120.0, -1.0 / 6.0, 1.0):
        poly = poly * x2 + coef * scale
    return poly * x


_DUR = {"t": 8, "u": 16, "k": 16, "i": 16, "m": 12, "g": 0, "c": 0, "j": 16}
_POST = {"t": 8.0, "u": 16.0, "k": 24.0, "i": 4.0, "j": 4.0, "m": 18.0}


def _plan_tokens(order, maxutil):
    lag, cap, pre, margin = 8, 60, 4, 3
    start, slots = {}, []
    for n in order:
        start[n] = len(slots)
        slots += [(n, r) for r in range(_DUR[n[0]])]
    nslot = len(slots) + lag
    free = [cap - (_POST[slots[i - lag][0][0]] if i >= lag else 0.0) for i in range(-pre, nslot)]
    units = []
    for n in order:
        kind, a, c = n
        if kind == "u":
            units += [(n + (g,), 94.0, start[n], -pre) for g in range(8)]
        elif kind == "g":
            units += [(n + (g,), 150.0, start[n], -pre) for g in range(8)]
        elif kind in "ic":
            src_ = [start[m] for m in (("u", a, c), ("k", a, c)) if m in start]
            for t in range(16):
                rel = max(max(src_) + 16, max(src_) + t + lag + 3) if src_ else -pre
                units.append((n + (t,), 32.0 * a + 48.0, nslot if kind == 'c' else start[n], rel))

    def simulate(util):
        left = [u[1] for u in units]
        done = [None] * len(units)
        for i in range(-pre, nslot):
            budget = util * free[i + pre]
            for j, u in enumerate(units):
                if budget <= 0.0:
                    break
                if done[j] is None and u[3] <= i:
                    use = min(budget, left[j])
                    left[j] -= use
                    budget -= use
                    if left[j] <= 1e-9:
                        done[j] = i + 1
        ok = all(u[2] < 8 or (d is not None and d <= max(u[2] - (1 if u[0][0] in 'cg' else margin), u[3] + 1))
                 for d, u in zip(done, units))
        return done, ok

    lo_, hi_ = 0.05, maxutil
    for _ in range(12):
        mid = 0.5 * (lo_ + hi_)
        if simulate(mid)[1]:
            hi_ = mid
        else:
            lo_ = mid
    done, _ = simulate(hi_)
    plan = {}
    for u, d in zip(units, done):
        if u[0][0] == "c":
            plan[u[0]] = slots[max((nslot - 1 if d is None else min(d, nslot - 1)) - lag, 0)]
        elif d is not None and 0 <= d < u[2]:
            plan.setdefault(slots[d], []).append(u[0])
    return plan


def _pack(x):
    return pltpu.bitcast(x.astype(BF16), U32)


def _unpack(w):
    return pltpu.bitcast(w, BF16)


def _dot(a, b):
    return jnp.dot(a, b, preferred_element_type=F32)


def _dot_nt(a, b):
    return jax.lax.dot_general(a, b, (((1,), (1,)), ((), ())), preferred_element_type=F32)


def _dot_fine(x, w, chunk, nt=False):
    if not chunk:
        return _dot_nt(x, w) if nt else _dot(x, w)
    n = w.shape[0] if nt else w.shape[1]
    head, last = (w[:n - 128], w[n - 128:]) if nt else (w[:, :n - 128], w[:, n - 128:])
    f = _dot_nt if nt else _dot
    parts = [f(x, head)] if n > 128 else []
    parts.append(jnp.concatenate([f(x[r:r + chunk], last) for r in range(0, x.shape[0], chunk)], axis=0))
    return jnp.concatenate(parts, axis=1)


def _lo(w):
    return pltpu.bitcast(w << 16, F32)


def _hi(w):
    return pltpu.bitcast(w & jnp.uint32(0xFFFF0000), F32)


def _ln_stats(x):
    m = jnp.sum(x, axis=-1, keepdims=True) * (1.0 / D)
    xc = x - m
    v = jnp.sum(xc * xc, axis=-1, keepdims=True) * (1.0 / D)
    return xc, jnp.exp(-0.5 * jnp.log(v + EPS))


def _ln(x):
    xc, r = _ln_stats(x)
    return xc * r


def _gelu(x):
    c0 = 0.7978845608028654
    c1 = c0 * 0.044715
    z = x * (c0 + c1 * (x * x))
    hx = 0.5 * x
    return hx + hx * jnp.tanh(z)


def _bfly(tr, ti, sign):
    s02r, s02i = tr[0] + tr[2], ti[0] + ti[2]
    d02r, d02i = tr[0] - tr[2], ti[0] - ti[2]
    s13r, s13i = tr[1] + tr[3], ti[1] + ti[3]
    d13r, d13i = tr[1] - tr[3], ti[1] - ti[3]
    x0r, x0i = s02r + s13r, s02i + s13i
    x2r, x2i = s02r - s13r, s02i - s13i
    ar, ai = d02r + d13i, d02i - d13r
    br, bi = d02r - d13i, d02i + d13r
    if sign < 0:
        return [x0r, ar, x2r, br], [x0i, ai, x2i, bi]
    return [x0r, br, x2r, ar], [x0i, bi, x2i, ai]


def _kernel(q_hbm, k_hbm, v_hbm, shift_hbm, ssmk_hbm, ssmd_hbm, w1_hbm, w2_hbm, w3t_hbm, w4_hbm,
            c_hbm, wmod_hbm,
            out_hbm,
            kbuf, vbuf, skbuf, fwdbuf, invbuf, permbuf,
            wmodbuf, w1buf, w2buf, w3buf, w4buf, qbuf,
            xs0, xs1, xs2, xs3, xs4, kraw, wbuf, zbuf, coefbuf, ybuf, modbuf, x2buf, hbuf, hhbuf, xnbuf, obuf, shiftbuf, dbuf, cbuf,
            sem_in, sem_out):
    cps = {}
    n_sem = [0]

    def start(name, src, dst):
        cp = pltpu.make_async_copy(src, dst, sem_in.at[n_sem[0]])
        n_sem[0] += 1
        cp.start()
        cps[name] = cp

    class Both:
        def __init__(self, a, b):
            self.cps = (a, b)

        def wait(self):
            for cp in self.cps:
                cp.wait()

    def start_w(name, src, dst, c0=0, n=NC):
        for e in range(2):
            start(name + str(e), src.at[:, e, pl.ds(c0, n)], dst.at[:, pl.ds(c0, n), pl.ds(8 * e, 8), :])
        cps[name] = Both(cps[name + "0"], cps[name + "1"])

    CH = P * NC
    HALO = 8 * NC

    def start_s(a):
        cols = pl.ds(a * P, P)
        start("s%d" % a, ssmk_hbm.at[:, cols], skbuf.at[:, cols])

    def start_kv(a):
        if a == 0:
            start("k0", k_hbm.at[pl.ds(0, CH), :], kbuf.at[0, pl.ds(HALO, CH), :])
        else:
            start("k%d" % a, k_hbm.at[pl.ds(a * CH - HALO, CH + HALO), :], kbuf.at[a, pl.ds(0, CH + HALO), :])
        start("v%d" % a, v_hbm.at[pl.ds(a * CH, CH), :], vbuf.at[a, pl.ds(0, CH), :])

    for n in "s0 x0 s1 k0 k1 s2 k2 s3 k3".split():
        if n[0] == "s":
            start_s(int(n[1]))
        elif n[0] == "k":
            start_kv(int(n[1]))
        else:
            start("d", ssmd_hbm, dbuf)
            start("shift", shift_hbm, shiftbuf)
            start("c", c_hbm, cbuf)
    QA = TS + LEAD
    XA = 128
    QB = 2 * TS + LEAD
    start("qa", q_hbm.at[pl.ds(0, QA + XA), :], qbuf.at[pl.ds(0, QA + XA), :])
    start_w("wmoda", wmod_hbm, wmodbuf, 0, 3 * NC)
    start_w("wmodb", wmod_hbm, wmodbuf, 3 * NC, 2 * NC)
    start_w("w1", w1_hbm, w1buf)
    start("qb", q_hbm.at[pl.ds(QA + XA, QB - QA - XA), :], qbuf.at[pl.ds(QA + XA, QB - QA - XA), :])
    start_w("w2", w2_hbm, w2buf)
    start_w("w3", w3t_hbm, w3buf)
    start_w("w4", w4_hbm, w4buf)
    start_w("wmodg", wmod_hbm, wmodbuf, 5 * NC, NC)
    start("q1", q_hbm.at[pl.ds(QB, S - QB), :], qbuf.at[pl.ds(QB, S - QB), :])

    kw = kbuf.bitcast(U32)
    vw = vbuf.bitcast(U32)
    kbuf[0, pl.ds(0, HALO), :] = jnp.zeros((HALO, 128), BF16)
    zbuf[...] = jnp.zeros(zbuf.shape, U32)
    for c in range(NC):
        ybuf[c, pl.ds(S, LEAD), :] = jnp.zeros((LEAD, 128), F32)
        hhbuf[c, pl.ds(0, 8), :] = jnp.zeros((8, 128), F32)
    qbuf[pl.ds(S, LEAD), :] = jnp.zeros((LEAD, D), BF16)

    def tables(p, carry):
        i0 = jax.lax.broadcasted_iota(jnp.int32, (128, 128), 0)
        n = R * jax.lax.broadcasted_iota(jnp.int32, (128, 128), 1) + p
        f2, off = _freq(2 * i0)
        j = f2 * n + off
        fwdbuf[p] = pltpu.pack_elementwise([_cos(j, 1.0), _cos(j + 4 * n, 1.0)], packed_dtype=BF16)
        return carry

    jax.lax.fori_loop(0, R, tables, 0)

    def unit_g(kt, r):
        col = jax.lax.broadcasted_iota(jnp.int32, (8, 128), 1) + 128 * kt
        f2, off = _freq((col & ~15) + 8 * (col & 1) + ((col >> 1) & 7))
        m = 2 * jax.lax.broadcasted_iota(jnp.int32, (8, 128), 0) + 16 * r
        j0 = f2 * (R * m) + off
        out = []
        for p in range(R):
            j = j0 + p * f2
            out.append(pltpu.pack_elementwise([_cos(j, 1.0 / P), _cos(j + R * f2, 1.0 / P)], packed_dtype=BF16))
            invbuf[p, pl.ds(8 * r, 8), pl.ds(128 * kt, 128)] = out[-1]
        return out

    i0 = jax.lax.broadcasted_iota(jnp.int32, (128, 128), 0)
    i1 = jax.lax.broadcasted_iota(jnp.int32, (128, 128), 1)
    permbuf[...] = _pack(jnp.where(i0 == (128 // R) * (i1 & (R - 1)) + (i1 >> 2), 1.0, 0.0).astype(F32))

    def fill_coef():
        coef = shiftbuf[...].astype(F32)
        dval = dbuf[...].astype(F32)
        for c in range(NC):
            for j in range(4):
                coefbuf[c, j] = jnp.broadcast_to(coef[j:j + 1, c * 128:(c + 1) * 128], (8, 128))
            coefbuf[c, 4] = jnp.broadcast_to(dval[c:c + 1, :], (8, 128))

    xs = (xs0, xs1, xs2, xs3, xs4)
    def split_ri(t):
        t = t.reshape(16, 2, 8, 128)
        return t[:, 0], t[:, 1]

    def get_never():
        return zbuf[pl.ds(0, 8), :] != 0

    def pack2(x, y):
        return pltpu.pack_elementwise([x, y], packed_dtype=BF16)

    def words(ref, a, c, r):
        return ref[a, pl.ds((r // 4) * 4 * NC + 4 * c + r % 4, 8, stride=4 * NC), :]

    def unit_u(a, c, g):
        c0, c1, c2, c3 = (coefbuf[c, pl.ds(j, 1)] for j in range(4))
        kk = jnp.stack([words(kw, a, c, 4 + 32 * g + d) for d in range(-2, 4)])
        vv = jnp.stack([words(vw, a, c, 32 * g + d) for d in range(4)])
        lo, hi = _lo(kk), _hi(kk)
        k0, k1, k2 = lo[2:], hi[1:5], lo[1:5]
        even = (((k0 * c0 + k1 * c1) + (k2 * c2 + hi[:4] * c3)) * _lo(vv)).reshape(32, 128)
        odd = (((hi[2:] * c0 + k0 * c1) + (k1 * c2 + k2 * c3)) * _hi(vv)).reshape(32, 128)
        e, o = pack2(even[:16], even[16:]), pack2(odd[:16], odd[16:])
        return [e[:8], o[:8], e[8:], o[8:]]

    def unit_i(a, c, t, z):
        x_c = xs[c].at[pl.ds(z, NA)]
        yr = yi = None
        for j in range(a + 1):
            ur, ui = x_c[j, :, t, 0], x_c[j, :, t, 1]
            kr, ki = x_c[a - j, :, t, 2], x_c[a - j, :, t, 3]
            pr = ur * kr - ui * ki
            pi = ur * ki + ui * kr
            yr = pr if yr is None else yr + pr
            yi = pi if yi is None else yi + pi
        halves = lambda x: (x[:x.shape[0] // 2], x[x.shape[0] // 2:])
        (ra, rb), (ia, ib) = halves(yr.reshape(32, 128)), halves(yi.reshape(32, 128))
        (sr0, sr1), (si0, si1), (dr0, dr1), (di0, di1) = (halves(x) for x in (ra + rb, ia + ib, ra - rb, ia - ib))
        return [pack2(sr0 + sr1, si0 + si1), pack2(dr0 - di1, di0 + dr1),
                pack2(sr0 - sr1, si0 - si1), pack2(dr0 + di1, di0 - dr1)]

    def segment(spec, z, maxutil=1.0, mod_fn=None):
        order = [(n[0], int(n[1]), int(n[2])) for n in spec.split()]
        plan = _plan_tokens(order, maxutil) if maxutil > 0 else {}
        never = get_never()
        units, res = {}, {}

        def unit(key):
            if key not in units:
                kind, a, c, j = key
                if kind == "u":
                    units[key] = unit_u(a, c, j)
                elif kind == "g":
                    units[key] = unit_g(a, j)
                else:
                    fresh = ("u", a, c) in order or ("k", a, c) in order
                    units[key] = unit_i(a, c, j, z if fresh else 0)
            return units[key]

        def lhs(name, p, full, r0=0):
            out, last = [], 0
            for r in range(full.shape[0] // 8):
                keys = plan.get((name, r0 + r), ())
                if keys:
                    if 8 * r > last:
                        out.append(full[last:8 * r])
                    v = full[8 * r:8 * r + 8]
                    for key in keys:
                        v = jax.lax.select(never, unit(key)[p], v)
                    out.append(v)
                    last = 8 * r + 8
            if last < full.shape[0]:
                out.append(full[last:] if last else full)
            return out[0] if len(out) == 1 else jnp.concatenate(out, axis=0)

        def dft(name, rhs):
            tr, ti = [], []
            for p in range(R):
                f = lhs(name, p, fwdbuf[p])
                r_, i_ = split_ri(_dot(_unpack(f), rhs[p]))
                if p == 0:
                    res.update({(name, r): (lambda r=r, v=r_: v[r]) for r in range(16)})
                tr.append(r_)
                ti.append(i_)
            return _bfly(tr, ti, -1)

        st = {}
        for name in order:
            kind, a, c = name
            x_c = xs[c]
            if kind == "g":
                for r in range(8):
                    unit(name + (r,))
            elif kind == "c":
                for t in range(16):
                    after = pltpu.bitcast(res[plan[name + (t,)]](), U32)
                    for p in range(R):
                        wbuf[c, p, pl.ds(8 * t, 8), :] = jax.lax.select(never, after, unit(name + (t,))[p])
            elif kind == "m":
                toks = {}
                for r in range(_DUR["m"]):
                    for n_, key in enumerate(plan.get((name, r), ())):
                        toks.setdefault(2 * r + n_ % 2, []).extend(unit(key))
                mod_fn(a, toks)
            elif kind == "t":
                trs = []
                for b in range(R):
                    pm = lhs(name, b, permbuf[...])
                    trs.append(_dot_nt(_unpack(pm), skbuf[pl.ds(c * 128, 128), pl.ds(a * P + b * 128, 128)]))
                res.update({(name, r): (lambda r=r, v=trs[0]: v[16 * r:16 * r + 8]) for r in range(8)})
                g_ = 128 // R
                st[a, c] = [jnp.concatenate([trs[b][p * g_:(p + 1) * g_] for b in range(R)], axis=0).astype(BF16)
                            for p in range(R)]
            elif kind == "u":
                rhs = [_unpack(jnp.concatenate([unit(name + (g,))[p] for g in range(8)], axis=0)) for p in range(R)]
                xr, xi = dft(name, rhs)
                for q in range(R):
                    x_c[a, q, :, 0] = xr[q]
                    x_c[a, q, :, 1] = xi[q]
            elif kind == "k":
                xr, xi = dft(name, st[a, c])
                for q in range(R):
                    if a == 0:
                        x_c[a, q, :, 2] = xr[q] + coefbuf[c, 4]
                        x_c[a, q, :, 3] = xi[q]
                    else:
                        pr, pi = kraw[c, a - 1, q, :, 0], kraw[c, a - 1, q, :, 1]
                        x_c[a, q, pl.ds(0, 8), 2] = xr[q][:8] - pi[:8]
                        x_c[a, q, pl.ds(0, 8), 3] = xi[q][:8] + pr[:8]
                        x_c[a, q, pl.ds(8, 8), 2] = xr[q][8:] + pi[8:]
                        x_c[a, q, pl.ds(8, 8), 3] = xi[q][8:] - pr[8:]
                    if a + 1 < NA:
                        kraw[c, a, q, :, 0] = xr[q]
                        kraw[c, a, q, :, 1] = xi[q]
            else:
                for p in range(R):
                    cols = [lhs(name, 2 * (p % 2) + kt,
                                invbuf[p, :, pl.ds(128 * kt, 128)], 8 * (p // 2))
                            for kt in range(2)]
                    g = _unpack(jnp.concatenate(cols, axis=1))
                    if kind == "j":
                        wp = _unpack(wbuf[c, p])
                    else:
                        wp = _unpack(jnp.concatenate([unit(name + (t,))[p] for t in range(16)], axis=0))
                    yp = _dot(g, wp)
                    if p % 2 == 0:
                        res.update({(name, 4 * p + r): (lambda r=r, v=yp: v[16 * r:16 * r + 8]) for r in range(8)})
                    ybuf[c, pl.ds(a * P + p, 128, stride=R), :] = yp

    one = jnp.minimum(pl.program_id(0) + 1, 1)

    def once(fn):
        def body(z, carry):
            fn(z)
            return carry
        jax.lax.fori_loop(0, one, body, 0)

    default = "t00 t01 t02 k00 t03 k01 t04 k02 k03 k04 g00|t10 t11 t12 k10 k11 k12 g10|t13 t14 k13 u00 k14 u01 u02 u03 i00 u04 i01 c02 c03|j02 j03 u10 i04 u11 u12 u13 i10 u14 i11 c12|t20 t21 j12 t22 t23 t24 k20 u20 k21 u21 k22 i13 k23 u22 k24 i14 u23 i20 u24 i21 c22|t30 t31 j22 t32 t33 t34 k30 u30 k31 u31 k32 i23 k33 u32 k34 i24 u33 i30 u34 i31 c32|m00 j32 m10 m20 i33 i34"
    specs = default.split("|")
    G5B = specs[-1]
    segs = list(zip("s0 d shift c|s1|k0 v0|k1 v1|s2 k2 v2|s3 k3 v3".split("|"), specs[:-1]))
    MU = 1.5
    for i, (waits, spec) in enumerate(segs):
        with jax.named_scope("g%d" % i):
            for n in waits.split():
                cps[n].wait()
            if i == 0:
                fill_coef()
            once(lambda z: segment(spec, z, MU))

    def mod_cols(lo, n, toks=None):
        cv = cbuf[...].astype(F32)
        sc = (cv * jax.nn.sigmoid(cv)).astype(BF16)
        m = _dot(jnp.broadcast_to(sc, (8, D)), weights(wmodbuf, lo * NC, (lo + n) * NC, toks=toks))
        return [m[:, j * D:(j + 1) * D] for j in range(n)]

    def mul_mod(x, j, cols=None):
        m = modbuf[j] if cols is None else modbuf[j, :, cols]
        return (x.reshape(-1, 8, x.shape[-1]) * m[None]).reshape(x.shape)

    def add_mod(x, j):
        return (x.reshape(-1, 8, x.shape[-1]) + modbuf[j][None]).reshape(x.shape)

    def slabs(ref, r0, n):
        return jnp.concatenate([ref[c, pl.ds(r0, n), :] for c in range(NC)], axis=1)

    def window(base, n):
        rows = pl.ds(base, n)
        return dict(q=qbuf.at[rows, :], y=ybuf.at[:, rows, :], x2=x2buf.at[rows, :], h=hbuf.at[rows, :],
                    hh=hhbuf.at[:, pl.ds(base, n + 8), :], xn=xnbuf.at[pl.ds(base, n - LEAD), :],
                    o=obuf.at[pl.ds(base, n - LEAD), :])

    def weights(ref, c0=0, c1=NC, r0=0, r1=None, toks=None):
        r1 = 16 * ref.shape[0] if r1 is None else r1
        view = ref.bitcast(U32)
        never = get_never() if toks else None
        rt = -(-(r1 - r0) // 128)
        cols = []
        for j in range(c0, c1):
            wu = view[pl.ds(r0 // 16, (r1 - r0) // 16), j].reshape((r1 - r0) // 2, 128)
            if toks:
                parts, last = [], 0
                for i in range(rt):
                    for n_, t in enumerate(toks.get((j - c0) * rt + i, ())):
                        r = 64 * i + 8 * n_
                        if r > last:
                            parts.append(wu[last:r])
                        parts.append(jax.lax.select(never, t, wu[r:r + 8]))
                        last = r + 8
                parts.append(wu[last:])
                wu = jnp.concatenate(parts, axis=0)
            cols.append(wu)
        return pltpu.bitcast(jnp.concatenate(cols, axis=1), BF16)

    def stage_a0(w, r0, n):
        rows = pl.ds(r0, n)
        x = w["q"][rows, :].astype(F32)
        y = slabs(w["y"], r0, n)
        x2 = x + add_mod(mul_mod(_ln(x), 1), 0) * y
        w["x2"][rows, :] = x2
        return _ln(x2)

    def stage_a1(w, r0, n, n2=None):
        if n2 is None:
            n2 = stage_a0(w, r0, n)
        h = add_mod(mul_mod(n2, 4), 3)
        w["h"][pl.ds(r0, n), :] = h
        return _ln(h).astype(BF16)

    def stage_a2(w, n3, r0, n, last_valid=None, fine=0):
        hh = _gelu(_dot_fine(n3, weights(w1buf), fine))
        for c in range(NC):
            blk = hh[:, c * 128:(c + 1) * 128]
            w["hh"][c, pl.ds(r0 + 8, n - LEAD), :] = blk[:n - LEAD]
            tail = blk[n - LEAD:]
            if last_valid is not None:
                tail = jnp.where(last_valid, tail, 0.0)
            w["hh"][c, pl.ds(r0 + 8 + n - LEAD, LEAD), :] = tail

    def stage_b1a(w, r0, n, fine=0):
        rows = pl.ds(r0, n)
        lane = jax.lax.broadcasted_iota(jnp.int32, (n, 128), 1)

        def sh(c, d):
            return w["hh"][c, pl.ds(r0 + 8 + d, n), :]

        g = [sh(0, -1),
             jnp.where(lane < 32, sh(1, -1), sh(1, 1)),
             jnp.where(lane < 64, sh(2, 1), sh(2, -2)),
             jnp.where(lane < 96, sh(3, -2), sh(3, 2)),
             sh(4, 2)]
        hs = _dot_fine(jnp.concatenate(g, axis=1).astype(BF16), weights(w2buf), fine)
        x1 = w["h"][rows, :] + hs
        w["h"][rows, :] = x1
        return x1

    def stage_b1b(w, x1, r0, n):
        w["xn"][pl.ds(r0, n), :] = _ln(x1).astype(BF16)

    def stage_b1(w, r0, n):
        stage_b1b(w, stage_b1a(w, r0, n), r0, n)

    def out_copy(r0, n):
        rows = pl.ds(r0, n)
        return pltpu.make_async_copy(obuf.at[rows, :], out_hbm.at[rows, :], sem_out.at[0])

    FM = (FF // 128) * 128
    FR = FF - FM

    NF = FM // 128

    def stage_b2h(w, r0, n):
        ht = _gelu(_dot_nt(weights(w3buf, r0=FM), w["xn"][pl.ds(r0, n), :]))
        ht = jnp.concatenate([ht, jnp.zeros((128 - FR, n), F32)], axis=0)
        return {NF: jnp.concatenate([ht[:, j:j + 128].T for j in range(0, n, 128)], axis=0).astype(BF16)}

    def stage_b2a(w, r0, n, lo=0, hi=NF, fine=0):
        xn = w["xn"][pl.ds(r0, n), :]
        return {lo: _gelu(_dot_fine(xn, weights(w3buf, r0=128 * lo, r1=128 * hi), fine, nt=True)).astype(BF16)}

    def stage_b2b(w, h3, r0, n, c0, c1, fine=0):
        rows = pl.ds(r0, n)
        cols = pl.ds(c0 * 128, (c1 - c0) * 128)
        w4 = jnp.concatenate([weights(w4buf, c0, c1), jnp.zeros((128 - FR, (c1 - c0) * 128), BF16)], axis=0)
        h2 = _dot_fine(jnp.concatenate([h3[j] for j in sorted(h3)], axis=1), w4, fine)
        w["o"][rows, cols] = (w["x2"][rows, cols] + mul_mod(w["h"][rows, cols] + h2, 5, cols)).astype(BF16)

    w = window(0, 2 * TS + LEAD)
    H = TS // 2
    with jax.named_scope("t0a"):
        cps["qa"].wait()
        cps["wmoda"].wait()

        mv = {}

        def mod_fn(j, toks):
            mv[j] = mod_cols(j, 1, toks)[0]
            if len(mv) == 3:
                modbuf[0] = mv[2] * mv[0]
                modbuf[1] = mv[2] * (1.0 + mv[1])

        segment(G5B, 0, MU, mod_fn=mod_fn)
        w["h"][pl.ds(0, QA), :] = stage_a0(w, 0, QA)
    with jax.named_scope("t0b"):
        cps["wmodb"].wait()
        sb, cb = mod_cols(3, 2)
        modbuf[3] = sb
        modbuf[4] = 1.0 + cb
        n3 = stage_a1(w, 0, QA, n2=w["h"][pl.ds(0, QA), :])
    XB = TS - XA
    FN = 32
    F4 = 64
    with jax.named_scope("t1"):
        cps["w1"].wait()
        n3a = stage_a1(w, QA, XA)
        stage_a2(w, n3, 0, QA)
        stage_a2(w, n3a, QA, XA, fine=FN)
    with jax.named_scope("t2"):
        cps["qb"].wait()
        cps["w2"].wait()
        n3b = stage_a1(w, QA + XA, XB)
        stage_b1(w, 0, TS)
        stage_a2(w, n3b, QA + XA, XB)
        stage_b1(w, TS, XA)
        stage_b1a(w, TS + XA, XB, fine=FN)
    L = TS + H
    with jax.named_scope("t3"):
        cps["w3"].wait()
        stage_b1b(w, w["h"][pl.ds(TS + XA, XB), :], TS + XA, XB)
        h3 = {**stage_b2h(w, 0, L), **stage_b2a(w, 0, L, fine=64)}
    with jax.named_scope("t4"):
        cps["w4"].wait()
        cps["wmodg"].wait()
        modbuf[5] = mod_cols(5, 1)[0]
        stage_b2b(w, h3, 0, L, 0, NC, fine=F4)
        out_copy(0, L).start()
        cps["q1"].wait()

    SUB = 64
    PART_B2 = {"a": (0, H), "b": (H, TS)}
    PART_B1 = {"a": (H, TS), "b": (L, H), "c": (H, H), "d": (TS, H)}
    BODY = "ha 3a w0 4a:0:1 w1 w2 2c w3 4a:1:2 2d 4a:2:5 3b hb w4 4b:0:2 w5 4b:2:3 2b 4b:3:5"

    def step(s, carry):
        r0 = pl.multiple_of(s * L, 128)
        w = window(r0, 2 * TS + LEAD)
        h3 = {"a": {}, "b": {}}
        for op in BODY.split():
            op, *rng = op.split(":")
            rng = [int(x) for x in rng]
            if op[0] == "3":
                h3[op[1]].update(stage_b2a(w, *PART_B2[op[1]], *rng))
            elif op[0] == "h":
                h3[op[1]].update(stage_b2h(w, *PART_B2[op[1]]))
            elif op[0] == "4":
                stage_b2b(w, h3[op[1]], *PART_B2[op[1]], *rng)
            elif op[0] == "2":
                stage_b1(w, *PART_B1[op[1]])
            else:
                j = int(op[1])
                ra = H + LEAD + j * SUB
                last = (j + 1) * SUB == L
                stage_a2(w, stage_a1(w, ra, SUB), ra, SUB, last_valid=(s < NL) if last else None)
        out_copy(r0, L).start()
        return carry

    NL = (S - H) // L - 1
    with jax.named_scope("p2main"):
        jax.lax.fori_loop(1, NL + 1, step, 0)
    with jax.named_scope("p2epi"):
        w = window(S - 2 * TS, 2 * TS + LEAD)
        h3 = {**stage_b2h(w, L, H), **stage_b2a(w, L, H)}
        rows = pl.ds(S - H, H)
        for c0, c1 in ((0, 4), (4, 5)):
            stage_b2b(w, h3, L, H, c0, c1)
            cols = pl.ds(c0 * 128, (c1 - c0) * 128)
            pltpu.make_async_copy(obuf.at[rows, cols], out_hbm.at[rows, cols], sem_out.at[0]).start()
        pltpu.make_async_copy(obuf, out_hbm, sem_out.at[0]).wait()


@jax.jit
def pallas_adaLN_cond__ssm_conv_h3__mixer_s_mlp__prompt_kernel(
    A_q: jax.Array,
    A_k: jax.Array,
    A_v: jax.Array,
    A_shift_k: jax.Array,
    A_ssm_k: jax.Array,
    A_ssm_D: jax.Array,
    B_x: jax.Array,
    B_w1: jax.Array,
    B_w2: jax.Array,
    B_w3: jax.Array,
    B_w4: jax.Array,
    c: jax.Array,
    w_mod: jax.Array,
):
    del B_x

    def tiles(x):
        return x.reshape(S // 8, 8, NC, 128).transpose(0, 2, 1, 3).reshape(S * NC, 128)

    def pairs(x):
        r, n = x.shape
        return x.reshape(r // 16, 2, 8, n // 128, 128).transpose(0, 1, 3, 2, 4)

    args = (
        A_q.reshape(S, D), tiles(A_k), tiles(A_v),
        A_shift_k.T, A_ssm_k, A_ssm_D.reshape(NC, 128),
        pairs(B_w1), pairs(B_w2), pairs(B_w3.T), pairs(B_w4), c, pairs(w_mod),
    )
    scratch = [
        pltpu.VMEM((NA, P * NC + 128, 128), BF16),
        pltpu.VMEM((NA, P * NC + 64, 128), BF16),
        pltpu.VMEM((D, S), BF16),
        pltpu.VMEM((R, 128, 128), U32),
        pltpu.VMEM((R, 64, 256), U32),
        pltpu.VMEM((64, 128), U32),
        pltpu.VMEM((D // 16, 6 * NC, 16, 128), BF16),
        pltpu.VMEM((D // 16, NC, 16, 128), BF16),
        pltpu.VMEM((D // 16, NC, 16, 128), BF16),
        pltpu.VMEM((FF // 16, NC, 16, 128), BF16),
        pltpu.VMEM((FF // 16, NC, 16, 128), BF16),
        pltpu.VMEM((S + 64, D), BF16),
        *[pltpu.VMEM((NA, R, 16, 4, 8, 128), F32) for _ in range(NC)],
        pltpu.VMEM((NC, NA - 1, R, 16, 2, 8, 128), F32),
        pltpu.VMEM((NC, R, 128, 128), U32),
        pltpu.VMEM((32, 128), U32),
        pltpu.VMEM((NC, 8, 8, 128), F32),
        pltpu.VMEM((NC, S + 32, 128), F32),
        pltpu.VMEM((8, 8, D), F32),
        pltpu.VMEM((S + 32, D), F32),
        pltpu.VMEM((S + 32, D), F32),
        pltpu.VMEM((NC, S + 32, 128), F32),
        pltpu.VMEM((S, D), BF16),
        pltpu.VMEM((S, D), BF16),
        pltpu.VMEM((4, D), BF16),
        pltpu.VMEM((NC, 128), BF16),
        pltpu.VMEM((1, D), BF16),
        pltpu.SemaphoreType.DMA((40,)),
        pltpu.SemaphoreType.DMA((1,)),
    ]
    out = pl.pallas_call(
        _kernel,
        out_shape=jax.ShapeDtypeStruct((S, D), BF16),
        in_specs=[pl.BlockSpec(memory_space=pl.ANY)] * len(args),
        out_specs=pl.BlockSpec(memory_space=pl.ANY),
        scratch_shapes=scratch,
        grid=(1,),
        compiler_params=pltpu.CompilerParams(vmem_limit_bytes=100 * 1024 * 1024, disable_semaphore_checks=True,
                                             disable_bounds_checks=True),
        name="adaln_h3_mixer",
    )(*args)
    return out.reshape(1, S, D)
```

```python
import numpy as np
import jax
import jax.numpy as jnp
import jax.experimental.pallas as pl
import jax.experimental.pallas.tpu as pltpu

F32 = jnp.float32
BF16 = jnp.bfloat16
U32 = jnp.uint32

S = 2048
D = 640
FF = 1728
NC = D // 128
R = 4
P = 128 * R
NA = S // P
TS = 256
NT = S // TS
LEAD = 16
EPS = 1e-5
P1_ORDER = "t0 t1 t2 t3 k0 k1 k2 k3 u0 i0 u1 i1 u2 i2 u3 i3"


def _freq(row):
    t, part, s = row >> 4, (row >> 3) & 1, row & 7
    return 32 * (t & 7) + 4 * s + 2 * (t >> 3) + 1, P * part


def _cos(j, scale):
    jf = (j & (4 * P - 1)).astype(F32)
    u = 2.0 * np.pi / (4 * P)
    x = jnp.abs(jf * u - np.pi) - 0.5 * np.pi
    x2 = x * x
    poly = scale / 362880.0 - x2 * (scale / 39916800.0)
    for coef in (-1.0 / 5040.0, 1.0 / 120.0, -1.0 / 6.0, 1.0):
        poly = poly * x2 + coef * scale
    return poly * x


_DUR = {"t": 8, "u": 16, "k": 16, "i": 16, "m": 12, "g": 0, "c": 0, "j": 16}
_POST = {"t": 8.0, "u": 16.0, "k": 24.0, "i": 4.0, "j": 4.0, "m": 18.0}


def _plan_tokens(order, maxutil):
    lag, cap, pre, margin = 8, 60, 4, 3
    start, slots = {}, []
    for n in order:
        start[n] = len(slots)
        slots += [(n, r) for r in range(_DUR[n[0]])]
    nslot = len(slots) + lag
    free = [cap - (_POST[slots[i - lag][0][0]] if i >= lag else 0.0) for i in range(-pre, nslot)]
    units = []
    for n in order:
        kind, a, c = n
        if kind == "u":
            units += [(n + (g,), 94.0, start[n], -pre) for g in range(8)]
        elif kind == "g":
            units += [(n + (g,), 150.0, start[n], -pre) for g in range(8)]
        elif kind in "ic":
            src_ = [start[m] for m in (("u", a, c), ("k", a, c)) if m in start]
            for t in range(16):
                rel = max(max(src_) + 16, max(src_) + t + lag + 3) if src_ else -pre
                units.append((n + (t,), 32.0 * a + 48.0, nslot if kind == 'c' else start[n], rel))

    def simulate(util):
        left = [u[1] for u in units]
        done = [None] * len(units)
        for i in range(-pre, nslot):
            budget = util * free[i + pre]
            for j, u in enumerate(units):
                if budget <= 0.0:
                    break
                if done[j] is None and u[3] <= i:
                    use = min(budget, left[j])
                    left[j] -= use
                    budget -= use
                    if left[j] <= 1e-9:
                        done[j] = i + 1
        ok = all(u[2] < 8 or (d is not None and d <= max(u[2] - (1 if u[0][0] in 'cg' else margin), u[3] + 1))
                 for d, u in zip(done, units))
        return done, ok

    lo_, hi_ = 0.05, maxutil
    for _ in range(12):
        mid = 0.5 * (lo_ + hi_)
        if simulate(mid)[1]:
            hi_ = mid
        else:
            lo_ = mid
    done, _ = simulate(hi_)
    plan = {}
    for u, d in zip(units, done):
        if u[0][0] == "c":
            plan[u[0]] = slots[max((nslot - 1 if d is None else min(d, nslot - 1)) - lag, 0)]
        elif d is not None and 0 <= d < u[2]:
            plan.setdefault(slots[d], []).append(u[0])
    return plan


def _pack(x):
    return pltpu.bitcast(x.astype(BF16), U32)


def _unpack(w):
    return pltpu.bitcast(w, BF16)


def _dot(a, b):
    return jnp.dot(a, b, preferred_element_type=F32)


def _dot_nt(a, b):
    return jax.lax.dot_general(a, b, (((1,), (1,)), ((), ())), preferred_element_type=F32)


def _dot_fine(x, w, chunk, nt=False):
    if not chunk:
        return _dot_nt(x, w) if nt else _dot(x, w)
    n = w.shape[0] if nt else w.shape[1]
    head, last = (w[:n - 128], w[n - 128:]) if nt else (w[:, :n - 128], w[:, n - 128:])
    f = _dot_nt if nt else _dot
    parts = [f(x, head)] if n > 128 else []
    parts.append(jnp.concatenate([f(x[r:r + chunk], last) for r in range(0, x.shape[0], chunk)], axis=0))
    return jnp.concatenate(parts, axis=1)


def _lo(w):
    return pltpu.bitcast(w << 16, F32)


def _hi(w):
    return pltpu.bitcast(w & jnp.uint32(0xFFFF0000), F32)


def _ln_stats(x):
    m = jnp.sum(x, axis=-1, keepdims=True) * (1.0 / D)
    xc = x - m
    v = jnp.sum(xc * xc, axis=-1, keepdims=True) * (1.0 / D)
    return xc, jnp.exp(-0.5 * jnp.log(v + EPS))


def _ln(x):
    xc, r = _ln_stats(x)
    return xc * r


def _gelu(x):
    c0 = 0.7978845608028654
    c1 = c0 * 0.044715
    z = x * (c0 + c1 * (x * x))
    hx = 0.5 * x
    return hx + hx * jnp.tanh(z)


def _bfly(tr, ti, sign):
    s02r, s02i = tr[0] + tr[2], ti[0] + ti[2]
    d02r, d02i = tr[0] - tr[2], ti[0] - ti[2]
    s13r, s13i = tr[1] + tr[3], ti[1] + ti[3]
    d13r, d13i = tr[1] - tr[3], ti[1] - ti[3]
    x0r, x0i = s02r + s13r, s02i + s13i
    x2r, x2i = s02r - s13r, s02i - s13i
    ar, ai = d02r + d13i, d02i - d13r
    br, bi = d02r - d13i, d02i + d13r
    if sign < 0:
        return [x0r, ar, x2r, br], [x0i, ai, x2i, bi]
    return [x0r, br, x2r, ar], [x0i, bi, x2i, ai]


def _kernel(q_hbm, k_hbm, v_hbm, shift_hbm, ssmk_hbm, ssmd_hbm, w1_hbm, w2_hbm, w3t_hbm, w4_hbm,
            c_hbm, wmod_hbm,
            out_hbm,
            kbuf, vbuf, skbuf, fwdbuf, invbuf, permbuf,
            wmodbuf, w1buf, w2buf, w3buf, w4buf, qbuf,
            xs0, xs1, xs2, xs3, xs4, kraw, wbuf, zbuf, coefbuf, ybuf, modbuf, x2buf, hbuf, hhbuf, xnbuf, obuf, shiftbuf, dbuf, cbuf,
            sem_in, sem_out):
    cps = {}
    n_sem = [0]

    def start(name, src, dst):
        cp = pltpu.make_async_copy(src, dst, sem_in.at[n_sem[0]])
        n_sem[0] += 1
        cp.start()
        cps[name] = cp

    class Both:
        def __init__(self, a, b):
            self.cps = (a, b)

        def wait(self):
            for cp in self.cps:
                cp.wait()

    def start_w(name, src, dst, c0=0, n=NC):
        for e in range(2):
            start(name + str(e), src.at[:, e, pl.ds(c0, n)], dst.at[:, pl.ds(c0, n), pl.ds(8 * e, 8), :])
        cps[name] = Both(cps[name + "0"], cps[name + "1"])

    CH = P * NC
    HALO = 8 * NC

    def start_s(a):
        cols = pl.ds(a * P, P)
        start("s%d" % a, ssmk_hbm.at[:, cols], skbuf.at[:, cols])

    def start_kv(a):
        if a == 0:
            start("k0", k_hbm.at[pl.ds(0, CH), :], kbuf.at[0, pl.ds(HALO, CH), :])
        else:
            start("k%d" % a, k_hbm.at[pl.ds(a * CH - HALO, CH + HALO), :], kbuf.at[a, pl.ds(0, CH + HALO), :])
        start("v%d" % a, v_hbm.at[pl.ds(a * CH, CH), :], vbuf.at[a, pl.ds(0, CH), :])

    for n in "s0 x0 s1 k0 k1 s2 k2 s3 k3".split():
        if n[0] == "s":
            start_s(int(n[1]))
        elif n[0] == "k":
            start_kv(int(n[1]))
        else:
            start("d", ssmd_hbm, dbuf)
            start("shift", shift_hbm, shiftbuf)
            start("c", c_hbm, cbuf)
    QA = TS + LEAD
    XA = 128
    QB = 2 * TS + LEAD
    W1A = 2
    QXPOS = "a"

    def start_q(name, r0, n):
        start(name, q_hbm.at[pl.ds(r0, n), :], qbuf.at[pl.ds(r0, n), :])

    start_q("qa", 0, QA)
    if QXPOS == "0":
        start_q("qx", QA, XA)
    start_w("wmoda", wmod_hbm, wmodbuf, 0, 3 * NC)
    start_w("wmodb", wmod_hbm, wmodbuf, 3 * NC, 2 * NC)
    if QXPOS == "a":
        start_q("qx", QA, XA)
    start_w("w1a", w1_hbm, w1buf, 0, W1A)
    if QXPOS == "b":
        start_q("qx", QA, XA)
    start_w("w1b", w1_hbm, w1buf, W1A, NC - W1A)
    start_q("qb", QA + XA, QB - QA - XA)
    start_w("w2", w2_hbm, w2buf)
    start_w("w3", w3t_hbm, w3buf)
    start_w("w4", w4_hbm, w4buf)
    start_w("wmodg", wmod_hbm, wmodbuf, 5 * NC, NC)
    start("q1", q_hbm.at[pl.ds(QB, S - QB), :], qbuf.at[pl.ds(QB, S - QB), :])

    kw = kbuf.bitcast(U32)
    vw = vbuf.bitcast(U32)
    kbuf[0, pl.ds(0, HALO), :] = jnp.zeros((HALO, 128), BF16)
    zbuf[...] = jnp.zeros(zbuf.shape, U32)
    for c in range(NC):
        ybuf[c, pl.ds(S, LEAD), :] = jnp.zeros((LEAD, 128), F32)
        hhbuf[c, pl.ds(0, 8), :] = jnp.zeros((8, 128), F32)
    qbuf[pl.ds(S, LEAD), :] = jnp.zeros((LEAD, D), BF16)

    def tables(p, carry):
        i0 = jax.lax.broadcasted_iota(jnp.int32, (128, 128), 0)
        n = R * jax.lax.broadcasted_iota(jnp.int32, (128, 128), 1) + p
        f2, off = _freq(2 * i0)
        j = f2 * n + off
        fwdbuf[p] = pltpu.pack_elementwise([_cos(j, 1.0), _cos(j + 4 * n, 1.0)], packed_dtype=BF16)
        return carry

    jax.lax.fori_loop(0, R, tables, 0)

    def unit_g(kt, r):
        col = jax.lax.broadcasted_iota(jnp.int32, (8, 128), 1) + 128 * kt
        f2, off = _freq((col & ~15) + 8 * (col & 1) + ((col >> 1) & 7))
        m = 2 * jax.lax.broadcasted_iota(jnp.int32, (8, 128), 0) + 16 * r
        j0 = f2 * (R * m) + off
        out = []
        for p in range(R):
            j = j0 + p * f2
            out.append(pltpu.pack_elementwise([_cos(j, 1.0 / P), _cos(j + R * f2, 1.0 / P)], packed_dtype=BF16))
            invbuf[p, pl.ds(8 * r, 8), pl.ds(128 * kt, 128)] = out[-1]
        return out

    i0 = jax.lax.broadcasted_iota(jnp.int32, (128, 128), 0)
    i1 = jax.lax.broadcasted_iota(jnp.int32, (128, 128), 1)
    permbuf[...] = _pack(jnp.where(i0 == (128 // R) * (i1 & (R - 1)) + (i1 >> 2), 1.0, 0.0).astype(F32))

    def fill_coef():
        coef = shiftbuf[...].astype(F32)
        dval = dbuf[...].astype(F32)
        for c in range(NC):
            for j in range(4):
                coefbuf[c, j] = jnp.broadcast_to(coef[j:j + 1, c * 128:(c + 1) * 128], (8, 128))
            coefbuf[c, 4] = jnp.broadcast_to(dval[c:c + 1, :], (8, 128))

    xs = (xs0, xs1, xs2, xs3, xs4)
    def split_ri(t):
        t = t.reshape(16, 2, 8, 128)
        return t[:, 0], t[:, 1]

    def get_never():
        return zbuf[pl.ds(0, 8), :] != 0

    def pack2(x, y):
        return pltpu.pack_elementwise([x, y], packed_dtype=BF16)

    def words(ref, a, c, r):
        return ref[a, pl.ds((r // 4) * 4 * NC + 4 * c + r % 4, 8, stride=4 * NC), :]

    def unit_u(a, c, g):
        c0, c1, c2, c3 = (coefbuf[c, pl.ds(j, 1)] for j in range(4))
        kk = jnp.stack([words(kw, a, c, 4 + 32 * g + d) for d in range(-2, 4)])
        vv = jnp.stack([words(vw, a, c, 32 * g + d) for d in range(4)])
        lo, hi = _lo(kk), _hi(kk)
        k0, k1, k2 = lo[2:], hi[1:5], lo[1:5]
        even = (((k0 * c0 + k1 * c1) + (k2 * c2 + hi[:4] * c3)) * _lo(vv)).reshape(32, 128)
        odd = (((hi[2:] * c0 + k0 * c1) + (k1 * c2 + k2 * c3)) * _hi(vv)).reshape(32, 128)
        e, o = pack2(even[:16], even[16:]), pack2(odd[:16], odd[16:])
        return [e[:8], o[:8], e[8:], o[8:]]

    def unit_i(a, c, t, z):
        x_c = xs[c].at[pl.ds(z, NA)]
        yr = yi = None
        for j in range(a + 1):
            ur, ui = x_c[j, :, t, 0], x_c[j, :, t, 1]
            kr, ki = x_c[a - j, :, t, 2], x_c[a - j, :, t, 3]
            pr = ur * kr - ui * ki
            pi = ur * ki + ui * kr
            yr = pr if yr is None else yr + pr
            yi = pi if yi is None else yi + pi
        halves = lambda x: (x[:x.shape[0] // 2], x[x.shape[0] // 2:])
        (ra, rb), (ia, ib) = halves(yr.reshape(32, 128)), halves(yi.reshape(32, 128))
        (sr0, sr1), (si0, si1), (dr0, dr1), (di0, di1) = (halves(x) for x in (ra + rb, ia + ib, ra - rb, ia - ib))
        return [pack2(sr0 + sr1, si0 + si1), pack2(dr0 - di1, di0 + dr1),
                pack2(sr0 - sr1, si0 - si1), pack2(dr0 + di1, di0 - dr1)]

    def segment(spec, z, maxutil=1.0, mod_fn=None):
        order = [(n[0], int(n[1]), int(n[2])) for n in spec.split()]
        plan = _plan_tokens(order, maxutil) if maxutil > 0 else {}
        never = get_never()
        units, res = {}, {}

        def unit(key):
            if key not in units:
                kind, a, c, j = key
                if kind == "u":
                    units[key] = unit_u(a, c, j)
                elif kind == "g":
                    units[key] = unit_g(a, j)
                else:
                    fresh = ("u", a, c) in order or ("k", a, c) in order
                    units[key] = unit_i(a, c, j, z if fresh else 0)
            return units[key]

        def lhs(name, p, full, r0=0):
            out, last = [], 0
            for r in range(full.shape[0] // 8):
                keys = plan.get((name, r0 + r), ())
                if keys:
                    if 8 * r > last:
                        out.append(full[last:8 * r])
                    v = full[8 * r:8 * r + 8]
                    for key in keys:
                        v = jax.lax.select(never, unit(key)[p], v)
                    out.append(v)
                    last = 8 * r + 8
            if last < full.shape[0]:
                out.append(full[last:] if last else full)
            return out[0] if len(out) == 1 else jnp.concatenate(out, axis=0)

        def dft(name, rhs):
            tr, ti = [], []
            for p in range(R):
                f = lhs(name, p, fwdbuf[p])
                r_, i_ = split_ri(_dot(_unpack(f), rhs[p]))
                if p == 0:
                    res.update({(name, r): (lambda r=r, v=r_: v[r]) for r in range(16)})
                tr.append(r_)
                ti.append(i_)
            return _bfly(tr, ti, -1)

        st = {}
        for name in order:
            kind, a, c = name
            x_c = xs[c]
            if kind == "g":
                for r in range(8):
                    unit(name + (r,))
            elif kind == "c":
                for t in range(16):
                    after = pltpu.bitcast(res[plan[name + (t,)]](), U32)
                    for p in range(R):
                        wbuf[c, p, pl.ds(8 * t, 8), :] = jax.lax.select(never, after, unit(name + (t,))[p])
            elif kind == "m":
                toks = {}
                for r in range(_DUR["m"]):
                    for n_, key in enumerate(plan.get((name, r), ())):
                        toks.setdefault(2 * r + n_ % 2, []).extend(unit(key))
                mod_fn(a, toks)
            elif kind == "t":
                trs = []
                for b in range(R):
                    pm = lhs(name, b, permbuf[...])
                    trs.append(_dot_nt(_unpack(pm), skbuf[pl.ds(c * 128, 128), pl.ds(a * P + b * 128, 128)]))
                res.update({(name, r): (lambda r=r, v=trs[0]: v[16 * r:16 * r + 8]) for r in range(8)})
                g_ = 128 // R
                st[a, c] = [jnp.concatenate([trs[b][p * g_:(p + 1) * g_] for b in range(R)], axis=0).astype(BF16)
                            for p in range(R)]
            elif kind == "u":
                rhs = [_unpack(jnp.concatenate([unit(name + (g,))[p] for g in range(8)], axis=0)) for p in range(R)]
                xr, xi = dft(name, rhs)
                for q in range(R):
                    x_c[a, q, :, 0] = xr[q]
                    x_c[a, q, :, 1] = xi[q]
            elif kind == "k":
                xr, xi = dft(name, st[a, c])
                for q in range(R):
                    if a == 0:
                        x_c[a, q, :, 2] = xr[q] + coefbuf[c, 4]
                        x_c[a, q, :, 3] = xi[q]
                    else:
                        pr, pi = kraw[c, a - 1, q, :, 0], kraw[c, a - 1, q, :, 1]
                        x_c[a, q, pl.ds(0, 8), 2] = xr[q][:8] - pi[:8]
                        x_c[a, q, pl.ds(0, 8), 3] = xi[q][:8] + pr[:8]
                        x_c[a, q, pl.ds(8, 8), 2] = xr[q][8:] + pi[8:]
                        x_c[a, q, pl.ds(8, 8), 3] = xi[q][8:] - pr[8:]
                    if a + 1 < NA:
                        kraw[c, a, q, :, 0] = xr[q]
                        kraw[c, a, q, :, 1] = xi[q]
            else:
                for p in range(R):
                    cols = [lhs(name, 2 * (p % 2) + kt,
                                invbuf[p, :, pl.ds(128 * kt, 128)], 8 * (p // 2))
                            for kt in range(2)]
                    g = _unpack(jnp.concatenate(cols, axis=1))
                    if kind == "j":
                        wp = _unpack(wbuf[c, p])
                    else:
                        wp = _unpack(jnp.concatenate([unit(name + (t,))[p] for t in range(16)], axis=0))
                    yp = _dot(g, wp)
                    if p % 2 == 0:
                        res.update({(name, 4 * p + r): (lambda r=r, v=yp: v[16 * r:16 * r + 8]) for r in range(8)})
                    ybuf[c, pl.ds(a * P + p, 128, stride=R), :] = yp

    one = jnp.minimum(pl.program_id(0) + 1, 1)

    def once(fn):
        def body(z, carry):
            fn(z)
            return carry
        jax.lax.fori_loop(0, one, body, 0)

    default = "t00 t01 t02 k00 t03 k01 t04 k02 k03 k04 g00|t10 t11 t12 k10 k11 k12 g10|t13 t14 k13 u00 k14 u01 u02 u03 i00 u04 i01 c02 c03|j02 j03 u10 i04 u11 u12 u13 i10 u14 i11 c12|t20 t21 j12 t22 t23 t24 k20 u20 k21 u21 k22 i13 k23 u22 k24 i14 u23 i20 u24 i21 c22|t30 t31 j22 t32 t33 t34 k30 u30 k31 u31 k32 i23 k33 u32 k34 i24 u33 i30 u34 i31 c32|m00 j32 m10 m20 i33 i34"
    specs = default.split("|")
    G5B = specs[-1]
    segs = list(zip("s0 d shift c|s1|k0 v0|k1 v1|s2 k2 v2|s3 k3 v3".split("|"), specs[:-1]))
    MU = 1.5
    for i, (waits, spec) in enumerate(segs):
        with jax.named_scope("g%d" % i):
            for n in waits.split():
                cps[n].wait()
            if i == 0:
                fill_coef()
            once(lambda z: segment(spec, z, MU))

    def mod_cols(lo, n, toks=None):
        cv = cbuf[...].astype(F32)
        sc = (cv * jax.nn.sigmoid(cv)).astype(BF16)
        m = _dot(jnp.broadcast_to(sc, (8, D)), weights(wmodbuf, lo * NC, (lo + n) * NC, toks=toks))
        return [m[:, j * D:(j + 1) * D] for j in range(n)]

    def mul_mod(x, j, cols=None):
        m = modbuf[j] if cols is None else modbuf[j, :, cols]
        return (x.reshape(-1, 8, x.shape[-1]) * m[None]).reshape(x.shape)

    def add_mod(x, j):
        return (x.reshape(-1, 8, x.shape[-1]) + modbuf[j][None]).reshape(x.shape)

    def slabs(ref, r0, n):
        return jnp.concatenate([ref[c, pl.ds(r0, n), :] for c in range(NC)], axis=1)

    def window(base, n):
        rows = pl.ds(base, n)
        return dict(q=qbuf.at[rows, :], y=ybuf.at[:, rows, :], x2=x2buf.at[rows, :], h=hbuf.at[rows, :],
                    hh=hhbuf.at[:, pl.ds(base, n + 8), :], xn=xnbuf.at[pl.ds(base, n - LEAD), :],
                    o=obuf.at[pl.ds(base, n - LEAD), :])

    def weights(ref, c0=0, c1=NC, r0=0, r1=None, toks=None):
        r1 = 16 * ref.shape[0] if r1 is None else r1
        view = ref.bitcast(U32)
        never = get_never() if toks else None
        rt = -(-(r1 - r0) // 128)
        cols = []
        for j in range(c0, c1):
            wu = view[pl.ds(r0 // 16, (r1 - r0) // 16), j].reshape((r1 - r0) // 2, 128)
            if toks:
                parts, last = [], 0
                for i in range(rt):
                    for n_, t in enumerate(toks.get((j - c0) * rt + i, ())):
                        r = 64 * i + 8 * n_
                        if r > last:
                            parts.append(wu[last:r])
                        parts.append(jax.lax.select(never, t, wu[r:r + 8]))
                        last = r + 8
                parts.append(wu[last:])
                wu = jnp.concatenate(parts, axis=0)
            cols.append(wu)
        return pltpu.bitcast(jnp.concatenate(cols, axis=1), BF16)

    def stage_a0(w, r0, n):
        rows = pl.ds(r0, n)
        x = w["q"][rows, :].astype(F32)
        y = slabs(w["y"], r0, n)
        x2 = x + add_mod(mul_mod(_ln(x), 1), 0) * y
        w["x2"][rows, :] = x2
        return _ln(x2)

    def stage_a1(w, r0, n, n2=None):
        if n2 is None:
            n2 = stage_a0(w, r0, n)
        h = add_mod(mul_mod(n2, 4), 3)
        w["h"][pl.ds(r0, n), :] = h
        return _ln(h).astype(BF16)

    def stage_a2(w, n3, r0, n, last_valid=None, fine=0, c0=0, c1=NC):
        hh = _gelu(_dot_fine(n3, weights(w1buf, c0, c1), fine))
        for c in range(c0, c1):
            blk = hh[:, (c - c0) * 128:(c - c0 + 1) * 128]
            w["hh"][c, pl.ds(r0 + 8, n - LEAD), :] = blk[:n - LEAD]
            tail = blk[n - LEAD:]
            if last_valid is not None:
                tail = jnp.where(last_valid, tail, 0.0)
            w["hh"][c, pl.ds(r0 + 8 + n - LEAD, LEAD), :] = tail

    def stage_b1a(w, r0, n, fine=0):
        rows = pl.ds(r0, n)
        lane = jax.lax.broadcasted_iota(jnp.int32, (n, 128), 1)

        def sh(c, d):
            return w["hh"][c, pl.ds(r0 + 8 + d, n), :]

        g = [sh(0, -1),
             jnp.where(lane < 32, sh(1, -1), sh(1, 1)),
             jnp.where(lane < 64, sh(2, 1), sh(2, -2)),
             jnp.where(lane < 96, sh(3, -2), sh(3, 2)),
             sh(4, 2)]
        hs = _dot_fine(jnp.concatenate(g, axis=1).astype(BF16), weights(w2buf), fine)
        x1 = w["h"][rows, :] + hs
        w["h"][rows, :] = x1
        return x1

    def stage_b1b(w, x1, r0, n):
        w["xn"][pl.ds(r0, n), :] = _ln(x1).astype(BF16)

    def stage_b1(w, r0, n):
        stage_b1b(w, stage_b1a(w, r0, n), r0, n)

    def out_copy(r0, n):
        rows = pl.ds(r0, n)
        return pltpu.make_async_copy(obuf.at[rows, :], out_hbm.at[rows, :], sem_out.at[0])

    FM = (FF // 128) * 128
    FR = FF - FM

    NF = FM // 128

    def stage_b2h(w, r0, n):
        ht = _gelu(_dot_nt(weights(w3buf, r0=FM), w["xn"][pl.ds(r0, n), :]))
        ht = jnp.concatenate([ht, jnp.zeros((128 - FR, n), F32)], axis=0)
        return {NF: jnp.concatenate([ht[:, j:j + 128].T for j in range(0, n, 128)], axis=0).astype(BF16)}

    def stage_b2a(w, r0, n, lo=0, hi=NF, fine=0):
        xn = w["xn"][pl.ds(r0, n), :]
        return {lo: _gelu(_dot_fine(xn, weights(w3buf, r0=128 * lo, r1=128 * hi), fine, nt=True)).astype(BF16)}

    def stage_b2b(w, h3, r0, n, c0, c1, fine=0):
        rows = pl.ds(r0, n)
        cols = pl.ds(c0 * 128, (c1 - c0) * 128)
        w4 = jnp.concatenate([weights(w4buf, c0, c1), jnp.zeros((128 - FR, (c1 - c0) * 128), BF16)], axis=0)
        h2 = _dot_fine(jnp.concatenate([h3[j] for j in sorted(h3)], axis=1), w4, fine)
        w["o"][rows, cols] = (w["x2"][rows, cols] + mul_mod(w["h"][rows, cols] + h2, 5, cols)).astype(BF16)

    w = window(0, 2 * TS + LEAD)
    H = TS // 2
    with jax.named_scope("t0a"):
        cps["qa"].wait()
        cps["wmoda"].wait()

        mv = {}

        def mod_fn(j, toks):
            mv[j] = mod_cols(j, 1, toks)[0]
            if len(mv) == 3:
                modbuf[0] = mv[2] * mv[0]
                modbuf[1] = mv[2] * (1.0 + mv[1])

        segment(G5B, 0, MU, mod_fn=mod_fn)
        w["h"][pl.ds(0, QA), :] = stage_a0(w, 0, QA)
    with jax.named_scope("t0b"):
        cps["wmodb"].wait()
        sb, cb = mod_cols(3, 2)
        modbuf[3] = sb
        modbuf[4] = 1.0 + cb
        n3 = stage_a1(w, 0, QA, n2=w["h"][pl.ds(0, QA), :])
    XB = TS - XA
    FN = 32
    F4 = 64
    with jax.named_scope("t1a"):
        cps["w1a"].wait()
        if QXPOS != "b":
            cps["qx"].wait()
            if "1" == "1":
                w["h"][pl.ds(QA, XA), :] = stage_a0(w, QA, XA)
            else:
                n3a = stage_a1(w, QA, XA)
        stage_a2(w, n3, 0, QA, c1=W1A, fine=80)
    with jax.named_scope("t1b"):
        cps["w1b"].wait()
        if QXPOS == "b":
            cps["qx"].wait()
            n3a = stage_a1(w, QA, XA)
        elif "1" == "1":
            n3a = stage_a1(w, QA, XA, n2=w["h"][pl.ds(QA, XA), :])
        stage_a2(w, n3, 0, QA, c0=W1A)
        if "0" == "1":
            stage_a2(w, n3a[:XA // 2], QA, XA // 2)
            stage_a2(w, n3a[XA // 2:], QA + XA // 2, XA // 2, fine=FN)
        else:
            stage_a2(w, n3a, QA, XA, fine=FN)
    with jax.named_scope("t2"):
        cps["qb"].wait()
        cps["w2"].wait()
        n3b = stage_a1(w, QA + XA, XB)
        stage_b1(w, 0, TS)
        stage_a2(w, n3b, QA + XA, XB)
        stage_b1(w, TS, XA)
        stage_b1a(w, TS + XA, XB, fine=FN)
    L = TS + H
    with jax.named_scope("t3"):
        cps["w3"].wait()
        stage_b1b(w, w["h"][pl.ds(TS + XA, XB), :], TS + XA, XB)
        h3 = {**stage_b2h(w, 0, L), **stage_b2a(w, 0, L, fine=64)}
    with jax.named_scope("t4"):
        cps["w4"].wait()
        cps["wmodg"].wait()
        modbuf[5] = mod_cols(5, 1)[0]
        stage_b2b(w, h3, 0, L, 0, NC, fine=F4)
        out_copy(0, L).start()
        cps["q1"].wait()

    SUB = 64
    PART_B2 = {"a": (0, H), "b": (H, TS)}
    PART_B1 = {"a": (H, TS), "b": (L, H), "c": (H, H), "d": (TS, H)}
    BODY = "ha 3a w0 4a:0:1 w1 w2 2c w3 4a:1:2 2d 4a:2:5 3b hb w4 4b:0:2 w5 4b:2:3 2b 4b:3:5"

    def step(s, carry):
        r0 = pl.multiple_of(s * L, 128)
        w = window(r0, 2 * TS + LEAD)
        h3 = {"a": {}, "b": {}}
        for op in BODY.split():
            op, *rng = op.split(":")
            rng = [int(x) for x in rng]
            if op[0] == "3":
                h3[op[1]].update(stage_b2a(w, *PART_B2[op[1]], *rng))
            elif op[0] == "h":
                h3[op[1]].update(stage_b2h(w, *PART_B2[op[1]]))
            elif op[0] == "4":
                stage_b2b(w, h3[op[1]], *PART_B2[op[1]], *rng)
            elif op[0] == "2":
                stage_b1(w, *PART_B1[op[1]])
            else:
                j = int(op[1])
                ra = H + LEAD + j * SUB
                last = (j + 1) * SUB == L
                stage_a2(w, stage_a1(w, ra, SUB), ra, SUB, last_valid=(s < NL) if last else None)
        out_copy(r0, L).start()
        return carry

    NL = (S - H) // L - 1
    with jax.named_scope("p2main"):
        jax.lax.fori_loop(1, NL + 1, step, 0)
    with jax.named_scope("p2epi"):
        w = window(S - 2 * TS, 2 * TS + LEAD)
        h3 = {**stage_b2h(w, L, H), **stage_b2a(w, L, H)}
        rows = pl.ds(S - H, H)
        for c0, c1 in ((0, 4), (4, 5)):
            stage_b2b(w, h3, L, H, c0, c1)
            cols = pl.ds(c0 * 128, (c1 - c0) * 128)
            pltpu.make_async_copy(obuf.at[rows, cols], out_hbm.at[rows, cols], sem_out.at[0]).start()
        pltpu.make_async_copy(obuf, out_hbm, sem_out.at[0]).wait()


@jax.jit
def pallas_adaLN_cond__ssm_conv_h3__mixer_s_mlp__prompt_kernel(
    A_q: jax.Array,
    A_k: jax.Array,
    A_v: jax.Array,
    A_shift_k: jax.Array,
    A_ssm_k: jax.Array,
    A_ssm_D: jax.Array,
    B_x: jax.Array,
    B_w1: jax.Array,
    B_w2: jax.Array,
    B_w3: jax.Array,
    B_w4: jax.Array,
    c: jax.Array,
    w_mod: jax.Array,
):
    del B_x

    def tiles(x):
        return x.reshape(S // 8, 8, NC, 128).transpose(0, 2, 1, 3).reshape(S * NC, 128)

    def pairs(x):
        r, n = x.shape
        return x.reshape(r // 16, 2, 8, n // 128, 128).transpose(0, 1, 3, 2, 4)

    args = (
        A_q.reshape(S, D), tiles(A_k), tiles(A_v),
        A_shift_k.T, A_ssm_k, A_ssm_D.reshape(NC, 128),
        pairs(B_w1), pairs(B_w2), pairs(B_w3.T), pairs(B_w4), c, pairs(w_mod),
    )
    scratch = [
        pltpu.VMEM((NA, P * NC + 128, 128), BF16),
        pltpu.VMEM((NA, P * NC + 64, 128), BF16),
        pltpu.VMEM((D, S), BF16),
        pltpu.VMEM((R, 128, 128), U32),
        pltpu.VMEM((R, 64, 256), U32),
        pltpu.VMEM((64, 128), U32),
        pltpu.VMEM((D // 16, 6 * NC, 16, 128), BF16),
        pltpu.VMEM((D // 16, NC, 16, 128), BF16),
        pltpu.VMEM((D // 16, NC, 16, 128), BF16),
        pltpu.VMEM((FF // 16, NC, 16, 128), BF16),
        pltpu.VMEM((FF // 16, NC, 16, 128), BF16),
        pltpu.VMEM((S + 64, D), BF16),
        *[pltpu.VMEM((NA, R, 16, 4, 8, 128), F32) for _ in range(NC)],
        pltpu.VMEM((NC, NA - 1, R, 16, 2, 8, 128), F32),
        pltpu.VMEM((NC, R, 128, 128), U32),
        pltpu.VMEM((32, 128), U32),
        pltpu.VMEM((NC, 8, 8, 128), F32),
        pltpu.VMEM((NC, S + 32, 128), F32),
        pltpu.VMEM((8, 8, D), F32),
        pltpu.VMEM((S + 32, D), F32),
        pltpu.VMEM((S + 32, D), F32),
        pltpu.VMEM((NC, S + 32, 128), F32),
        pltpu.VMEM((S, D), BF16),
        pltpu.VMEM((S, D), BF16),
        pltpu.VMEM((4, D), BF16),
        pltpu.VMEM((NC, 128), BF16),
        pltpu.VMEM((1, D), BF16),
        pltpu.SemaphoreType.DMA((40,)),
        pltpu.SemaphoreType.DMA((1,)),
    ]
    out = pl.pallas_call(
        _kernel,
        out_shape=jax.ShapeDtypeStruct((S, D), BF16),
        in_specs=[pl.BlockSpec(memory_space=pl.ANY)] * len(args),
        out_specs=pl.BlockSpec(memory_space=pl.ANY),
        scratch_shapes=scratch,
        grid=(1,),
        compiler_params=pltpu.CompilerParams(vmem_limit_bytes=100 * 1024 * 1024, disable_semaphore_checks=True,
                                             disable_bounds_checks=True),
        name="adaln_h3_mixer",
    )(*args)
    return out.reshape(1, S, D)
```

```python
import numpy as np
import jax
import jax.numpy as jnp
import jax.experimental.pallas as pl
import jax.experimental.pallas.tpu as pltpu

F32 = jnp.float32
BF16 = jnp.bfloat16
U32 = jnp.uint32

S = 2048
D = 640
FF = 1728
NC = D // 128
R = 4
P = 128 * R
NA = S // P
TS = 256
NT = S // TS
LEAD = 16
EPS = 1e-5
KEEP3 = 0
KEEP4 = 0
FAST = ""
FM = (FF // 128) * 128
FR = FF - FM
P1_ORDER = "t0 t1 t2 t3 k0 k1 k2 k3 u0 i0 u1 i1 u2 i2 u3 i3"


def _freq(row):
    t, part, s = row >> 4, (row >> 3) & 1, row & 7
    return 32 * (t & 7) + 4 * s + 2 * (t >> 3) + 1, P * part


def _cos(j, scale):
    jf = (j & (4 * P - 1)).astype(F32)
    u = 2.0 * np.pi / (4 * P)
    x = jnp.abs(jf * u - np.pi) - 0.5 * np.pi
    x2 = x * x
    poly = scale / 362880.0 - x2 * (scale / 39916800.0)
    for coef in (-1.0 / 5040.0, 1.0 / 120.0, -1.0 / 6.0, 1.0):
        poly = poly * x2 + coef * scale
    return poly * x


_DUR = {"t": 8, "u": 16, "k": 16, "i": 16, "m": 12, "g": 0, "c": 0, "j": 16}
_POST = {"t": 8.0, "u": 16.0, "k": 24.0, "i": 4.0, "j": 4.0, "m": 18.0}


def _plan_tokens(order, maxutil):
    lag, cap, pre, margin = 8, 60, 4, 3
    start, slots = {}, []
    for n in order:
        start[n] = len(slots)
        slots += [(n, r) for r in range(_DUR[n[0]])]
    nslot = len(slots) + lag
    free = [cap - (_POST[slots[i - lag][0][0]] if i >= lag else 0.0) for i in range(-pre, nslot)]
    units = []
    for n in order:
        kind, a, c = n
        if kind == "u":
            units += [(n + (g,), 94.0, start[n], -pre) for g in range(8)]
        elif kind == "g":
            units += [(n + (g,), 150.0, start[n], -pre) for g in range(8)]
        elif kind in "ic":
            src_ = [start[m] for m in (("u", a, c), ("k", a, c)) if m in start]
            for t in range(16):
                rel = max(max(src_) + 16, max(src_) + t + lag + 3) if src_ else -pre
                units.append((n + (t,), 32.0 * a + 48.0, nslot if kind == 'c' else start[n], rel))

    def simulate(util):
        left = [u[1] for u in units]
        done = [None] * len(units)
        for i in range(-pre, nslot):
            budget = util * free[i + pre]
            for j, u in enumerate(units):
                if budget <= 0.0:
                    break
                if done[j] is None and u[3] <= i:
                    use = min(budget, left[j])
                    left[j] -= use
                    budget -= use
                    if left[j] <= 1e-9:
                        done[j] = i + 1
        ok = all(u[2] < 8 or (d is not None and d <= max(u[2] - (1 if u[0][0] in 'cg' else margin), u[3] + 1))
                 for d, u in zip(done, units))
        return done, ok

    lo_, hi_ = 0.05, maxutil
    for _ in range(12):
        mid = 0.5 * (lo_ + hi_)
        if simulate(mid)[1]:
            hi_ = mid
        else:
            lo_ = mid
    done, _ = simulate(hi_)
    plan = {}
    for u, d in zip(units, done):
        if u[0][0] == "c":
            plan[u[0]] = slots[max((nslot - 1 if d is None else min(d, nslot - 1)) - lag, 0)]
        elif d is not None and 0 <= d < u[2]:
            plan.setdefault(slots[d], []).append(u[0])
    return plan


def _pack(x):
    return pltpu.bitcast(x.astype(BF16), U32)


def _unpack(w):
    return pltpu.bitcast(w, BF16)


_CLOCK = []


def _tick(r, k):
    t = (_CLOCK[-1][0] if _CLOCK else 0) + r.shape[0] * (-(-k // 128)) * (-(-r.shape[1] // 128)) // 4
    _CLOCK.append((t, r))
    return r


def _dot(a, b):
    return _tick(jnp.dot(a.astype(BF16), b, preferred_element_type=F32), a.shape[1])


def _dot_nt(a, b):
    return _tick(jax.lax.dot_general(a.astype(BF16), b, (((1,), (1,)), ((), ())), preferred_element_type=F32),
                 a.shape[1])


def _dot_fine(x, w, chunk, nt=False):
    if not chunk:
        return _dot_nt(x, w) if nt else _dot(x, w)
    n = w.shape[0] if nt else w.shape[1]
    head, last = (w[:n - 128], w[n - 128:]) if nt else (w[:, :n - 128], w[:, n - 128:])
    f = _dot_nt if nt else _dot
    parts = [f(x, head)] if n > 128 else []
    parts.append(jnp.concatenate([f(x[r:r + chunk], last) for r in range(0, x.shape[0], chunk)], axis=0))
    return jnp.concatenate(parts, axis=1)


def _rows2(x):
    n, c = x.shape
    x = x.reshape(n // 32, 2, 16, c)
    return x[:, 0].reshape(n // 2, c), x[:, 1].reshape(n // 2, c)


def _unrows2(top, bot):
    n, c = top.shape
    return jnp.stack([top.reshape(n // 16, 16, c), bot.reshape(n // 16, 16, c)], axis=1).reshape(2 * n, c)


def _sums_a(a11, a12, a21, a22):
    return [a11 + a22, a21 + a22, a11 + a12, a21 - a11, a12 - a22]


def _sums_b(b11, b12, b21, b22):
    return [b11 + b22, b12 - b22, b21 - b11, b11 + b12, b21 + b22]


_STRASSEN = ((0, 0), (1, 5), (5, 1), (6, 2), (2, 6), (3, 3), (4, 4))


def _combine(m1, m2, m3, m4, m5, m6, m7):
    return (m1 + m4) + (m7 - m5), m3 + m5, m2 + m4, (m1 - m2) + (m3 + m6)


def _lo(w):
    return pltpu.bitcast(w << 16, F32)


def _hi(w):
    return pltpu.bitcast(w & jnp.uint32(0xFFFF0000), F32)


def _ln_stats(x):
    m = jnp.sum(x, axis=-1, keepdims=True) * (1.0 / D)
    xc = x - m
    v = jnp.sum(xc * xc, axis=-1, keepdims=True) * (1.0 / D)
    return xc, jnp.exp(-0.5 * jnp.log(v + EPS))


def _ln(x, fast=False):
    if fast:
        m = jnp.sum(x, axis=-1, keepdims=True) * (1.0 / D)
        v = jnp.maximum(jnp.sum(x * x, axis=-1, keepdims=True) * (1.0 / D) - m * m, 0.0)
        return (x - m) * jnp.exp(-0.5 * jnp.log(v + EPS))
    xc, r = _ln_stats(x)
    return xc * r


def _gelu(x):
    c0 = 0.7978845608028654
    c1 = c0 * 0.044715
    z = x * (c0 + c1 * (x * x))
    hx = 0.5 * x
    return hx + hx * jnp.tanh(z)


def _bfly(tr, ti, sign):
    s02r, s02i = tr[0] + tr[2], ti[0] + ti[2]
    d02r, d02i = tr[0] - tr[2], ti[0] - ti[2]
    s13r, s13i = tr[1] + tr[3], ti[1] + ti[3]
    d13r, d13i = tr[1] - tr[3], ti[1] - ti[3]
    x0r, x0i = s02r + s13r, s02i + s13i
    x2r, x2i = s02r - s13r, s02i - s13i
    ar, ai = d02r + d13i, d02i - d13r
    br, bi = d02r - d13i, d02i + d13r
    if sign < 0:
        return [x0r, ar, x2r, br], [x0i, ai, x2i, bi]
    return [x0r, br, x2r, ar], [x0i, bi, x2i, ai]


def _kernel(q_hbm, k_hbm, v_hbm, shift_hbm, ssmk_hbm, ssmd_hbm, w1_hbm, w2_hbm, w3t_hbm, w4_hbm,
            c_hbm, wmod_hbm,
            out_hbm,
            kbuf, vbuf, skbuf, fwdbuf, invbuf, permbuf,
            wmodbuf, w1buf, w2buf, w3buf, w4buf, qbuf,
            xs0, xs1, xs2, xs3, xs4, kraw, wbuf, zbuf, coefbuf, ybuf, modbuf, x2buf, hbuf, hhbuf, xnbuf, xsbuf, w1s, w2s, w3s, w4s, hba, hbb, obuf, shiftbuf, dbuf, cbuf,
            zsm, sem_in, sem_out):
    cps = {}
    n_sem = [0]

    def start(name, src, dst):
        cp = pltpu.make_async_copy(src, dst, sem_in.at[n_sem[0]])
        n_sem[0] += 1
        cp.start()
        cps[name] = cp

    class Both:
        def __init__(self, a, b):
            self.cps = (a, b)

        def wait(self):
            for cp in self.cps:
                cp.wait()

    def start_w(name, src, dst, c0=0, n=NC):
        for e in range(2):
            start(name + str(e), src.at[:, e, pl.ds(c0, n)], dst.at[:, pl.ds(c0, n), pl.ds(8 * e, 8), :])
        cps[name] = Both(cps[name + "0"], cps[name + "1"])

    CH = P * NC
    HALO = 8 * NC

    def start_s(a):
        cols = pl.ds(a * P, P)
        start("s%d" % a, ssmk_hbm.at[:, cols], skbuf.at[:, cols])

    def start_kv(a):
        if a == 0:
            start("k0", k_hbm.at[pl.ds(0, CH), :], kbuf.at[0, pl.ds(HALO, CH), :])
        else:
            start("k%d" % a, k_hbm.at[pl.ds(a * CH - HALO, CH + HALO), :], kbuf.at[a, pl.ds(0, CH + HALO), :])
        start("v%d" % a, v_hbm.at[pl.ds(a * CH, CH), :], vbuf.at[a, pl.ds(0, CH), :])

    for n in "s0 x0 s1 k0 k1 s2 k2 s3 k3".split():
        if n[0] == "s":
            start_s(int(n[1]))
        elif n[0] == "k":
            start_kv(int(n[1]))
        else:
            start("d", ssmd_hbm, dbuf)
            start("shift", shift_hbm, shiftbuf)
            start("c", c_hbm, cbuf)
    QA = TS + LEAD
    XA = 128
    QB = 2 * TS + LEAD
    W1A = 2
    QXPOS = "a"

    def start_q(name, r0, n):
        start(name, q_hbm.at[pl.ds(r0, n), :], qbuf.at[pl.ds(r0, n), :])

    start_q("qa", 0, QA)
    if QXPOS == "0":
        start_q("qx", QA, XA)
    start_w("wmoda", wmod_hbm, wmodbuf, 0, 3 * NC)
    start_w("wmodb", wmod_hbm, wmodbuf, 3 * NC, 2 * NC)
    if QXPOS == "a":
        start_q("qx", QA, XA)
    start_w("w1a", w1_hbm, w1buf, 0, W1A)
    if QXPOS == "b":
        start_q("qx", QA, XA)
    start_w("w1b", w1_hbm, w1buf, W1A, NC - W1A)
    start_q("qb", QA + XA, QB - QA - XA)
    start_w("w2", w2_hbm, w2buf)
    start_w("w3", w3t_hbm, w3buf)
    start_w("w4", w4_hbm, w4buf)
    start_w("wmodg", wmod_hbm, wmodbuf, 5 * NC, NC)
    start("q1", q_hbm.at[pl.ds(QB, S - QB), :], qbuf.at[pl.ds(QB, S - QB), :])

    kw = kbuf.bitcast(U32)
    vw = vbuf.bitcast(U32)
    kbuf[0, pl.ds(0, HALO), :] = jnp.zeros((HALO, 128), BF16)
    zbuf[...] = jnp.zeros(zbuf.shape, U32)
    for j in range(8):
        zsm[j] = 0
    for c in range(NC):
        ybuf[c, pl.ds(S, LEAD), :] = jnp.zeros((LEAD, 128), F32)
        hhbuf[c, pl.ds(0, 8), :] = jnp.zeros((8, 128), F32)
    qbuf[pl.ds(S, LEAD), :] = jnp.zeros((LEAD, D), BF16)

    def tables(p, carry):
        i0 = jax.lax.broadcasted_iota(jnp.int32, (128, 128), 0)
        n = R * jax.lax.broadcasted_iota(jnp.int32, (128, 128), 1) + p
        f2, off = _freq(2 * i0)
        j = f2 * n + off
        fwdbuf[p] = pltpu.pack_elementwise([_cos(j, 1.0), _cos(j + 4 * n, 1.0)], packed_dtype=BF16)
        return carry

    jax.lax.fori_loop(0, R, tables, 0)

    def unit_g(kt, r):
        col = jax.lax.broadcasted_iota(jnp.int32, (8, 128), 1) + 128 * kt
        f2, off = _freq((col & ~15) + 8 * (col & 1) + ((col >> 1) & 7))
        m = 2 * jax.lax.broadcasted_iota(jnp.int32, (8, 128), 0) + 16 * r
        j0 = f2 * (R * m) + off
        out = []
        for p in range(R):
            j = j0 + p * f2
            out.append(pltpu.pack_elementwise([_cos(j, 1.0 / P), _cos(j + R * f2, 1.0 / P)], packed_dtype=BF16))
            invbuf[p, pl.ds(8 * r, 8), pl.ds(128 * kt, 128)] = out[-1]
        return out

    i0 = jax.lax.broadcasted_iota(jnp.int32, (128, 128), 0)
    i1 = jax.lax.broadcasted_iota(jnp.int32, (128, 128), 1)
    permbuf[...] = _pack(jnp.where(i0 == (128 // R) * (i1 & (R - 1)) + (i1 >> 2), 1.0, 0.0).astype(F32))

    def fill_coef():
        coef = shiftbuf[...].astype(F32)
        dval = dbuf[...].astype(F32)
        for c in range(NC):
            for j in range(4):
                coefbuf[c, j] = jnp.broadcast_to(coef[j:j + 1, c * 128:(c + 1) * 128], (8, 128))
            coefbuf[c, 4] = jnp.broadcast_to(dval[c:c + 1, :], (8, 128))

    xs = (xs0, xs1, xs2, xs3, xs4)
    wsbufs = dict(w1=w1s, w2=w2s, w3=w3s, w4=w4s)
    def split_ri(t):
        t = t.reshape(16, 2, 8, 128)
        return t[:, 0], t[:, 1]

    def get_never():
        return zbuf[pl.ds(0, 8), :] != 0

    def pack2(x, y):
        return pltpu.pack_elementwise([x, y], packed_dtype=BF16)

    def words(ref, a, c, r):
        return ref[a, pl.ds((r // 4) * 4 * NC + 4 * c + r % 4, 8, stride=4 * NC), :]

    def unit_u(a, c, g):
        c0, c1, c2, c3 = (coefbuf[c, pl.ds(j, 1)] for j in range(4))
        kk = jnp.stack([words(kw, a, c, 4 + 32 * g + d) for d in range(-2, 4)])
        vv = jnp.stack([words(vw, a, c, 32 * g + d) for d in range(4)])
        lo, hi = _lo(kk), _hi(kk)
        k0, k1, k2 = lo[2:], hi[1:5], lo[1:5]
        even = (((k0 * c0 + k1 * c1) + (k2 * c2 + hi[:4] * c3)) * _lo(vv)).reshape(32, 128)
        odd = (((hi[2:] * c0 + k0 * c1) + (k1 * c2 + k2 * c3)) * _hi(vv)).reshape(32, 128)
        e, o = pack2(even[:16], even[16:]), pack2(odd[:16], odd[16:])
        return [e[:8], o[:8], e[8:], o[8:]]

    def unit_i(a, c, t, z):
        x_c = xs[c].at[pl.ds(z, NA)]
        yr = yi = None
        for j in range(a + 1):
            ur, ui = x_c[j, :, t, 0], x_c[j, :, t, 1]
            kr, ki = x_c[a - j, :, t, 2], x_c[a - j, :, t, 3]
            pr = ur * kr - ui * ki
            pi = ur * ki + ui * kr
            yr = pr if yr is None else yr + pr
            yi = pi if yi is None else yi + pi
        halves = lambda x: (x[:x.shape[0] // 2], x[x.shape[0] // 2:])
        (ra, rb), (ia, ib) = halves(yr.reshape(32, 128)), halves(yi.reshape(32, 128))
        (sr0, sr1), (si0, si1), (dr0, dr1), (di0, di1) = (halves(x) for x in (ra + rb, ia + ib, ra - rb, ia - ib))
        return [pack2(sr0 + sr1, si0 + si1), pack2(dr0 - di1, di0 + dr1),
                pack2(sr0 - sr1, si0 - si1), pack2(dr0 + di1, di0 - dr1)]

    def segment(spec, z, maxutil=1.0, mod_fn=None):
        order = [(n[0], int(n[1]), int(n[2])) for n in spec.split()]
        plan = _plan_tokens(order, maxutil) if maxutil > 0 else {}
        never = get_never()
        units, res = {}, {}

        def unit(key):
            if key not in units:
                kind, a, c, j = key
                if kind == "u":
                    units[key] = unit_u(a, c, j)
                elif kind == "g":
                    units[key] = unit_g(a, j)
                else:
                    fresh = ("u", a, c) in order or ("k", a, c) in order
                    units[key] = unit_i(a, c, j, z if fresh else 0)
            return units[key]

        def lhs(name, p, full, r0=0):
            out, last = [], 0
            for r in range(full.shape[0] // 8):
                keys = plan.get((name, r0 + r), ())
                if keys:
                    if 8 * r > last:
                        out.append(full[last:8 * r])
                    v = full[8 * r:8 * r + 8]
                    for key in keys:
                        v = jax.lax.select(never, unit(key)[p], v)
                    out.append(v)
                    last = 8 * r + 8
            if last < full.shape[0]:
                out.append(full[last:] if last else full)
            return out[0] if len(out) == 1 else jnp.concatenate(out, axis=0)

        def dft(name, rhs):
            tr, ti = [], []
            for p in range(R):
                f = lhs(name, p, fwdbuf[p])
                r_, i_ = split_ri(_dot(_unpack(f), rhs[p]))
                if p == 0:
                    res.update({(name, r): (lambda r=r, v=r_: v[r]) for r in range(16)})
                tr.append(r_)
                ti.append(i_)
            return _bfly(tr, ti, -1)

        st = {}
        for name in order:
            kind, a, c = name
            x_c = xs[c]
            if kind == "g":
                for r in range(8):
                    unit(name + (r,))
            elif kind == "c":
                for t in range(16):
                    after = pltpu.bitcast(res[plan[name + (t,)]](), U32)
                    for p in range(R):
                        wbuf[c, p, pl.ds(8 * t, 8), :] = jax.lax.select(never, after, unit(name + (t,))[p])
            elif kind == "m":
                toks = {}
                for r in range(_DUR["m"]):
                    for n_, key in enumerate(plan.get((name, r), ())):
                        toks.setdefault(2 * r + n_ % 2, []).extend(unit(key))
                mod_fn(a, toks)
            elif kind == "t":
                trs = []
                for b in range(R):
                    pm = lhs(name, b, permbuf[...])
                    trs.append(_dot_nt(_unpack(pm), skbuf[pl.ds(c * 128, 128), pl.ds(a * P + b * 128, 128)]))
                res.update({(name, r): (lambda r=r, v=trs[0]: v[16 * r:16 * r + 8]) for r in range(8)})
                g_ = 128 // R
                st[a, c] = [jnp.concatenate([trs[b][p * g_:(p + 1) * g_] for b in range(R)], axis=0).astype(BF16)
                            for p in range(R)]
            elif kind == "u":
                rhs = [_unpack(jnp.concatenate([unit(name + (g,))[p] for g in range(8)], axis=0)) for p in range(R)]
                xr, xi = dft(name, rhs)
                for q in range(R):
                    x_c[a, q, :, 0] = xr[q]
                    x_c[a, q, :, 1] = xi[q]
            elif kind == "k":
                xr, xi = dft(name, st[a, c])
                for q in range(R):
                    if a == 0:
                        x_c[a, q, :, 2] = xr[q] + coefbuf[c, 4]
                        x_c[a, q, :, 3] = xi[q]
                    else:
                        pr, pi = kraw[c, a - 1, q, :, 0], kraw[c, a - 1, q, :, 1]
                        x_c[a, q, pl.ds(0, 8), 2] = xr[q][:8] - pi[:8]
                        x_c[a, q, pl.ds(0, 8), 3] = xi[q][:8] + pr[:8]
                        x_c[a, q, pl.ds(8, 8), 2] = xr[q][8:] + pi[8:]
                        x_c[a, q, pl.ds(8, 8), 3] = xi[q][8:] - pr[8:]
                    if a + 1 < NA:
                        kraw[c, a, q, :, 0] = xr[q]
                        kraw[c, a, q, :, 1] = xi[q]
            else:
                for p in range(R):
                    cols = [lhs(name, 2 * (p % 2) + kt,
                                invbuf[p, :, pl.ds(128 * kt, 128)], 8 * (p // 2))
                            for kt in range(2)]
                    g = _unpack(jnp.concatenate(cols, axis=1))
                    if kind == "j":
                        wp = _unpack(wbuf[c, p])
                    else:
                        wp = _unpack(jnp.concatenate([unit(name + (t,))[p] for t in range(16)], axis=0))
                    yp = _dot(g, wp)
                    if p % 2 == 0:
                        res.update({(name, 4 * p + r): (lambda r=r, v=yp: v[16 * r:16 * r + 8]) for r in range(8)})
                    ybuf[c, pl.ds(a * P + p, 128, stride=R), :] = yp

    one = jnp.minimum(pl.program_id(0) + 1, 1)

    def once(fn):
        def body(z, carry):
            fn(z)
            return carry
        jax.lax.fori_loop(0, one, body, 0)

    default = "t00 t01 t02 k00 t03 k01 t04 k02 k03 k04 g00|t10 t11 t12 k10 k11 k12 g10|t13 t14 k13 u00 k14 u01 u02 u03 i00 u04 i01 c02 c03|j02 j03 u10 i04 u11 u12 u13 i10 u14 i11 c12|t20 t21 j12 t22 t23 t24 k20 u20 k21 u21 k22 i13 k23 u22 k24 i14 u23 i20 u24 i21 c22|t30 t31 j22 t32 t33 t34 k30 u30 k31 u31 k32 i23 k33 u32 k34 i24 u33 i30 u34 i31 c32|m00 j32 m10 m20 i33 i34"
    specs = default.split("|")
    G5B = specs[-1]
    segs = list(zip("s0 d shift c|s1|k0 v0|k1 v1|s2 k2 v2|s3 k3 v3".split("|"), specs[:-1]))
    MU = 1.5
    for i, (waits, spec) in enumerate(segs):
        with jax.named_scope("g%d" % i):
            for n in waits.split():
                cps[n].wait()
            if i == 0:
                fill_coef()
            once(lambda z: segment(spec, z, MU))

    def mod_cols(lo, n, toks=None):
        cv = cbuf[...].astype(F32)
        sc = (cv * jax.nn.sigmoid(cv)).astype(BF16)
        m = _dot(jnp.broadcast_to(sc, (8, D)), weights(wmodbuf, lo * NC, (lo + n) * NC, toks=toks))
        return [m[:, j * D:(j + 1) * D] for j in range(n)]

    def mul_mod(x, j, cols=None):
        m = modbuf[j] if cols is None else modbuf[j, :, cols]
        return (x.reshape(-1, 8, x.shape[-1]) * m[None]).reshape(x.shape)

    def add_mod(x, j):
        return (x.reshape(-1, 8, x.shape[-1]) + modbuf[j][None]).reshape(x.shape)

    def slabs(ref, r0, n):
        return jnp.concatenate([ref[c, pl.ds(r0, n), :] for c in range(NC)], axis=1)

    def put(ref, rows, x):
        for c in range(NC):
            ref[c, rows, :] = x[:, c * 128:(c + 1) * 128]

    def parity(ref, r0, n, e):
        return jnp.concatenate([ref[c, pl.ds(r0 + e, n // 2, stride=2), :] for c in range(NC)], axis=1)

    def window(base, n, half):
        rows = pl.ds(base, n)
        return dict(xs=xsbuf.at[pl.ds(half, (n - LEAD) // 2), :],
                    q=qbuf.at[rows, :], y=ybuf.at[:, rows, :], x2=x2buf.at[rows, :], h=hbuf.at[:, rows, :],
                    hh=hhbuf.at[:, pl.ds(base, n + 8), :], xn=xnbuf.at[:, pl.ds(half, (n - LEAD) // 2), :],
                    o=obuf.at[pl.ds(base, n - LEAD), :])

    def weights(ref, c0=0, c1=NC, r0=0, r1=None, toks=None, raw=False, z=None):
        r1 = 16 * ref.shape[0] if r1 is None else r1
        view = ref.bitcast(U32)
        if z is not None:
            view = view.at[pl.ds(z, ref.shape[0])]
        never = get_never() if toks else None
        rt = -(-(r1 - r0) // 128)
        cols = []
        for j in range(c0, c1):
            wu = view[pl.ds(r0 // 16, (r1 - r0) // 16), j].reshape((r1 - r0) // 2, 128)
            if toks:
                parts, last = [], 0
                for i in range(rt):
                    for n_, t in enumerate(toks.get((j - c0) * rt + i, ())):
                        r = 64 * i + 8 * n_
                        if r > last:
                            parts.append(wu[last:r])
                        parts.append(jax.lax.select(never, t, wu[r:r + 8]))
                        last = r + 8
                parts.append(wu[last:])
                wu = jnp.concatenate(parts, axis=0)
            cols.append(wu)
        wu = jnp.concatenate(cols, axis=1)
        return wu if raw else _unpack(wu)

    def wblocks(name, j, z=None):
        if name == "w3":
            blk = lambda kh, nh: weights(w3buf, 2 * kh, 2 * kh + 2, 128 * (j + 6 * nh), 128 * (j + 6 * nh + 1), raw=True, z=z)
        elif name == "w4":
            def blk(kh, nh):
                c = j + 2 * nh
                parts = [weights(w4buf, c, c + 1, 768 * kh, 768 * (kh + 1), raw=True, z=z),
                         weights(w4buf, c, c + 1, 1536 + 128 * kh, min(1664 + 128 * kh, FF), raw=True, z=z)]
                if kh:
                    parts.append(jnp.zeros(((128 - FR) // 2, 128), U32))
                return jnp.concatenate(parts, axis=0)
        else:
            ref = w1buf if name == "w1" else w2buf
            blk = lambda kh, nh: weights(ref, j + 2 * nh, j + 2 * nh + 1, 256 * kh, 256 * (kh + 1), raw=True, z=z)
        return blk

    def wsums(name, j):
        blk = wblocks(name, j)
        bs = [blk(0, 0), blk(0, 1), blk(1, 0), blk(1, 1)]
        return [pack2(x, y) for x, y in zip(_sums_b(*[_lo(b) for b in bs]), _sums_b(*[_hi(b) for b in bs]))]

    def wsum(name, j, k):
        blk = wblocks(name, j, zsm[k])
        p, q, sign = ((0, 3, 1), (1, 3, -1), (2, 0, -1), (0, 1, 1), (2, 3, 1))[k]
        x, y = blk(p // 2, p % 2), blk(q // 2, q % 2)
        if sign > 0:
            return pack2(_lo(x) + _lo(y), _hi(x) + _hi(y))
        return pack2(_lo(x) - _lo(y), _hi(x) - _hi(y))

    def keep(dst, val, after):
        tok = pltpu.bitcast(after[:8, :128], U32)
        r, c = val.shape
        tok = jnp.broadcast_to(jnp.concatenate([tok] * (c // 128), axis=1)[None], (r // 8, 8, c))
        nv = get_never()
        nv = jnp.broadcast_to(jnp.concatenate([nv.astype(U32)] * (c // 128), axis=1)[None], (r // 8, 8, c)) != 0
        dst[...] = jax.lax.select(nv, tok, val.reshape(r // 8, 8, c)).reshape(r, c)

    def sprods(name, j, lhs, k0=0, k1=7, prep=False):
        blk, buf = wblocks(name, j), wsbufs[name]
        out = []
        for ia, ib in _STRASSEN[k0:k1]:
            wv = blk(ib - 5, ib - 5) if ib >= 5 else (wsum(name, j, ib) if prep else buf[ib, j])
            out.append((_dot_nt if name == "w3" else _dot)(lhs(ia), _unpack(wv)))
            if prep and ib < 5:
                back = KEEP3 if name == "w3" else KEEP4
                if back == 0 or len(_CLOCK) < back:
                    buf[ib, j] = wv
                else:
                    keep(buf.at[ib, j], wv, _CLOCK[-back][1])
        return out

    def spair(name, j, lhs, prep=False):
        return _combine(*sprods(name, j, lhs, prep=prep))

    def dd_rest(name, t, b):
        ref = w1buf if name == "w1" else w2buf
        m = t.shape[0]
        xb = jnp.concatenate([t, b], axis=0)
        last = _dot(xb, weights(ref, 4, 5))
        rem = _dot(xb[:, 512:], weights(ref, 0, 4, r0=512))
        return t, b, rem[:m], rem[m:], last[:m], last[m:]

    def dd_main(name, parts, prep=False):
        t, b, rt, rb, lt, lb = (jnp.concatenate(v, axis=0) for v in zip(*parts))
        ops = _sums_a(t[:, :256], t[:, 256:512], b[:, :256], b[:, 256:512]) + [t[:, :256], b[:, 256:512]]
        top, bot = [None] * 4, [None] * 4
        for j in range(2):
            top[j], top[j + 2], bot[j], bot[j + 2] = spair(name, j, lambda i: ops[i], prep)
        return (jnp.concatenate([jnp.concatenate(top, axis=1) + rt, lt], axis=1),
                jnp.concatenate([jnp.concatenate(bot, axis=1) + rb, lb], axis=1))

    def stage_a0(w, r0, n, span=None):
        rows = pl.ds(r0, n)
        x = w["q"][rows, :].astype(F32)
        y = slabs(w["y"], r0, n)
        x2 = x + add_mod(mul_mod(_ln(x, "1" in FAST), 1), 0) * y
        w["x2"][rows, :] = x2
        return _ln(x2, "2" in FAST)

    def stage_a1(w, r0, n, n2=None, f32=False, span=None):
        if n2 is None:
            n2 = stage_a0(w, r0, n, span)
        h = add_mod(mul_mod(n2, 4), 3)
        put(w["h"], pl.ds(r0, n), h)
        n3 = _ln(h, "3" in FAST)
        return n3 if f32 else n3.astype(BF16)

    def stage_a2(w, n3, r0, n, last_valid=None, fine=0, c0=0, c1=NC, prep=False):
        hh = _gelu(_unrows2(*dd_main("w1", n3, prep)) if isinstance(n3, list) else _dot_fine(n3, weights(w1buf, c0, c1), fine))
        for c in range(c0, c1):
            blk = hh[:, (c - c0) * 128:(c - c0 + 1) * 128]
            w["hh"][c, pl.ds(r0 + 8, n - LEAD), :] = blk[:n - LEAD]
            tail = blk[n - LEAD:]
            if last_valid is not None:
                tail = jnp.where(last_valid, tail, 0.0)
            w["hh"][c, pl.ds(r0 + 8 + n - LEAD, LEAD), :] = tail

    def stage_b1a(w, r0, n, fine=0, fast=False, prep=False):
        m = n // 2
        lane = jax.lax.broadcasted_iota(jnp.int32, (m, 128), 1)
        g = []
        for e in range(2):
            sh = lambda c, d: w["hh"][c, pl.ds(r0 + 8 + e + d, m, stride=2), :]
            g.append(jnp.concatenate([sh(0, -1),
                                      jnp.where(lane < 32, sh(1, -1), sh(1, 1)),
                                      jnp.where(lane < 64, sh(2, 1), sh(2, -2)),
                                      jnp.where(lane < 96, sh(3, -2), sh(3, 2)),
                                      sh(4, 2)], axis=1))
        if fast:
            hs = dd_main("w2", [dd_rest("w2", *g)], prep)
        else:
            hs = _dot_fine(jnp.concatenate(g, axis=0), weights(w2buf), fine)
            hs = hs[:m], hs[m:]
        x1 = [parity(w["h"], r0, n, e) + hs[e] for e in range(2)]
        for e in range(2):
            put(w["h"], pl.ds(r0 + e, m, stride=2), x1[e])
        return x1

    def stage_b1b(w, x1, r0, n):
        xn = jnp.stack([_ln(x).reshape(n // 16, 8, D) for x in x1], axis=1).reshape(n, D)
        t, b = _rows2(xn)
        w["xn"][0, pl.ds(r0 // 2, n // 2), :] = t.astype(BF16)
        w["xn"][1, pl.ds(r0 // 2, n // 2), :] = b.astype(BF16)
        sa = _sums_a(t[:, :256], t[:, 256:512], b[:, :256], b[:, 256:512])
        w["xs"][pl.ds(r0 // 2, n // 2), :] = jnp.concatenate(sa, axis=1).astype(BF16)

    def stage_b1(w, r0, n, fast=False, prep=False):
        stage_b1b(w, stage_b1a(w, r0, n, fast=fast, prep=prep), r0, n)

    def out_copy(r0, n):
        rows = pl.ds(r0, n)
        return pltpu.make_async_copy(obuf.at[rows, :], out_hbm.at[rows, :], sem_out.at[0])


    def emit(h3, j, left, right):
        m = left.shape[0] // 2
        g = [left[:m], right[:m], left[m:], right[m:]]
        for k, v in enumerate(_sums_a(*g) + g):
            v = v.reshape(m // 16, 2, 8, 128)
            h3[0][j, k, pl.ds(0, m // 2), :] = pack2(v[:, 0], v[:, 1]).reshape(m // 2, 128)

    def load_xn(w, r0, n):
        return w["xn"][:, pl.ds(r0 // 2, n // 2), :].reshape(n, D)

    def stage_b2h(w, h3, r0, n, fine=0):
        xn = load_xn(w, r0, n)
        ht = _gelu(_dot_nt(weights(w3buf, r0=FM), xn))
        ht = jnp.concatenate([ht, jnp.zeros((128 - FR, n), F32)], axis=0)
        hl = jnp.concatenate([ht[:, j:j + 128].T for j in range(0, n, 128)], axis=0)
        emit(h3, 6, _gelu(_dot_fine(xn, weights(w3buf, r0=FM - 128, r1=FM), fine, nt=True)), hl)

    def stage_b2a(w, h3, r0, n, lo=0, hi=6, prep=False):
        xn = load_xn(w, r0, n)
        xsum = w["xs"][pl.ds(r0 // 2, n // 2), :]
        m = n // 2
        ops = [xsum[:, 256 * k:256 * (k + 1)] for k in range(5)] + [xn[:m, :256], xn[m:, 256:512]]
        for j in range(lo, hi):
            r1, r2 = (_dot_nt(xn[:, 512:], weights(w3buf, 4, 5, 128 * t, 128 * (t + 1))) for t in (j, j + 6))
            c11, c12, c21, c22 = spair("w3", j, lambda i: ops[i], prep)
            emit(h3, j, _gelu(jnp.concatenate([c11, c21], axis=0) + r1), _gelu(jnp.concatenate([c12, c22], axis=0) + r2))

    def finish(w, h2, r0, n, c):
        rows, cols = pl.ds(r0, n), pl.ds(c * 128, 128)
        w["o"][rows, cols] = (w["x2"][rows, cols] + mul_mod(w["h"][c, rows, :] + h2, 5, cols)).astype(BF16)

    def stage_b2b(w, h3, r0, n, j, k0=0, k1=7, done=None, prep=False, fine=0):
        hv = h3[0].at[pl.ds(h3[1][j], 7)]
        blk = lambda k: jnp.concatenate([hv[p, k, pl.ds(0, n // 4), :] for p in range(7)], axis=1)
        if j < 2:
            done = [] if done is None else done
            done += sprods("w4", j, lambda i: _unpack(blk(8 if i == 6 else i)), k0, k1, prep)
            if k1 == 7:
                c11, c12, c21, c22 = _combine(*done)
                finish(w, _unrows2(c11, c21), r0, n, j)
                finish(w, _unrows2(c12, c22), r0, n, j + 2)
            return done
        wb = wblocks("w4", 4)
        lhs = jnp.concatenate([jnp.concatenate([blk(5), blk(6)], axis=1),
                               jnp.concatenate([blk(7), blk(8)], axis=1)], axis=0)
        h2 = _dot_fine(_unpack(lhs), _unpack(jnp.concatenate([wb(0, 0), wb(1, 0)], axis=0)), fine)
        finish(w, _unrows2(h2[:n // 2], h2[n // 2:]), r0, n, 4)

    w = window(0, 2 * TS + LEAD, 0)
    H = TS // 2
    with jax.named_scope("t0a"):
        cps["qa"].wait()
        cps["wmoda"].wait()

        mv = {}

        def mod_fn(j, toks):
            mv[j] = mod_cols(j, 1, toks)[0]
            if len(mv) == 3:
                modbuf[0] = mv[2] * mv[0]
                modbuf[1] = mv[2] * (1.0 + mv[1])

        segment(G5B, 0, MU, mod_fn=mod_fn)
        put(w["h"], pl.ds(0, QA), stage_a0(w, 0, QA))
    with jax.named_scope("t0b"):
        cps["wmodb"].wait()
        sb, cb = mod_cols(3, 2)
        modbuf[3] = sb
        modbuf[4] = 1.0 + cb
        n3 = stage_a1(w, 0, QA, n2=slabs(w["h"], 0, QA))
    XB = TS - XA
    FN = 32
    F4 = 64
    with jax.named_scope("t1a"):
        cps["w1a"].wait()
        if QXPOS != "b":
            cps["qx"].wait()
            if "1" == "1":
                put(w["h"], pl.ds(QA, XA), stage_a0(w, QA, XA))
            else:
                n3a = stage_a1(w, QA, XA)
        stage_a2(w, n3, 0, QA, c1=W1A, fine=80)
    with jax.named_scope("t1b"):
        cps["w1b"].wait()
        if QXPOS == "b":
            cps["qx"].wait()
            n3a = stage_a1(w, QA, XA)
        elif "1" == "1":
            n3a = stage_a1(w, QA, XA, n2=slabs(w["h"], QA, XA))
        stage_a2(w, n3, 0, QA, c0=W1A)
        if "0" == "1":
            stage_a2(w, n3a[:XA // 2], QA, XA // 2)
            stage_a2(w, n3a[XA // 2:], QA + XA // 2, XA // 2, fine=FN)
        else:
            stage_a2(w, n3a, QA, XA, fine=FN)
    with jax.named_scope("t2"):
        cps["qb"].wait()
        cps["w2"].wait()
        T2V = "1"
        n3b = stage_a1(w, QA + XA, XB, f32=True)
        if T2V == "1":
            stage_b1(w, 0, TS, fast=True, prep=True)
            stage_a2(w, [dd_rest("w1", *_rows2(n3b))], QA + XA, XB, prep=True)
            stage_b1(w, TS, XA, fast=True)
            stage_b1a(w, TS + XA, XB, fast=True)
        elif T2V == "2":
            stage_b1(w, 0, TS)
            stage_a2(w, [dd_rest("w1", *_rows2(n3b))], QA + XA, XB, prep=True)
            stage_b1(w, TS, XA)
            stage_b1a(w, TS + XA, XB, fast=True, prep=True)
        elif T2V == "3":
            stage_b1(w, 0, TS)
            stage_a2(w, [dd_rest("w1", *_rows2(n3b))], QA + XA, XB, prep=True)
            stage_b1(w, TS, XA, fast=True, prep=True)
            stage_b1a(w, TS + XA, XB, fast=True)
    PREP = "1" == "1"
    zs = [zsm[j] for j in range(3)]
    ha, hb = (hba, zs), (hbb, zs)
    with jax.named_scope("t3"):
        cps["w3"].wait()
        _CLOCK.clear()
        stage_b1b(w, [parity(w["h"], TS + XA, XB, e) for e in range(2)], TS + XA, XB)
        stage_b2h(w, ha, 0, TS)
        stage_b2a(w, ha, 0, TS, prep=PREP)
        stage_b2h(w, hb, TS, TS)
        for j in range(6):
            stage_b2a(w, hb, TS, TS, j, j + 1)
            if PREP and j < 4 and "no" == "t3":
                name = ("w1", "w2")[j // 2]
                for k in range(5):
                    keep(wsbufs[name].at[k, j % 2], wsum(name, j % 2, k), _CLOCK[-9 + k][1])
    with jax.named_scope("t4"):
        cps["w4"].wait()
        cps["wmodg"].wait()
        _CLOCK.clear()
        modbuf[5] = mod_cols(5, 1)[0]
        for j in (0, 1, 2):
            stage_b2b(w, ha, 0, TS, j, prep=PREP, fine=F4)
        out_copy(0, TS).start()
        cps["q1"].wait()

    CBS = (96, 96, 64)
    PART = {"a": (TS, TS), "c": (TS, H), "d": (TS + H, H)}
    BODY = "4:0:0:5 r0 4:0:5:7 4:1:0:2 r1 4:1:2:5 r2 1a 4:1:5:7 2a na 4:2 3a:0:3 ha 3a:3:6"

    def step(s, carry):
        r0 = pl.multiple_of(s * TS, TS)
        w = window(r0, 2 * TS + LEAD, pl.multiple_of(s * H, H))
        x1, rest, done = {}, {}, {0: [], 1: [], 2: None}
        for op in BODY.split():
            op, *rng = op.split(":")
            rng = [int(x) for x in rng]
            if op[0] == "3":
                stage_b2a(w, hb, TS, TS, *rng)
            elif op[0] == "h":
                stage_b2h(w, hb, TS, TS)
            elif op[0] == "4":
                stage_b2b(w, hb, 0, TS, *rng, done=done[rng[0]])
            elif op[0] == "2":
                x1[op[1]] = stage_b1a(w, *PART[op[1]], fast=True)
            elif op[0] == "n":
                stage_b1b(w, x1[op[1]], *PART[op[1]])
            elif op[0] == "r":
                j = int(op[1])
                rest[j] = dd_rest("w1", *_rows2(stage_a1(w, TS + LEAD + sum(CBS[:j]), CBS[j], f32=True)))
            else:
                ra, n = PART[op[1]]
                parts = [rest[j] for j in range(len(CBS)) if ra - TS <= sum(CBS[:j]) < ra - TS + n]
                stage_a2(w, parts, ra + LEAD, n, last_valid=(s < NT - 2) if ra + n == 2 * TS else None)
        out_copy(r0, TS).start()
        return carry

    with jax.named_scope("p2main"):
        jax.lax.fori_loop(1, NT - 1, step, 0)
    with jax.named_scope("p2epi"):
        w = window(S - 2 * TS, 2 * TS + LEAD, S // 2 - TS)
        rows = pl.ds(S - TS, TS)
        for j in range(3):
            stage_b2b(w, hb, TS, TS, j)
            if j > 0:
                cols = pl.ds(0, 512) if j == 1 else pl.ds(512, 128)
                pltpu.make_async_copy(obuf.at[rows, cols], out_hbm.at[rows, cols], sem_out.at[0]).start()
        pltpu.make_async_copy(obuf, out_hbm, sem_out.at[0]).wait()


@jax.jit
def pallas_adaLN_cond__ssm_conv_h3__mixer_s_mlp__prompt_kernel(
    A_q: jax.Array,
    A_k: jax.Array,
    A_v: jax.Array,
    A_shift_k: jax.Array,
    A_ssm_k: jax.Array,
    A_ssm_D: jax.Array,
    B_x: jax.Array,
    B_w1: jax.Array,
    B_w2: jax.Array,
    B_w3: jax.Array,
    B_w4: jax.Array,
    c: jax.Array,
    w_mod: jax.Array,
):
    del B_x

    def tiles(x):
        return x.reshape(S // 8, 8, NC, 128).transpose(0, 2, 1, 3).reshape(S * NC, 128)

    def pairs(x):
        r, n = x.shape
        return x.reshape(r // 16, 2, 8, n // 128, 128).transpose(0, 1, 3, 2, 4)

    args = (
        A_q.reshape(S, D), tiles(A_k), tiles(A_v),
        A_shift_k.T, A_ssm_k, A_ssm_D.reshape(NC, 128),
        pairs(B_w1), pairs(B_w2), pairs(B_w3.T), pairs(B_w4), c, pairs(w_mod),
    )
    scratch = [
        pltpu.VMEM((NA, P * NC + 128, 128), BF16),
        pltpu.VMEM((NA, P * NC + 64, 128), BF16),
        pltpu.VMEM((D, S), BF16),
        pltpu.VMEM((R, 128, 128), U32),
        pltpu.VMEM((R, 64, 256), U32),
        pltpu.VMEM((64, 128), U32),
        pltpu.VMEM((D // 16, 6 * NC, 16, 128), BF16),
        pltpu.VMEM((D // 16, NC, 16, 128), BF16),
        pltpu.VMEM((D // 16, NC, 16, 128), BF16),
        pltpu.VMEM((FF // 16, NC, 16, 128), BF16),
        pltpu.VMEM((FF // 16, NC, 16, 128), BF16),
        pltpu.VMEM((S + 64, D), BF16),
        *[pltpu.VMEM((NA, R, 16, 4, 8, 128), F32) for _ in range(NC)],
        pltpu.VMEM((NC, NA - 1, R, 16, 2, 8, 128), F32),
        pltpu.VMEM((NC, R, 128, 128), U32),
        pltpu.VMEM((32, 128), U32),
        pltpu.VMEM((NC, 8, 8, 128), F32),
        pltpu.VMEM((NC, S + 32, 128), F32),
        pltpu.VMEM((8, 8, D), F32),
        pltpu.VMEM((S + 32, D), F32),
        pltpu.VMEM((NC, S + 32, 128), F32),
        pltpu.VMEM((NC, S + 32, 128), F32),
        pltpu.VMEM((2, S // 2, D), BF16),
        pltpu.VMEM((S // 2, 5 * 256), BF16),
        pltpu.VMEM((5, 2, 128, 128), U32),
        pltpu.VMEM((5, 2, 128, 128), U32),
        pltpu.VMEM((5, 6, 64, 256), U32),
        pltpu.VMEM((5, 2, 448, 128), U32),
        pltpu.VMEM((8, 9, 72, 128), U32),
        pltpu.VMEM((8, 9, 72, 128), U32),
        pltpu.VMEM((S, D), BF16),
        pltpu.VMEM((4, D), BF16),
        pltpu.VMEM((NC, 128), BF16),
        pltpu.VMEM((1, D), BF16),
        pltpu.SMEM((8,), jnp.int32),
        pltpu.SemaphoreType.DMA((40,)),
        pltpu.SemaphoreType.DMA((1,)),
    ]
    out = pl.pallas_call(
        _kernel,
        out_shape=jax.ShapeDtypeStruct((S, D), BF16),
        in_specs=[pl.BlockSpec(memory_space=pl.ANY)] * len(args),
        out_specs=pl.BlockSpec(memory_space=pl.ANY),
        scratch_shapes=scratch,
        grid=(1,),
        compiler_params=pltpu.CompilerParams(vmem_limit_bytes=100 * 1024 * 1024, disable_semaphore_checks=True,
                                             disable_bounds_checks=True),
        name="adaln_h3_mixer",
    )(*args)
    return out.reshape(1, S, D)
```

```python
import numpy as np
import jax
import jax.numpy as jnp
import jax.experimental.pallas as pl
import jax.experimental.pallas.tpu as pltpu

F32 = jnp.float32
BF16 = jnp.bfloat16
U32 = jnp.uint32

S = 2048
D = 640
FF = 1728
NC = D // 128
R = 4
P = 128 * R
NA = S // P
TS = 256
NT = S // TS
LEAD = 16
EPS = 1e-5
FT = (FF - 1536) // 2
FM = (FF // 128) * 128
FR = FF - FM
P1_ORDER = "t0 t1 t2 t3 k0 k1 k2 k3 u0 i0 u1 i1 u2 i2 u3 i3"


def _freq(row):
    t, part, s = row >> 4, (row >> 3) & 1, row & 7
    return 32 * (t & 7) + 4 * s + 2 * (t >> 3) + 1, P * part


def _cos(j, scale):
    jf = (j & (4 * P - 1)).astype(F32)
    u = 2.0 * np.pi / (4 * P)
    x = jnp.abs(jf * u - np.pi) - 0.5 * np.pi
    x2 = x * x
    poly = scale / 362880.0 - x2 * (scale / 39916800.0)
    for coef in (-1.0 / 5040.0, 1.0 / 120.0, -1.0 / 6.0, 1.0):
        poly = poly * x2 + coef * scale
    return poly * x


_DUR = {"t": 8, "u": 16, "k": 16, "i": 16, "m": 12, "g": 0, "c": 0, "j": 16}
_POST = {"t": 8.0, "u": 16.0, "k": 24.0, "i": 4.0, "j": 4.0, "m": 18.0}


def _plan_tokens(order, maxutil):
    lag, cap, pre, margin = 8, 60, 4, 3
    start, slots = {}, []
    for n in order:
        start[n] = len(slots)
        slots += [(n, r) for r in range(_DUR[n[0]])]
    nslot = len(slots) + lag
    free = [cap - (_POST[slots[i - lag][0][0]] if i >= lag else 0.0) for i in range(-pre, nslot)]
    units = []
    for n in order:
        kind, a, c = n
        if kind == "u":
            units += [(n + (g,), 94.0, start[n], -pre) for g in range(8)]
        elif kind == "g":
            units += [(n + (g,), 150.0, start[n], -pre) for g in range(8)]
        elif kind in "ic":
            src_ = [start[m] for m in (("u", a, c), ("k", a, c)) if m in start]
            for t in range(16):
                rel = max(max(src_) + 16, max(src_) + t + lag + 3) if src_ else -pre
                units.append((n + (t,), 32.0 * a + 48.0, nslot if kind == 'c' else start[n], rel))

    def simulate(util):
        left = [u[1] for u in units]
        done = [None] * len(units)
        for i in range(-pre, nslot):
            budget = util * free[i + pre]
            for j, u in enumerate(units):
                if budget <= 0.0:
                    break
                if done[j] is None and u[3] <= i:
                    use = min(budget, left[j])
                    left[j] -= use
                    budget -= use
                    if left[j] <= 1e-9:
                        done[j] = i + 1
        ok = all(u[2] < 8 or (d is not None and d <= max(u[2] - (1 if u[0][0] in 'cg' else margin), u[3] + 1))
                 for d, u in zip(done, units))
        return done, ok

    lo_, hi_ = 0.05, maxutil
    for _ in range(12):
        mid = 0.5 * (lo_ + hi_)
        if simulate(mid)[1]:
            hi_ = mid
        else:
            lo_ = mid
    done, _ = simulate(hi_)
    plan = {}
    for u, d in zip(units, done):
        if u[0][0] == "c":
            plan[u[0]] = slots[max((nslot - 1 if d is None else min(d, nslot - 1)) - lag, 0)]
        elif d is not None and 0 <= d < u[2]:
            plan.setdefault(slots[d], []).append(u[0])
    return plan


def _pack(x):
    return pltpu.bitcast(x.astype(BF16), U32)


def _unpack(w):
    return pltpu.bitcast(w, BF16)


def _dot(a, b):
    return jnp.dot(a.astype(BF16), b, preferred_element_type=F32)


def _dot_nt(a, b):
    return jax.lax.dot_general(a.astype(BF16), b, (((1,), (1,)), ((), ())), preferred_element_type=F32)


def _dot_fine(x, w, chunk, nt=False):
    if not chunk:
        return _dot_nt(x, w) if nt else _dot(x, w)
    n = w.shape[0] if nt else w.shape[1]
    head, last = (w[:n - 128], w[n - 128:]) if nt else (w[:, :n - 128], w[:, n - 128:])
    f = _dot_nt if nt else _dot
    parts = [f(x, head)] if n > 128 else []
    parts.append(jnp.concatenate([f(x[r:r + chunk], last) for r in range(0, x.shape[0], chunk)], axis=0))
    return jnp.concatenate(parts, axis=1)


def _rows2(x):
    n, c = x.shape
    x = x.reshape(n // 32, 2, 16, c)
    return x[:, 0].reshape(n // 2, c), x[:, 1].reshape(n // 2, c)


def _unrows2(top, bot):
    n, c = top.shape
    return jnp.stack([top.reshape(n // 16, 16, c), bot.reshape(n // 16, 16, c)], axis=1).reshape(2 * n, c)


def _sums_a(a11, a12, a21, a22):
    return [a11 + a22, a21 + a22, a11 + a12, a21 - a11, a12 - a22]


def _sums_b(b11, b12, b21, b22):
    return [b11 + b22, b12 - b22, b21 - b11, b11 + b12, b21 + b22]


_STRASSEN = ((0, 0), (1, 5), (5, 1), (6, 2), (2, 6), (3, 3), (4, 4))


def _combine(m1, m2, m3, m4, m5, m6, m7):
    return (m1 + m4) + (m7 - m5), m3 + m5, m2 + m4, (m1 - m2) + (m3 + m6)


def _lo(w):
    return pltpu.bitcast(w << 16, F32)


def _hi(w):
    return pltpu.bitcast(w & jnp.uint32(0xFFFF0000), F32)


def _ln(x, eps=EPS):
    m = jnp.sum(x, axis=-1, keepdims=True) * (1.0 / D)
    xc = x - m
    v = jnp.sum(xc * xc, axis=-1, keepdims=True) * (1.0 / D)
    return xc * jnp.exp(-0.5 * jnp.log(v + eps))


def _gelu2(x):
    c0 = 0.7978845608028654
    c1 = c0 * 0.044715
    return x + x * jnp.tanh(x * (c0 + c1 * (x * x)))


def _bfly(tr, ti, sign):
    s02r, s02i = tr[0] + tr[2], ti[0] + ti[2]
    d02r, d02i = tr[0] - tr[2], ti[0] - ti[2]
    s13r, s13i = tr[1] + tr[3], ti[1] + ti[3]
    d13r, d13i = tr[1] - tr[3], ti[1] - ti[3]
    x0r, x0i = s02r + s13r, s02i + s13i
    x2r, x2i = s02r - s13r, s02i - s13i
    ar, ai = d02r + d13i, d02i - d13r
    br, bi = d02r - d13i, d02i + d13r
    if sign < 0:
        return [x0r, ar, x2r, br], [x0i, ai, x2i, bi]
    return [x0r, br, x2r, ar], [x0i, bi, x2i, ai]


def _kernel(q_hbm, k_hbm, v_hbm, shift_hbm, ssmk_hbm, ssmd_hbm, w1_hbm, w2_hbm, w3t_hbm, w4_hbm,
            c_hbm, wmod_hbm,
            out_hbm,
            kbuf, vbuf, skbuf, fwdbuf, invbuf, permbuf,
            wmodbuf, w1buf, w2buf, w3buf, w4buf, qbuf,
            xs0, xs1, xs2, xs3, xs4, kraw, wbuf, zbuf, coefbuf, ybuf, modbuf, x2buf, hbuf, hhbuf, xnbuf, xsbuf,
             w1s, w2s, w3s, w3ts, w4s, hba, hbb, obuf, shiftbuf, dbuf, cbuf,
            zsm, sem_in, sem_out):
    cps = {}
    n_sem = [0]

    def start(name, src, dst):
        cp = pltpu.make_async_copy(src, dst, sem_in.at[n_sem[0]])
        n_sem[0] += 1
        cp.start()
        cps[name] = cp

    class Both:
        def __init__(self, a, b):
            self.cps = (a, b)

        def wait(self):
            for cp in self.cps:
                cp.wait()

    def start_w(name, src, dst, c0=0, n=NC):
        for e in range(2):
            start(name + str(e), src.at[:, e, pl.ds(c0, n)], dst.at[:, pl.ds(c0, n), pl.ds(8 * e, 8), :])
        cps[name] = Both(cps[name + "0"], cps[name + "1"])

    CH = P * NC
    HALO = 8 * NC

    def start_s(a):
        cols = pl.ds(a * P, P)
        start("s%d" % a, ssmk_hbm.at[:, cols], skbuf.at[:, cols])

    def start_kv(a):
        if a == 0:
            start("k0", k_hbm.at[pl.ds(0, CH), :], kbuf.at[0, pl.ds(HALO, CH), :])
        else:
            start("k%d" % a, k_hbm.at[pl.ds(a * CH - HALO, CH + HALO), :], kbuf.at[a, pl.ds(0, CH + HALO), :])
        start("v%d" % a, v_hbm.at[pl.ds(a * CH, CH), :], vbuf.at[a, pl.ds(0, CH), :])

    for n in "s0 x0 s1 k0 k1 s2 k2 s3 k3".split():
        if n[0] == "s":
            start_s(int(n[1]))
        elif n[0] == "k":
            start_kv(int(n[1]))
        else:
            start("d", ssmd_hbm, dbuf)
            start("shift", shift_hbm, shiftbuf)
            start("c", c_hbm, cbuf)
    QA = TS + LEAD
    XA = 128
    QB = 2 * TS + LEAD
    W1A = 2
    QXPOS = "a"

    def start_q(name, r0, n):
        start(name, q_hbm.at[pl.ds(r0, n), :], qbuf.at[pl.ds(r0, n), :])

    start_q("qa", 0, QA)
    if QXPOS == "0":
        start_q("qx", QA, XA)
    start_w("wmoda", wmod_hbm, wmodbuf, 0, 3 * NC)
    start_w("wmodb", wmod_hbm, wmodbuf, 3 * NC, 2 * NC)
    if QXPOS == "a":
        start_q("qx", QA, XA)
    start_w("w1a", w1_hbm, w1buf, 0, W1A)
    if QXPOS == "b":
        start_q("qx", QA, XA)
    start_w("w1b", w1_hbm, w1buf, W1A, NC - W1A)
    start_q("qb", QA + XA, QB - QA - XA)
    start_w("w2", w2_hbm, w2buf)
    start_w("w3", w3t_hbm, w3buf)
    start_w("w4", w4_hbm, w4buf)
    start_w("wmodg", wmod_hbm, wmodbuf, 5 * NC, NC)
    start_q("q1", QB, S - QB)

    kw = kbuf.bitcast(U32)
    vw = vbuf.bitcast(U32)
    kbuf[0, pl.ds(0, HALO), :] = jnp.zeros((HALO, 128), BF16)
    zbuf[...] = jnp.zeros(zbuf.shape, U32)
    for j in range(8):
        zsm[j] = 0
    for c in range(NC):
        ybuf[c, pl.ds(S, LEAD), :] = jnp.zeros((LEAD, 128), F32)
        hhbuf[c, pl.ds(0, 8), :] = jnp.zeros((8, 128), F32)
    qbuf[pl.ds(S, LEAD), :] = jnp.zeros((LEAD, D), BF16)

    def tables(p, carry):
        i0 = jax.lax.broadcasted_iota(jnp.int32, (128, 128), 0)
        n = R * jax.lax.broadcasted_iota(jnp.int32, (128, 128), 1) + p
        f2, off = _freq(2 * i0)
        j = f2 * n + off
        fwdbuf[p] = pltpu.pack_elementwise([_cos(j, 1.0), _cos(j + 4 * n, 1.0)], packed_dtype=BF16)
        return carry

    jax.lax.fori_loop(0, R, tables, 0)

    def unit_g(kt, r):
        col = jax.lax.broadcasted_iota(jnp.int32, (8, 128), 1) + 128 * kt
        f2, off = _freq((col & ~15) + 8 * (col & 1) + ((col >> 1) & 7))
        m = 2 * jax.lax.broadcasted_iota(jnp.int32, (8, 128), 0) + 16 * r
        j0 = f2 * (R * m) + off
        out = []
        for p in range(R):
            j = j0 + p * f2
            out.append(pltpu.pack_elementwise([_cos(j, 1.0 / P), _cos(j + R * f2, 1.0 / P)], packed_dtype=BF16))
            invbuf[p, pl.ds(8 * r, 8), pl.ds(128 * kt, 128)] = out[-1]
        return out

    i0 = jax.lax.broadcasted_iota(jnp.int32, (128, 128), 0)
    i1 = jax.lax.broadcasted_iota(jnp.int32, (128, 128), 1)
    permbuf[...] = _pack(jnp.where(i0 == (128 // R) * (i1 & (R - 1)) + (i1 >> 2), 1.0, 0.0).astype(F32))

    def fill_coef():
        coef = shiftbuf[...].astype(F32)
        dval = dbuf[...].astype(F32)
        for c in range(NC):
            for j in range(4):
                coefbuf[c, j] = jnp.broadcast_to(coef[j:j + 1, c * 128:(c + 1) * 128], (8, 128))
            coefbuf[c, 4] = jnp.broadcast_to(dval[c:c + 1, :], (8, 128))

    xs = (xs0, xs1, xs2, xs3, xs4)
    wsbufs = dict(w1=w1s, w2=w2s, w3=w3s, w4=w4s, w3t=w3ts)
    def split_ri(t):
        t = t.reshape(16, 2, 8, 128)
        return t[:, 0], t[:, 1]

    def get_never():
        return zbuf[pl.ds(0, 8), :] != 0

    def pack2(x, y):
        return pltpu.pack_elementwise([x, y], packed_dtype=BF16)

    def words(ref, a, c, r):
        return ref[a, pl.ds((r // 4) * 4 * NC + 4 * c + r % 4, 8, stride=4 * NC), :]

    def unit_u(a, c, g):
        c0, c1, c2, c3 = (coefbuf[c, pl.ds(j, 1)] for j in range(4))
        kk = jnp.stack([words(kw, a, c, 4 + 32 * g + d) for d in range(-2, 4)])
        vv = jnp.stack([words(vw, a, c, 32 * g + d) for d in range(4)])
        lo, hi = _lo(kk), _hi(kk)
        k0, k1, k2 = lo[2:], hi[1:5], lo[1:5]
        even = (((k0 * c0 + k1 * c1) + (k2 * c2 + hi[:4] * c3)) * _lo(vv)).reshape(32, 128)
        odd = (((hi[2:] * c0 + k0 * c1) + (k1 * c2 + k2 * c3)) * _hi(vv)).reshape(32, 128)
        e, o = pack2(even[:16], even[16:]), pack2(odd[:16], odd[16:])
        return [e[:8], o[:8], e[8:], o[8:]]

    def unit_i(a, c, t, z):
        x_c = xs[c].at[pl.ds(z, NA)]
        yr = yi = None
        for j in range(a + 1):
            ur, ui = x_c[j, :, t, 0], x_c[j, :, t, 1]
            kr, ki = x_c[a - j, :, t, 2], x_c[a - j, :, t, 3]
            pr = ur * kr - ui * ki
            pi = ur * ki + ui * kr
            yr = pr if yr is None else yr + pr
            yi = pi if yi is None else yi + pi
        halves = lambda x: (x[:x.shape[0] // 2], x[x.shape[0] // 2:])
        (ra, rb), (ia, ib) = halves(yr.reshape(32, 128)), halves(yi.reshape(32, 128))
        (sr0, sr1), (si0, si1), (dr0, dr1), (di0, di1) = (halves(x) for x in (ra + rb, ia + ib, ra - rb, ia - ib))
        return [pack2(sr0 + sr1, si0 + si1), pack2(dr0 - di1, di0 + dr1),
                pack2(sr0 - sr1, si0 - si1), pack2(dr0 + di1, di0 - dr1)]

    def segment(spec, z, maxutil=1.0, mod_fn=None):
        order = [(n[0], int(n[1]), int(n[2])) for n in spec.split()]
        plan = _plan_tokens(order, maxutil) if maxutil > 0 else {}
        never = get_never()
        units, res = {}, {}

        def unit(key):
            if key not in units:
                kind, a, c, j = key
                if kind == "u":
                    units[key] = unit_u(a, c, j)
                elif kind == "g":
                    units[key] = unit_g(a, j)
                else:
                    fresh = ("u", a, c) in order or ("k", a, c) in order
                    units[key] = unit_i(a, c, j, z if fresh else 0)
            return units[key]

        def lhs(name, p, full, r0=0):
            out, last = [], 0
            for r in range(full.shape[0] // 8):
                keys = plan.get((name, r0 + r), ())
                if keys:
                    if 8 * r > last:
                        out.append(full[last:8 * r])
                    v = full[8 * r:8 * r + 8]
                    for key in keys:
                        v = jax.lax.select(never, unit(key)[p], v)
                    out.append(v)
                    last = 8 * r + 8
            if last < full.shape[0]:
                out.append(full[last:] if last else full)
            return out[0] if len(out) == 1 else jnp.concatenate(out, axis=0)

        def dft(name, rhs):
            tr, ti = [], []
            for p in range(R):
                f = lhs(name, p, fwdbuf[p])
                r_, i_ = split_ri(_dot(_unpack(f), rhs[p]))
                if p == 0:
                    res.update({(name, r): (lambda r=r, v=r_: v[r]) for r in range(16)})
                tr.append(r_)
                ti.append(i_)
            return _bfly(tr, ti, -1)

        st = {}
        for name in order:
            kind, a, c = name
            x_c = xs[c]
            if kind == "g":
                for r in range(8):
                    unit(name + (r,))
            elif kind == "c":
                for t in range(16):
                    after = pltpu.bitcast(res[plan[name + (t,)]](), U32)
                    for p in range(R):
                        wbuf[c, p, pl.ds(8 * t, 8), :] = jax.lax.select(never, after, unit(name + (t,))[p])
            elif kind == "m":
                toks = {}
                for r in range(_DUR["m"]):
                    for n_, key in enumerate(plan.get((name, r), ())):
                        toks.setdefault(2 * r + n_ % 2, []).extend(unit(key))
                mod_fn(a, toks)
            elif kind == "t":
                trs = []
                for b in range(R):
                    pm = lhs(name, b, permbuf[...])
                    trs.append(_dot_nt(_unpack(pm), skbuf[pl.ds(c * 128, 128), pl.ds(a * P + b * 128, 128)]))
                res.update({(name, r): (lambda r=r, v=trs[0]: v[16 * r:16 * r + 8]) for r in range(8)})
                g_ = 128 // R
                st[a, c] = [jnp.concatenate([trs[b][p * g_:(p + 1) * g_] for b in range(R)], axis=0).astype(BF16)
                            for p in range(R)]
            elif kind == "u":
                rhs = [_unpack(jnp.concatenate([unit(name + (g,))[p] for g in range(8)], axis=0)) for p in range(R)]
                xr, xi = dft(name, rhs)
                for q in range(R):
                    x_c[a, q, :, 0] = xr[q]
                    x_c[a, q, :, 1] = xi[q]
            elif kind == "k":
                xr, xi = dft(name, st[a, c])
                for q in range(R):
                    if a == 0:
                        x_c[a, q, :, 2] = xr[q] + coefbuf[c, 4]
                        x_c[a, q, :, 3] = xi[q]
                    else:
                        pr, pi = kraw[c, a - 1, q, :, 0], kraw[c, a - 1, q, :, 1]
                        x_c[a, q, pl.ds(0, 8), 2] = xr[q][:8] - pi[:8]
                        x_c[a, q, pl.ds(0, 8), 3] = xi[q][:8] + pr[:8]
                        x_c[a, q, pl.ds(8, 8), 2] = xr[q][8:] + pi[8:]
                        x_c[a, q, pl.ds(8, 8), 3] = xi[q][8:] - pr[8:]
                    if a + 1 < NA:
                        kraw[c, a, q, :, 0] = xr[q]
                        kraw[c, a, q, :, 1] = xi[q]
            else:
                for p in range(R):
                    cols = [lhs(name, 2 * (p % 2) + kt,
                                invbuf[p, :, pl.ds(128 * kt, 128)], 8 * (p // 2))
                            for kt in range(2)]
                    g = _unpack(jnp.concatenate(cols, axis=1))
                    if kind == "j":
                        wp = _unpack(wbuf[c, p])
                    else:
                        wp = _unpack(jnp.concatenate([unit(name + (t,))[p] for t in range(16)], axis=0))
                    yp = _dot(g, wp)
                    if p % 2 == 0:
                        res.update({(name, 4 * p + r): (lambda r=r, v=yp: v[16 * r:16 * r + 8]) for r in range(8)})
                    ybuf[c, pl.ds(a * P + p, 128, stride=R), :] = yp

    one = jnp.minimum(pl.program_id(0) + 1, 1)

    def once(fn):
        def body(z, carry):
            fn(z)
            return carry
        jax.lax.fori_loop(0, one, body, 0)

    default = "t00 t01 t02 k00 t03 k01 t04 k02 k03 k04 g00|t10 t11 t12 k10 k11 k12 g10|t13 t14 k13 u00 k14 u01 u02 u03 i00 u04 i01 c02 c03|j02 j03 u10 i04 u11 u12 u13 i10 u14 i11 c12|t20 t21 j12 t22 t23 t24 k20 u20 k21 u21 k22 i13 k23 u22 k24 i14 u23 i20 u24 i21 c22|t30 t31 j22 t32 t33 t34 k30 u30 k31 u31 k32 i23 k33 u32 k34 i24 u33 i30 u34 i31 c32|m00 j32 m10 m20 i33 i34"
    specs = default.split("|")
    G5B = specs[-1]
    segs = list(zip("s0 d shift c|s1|k0 v0|k1 v1|s2 k2 v2|s3 k3 v3".split("|"), specs[:-1]))
    MU = 1.5
    for i, (waits, spec) in enumerate(segs):
        with jax.named_scope("g%d" % i):
            for n in waits.split():
                cps[n].wait()
            if i == 0:
                fill_coef()
            once(lambda z: segment(spec, z, MU))

    def mod_cols(lo, n, toks=None):
        cv = cbuf[...].astype(F32)
        sc = (cv * jax.nn.sigmoid(cv)).astype(BF16)
        m = _dot(jnp.broadcast_to(sc, (8, D)), weights(wmodbuf, lo * NC, (lo + n) * NC, toks=toks))
        return [m[:, j * D:(j + 1) * D] for j in range(n)]

    def mul_mod(x, j, cols=None):
        m = modbuf[j] if cols is None else modbuf[j, :, cols]
        return (x.reshape(-1, 8, x.shape[-1]) * m[None]).reshape(x.shape)

    def add_mod(x, j):
        return (x.reshape(-1, 8, x.shape[-1]) + modbuf[j][None]).reshape(x.shape)

    def slabs(ref, r0, n):
        return jnp.concatenate([ref[c, pl.ds(r0, n), :] for c in range(NC)], axis=1)

    def put(ref, rows, x):
        for c in range(NC):
            ref[c, rows, :] = x[:, c * 128:(c + 1) * 128]

    def parity(ref, r0, n, e):
        return jnp.concatenate([ref[c, pl.ds(r0 + e, n // 2, stride=2), :] for c in range(NC)], axis=1)

    def window(base, n, half):
        rows = pl.ds(base, n)
        return dict(xs=xsbuf.at[pl.ds(half, (n - LEAD) // 2), :],
                    q=qbuf.at[rows, :], y=ybuf.at[:, rows, :], x2=x2buf.at[rows, :], h=hbuf.at[:, rows, :],
                    hh=hhbuf.at[:, pl.ds(base, n + 8), :], xn=xnbuf.at[:, pl.ds(half, (n - LEAD) // 2), :],
                    o=obuf.at[pl.ds(base, n - LEAD), :])

    def weights(ref, c0=0, c1=NC, r0=0, r1=None, toks=None, raw=False, z=None):
        r1 = 16 * ref.shape[0] if r1 is None else r1
        view = ref.bitcast(U32)
        if z is not None:
            view = view.at[pl.ds(z, ref.shape[0])]
        never = get_never() if toks else None
        rt = -(-(r1 - r0) // 128)
        cols = []
        for j in range(c0, c1):
            wu = view[pl.ds(r0 // 16, (r1 - r0) // 16), j].reshape((r1 - r0) // 2, 128)
            if toks:
                parts, last = [], 0
                for i in range(rt):
                    for n_, t in enumerate(toks.get((j - c0) * rt + i, ())):
                        r = 64 * i + 8 * n_
                        if r > last:
                            parts.append(wu[last:r])
                        parts.append(jax.lax.select(never, t, wu[r:r + 8]))
                        last = r + 8
                parts.append(wu[last:])
                wu = jnp.concatenate(parts, axis=0)
            cols.append(wu)
        wu = jnp.concatenate(cols, axis=1)
        return wu if raw else _unpack(wu)

    def wblocks(name, j, z=None):
        if name == "w3":
            blk = lambda kh, nh: weights(w3buf, 2 * kh, 2 * kh + 2, 128 * (j + 6 * nh), 128 * (j + 6 * nh + 1), raw=True, z=z)
        elif name == "w4":
            def blk(kh, nh):
                c = j + 2 * nh
                parts = [weights(w4buf, c, c + 1, 768 * kh, 768 * (kh + 1), raw=True, z=z),
                         weights(w4buf, c, c + 1, 1536 + FT * kh, 1536 + FT * (kh + 1), raw=True, z=z),
                         jnp.zeros(((128 - FT) // 2, 128), U32)]
                return jnp.concatenate(parts, axis=0)
        elif name == "w3t":
            blk = lambda kh, nh: weights(w3buf, 2 * kh, 2 * kh + 2, 1536 + FT * nh, 1536 + FT * (nh + 1), raw=True, z=z)
        else:
            ref = w1buf if name == "w1" else w2buf
            blk = lambda kh, nh: weights(ref, j + 2 * nh, j + 2 * nh + 1, 256 * kh, 256 * (kh + 1), raw=True, z=z)
        return blk

    def wsum(name, j, k):
        blk = wblocks(name, j, zsm[k])
        p, q, sign = ((0, 3, 1), (1, 3, -1), (2, 0, -1), (0, 1, 1), (2, 3, 1))[k]
        x, y = blk(p // 2, p % 2), blk(q // 2, q % 2)
        if sign > 0:
            return pack2(_lo(x) + _lo(y), _hi(x) + _hi(y))
        return pack2(_lo(x) - _lo(y), _hi(x) - _hi(y))

    pending = []

    def attach(wv):
        if not pending:
            return wv
        never = get_never()
        rows = [wv[8 * i:8 * i + 8, :128] for i in range(8)]
        for i, t in enumerate(pending):
            rows[i % 8] = jax.lax.select(never, pltpu.bitcast(t, U32), rows[i % 8])
        pending.clear()
        first = jnp.concatenate(rows + ([wv[64:, :128]] if wv.shape[0] > 64 else []), axis=0)
        return first if wv.shape[1] == 128 else jnp.concatenate([first, wv[:, 128:]], axis=1)

    def sprods(name, j, lhs, k0=0, k1=7, prep=False):
        blk, buf = wblocks(name, j), wsbufs[name]
        out = []
        for ia, ib in _STRASSEN[k0:k1]:
            wv = blk(ib - 5, ib - 5) if ib >= 5 else (wsum(name, j, ib) if prep else buf[ib, j])
            if name == "w3t":
                out.append(_dot_nt(_unpack(wv), lhs(ia)))
            else:
                out.append((_dot_nt if name == "w3" else _dot)(lhs(ia), _unpack(attach(wv))))
            if prep and ib < 5:
                buf[ib, j] = wv
        return out

    def spair(name, j, lhs, prep=False):
        return _combine(*sprods(name, j, lhs, prep=prep))

    def dd_rest(name, t, b):
        ref = w1buf if name == "w1" else w2buf
        m = t.shape[0]
        xb = jnp.concatenate([t, b], axis=0)
        last = _dot(xb, weights(ref, 4, 5))
        rem = _dot(xb[:, 512:], weights(ref, 0, 4, r0=512))
        return t, b, rem[:m], rem[m:], last[:m], last[m:]

    def dd_main(name, parts, prep=False):
        t, b, rt, rb, lt, lb = (jnp.concatenate(v, axis=0) for v in zip(*parts))
        ops = _sums_a(t[:, :256], t[:, 256:512], b[:, :256], b[:, 256:512]) + [t[:, :256], b[:, 256:512]]
        top, bot = [None] * 4, [None] * 4
        for j in range(2):
            top[j], top[j + 2], bot[j], bot[j + 2] = spair(name, j, lambda i: ops[i], prep)
        return (jnp.concatenate([jnp.concatenate(top, axis=1) + rt, lt], axis=1),
                jnp.concatenate([jnp.concatenate(bot, axis=1) + rb, lb], axis=1))

    def stage_a0(w, r0, n):
        rows = pl.ds(r0, n)
        x = w["q"][rows, :].astype(F32)
        x2 = x + add_mod(mul_mod(_ln(x), 1), 0) * slabs(w["y"], r0, n)
        w["x2"][rows, :] = x2
        return _ln(x2)

    def stage_a1(w, r0, n, n2=None, f32=False):
        if n2 is None:
            n2 = stage_a0(w, r0, n)
        h = add_mod(mul_mod(n2, 4), 3)
        put(w["h"], pl.ds(r0, n), h)
        n3 = _ln(h, 4 * EPS)
        return n3 if f32 else n3.astype(BF16)

    def stage_a2(w, n3, r0, n, last_valid=None, fine=0, c0=0, c1=NC, prep=False):
        hh = _gelu2(_unrows2(*dd_main("w1", n3, prep)) if isinstance(n3, list) else _dot_fine(n3, weights(w1buf, c0, c1), fine))
        for c in range(c0, c1):
            blk = hh[:, (c - c0) * 128:(c - c0 + 1) * 128]
            w["hh"][c, pl.ds(r0 + 8, n - LEAD), :] = blk[:n - LEAD]
            tail = blk[n - LEAD:]
            if last_valid is not None:
                tail = jnp.where(last_valid, tail, 0.0)
            w["hh"][c, pl.ds(r0 + 8 + n - LEAD, LEAD), :] = tail

    def stage_b1a(w, r0, n, fine=0, fast=False, prep=False):
        m = n // 2
        lane = jax.lax.broadcasted_iota(jnp.int32, (m, 128), 1)
        g = []
        for e in range(2):
            sh = lambda c, d: w["hh"][c, pl.ds(r0 + 8 + e + d, m, stride=2), :]
            g.append(jnp.concatenate([sh(0, -1),
                                      jnp.where(lane < 32, sh(1, -1), sh(1, 1)),
                                      jnp.where(lane < 64, sh(2, 1), sh(2, -2)),
                                      jnp.where(lane < 96, sh(3, -2), sh(3, 2)),
                                      sh(4, 2)], axis=1))
        if fast:
            hs = dd_main("w2", [dd_rest("w2", *g)], prep)
        else:
            hs = _dot_fine(jnp.concatenate(g, axis=0), weights(w2buf), fine)
            hs = hs[:m], hs[m:]
        x1 = [parity(w["h"], r0, n, e) + hs[e] for e in range(2)]
        for e in range(2):
            put(w["h"], pl.ds(r0 + e, m, stride=2), x1[e])
        return x1

    def stage_b1b(w, x1, r0, n):
        xn = jnp.stack([_ln(x, 4 * EPS).reshape(n // 16, 8, D) for x in x1], axis=1).reshape(n, D)
        t, b = _rows2(xn)
        w["xn"][0, pl.ds(r0 // 2, n // 2), :] = t.astype(BF16)
        w["xn"][1, pl.ds(r0 // 2, n // 2), :] = b.astype(BF16)
        sa = _sums_a(t[:, :256], t[:, 256:512], b[:, :256], b[:, 256:512])
        w["xs"][pl.ds(r0 // 2, n // 2), :] = jnp.concatenate(sa, axis=1).astype(BF16)

    def stage_b1(w, r0, n, fast=False, prep=False):
        stage_b1b(w, stage_b1a(w, r0, n, fast=fast, prep=prep), r0, n)

    def out_copy(r0, n):
        rows = pl.ds(r0, n)
        return pltpu.make_async_copy(obuf.at[rows, :], out_hbm.at[rows, :], sem_out.at[0])


    def packrows(v):
        v = v.reshape(v.shape[0] // 16, 2, 8, 128)
        return pack2(v[:, 0], v[:, 1]).reshape(-1, 128)

    def emit(h3, j, left, right):
        m = left.shape[0] // 2
        g = [left[:m], right[:m], left[m:], right[m:]]
        for k, v in enumerate(_sums_a(*g) + g):
            h3[j, k, pl.ds(0, m // 2), :] = packrows(v)

    def load_xn(w, r0, n):
        return w["xn"][:, pl.ds(r0 // 2, n // 2), :].reshape(n, D)

    def w3_operands(w, r0, n):
        xn = load_xn(w, r0, n)
        xsum = w["xs"][pl.ds(r0 // 2, n // 2), :]
        m = n // 2
        return xn, [xsum[:, 256 * k:256 * (k + 1)] for k in range(5)] + [xn[:m, :256], xn[m:, 256:512]]

    def stage_b2h(w, h3, r0, n, prep=False):
        xn, ops = w3_operands(w, r0, n)
        m = n // 2
        rem = _dot_nt(weights(w3buf, 4, 5, r0=1536), xn[:, 512:])
        c11, c12, c21, c22 = spair("w3t", 0, lambda i: ops[i], prep)
        pad = jnp.zeros((128 - FT, m), F32)
        g11, g12, g21, g22 = (jnp.concatenate([_gelu2(c + r), pad], axis=0).T for c, r in (
            (c11, rem[:FT, :m]), (c12, rem[FT:, :m]), (c21, rem[:FT, m:]), (c22, rem[FT:, m:])))
        emit(h3, 6, jnp.concatenate([g11, g21], axis=0), jnp.concatenate([g12, g22], axis=0))

    def stage_b2a(w, h3, r0, n, lo=0, hi=6, prep=False):
        xn, ops = w3_operands(w, r0, n)
        for j in range(lo, hi):
            r1, r2 = (_dot_nt(xn[:, 512:], weights(w3buf, 4, 5, 128 * t, 128 * (t + 1))) for t in (j, j + 6))
            c11, c12, c21, c22 = spair("w3", j, lambda i: ops[i], prep)
            emit(h3, j, _gelu2(jnp.concatenate([c11, c21], axis=0) + r1), _gelu2(jnp.concatenate([c12, c22], axis=0) + r2))

    def finish(w, h2, r0, n, c):
        rows, cols = pl.ds(r0, n), pl.ds(c * 128, 128)
        w["o"][rows, cols] = (w["x2"][rows, cols] + mul_mod(w["h"][c, rows, :] + h2, 5, cols)).astype(BF16)

    def stage_b2b(w, h3, r0, n, j, k0=0, k1=7, done=None, prep=False, fine=0):
        hv = h3.at[pl.ds(zsm[j], 7)]
        blk = lambda k: jnp.concatenate([hv[p, k, pl.ds(0, n // 4), :] for p in range(7)], axis=1)
        if j < 2:
            done = [] if done is None else done
            done += sprods("w4", j, lambda i: _unpack(blk(8 if i == 6 else i)), k0, k1, prep)
            if k1 == 7:
                c11, c12, c21, c22 = _combine(*done)
                finish(w, _unrows2(c11, c21), r0, n, j)
                finish(w, _unrows2(c12, c22), r0, n, j + 2)
            return done
        wb = wblocks("w4", 4)
        lhs = jnp.concatenate([jnp.concatenate([blk(5), blk(6)], axis=1),
                               jnp.concatenate([blk(7), blk(8)], axis=1)], axis=0)
        h2 = _dot_fine(_unpack(lhs), _unpack(jnp.concatenate([wb(0, 0), wb(1, 0)], axis=0)), fine)
        finish(w, _unrows2(h2[:n // 2], h2[n // 2:]), r0, n, 4)

    w = window(0, 2 * TS + LEAD, 0)
    H = TS // 2
    with jax.named_scope("t0a"):
        cps["qa"].wait()
        cps["wmoda"].wait()

        mv = {}

        def mod_fn(j, toks):
            mv[j] = mod_cols(j, 1, toks)[0]
            if len(mv) == 3:
                modbuf[0] = mv[2] * mv[0]
                modbuf[1] = mv[2] * (1.0 + mv[1])

        segment(G5B, 0, MU, mod_fn=mod_fn)
        put(w["h"], pl.ds(0, QA), stage_a0(w, 0, QA))
    with jax.named_scope("t0b"):
        cps["wmodb"].wait()
        sb, cb = mod_cols(3, 2)
        modbuf[3] = 2.0 * sb
        modbuf[4] = 2.0 + 2.0 * cb
        n3 = stage_a1(w, 0, QA, n2=slabs(w["h"], 0, QA))
    XB = TS - XA
    FN = 32
    F4 = 64
    with jax.named_scope("t1a"):
        cps["w1a"].wait()
        if QXPOS != "b":
            cps["qx"].wait()
            if "1" == "1":
                put(w["h"], pl.ds(QA, XA), stage_a0(w, QA, XA))
            else:
                n3a = stage_a1(w, QA, XA)
        stage_a2(w, n3, 0, QA, c1=W1A, fine=80)
    with jax.named_scope("t1b"):
        cps["w1b"].wait()
        if QXPOS == "b":
            cps["qx"].wait()
            n3a = stage_a1(w, QA, XA)
        elif "1" == "1":
            n3a = stage_a1(w, QA, XA, n2=slabs(w["h"], QA, XA))
        stage_a2(w, n3, 0, QA, c0=W1A)
        if "0" == "1":
            stage_a2(w, n3a[:XA // 2], QA, XA // 2)
            stage_a2(w, n3a[XA // 2:], QA + XA // 2, XA // 2, fine=FN)
        else:
            stage_a2(w, n3a, QA, XA, fine=FN)
    with jax.named_scope("t2"):
        cps["qb"].wait()
        cps["w2"].wait()
        T2V = "1"
        n3b = stage_a1(w, QA + XA, XB, f32=True)
        if T2V == "1":
            stage_b1(w, 0, TS, fast=True, prep=True)
            stage_a2(w, [dd_rest("w1", *_rows2(n3b))], QA + XA, XB, prep=True)
            stage_b1(w, TS, XA, fast=True)
            stage_b1a(w, TS + XA, XB, fast=True)
        elif T2V == "2":
            stage_b1(w, 0, TS)
            stage_a2(w, [dd_rest("w1", *_rows2(n3b))], QA + XA, XB, prep=True)
            stage_b1(w, TS, XA)
            stage_b1a(w, TS + XA, XB, fast=True, prep=True)
        elif T2V == "3":
            stage_b1(w, 0, TS)
            stage_a2(w, [dd_rest("w1", *_rows2(n3b))], QA + XA, XB, prep=True)
            stage_b1(w, TS, XA, fast=True, prep=True)
            stage_b1a(w, TS + XA, XB, fast=True)
    ha, hb = hba, hbb
    with jax.named_scope("t3"):
        cps["w3"].wait()
        stage_b1b(w, [parity(w["h"], TS + XA, XB, e) for e in range(2)], TS + XA, XB)
        for op in "ha 3a:0:6 hb 3b:0:6".split():
            op, *rng = op.split(":")
            rng = [int(x) for x in rng]
            hx, r = (ha, 0) if op[1] == "a" else (hb, TS)
            if op[0] == "h":
                stage_b2h(w, hx, r, TS, prep=op[1] == "a")
            else:
                stage_b2a(w, hx, r, TS, *rng, prep=op[1] == "a")
    with jax.named_scope("t4"):
        cps["w4"].wait()
        cps["wmodg"].wait()
        modbuf[5] = 0.5 * mod_cols(5, 1)[0]
        for j in range(3):
            stage_b2b(w, ha, 0, TS, j, prep=True, fine=F4)
        out_copy(0, TS).start()
        cps["q1"].wait()

    CBS = (160, 96)
    PART = {"a": (TS, TS), "c": (TS, H), "d": (TS + H, H)}
    BODY = "4:0:0:7 r0 4:1:0:5 r1 1a 4:1:5:7 2a na 4:2 3a:0:2 ha 3a:2:6"

    def step(s, carry):
        r0 = pl.multiple_of(s * TS, TS)
        w = window(r0, 2 * TS + LEAD, pl.multiple_of(s * H, H))
        x1, rest, done = {}, {}, {0: [], 1: [], 2: None}
        for op in BODY.split():
            op, *rng = op.split(":")
            rng = [int(x) for x in rng]
            if op[0] == "3":
                stage_b2a(w, hb, TS, TS, *rng)
            elif op[0] == "h":
                stage_b2h(w, hb, TS, TS)
            elif op[0] == "4":
                stage_b2b(w, hb, 0, TS, *rng, done=done[rng[0]])
            elif op[0] == "2":
                x1[op[1]] = stage_b1a(w, *PART[op[1]], fast=True)
            elif op[0] == "n":
                stage_b1b(w, x1[op[1]], *PART[op[1]])
            elif op[0] == "r":
                j = int(op[1])
                rest[j] = dd_rest("w1", *_rows2(stage_a1(w, TS + LEAD + sum(CBS[:j]), CBS[j], f32=True)))
            else:
                ra, n = PART[op[1]]
                parts = [rest[j] for j in range(len(CBS)) if ra - TS <= sum(CBS[:j]) < ra - TS + n]
                stage_a2(w, parts, ra + LEAD, n, last_valid=(s < NT - 2) if ra + n == 2 * TS else None)
        out_copy(r0, TS).start()
        return carry

    with jax.named_scope("p2main"):
        jax.lax.fori_loop(1, NT - 1, step, 0)
    with jax.named_scope("p2epi"):
        w = window(S - 2 * TS, 2 * TS + LEAD, S // 2 - TS)
        rows = pl.ds(S - TS, TS)
        pending.append(hhbuf[0, pl.ds(S, 8), :])
        for j in range(3):
            stage_b2b(w, hb, TS, TS, j)
            if j > 0:
                cols = pl.ds(0, 512) if j == 1 else pl.ds(512, 128)
                pltpu.make_async_copy(obuf.at[rows, cols], out_hbm.at[rows, cols], sem_out.at[0]).start()
        pltpu.make_async_copy(obuf, out_hbm, sem_out.at[0]).wait()


@jax.jit
def pallas_adaLN_cond__ssm_conv_h3__mixer_s_mlp__prompt_kernel(
    A_q: jax.Array,
    A_k: jax.Array,
    A_v: jax.Array,
    A_shift_k: jax.Array,
    A_ssm_k: jax.Array,
    A_ssm_D: jax.Array,
    B_x: jax.Array,
    B_w1: jax.Array,
    B_w2: jax.Array,
    B_w3: jax.Array,
    B_w4: jax.Array,
    c: jax.Array,
    w_mod: jax.Array,
):
    del B_x

    def tiles(x):
        return x.reshape(S // 8, 8, NC, 128).transpose(0, 2, 1, 3).reshape(S * NC, 128)

    def pairs(x):
        r, n = x.shape
        return x.reshape(r // 16, 2, 8, n // 128, 128).transpose(0, 1, 3, 2, 4)

    args = (
        A_q.reshape(S, D), tiles(A_k), tiles(A_v),
        A_shift_k.T, A_ssm_k, A_ssm_D.reshape(NC, 128),
        pairs(B_w1), pairs(B_w2), pairs(B_w3.T), pairs(B_w4), c, pairs(w_mod),
    )
    scratch = [
        pltpu.VMEM((NA, P * NC + 128, 128), BF16),
        pltpu.VMEM((NA, P * NC + 64, 128), BF16),
        pltpu.VMEM((D, S), BF16),
        pltpu.VMEM((R, 128, 128), U32),
        pltpu.VMEM((R, 64, 256), U32),
        pltpu.VMEM((64, 128), U32),
        pltpu.VMEM((D // 16, 6 * NC, 16, 128), BF16),
        pltpu.VMEM((D // 16, NC, 16, 128), BF16),
        pltpu.VMEM((D // 16, NC, 16, 128), BF16),
        pltpu.VMEM((FF // 16, NC, 16, 128), BF16),
        pltpu.VMEM((FF // 16, NC, 16, 128), BF16),
        pltpu.VMEM((S + 64, D), BF16),
        *[pltpu.VMEM((NA, R, 16, 4, 8, 128), F32) for _ in range(NC)],
        pltpu.VMEM((NC, NA - 1, R, 16, 2, 8, 128), F32),
        pltpu.VMEM((NC, R, 128, 128), U32),
        pltpu.VMEM((32, 128), U32),
        pltpu.VMEM((NC, 8, 8, 128), F32),
        pltpu.VMEM((NC, S + 32, 128), F32),
        pltpu.VMEM((8, 8, D), F32),
        pltpu.VMEM((S + 32, D), F32),
        pltpu.VMEM((NC, S + 32, 128), F32),
        pltpu.VMEM((NC, S + 32, 128), F32),
        pltpu.VMEM((2, S // 2, D), BF16),
        pltpu.VMEM((S // 2, 5 * 256), BF16),
        pltpu.VMEM((5, 2, 128, 128), U32),
        pltpu.VMEM((5, 2, 128, 128), U32),
        pltpu.VMEM((5, 6, 64, 256), U32),
        pltpu.VMEM((5, 2, FT // 2, 256), U32),
        pltpu.VMEM((5, 2, 448, 128), U32),
        pltpu.VMEM((8, 9, 72, 128), U32),
        pltpu.VMEM((8, 9, 72, 128), U32),
        pltpu.VMEM((S, D), BF16),
        pltpu.VMEM((4, D), BF16),
        pltpu.VMEM((NC, 128), BF16),
        pltpu.VMEM((1, D), BF16),
        pltpu.SMEM((8,), jnp.int32),
        pltpu.SemaphoreType.DMA((40,)),
        pltpu.SemaphoreType.DMA((1,)),
    ]
    out = pl.pallas_call(
        _kernel,
        out_shape=jax.ShapeDtypeStruct((S, D), BF16),
        in_specs=[pl.BlockSpec(memory_space=pl.ANY)] * len(args),
        out_specs=pl.BlockSpec(memory_space=pl.ANY),
        scratch_shapes=scratch,
        grid=(1,),
        compiler_params=pltpu.CompilerParams(vmem_limit_bytes=100 * 1024 * 1024, disable_semaphore_checks=True,
                                             disable_bounds_checks=True),
        name="adaln_h3_mixer",
    )(*args)
    return out.reshape(1, S, D)
```

```python
import numpy as np
import jax
import jax.numpy as jnp
import jax.experimental.pallas as pl
import jax.experimental.pallas.tpu as pltpu

F32 = jnp.float32
BF16 = jnp.bfloat16
U32 = jnp.uint32

S = 2048
D = 640
FF = 1728
NC = D // 128
R = 4
P = 128 * R
NA = S // P
TS = 256
NT = S // TS
LEAD = 16
EPS = 1e-5
FT = (FF - 1536) // 2
FM = (FF // 128) * 128
FR = FF - FM
P1_ORDER = "t0 t1 t2 t3 k0 k1 k2 k3 u0 i0 u1 i1 u2 i2 u3 i3"


def _freq(row):
    t, part, s = row >> 4, (row >> 3) & 1, row & 7
    return 32 * (t & 7) + 4 * s + 2 * (t >> 3) + 1, P * part


def _cos(j, scale):
    jf = (j & (4 * P - 1)).astype(F32)
    u = 2.0 * np.pi / (4 * P)
    x = jnp.abs(jf * u - np.pi) - 0.5 * np.pi
    x2 = x * x
    poly = scale / 362880.0 - x2 * (scale / 39916800.0)
    for coef in (-1.0 / 5040.0, 1.0 / 120.0, -1.0 / 6.0, 1.0):
        poly = poly * x2 + coef * scale
    return poly * x


_DUR = {"t": 8, "u": 16, "k": 16, "i": 16, "m": 12, "g": 0, "c": 0, "j": 16}
_POST = {"t": 8.0, "u": 16.0, "k": 24.0, "i": 4.0, "j": 4.0, "m": 18.0}


def _plan_tokens(order, maxutil):
    lag, cap, pre, margin = 8, 60, 4, 3
    start, slots = {}, []
    for n in order:
        start[n] = len(slots)
        slots += [(n, r) for r in range(_DUR[n[0]])]
    nslot = len(slots) + lag
    free = [cap - (_POST[slots[i - lag][0][0]] if i >= lag else 0.0) for i in range(-pre, nslot)]
    units = []
    for n in order:
        kind, a, c = n
        if kind == "u":
            units += [(n + (g,), 94.0, start[n], -pre) for g in range(8)]
        elif kind == "g":
            units += [(n + (g,), 150.0, start[n], -pre) for g in range(8)]
        elif kind in "ic":
            src_ = [start[m] for m in (("u", a, c), ("k", a, c)) if m in start]
            for t in range(16):
                rel = max(max(src_) + 16, max(src_) + t + lag + 3) if src_ else -pre
                units.append((n + (t,), 32.0 * a + 48.0, nslot if kind == 'c' else start[n], rel))

    def simulate(util):
        left = [u[1] for u in units]
        done = [None] * len(units)
        for i in range(-pre, nslot):
            budget = util * free[i + pre]
            for j, u in enumerate(units):
                if budget <= 0.0:
                    break
                if done[j] is None and u[3] <= i:
                    use = min(budget, left[j])
                    left[j] -= use
                    budget -= use
                    if left[j] <= 1e-9:
                        done[j] = i + 1
        ok = all(u[2] < 8 or (d is not None and d <= max(u[2] - (1 if u[0][0] in 'cg' else margin), u[3] + 1))
                 for d, u in zip(done, units))
        return done, ok

    lo_, hi_ = 0.05, maxutil
    for _ in range(12):
        mid = 0.5 * (lo_ + hi_)
        if simulate(mid)[1]:
            hi_ = mid
        else:
            lo_ = mid
    done, _ = simulate(hi_)
    plan = {}
    for u, d in zip(units, done):
        if u[0][0] == "c":
            plan[u[0]] = slots[max((nslot - 1 if d is None else min(d, nslot - 1)) - lag, 0)]
        elif d is not None and 0 <= d < u[2]:
            plan.setdefault(slots[d], []).append(u[0])
    return plan


def _pack(x):
    return pltpu.bitcast(x.astype(BF16), U32)


def _unpack(w):
    return pltpu.bitcast(w, BF16)


def _dot(a, b):
    return jnp.dot(a.astype(BF16), b, preferred_element_type=F32)


def _dot_nt(a, b):
    return jax.lax.dot_general(a.astype(BF16), b, (((1,), (1,)), ((), ())), preferred_element_type=F32)


def _dot_fine(x, w, chunk, nt=False):
    if not chunk:
        return _dot_nt(x, w) if nt else _dot(x, w)
    n = w.shape[0] if nt else w.shape[1]
    head, last = (w[:n - 128], w[n - 128:]) if nt else (w[:, :n - 128], w[:, n - 128:])
    f = _dot_nt if nt else _dot
    parts = [f(x, head)] if n > 128 else []
    parts.append(jnp.concatenate([f(x[r:r + chunk], last) for r in range(0, x.shape[0], chunk)], axis=0))
    return jnp.concatenate(parts, axis=1)


def _rows2(x):
    n, c = x.shape
    x = x.reshape(n // 32, 2, 16, c)
    return x[:, 0].reshape(n // 2, c), x[:, 1].reshape(n // 2, c)


def _unrows2(top, bot):
    n, c = top.shape
    return jnp.stack([top.reshape(n // 16, 16, c), bot.reshape(n // 16, 16, c)], axis=1).reshape(2 * n, c)


def _sums_a(a11, a12, a21, a22):
    return [a11 + a22, a21 + a22, a11 + a12, a21 - a11, a12 - a22]


def _sums_b(b11, b12, b21, b22):
    return [b11 + b22, b12 - b22, b21 - b11, b11 + b12, b21 + b22]


_STRASSEN = ((0, 0), (1, 5), (5, 1), (6, 2), (2, 6), (3, 3), (4, 4))


def _combine(m1, m2, m3, m4, m5, m6, m7):
    return (m1 + m4) + (m7 - m5), m3 + m5, m2 + m4, (m1 - m2) + (m3 + m6)


def _lo(w):
    return pltpu.bitcast(w << 16, F32)


def _hi(w):
    return pltpu.bitcast(w & jnp.uint32(0xFFFF0000), F32)


def _ln(x, eps=EPS):
    m = jnp.sum(x, axis=-1, keepdims=True) * (1.0 / D)
    xc = x - m
    v = jnp.sum(xc * xc, axis=-1, keepdims=True) * (1.0 / D)
    return xc * jnp.exp(-0.5 * jnp.log(v + eps))


def _gelu2(x):
    c0 = 0.7978845608028654
    c1 = c0 * 0.044715
    return x + x * jnp.tanh(x * (c0 + c1 * (x * x)))


def _bfly(tr, ti, sign):
    s02r, s02i = tr[0] + tr[2], ti[0] + ti[2]
    d02r, d02i = tr[0] - tr[2], ti[0] - ti[2]
    s13r, s13i = tr[1] + tr[3], ti[1] + ti[3]
    d13r, d13i = tr[1] - tr[3], ti[1] - ti[3]
    x0r, x0i = s02r + s13r, s02i + s13i
    x2r, x2i = s02r - s13r, s02i - s13i
    ar, ai = d02r + d13i, d02i - d13r
    br, bi = d02r - d13i, d02i + d13r
    if sign < 0:
        return [x0r, ar, x2r, br], [x0i, ai, x2i, bi]
    return [x0r, br, x2r, ar], [x0i, bi, x2i, ai]


def _kernel(q_hbm, k_hbm, v_hbm, shift_hbm, ssmk_hbm, ssmd_hbm, w1_hbm, w2_hbm, w3t_hbm, w4_hbm,
            c_hbm, wmod_hbm,
            out_hbm,
            kbuf, vbuf, skbuf, fwdbuf, invbuf, permbuf,
            wmodbuf, w1buf, w2buf, w3buf, w4buf, qbuf,
            xs0, xs1, xs2, xs3, xs4, kraw, wbuf, zbuf, coefbuf, ybuf, modbuf, x2buf, hbuf, hhbuf, xnbuf, xsbuf,
             w1s, w2s, w3s, w3ts, w4s, hba, hbb, obuf, shiftbuf, dbuf, cbuf,
            zsm, sem_in, sem_out):
    cps = {}
    n_sem = [0]

    def start(name, src, dst):
        cp = pltpu.make_async_copy(src, dst, sem_in.at[n_sem[0]])
        n_sem[0] += 1
        cp.start()
        cps[name] = cp

    class Both:
        def __init__(self, a, b):
            self.cps = (a, b)

        def wait(self):
            for cp in self.cps:
                cp.wait()

    def start_w(name, src, dst, c0=0, n=NC):
        for e in range(2):
            start(name + str(e), src.at[:, e, pl.ds(c0, n)], dst.at[:, pl.ds(c0, n), pl.ds(8 * e, 8), :])
        cps[name] = Both(cps[name + "0"], cps[name + "1"])

    CH = P * NC
    HALO = 8 * NC

    def start_s(a):
        cols = pl.ds(a * P, P)
        start("s%d" % a, ssmk_hbm.at[:, cols], skbuf.at[:, cols])

    def start_kv(a):
        if a == 0:
            kbuf[0, pl.ds(0, HALO + 8), :] = jnp.zeros((HALO + 8, 128), BF16)
            start("k0", k_hbm.at[pl.ds(0, CH), :], kbuf.at[0, pl.ds(HALO, CH), :])
        else:
            start("k%d" % a, k_hbm.at[pl.ds(a * CH - HALO, CH + HALO), :], kbuf.at[a, pl.ds(0, CH + HALO), :])
        start("v%d" % a, v_hbm.at[pl.ds(a * CH, CH), :], vbuf.at[a, pl.ds(0, CH), :])

    for n in "s0 x0 s1 k0 k1 s2 k2 s3 k3".split():
        if n[0] == "s":
            start_s(int(n[1]))
        elif n[0] == "k":
            start_kv(int(n[1]))
        else:
            start("d", ssmd_hbm, dbuf)
            start("shift", shift_hbm, shiftbuf)
            start("c", c_hbm, cbuf)
    QA = TS + LEAD
    XA = 128
    QB = 2 * TS + LEAD
    W1A = 2

    def start_q(name, r0, n):
        start(name, q_hbm.at[pl.ds(r0, n), :], qbuf.at[pl.ds(r0, n), :])

    start_q("qa", 0, QA)
    start_w("wmoda", wmod_hbm, wmodbuf, 0, 3 * NC)
    start_w("wmodb", wmod_hbm, wmodbuf, 3 * NC, 2 * NC)
    start_q("qx", QA, XA)
    start_w("w1a", w1_hbm, w1buf, 0, W1A)
    start_w("w1b", w1_hbm, w1buf, W1A, NC - W1A)
    start_q("qb", QA + XA, QB - QA - XA)
    start_w("w2", w2_hbm, w2buf)
    start_w("w3", w3t_hbm, w3buf)
    start_w("w4", w4_hbm, w4buf)
    start_w("wmodg", wmod_hbm, wmodbuf, 5 * NC, NC)
    start_q("q1", QB, S - QB)

    kw = kbuf.bitcast(U32)
    vw = vbuf.bitcast(U32)
    zbuf[...] = jnp.zeros(zbuf.shape, U32)
    for j in range(8):
        zsm[j] = 0
    for c in range(NC):
        ybuf[c, pl.ds(S, LEAD), :] = jnp.zeros((LEAD, 128), F32)
        hhbuf[c, pl.ds(0, 8), :] = jnp.zeros((8, 128), F32)
    qbuf[pl.ds(S, LEAD), :] = jnp.zeros((LEAD, D), BF16)

    def tables(p, carry):
        i0 = jax.lax.broadcasted_iota(jnp.int32, (128, 128), 0)
        n = R * jax.lax.broadcasted_iota(jnp.int32, (128, 128), 1) + p
        f2, off = _freq(2 * i0)
        j = f2 * n + off
        fwdbuf[p] = pltpu.pack_elementwise([_cos(j, 1.0), _cos(j + 4 * n, 1.0)], packed_dtype=BF16)
        return carry

    jax.lax.fori_loop(0, R, tables, 0)

    def unit_g(kt, r):
        col = jax.lax.broadcasted_iota(jnp.int32, (8, 128), 1) + 128 * kt
        f2, off = _freq((col & ~15) + 8 * (col & 1) + ((col >> 1) & 7))
        m = 2 * jax.lax.broadcasted_iota(jnp.int32, (8, 128), 0) + 16 * r
        j0 = f2 * (R * m) + off
        out = []
        for p in range(R):
            j = j0 + p * f2
            out.append(pltpu.pack_elementwise([_cos(j, 1.0 / P), _cos(j + R * f2, 1.0 / P)], packed_dtype=BF16))
            invbuf[p, pl.ds(8 * r, 8), pl.ds(128 * kt, 128)] = out[-1]
        return out

    i0 = jax.lax.broadcasted_iota(jnp.int32, (128, 128), 0)
    i1 = jax.lax.broadcasted_iota(jnp.int32, (128, 128), 1)
    permbuf[...] = _pack(jnp.where(i0 == (128 // R) * (i1 & (R - 1)) + (i1 >> 2), 1.0, 0.0).astype(F32))

    def fill_coef():
        cv = cbuf[...].astype(F32)
        modbuf[6] = jnp.broadcast_to(cv * jax.nn.sigmoid(cv), (8, D))
        coef = shiftbuf[...].astype(F32)
        dval = dbuf[...].astype(F32)
        for c in range(NC):
            for j in range(4):
                coefbuf[c, j] = jnp.broadcast_to(coef[j:j + 1, c * 128:(c + 1) * 128], (8, 128))
            coefbuf[c, 4] = jnp.broadcast_to(dval[c:c + 1, :], (8, 128))

    xs = (xs0, xs1, xs2, xs3, xs4)
    wsbufs = dict(w1=w1s, w2=w2s, w3=w3s, w4=w4s, w3t=w3ts)
    def split_ri(t):
        t = t.reshape(16, 2, 8, 128)
        return t[:, 0], t[:, 1]

    def get_never():
        return zbuf[pl.ds(0, 8), :] != 0

    def pack2(x, y):
        return pltpu.pack_elementwise([x, y], packed_dtype=BF16)

    def words(ref, a, c, r):
        return ref[a, pl.ds((r // 4) * 4 * NC + 4 * c + r % 4, 8, stride=4 * NC), :]

    def unit_u(a, c, g):
        c0, c1, c2, c3 = (coefbuf[c, pl.ds(j, 1)] for j in range(4))
        kk = jnp.stack([words(kw, a, c, 4 + 32 * g + d) for d in range(-2, 4)])
        vv = jnp.stack([words(vw, a, c, 32 * g + d) for d in range(4)])
        lo, hi = _lo(kk), _hi(kk)
        k0, k1, k2 = lo[2:], hi[1:5], lo[1:5]
        even = (((k0 * c0 + k1 * c1) + (k2 * c2 + hi[:4] * c3)) * _lo(vv)).reshape(32, 128)
        odd = (((hi[2:] * c0 + k0 * c1) + (k1 * c2 + k2 * c3)) * _hi(vv)).reshape(32, 128)
        e, o = pack2(even[:16], even[16:]), pack2(odd[:16], odd[16:])
        return [e[:8], o[:8], e[8:], o[8:]]

    def unit_i(a, c, t, z):
        x_c = xs[c].at[pl.ds(z, NA)]
        yr = yi = None
        for j in range(a + 1):
            ur, ui = x_c[j, :, t, 0], x_c[j, :, t, 1]
            kr, ki = x_c[a - j, :, t, 2], x_c[a - j, :, t, 3]
            pr = ur * kr - ui * ki
            pi = ur * ki + ui * kr
            yr = pr if yr is None else yr + pr
            yi = pi if yi is None else yi + pi
        halves = lambda x: (x[:x.shape[0] // 2], x[x.shape[0] // 2:])
        (ra, rb), (ia, ib) = halves(yr.reshape(32, 128)), halves(yi.reshape(32, 128))
        (sr0, sr1), (si0, si1), (dr0, dr1), (di0, di1) = (halves(x) for x in (ra + rb, ia + ib, ra - rb, ia - ib))
        return [pack2(sr0 + sr1, si0 + si1), pack2(dr0 - di1, di0 + dr1),
                pack2(sr0 - sr1, si0 - si1), pack2(dr0 + di1, di0 - dr1)]

    def segment(spec, z, maxutil=1.0, mod_fn=None):
        order = [(n[0], int(n[1]), int(n[2])) for n in spec.split()]
        plan = _plan_tokens(order, maxutil) if maxutil > 0 else {}
        never = get_never()
        units, res = {}, {}

        def unit(key):
            if key not in units:
                kind, a, c, j = key
                if kind == "u":
                    units[key] = unit_u(a, c, j)
                elif kind == "g":
                    units[key] = unit_g(a, j)
                else:
                    fresh = ("u", a, c) in order or ("k", a, c) in order
                    units[key] = unit_i(a, c, j, z if fresh else 0)
            return units[key]

        def lhs(name, p, full, r0=0):
            out, last = [], 0
            for r in range(full.shape[0] // 8):
                keys = plan.get((name, r0 + r), ())
                if keys:
                    if 8 * r > last:
                        out.append(full[last:8 * r])
                    v = full[8 * r:8 * r + 8]
                    for key in keys:
                        v = jax.lax.select(never, unit(key)[p], v)
                    out.append(v)
                    last = 8 * r + 8
            if last < full.shape[0]:
                out.append(full[last:] if last else full)
            return out[0] if len(out) == 1 else jnp.concatenate(out, axis=0)

        def dft(name, rhs):
            tr, ti = [], []
            for p in range(R):
                f = lhs(name, p, fwdbuf[p])
                r_, i_ = split_ri(_dot(_unpack(f), rhs[p]))
                if p == 0:
                    res.update({(name, r): (lambda r=r, v=r_: v[r]) for r in range(16)})
                tr.append(r_)
                ti.append(i_)
            return _bfly(tr, ti, -1)

        st = {}
        for name in order:
            kind, a, c = name
            x_c = xs[c]
            if kind == "g":
                for r in range(8):
                    unit(name + (r,))
            elif kind == "c":
                for t in range(16):
                    after = pltpu.bitcast(res[plan[name + (t,)]](), U32)
                    for p in range(R):
                        wbuf[c, p, pl.ds(8 * t, 8), :] = jax.lax.select(never, after, unit(name + (t,))[p])
            elif kind == "m":
                toks = {}
                for r in range(_DUR["m"]):
                    for n_, key in enumerate(plan.get((name, r), ())):
                        toks.setdefault(2 * r + n_ % 2, []).extend(unit(key))
                mod_fn(a, toks)
            elif kind == "t":
                trs = []
                for b in range(R):
                    pm = lhs(name, b, permbuf[...])
                    trs.append(_dot_nt(_unpack(pm), skbuf[pl.ds(c * 128, 128), pl.ds(a * P + b * 128, 128)]))
                res.update({(name, r): (lambda r=r, v=trs[0]: v[16 * r:16 * r + 8]) for r in range(8)})
                g_ = 128 // R
                st[a, c] = [jnp.concatenate([trs[b][p * g_:(p + 1) * g_] for b in range(R)], axis=0).astype(BF16)
                            for p in range(R)]
            elif kind == "u":
                rhs = [_unpack(jnp.concatenate([unit(name + (g,))[p] for g in range(8)], axis=0)) for p in range(R)]
                xr, xi = dft(name, rhs)
                for q in range(R):
                    x_c[a, q, :, 0] = xr[q]
                    x_c[a, q, :, 1] = xi[q]
            elif kind == "k":
                xr, xi = dft(name, st[a, c])
                for q in range(R):
                    if a == 0:
                        x_c[a, q, :, 2] = xr[q] + coefbuf[c, 4]
                        x_c[a, q, :, 3] = xi[q]
                    else:
                        pr, pi = kraw[c, a - 1, q, :, 0], kraw[c, a - 1, q, :, 1]
                        x_c[a, q, pl.ds(0, 8), 2] = xr[q][:8] - pi[:8]
                        x_c[a, q, pl.ds(0, 8), 3] = xi[q][:8] + pr[:8]
                        x_c[a, q, pl.ds(8, 8), 2] = xr[q][8:] + pi[8:]
                        x_c[a, q, pl.ds(8, 8), 3] = xi[q][8:] - pr[8:]
                    if a + 1 < NA:
                        kraw[c, a, q, :, 0] = xr[q]
                        kraw[c, a, q, :, 1] = xi[q]
            else:
                for p in range(R):
                    cols = [lhs(name, 2 * (p % 2) + kt,
                                invbuf[p, :, pl.ds(128 * kt, 128)], 8 * (p // 2))
                            for kt in range(2)]
                    g = _unpack(jnp.concatenate(cols, axis=1))
                    if kind == "j":
                        wp = _unpack(wbuf[c, p])
                    else:
                        wp = _unpack(jnp.concatenate([unit(name + (t,))[p] for t in range(16)], axis=0))
                    yp = _dot(g, wp)
                    if p % 2 == 0:
                        res.update({(name, 4 * p + r): (lambda r=r, v=yp: v[16 * r:16 * r + 8]) for r in range(8)})
                    ybuf[c, pl.ds(a * P + p, 128, stride=R), :] = yp

    one = jnp.minimum(pl.program_id(0) + 1, 1)

    def once(fn):
        def body(z, carry):
            fn(z)
            return carry
        jax.lax.fori_loop(0, one, body, 0)

    default = "t00 t01 t02 k00 t03 k01 t04 k02 k03 k04 g00|t10 t11 t12 k10 k11 k12 g10|t13 t14 k13 u00 k14 u01 u02 u03 i00 u04 i01 c02 c03|j02 j03 u10 i04 u11 u12 u13 i10 u14 i11 c12|t20 t21 j12 t22 t23 t24 k20 u20 k21 u21 k22 i13 k23 u22 k24 i14 u23 i20 u24 i21 c22|t30 t31 j22 t32 t33 t34 k30 u30 k31 u31 k32 i23 k33 u32 k34 i24 u33 i30 u34 i31 c32|m00 j32 m10 m20 i33 i34"
    specs = default.split("|")
    G5B = specs[-1]
    segs = list(zip("s0 d shift c|s1|k0 v0|k1 v1|s2 k2 v2|s3 k3 v3".split("|"), specs[:-1]))
    MU = 1.5
    for i, (waits, spec) in enumerate(segs):
        with jax.named_scope("g%d" % i):
            for n in waits.split():
                cps[n].wait()
            if i == 0:
                fill_coef()
            once(lambda z: segment(spec, z, MU))

    def mod_cols(lo, n, toks=None):
        m = _dot(modbuf[6], weights(wmodbuf, lo * NC, (lo + n) * NC, toks=toks))
        return [m[:, j * D:(j + 1) * D] for j in range(n)]

    def mul_mod(x, j, cols=None):
        m = modbuf[j] if cols is None else modbuf[j, :, cols]
        return (x.reshape(-1, 8, x.shape[-1]) * m[None]).reshape(x.shape)

    def add_mod(x, j):
        return (x.reshape(-1, 8, x.shape[-1]) + modbuf[j][None]).reshape(x.shape)

    def slabs(ref, r0, n):
        return jnp.concatenate([ref[c, pl.ds(r0, n), :] for c in range(NC)], axis=1)

    def put(ref, rows, x):
        for c in range(NC):
            ref[c, rows, :] = x[:, c * 128:(c + 1) * 128]

    def parity(ref, r0, n, e):
        return jnp.concatenate([ref[c, pl.ds(r0 + e, n // 2, stride=2), :] for c in range(NC)], axis=1)

    def window(base, n, half):
        rows = pl.ds(base, n)
        return dict(xs=xsbuf.at[pl.ds(half, (n - LEAD) // 2), :],
                    q=qbuf.at[rows, :], y=ybuf.at[:, rows, :], x2=x2buf.at[rows, :], h=hbuf.at[:, rows, :],
                    hh=hhbuf.at[:, pl.ds(base, n + 8), :], xn=xnbuf.at[:, pl.ds(half, (n - LEAD) // 2), :],
                    o=obuf.at[pl.ds(base, n - LEAD), :])

    def weights(ref, c0=0, c1=NC, r0=0, r1=None, toks=None, raw=False, z=None):
        r1 = 16 * ref.shape[0] if r1 is None else r1
        view = ref.bitcast(U32)
        if z is not None:
            view = view.at[pl.ds(z, ref.shape[0])]
        never = get_never() if toks else None
        rt = -(-(r1 - r0) // 128)
        cols = []
        for j in range(c0, c1):
            wu = view[pl.ds(r0 // 16, (r1 - r0) // 16), j].reshape((r1 - r0) // 2, 128)
            if toks:
                parts, last = [], 0
                for i in range(rt):
                    for n_, t in enumerate(toks.get((j - c0) * rt + i, ())):
                        r = 64 * i + 8 * n_
                        if r > last:
                            parts.append(wu[last:r])
                        parts.append(jax.lax.select(never, t, wu[r:r + 8]))
                        last = r + 8
                parts.append(wu[last:])
                wu = jnp.concatenate(parts, axis=0)
            cols.append(wu)
        wu = jnp.concatenate(cols, axis=1)
        return wu if raw else _unpack(wu)

    def wblocks(name, j, z=None):
        if name == "w3":
            blk = lambda kh, nh: weights(w3buf, 2 * kh, 2 * kh + 2, 128 * (j + 6 * nh), 128 * (j + 6 * nh + 1), raw=True, z=z)
        elif name == "w4":
            def blk(kh, nh):
                c = j + 2 * nh
                parts = [weights(w4buf, c, c + 1, 768 * kh, 768 * (kh + 1), raw=True, z=z),
                         weights(w4buf, c, c + 1, 1536 + FT * kh, 1536 + FT * (kh + 1), raw=True, z=z),
                         jnp.zeros(((128 - FT) // 2, 128), U32)]
                return jnp.concatenate(parts, axis=0)
        elif name == "w3t":
            blk = lambda kh, nh: weights(w3buf, 2 * kh, 2 * kh + 2, 1536 + FT * nh, 1536 + FT * (nh + 1), raw=True, z=z)
        else:
            ref = w1buf if name == "w1" else w2buf
            blk = lambda kh, nh: weights(ref, j + 2 * nh, j + 2 * nh + 1, 256 * kh, 256 * (kh + 1), raw=True, z=z)
        return blk

    def wsum(name, j, k):
        blk = wblocks(name, j, zsm[k])
        p, q, sign = ((0, 3, 1), (1, 3, -1), (2, 0, -1), (0, 1, 1), (2, 3, 1))[k]
        x, y = blk(p // 2, p % 2), blk(q // 2, q % 2)
        if sign > 0:
            return pack2(_lo(x) + _lo(y), _hi(x) + _hi(y))
        return pack2(_lo(x) - _lo(y), _hi(x) - _hi(y))

    pending = []

    def attach(wv):
        if not pending:
            return wv
        never = get_never()
        rows = [wv[8 * i:8 * i + 8, :128] for i in range(8)]
        for i, t in enumerate(pending):
            rows[i % 8] = jax.lax.select(never, pltpu.bitcast(t, U32), rows[i % 8])
        pending.clear()
        first = jnp.concatenate(rows + ([wv[64:, :128]] if wv.shape[0] > 64 else []), axis=0)
        return first if wv.shape[1] == 128 else jnp.concatenate([first, wv[:, 128:]], axis=1)

    def sprods(name, j, lhs, k0=0, k1=7, prep=False):
        blk, buf = wblocks(name, j), wsbufs[name]
        out = []
        for ia, ib in _STRASSEN[k0:k1]:
            wv = blk(ib - 5, ib - 5) if ib >= 5 else (wsum(name, j, ib) if prep else buf[ib, j])
            if name == "w3t":
                out.append(_dot_nt(_unpack(wv), lhs(ia)))
            else:
                out.append((_dot_nt if name == "w3" else _dot)(lhs(ia), _unpack(attach(wv))))
            if prep and ib < 5:
                buf[ib, j] = wv
        return out

    def spair(name, j, lhs, prep=False):
        return _combine(*sprods(name, j, lhs, prep=prep))

    def dd_rest(name, t, b):
        ref = w1buf if name == "w1" else w2buf
        m = t.shape[0]
        xb = jnp.concatenate([t, b], axis=0)
        last = _dot(xb, weights(ref, 4, 5))
        rem = _dot(xb[:, 512:], weights(ref, 0, 4, r0=512))
        return t, b, rem[:m], rem[m:], last[:m], last[m:]

    def dd_main(name, parts, prep=False):
        t, b, rt, rb, lt, lb = (jnp.concatenate(v, axis=0) for v in zip(*parts))
        ops = _sums_a(t[:, :256], t[:, 256:512], b[:, :256], b[:, 256:512]) + [t[:, :256], b[:, 256:512]]
        top, bot = [None] * 4, [None] * 4
        for j in range(2):
            top[j], top[j + 2], bot[j], bot[j + 2] = spair(name, j, lambda i: ops[i], prep)
        return (jnp.concatenate([jnp.concatenate(top, axis=1) + rt, lt], axis=1),
                jnp.concatenate([jnp.concatenate(bot, axis=1) + rb, lb], axis=1))

    def stage_a0(w, r0, n):
        rows = pl.ds(r0, n)
        x = w["q"][rows, :].astype(F32)
        x2 = x + add_mod(mul_mod(_ln(x), 1), 0) * slabs(w["y"], r0, n)
        w["x2"][rows, :] = x2
        return _ln(x2)

    def stage_a1(w, r0, n, n2=None, f32=False):
        if n2 is None:
            n2 = stage_a0(w, r0, n)
        h = add_mod(mul_mod(n2, 4), 3)
        put(w["h"], pl.ds(r0, n), h)
        n3 = _ln(h, 4 * EPS)
        return n3 if f32 else n3.astype(BF16)

    def stage_a2(w, n3, r0, n, last_valid=None, fine=0, c0=0, c1=NC, prep=False):
        hh = _gelu2(_unrows2(*dd_main("w1", n3, prep)) if isinstance(n3, list) else _dot_fine(n3, weights(w1buf, c0, c1), fine))
        for c in range(c0, c1):
            blk = hh[:, (c - c0) * 128:(c - c0 + 1) * 128]
            w["hh"][c, pl.ds(r0 + 8, n - LEAD), :] = blk[:n - LEAD]
            tail = blk[n - LEAD:]
            if last_valid is not None:
                tail = jnp.where(last_valid, tail, 0.0)
            w["hh"][c, pl.ds(r0 + 8 + n - LEAD, LEAD), :] = tail

    def stage_b1a(w, r0, n, fine=0, fast=False, prep=False):
        m = n // 2
        lane = jax.lax.broadcasted_iota(jnp.int32, (m, 128), 1)
        g = []
        for e in range(2):
            sh = lambda c, d: w["hh"][c, pl.ds(r0 + 8 + e + d, m, stride=2), :]
            g.append(jnp.concatenate([sh(0, -1),
                                      jnp.where(lane < 32, sh(1, -1), sh(1, 1)),
                                      jnp.where(lane < 64, sh(2, 1), sh(2, -2)),
                                      jnp.where(lane < 96, sh(3, -2), sh(3, 2)),
                                      sh(4, 2)], axis=1))
        if fast:
            hs = dd_main("w2", [dd_rest("w2", *g)], prep)
        else:
            hs = _dot_fine(jnp.concatenate(g, axis=0), weights(w2buf), fine)
            hs = hs[:m], hs[m:]
        x1 = [parity(w["h"], r0, n, e) + hs[e] for e in range(2)]
        for e in range(2):
            put(w["h"], pl.ds(r0 + e, m, stride=2), x1[e])
        return x1

    def stage_b1b(w, x1, r0, n):
        xn = jnp.stack([_ln(x, 4 * EPS).reshape(n // 16, 8, D) for x in x1], axis=1).reshape(n, D)
        t, b = _rows2(xn)
        w["xn"][0, pl.ds(r0 // 2, n // 2), :] = t.astype(BF16)
        w["xn"][1, pl.ds(r0 // 2, n // 2), :] = b.astype(BF16)
        sa = _sums_a(t[:, :256], t[:, 256:512], b[:, :256], b[:, 256:512])
        w["xs"][pl.ds(r0 // 2, n // 2), :] = jnp.concatenate(sa, axis=1).astype(BF16)

    def stage_b1(w, r0, n, fast=False, prep=False):
        stage_b1b(w, stage_b1a(w, r0, n, fast=fast, prep=prep), r0, n)

    def out_copy(r0, n):
        rows = pl.ds(r0, n)
        return pltpu.make_async_copy(obuf.at[rows, :], out_hbm.at[rows, :], sem_out.at[0])


    def packrows(v):
        v = v.reshape(v.shape[0] // 16, 2, 8, 128)
        return pack2(v[:, 0], v[:, 1]).reshape(-1, 128)

    def emit(h3, j, left, right):
        m = left.shape[0] // 2
        g = [left[:m], right[:m], left[m:], right[m:]]
        for k, v in enumerate(_sums_a(*g) + g):
            h3[j, k, pl.ds(0, m // 2), :] = packrows(v)

    def load_xn(w, r0, n):
        return w["xn"][:, pl.ds(r0 // 2, n // 2), :].reshape(n, D)

    def w3_operands(w, r0, n):
        xn = load_xn(w, r0, n)
        xsum = w["xs"][pl.ds(r0 // 2, n // 2), :]
        m = n // 2
        return xn, [xsum[:, 256 * k:256 * (k + 1)] for k in range(5)] + [xn[:m, :256], xn[m:, 256:512]]

    def stage_b2h(w, h3, r0, n, prep=False):
        xn, ops = w3_operands(w, r0, n)
        m = n // 2
        rem = _dot_nt(weights(w3buf, 4, 5, r0=1536), xn[:, 512:])
        c11, c12, c21, c22 = spair("w3t", 0, lambda i: ops[i], prep)
        pad = jnp.zeros((128 - FT, m), F32)
        g11, g12, g21, g22 = (jnp.concatenate([_gelu2(c + r), pad], axis=0).T for c, r in (
            (c11, rem[:FT, :m]), (c12, rem[FT:, :m]), (c21, rem[:FT, m:]), (c22, rem[FT:, m:])))
        emit(h3, 6, jnp.concatenate([g11, g21], axis=0), jnp.concatenate([g12, g22], axis=0))

    def stage_b2a(w, h3, r0, n, lo=0, hi=6, prep=False):
        xn, ops = w3_operands(w, r0, n)
        for j in range(lo, hi):
            r1, r2 = (_dot_nt(xn[:, 512:], weights(w3buf, 4, 5, 128 * t, 128 * (t + 1))) for t in (j, j + 6))
            c11, c12, c21, c22 = spair("w3", j, lambda i: ops[i], prep)
            emit(h3, j, _gelu2(jnp.concatenate([c11, c21], axis=0) + r1), _gelu2(jnp.concatenate([c12, c22], axis=0) + r2))

    def finish(w, h2, r0, n, c):
        rows, cols = pl.ds(r0, n), pl.ds(c * 128, 128)
        w["o"][rows, cols] = (w["x2"][rows, cols] + mul_mod(w["h"][c, rows, :] + h2, 5, cols)).astype(BF16)

    def stage_b2b(w, h3, r0, n, j, k0=0, k1=7, done=None, prep=False, fine=0, sub=0):
        hv = h3.at[pl.ds(zsm[j], 7)]
        blk = lambda k: jnp.concatenate([hv[p, k, pl.ds(sub // 4, n // 4), :] for p in range(7)], axis=1)
        r0 += sub
        if j < 2:
            done = [] if done is None else done
            done += sprods("w4", j, lambda i: _unpack(blk(8 if i == 6 else i)), k0, k1, prep)
            if k1 == 7:
                c11, c12, c21, c22 = _combine(*done)
                finish(w, _unrows2(c11, c21), r0, n, j)
                finish(w, _unrows2(c12, c22), r0, n, j + 2)
            return done
        wb = wblocks("w4", 4)
        lhs = jnp.concatenate([jnp.concatenate([blk(5), blk(6)], axis=1),
                               jnp.concatenate([blk(7), blk(8)], axis=1)], axis=0)
        h2 = _dot_fine(_unpack(lhs), _unpack(jnp.concatenate([wb(0, 0), wb(1, 0)], axis=0)), fine)
        finish(w, _unrows2(h2[:n // 2], h2[n // 2:]), r0, n, 4)

    w = window(0, 2 * TS + LEAD, 0)
    H = TS // 2
    with jax.named_scope("t0a"):
        cps["qa"].wait()
        cps["wmoda"].wait()

        mv = {}

        def mod_fn(j, toks):
            mv[j] = mod_cols(j, 1, toks)[0]
            if len(mv) == 3:
                modbuf[0] = mv[2] * mv[0]
                modbuf[1] = mv[2] * (1.0 + mv[1])

        segment(G5B, 0, MU, mod_fn=mod_fn)
        put(w["h"], pl.ds(0, QA), stage_a0(w, 0, QA))
    with jax.named_scope("t0b"):
        cps["wmodb"].wait()
        sb, cb = mod_cols(3, 2)
        modbuf[3] = 2.0 * sb
        modbuf[4] = 2.0 + 2.0 * cb
        n3 = stage_a1(w, 0, QA, n2=slabs(w["h"], 0, QA))
    XB = TS - XA
    FN = 32
    F4 = 64
    P1B = "1" == "1"
    with jax.named_scope("t1a"):
        cps["w1a"].wait()
        cps["qx"].wait()
        put(w["h"], pl.ds(QA, XA), stage_a0(w, QA, XA))
        stage_a2(w, n3, 0, QA, c1=W1A, fine=80)
    with jax.named_scope("t1b"):
        cps["w1b"].wait()
        n3a = stage_a1(w, QA, XA, n2=slabs(w["h"], QA, XA), f32=True)
        stage_a2(w, n3, 0, QA, c0=W1A)
        if P1B:
            stage_a2(w, [dd_rest("w1", *_rows2(n3a))], QA, XA, prep=True)
        else:
            stage_a2(w, n3a, QA, XA, fine=FN)
    with jax.named_scope("t2"):
        cps["qb"].wait()
        cps["w2"].wait()
        n3b = stage_a1(w, QA + XA, XB, f32=True)
        x1 = {}
        for op in "2aP na 1 2bF nb 2cF".split():
            r, n = dict(a=(0, TS), b=(TS, XA), c=(TS + XA, XB), d=(0, H), e=(H, H), f=(H, TS), g=(TS, TS)).get(op[1:2], (0, 0))
            if op == "1":
                stage_a2(w, [dd_rest("w1", *_rows2(n3b))], QA + XA, XB, prep=not P1B)
            elif op[0] == "n":
                stage_b1b(w, x1[op[1]], r, n)
            else:
                x1[op[1]] = stage_b1a(w, r, n, fast=op[2] in "PF", prep=op[2] == "P", fine=FN if op[2] == "f" else 0)
    ha, hb = hba, hbb
    with jax.named_scope("t3"):
        cps["w3"].wait()
        r, n = (TS + XA, XB)
        stage_b1b(w, [parity(w["h"], r, n, e) for e in range(2)], r, n)
        for op in "ha 3a:0:6 hb 3b:0:6".split():
            op, *rng = op.split(":")
            rng = [int(x) for x in rng]
            hx, r = (ha, 0) if op[1] == "a" else (hb, TS)
            if op[0] == "h":
                stage_b2h(w, hx, r, TS, prep=op[1] == "a")
            else:
                stage_b2a(w, hx, r, TS, *rng, prep=op[1] == "a")
    with jax.named_scope("t4"):
        cps["w4"].wait()
        cps["wmodg"].wait()
        done = []
        for op in "m0 p m2 p m1 p m3 p m4 p p p".split():
            if op == "p":
                stage_b2b(w, ha, 0, TS, 0, len(done), len(done) + 1, done=done, prep=True)
            else:
                c = int(op[1])
                modbuf[5, :, pl.ds(c * 128, 128)] = 0.5 * _dot(modbuf[6], weights(wmodbuf, 5 * NC + c, 5 * NC + c + 1))
        for j in range(1, 3):
            stage_b2b(w, ha, 0, TS, j, prep=True, fine=F4)
        out_copy(0, TS).start()
        cps["q1"].wait()

    CBS = (128, 128)
    PART = {"a": (TS, TS), "c": (TS, H), "d": (TS + H, H)}
    BODY = "4:2 4:0:0:4 r0 4:0:4:7 r1 1a 4:1:0:3 2a na 4:1:3:7 3a:0:1 ha 3a:1:6"

    def step(s, carry):
        r0 = pl.multiple_of(s * TS, TS)
        w = window(r0, 2 * TS + LEAD, pl.multiple_of(s * H, H))
        x1, rest, done = {}, {}, {0: [], 1: [], 2: None}
        for op in BODY.split():
            op, *rng = op.split(":")
            rng = [int(x) for x in rng]
            if op[0] == "3":
                stage_b2a(w, hb, TS, TS, *rng)
            elif op[0] == "h":
                stage_b2h(w, hb, TS, TS)
            elif op[0] == "4":
                stage_b2b(w, hb, 0, TS, *rng, done=done[rng[0]])
            elif op[0] == "2":
                x1[op[1]] = stage_b1a(w, *PART[op[1]], fast=True)
            elif op[0] == "n":
                stage_b1b(w, x1[op[1]], *PART[op[1]])
            elif op[0] == "r":
                j = int(op[1])
                rest[j] = dd_rest("w1", *_rows2(stage_a1(w, TS + LEAD + sum(CBS[:j]), CBS[j], f32=True)))
            else:
                ra, n = PART[op[1]]
                parts = [rest[j] for j in range(len(CBS)) if ra - TS <= sum(CBS[:j]) < ra - TS + n]
                stage_a2(w, parts, ra + LEAD, n, last_valid=(s < NT - 2) if ra + n == 2 * TS else None)
        out_copy(r0, TS).start()
        return carry

    with jax.named_scope("p2main"):
        jax.lax.fori_loop(1, NT - 1, step, 0)
    with jax.named_scope("p2epi"):
        w = window(S - 2 * TS, 2 * TS + LEAD, S // 2 - TS)
        rows = pl.ds(S - TS, TS)
        pending.append(hhbuf[0, pl.ds(S, 8), :])
        def flush(rows, cols):
            pltpu.make_async_copy(obuf.at[rows, cols], out_hbm.at[rows, cols], sem_out.at[0]).start()

        for j in range(2):
            stage_b2b(w, hb, TS, TS, j)
        flush(rows, pl.ds(0, 512))
        sub = 0
        for n in (128, 64, 64):
            stage_b2b(w, hb, TS, n, 2, sub=sub)
            flush(pl.ds(S - TS + sub, n), pl.ds(512, 128))
            sub += n
        pltpu.make_async_copy(obuf, out_hbm, sem_out.at[0]).wait()


@jax.jit
def pallas_adaLN_cond__ssm_conv_h3__mixer_s_mlp__prompt_kernel(
    A_q: jax.Array,
    A_k: jax.Array,
    A_v: jax.Array,
    A_shift_k: jax.Array,
    A_ssm_k: jax.Array,
    A_ssm_D: jax.Array,
    B_x: jax.Array,
    B_w1: jax.Array,
    B_w2: jax.Array,
    B_w3: jax.Array,
    B_w4: jax.Array,
    c: jax.Array,
    w_mod: jax.Array,
):
    del B_x

    def tiles(x):
        return x.reshape(S // 8, 8, NC, 128).transpose(0, 2, 1, 3).reshape(S * NC, 128)

    def pairs(x):
        r, n = x.shape
        return x.reshape(r // 16, 2, 8, n // 128, 128).transpose(0, 1, 3, 2, 4)

    args = (
        A_q.reshape(S, D), tiles(A_k), tiles(A_v),
        A_shift_k.T, A_ssm_k, A_ssm_D.reshape(NC, 128),
        pairs(B_w1), pairs(B_w2), pairs(B_w3.T), pairs(B_w4), c, pairs(w_mod),
    )
    scratch = [
        pltpu.VMEM((NA, P * NC + 128, 128), BF16),
        pltpu.VMEM((NA, P * NC + 64, 128), BF16),
        pltpu.VMEM((D, S), BF16),
        pltpu.VMEM((R, 128, 128), U32),
        pltpu.VMEM((R, 64, 256), U32),
        pltpu.VMEM((64, 128), U32),
        pltpu.VMEM((D // 16, 6 * NC, 16, 128), BF16),
        pltpu.VMEM((D // 16, NC, 16, 128), BF16),
        pltpu.VMEM((D // 16, NC, 16, 128), BF16),
        pltpu.VMEM((FF // 16, NC, 16, 128), BF16),
        pltpu.VMEM((FF // 16, NC, 16, 128), BF16),
        pltpu.VMEM((S + 64, D), BF16),
        *[pltpu.VMEM((NA, R, 16, 4, 8, 128), F32) for _ in range(NC)],
        pltpu.VMEM((NC, NA - 1, R, 16, 2, 8, 128), F32),
        pltpu.VMEM((NC, R, 128, 128), U32),
        pltpu.VMEM((32, 128), U32),
        pltpu.VMEM((NC, 8, 8, 128), F32),
        pltpu.VMEM((NC, S + 32, 128), F32),
        pltpu.VMEM((8, 8, D), F32),
        pltpu.VMEM((S + 32, D), F32),
        pltpu.VMEM((NC, S + 32, 128), F32),
        pltpu.VMEM((NC, S + 32, 128), F32),
        pltpu.VMEM((2, S // 2, D), BF16),
        pltpu.VMEM((S // 2, 5 * 256), BF16),
        pltpu.VMEM((5, 2, 128, 128), U32),
        pltpu.VMEM((5, 2, 128, 128), U32),
        pltpu.VMEM((5, 6, 64, 256), U32),
        pltpu.VMEM((5, 2, FT // 2, 256), U32),
        pltpu.VMEM((5, 2, 448, 128), U32),
        pltpu.VMEM((8, 9, 72, 128), U32),
        pltpu.VMEM((8, 9, 72, 128), U32),
        pltpu.VMEM((S, D), BF16),
        pltpu.VMEM((4, D), BF16),
        pltpu.VMEM((NC, 128), BF16),
        pltpu.VMEM((1, D), BF16),
        pltpu.SMEM((8,), jnp.int32),
        pltpu.SemaphoreType.DMA((40,)),
        pltpu.SemaphoreType.DMA((1,)),
    ]
    out = pl.pallas_call(
        _kernel,
        out_shape=jax.ShapeDtypeStruct((S, D), BF16),
        in_specs=[pl.BlockSpec(memory_space=pl.ANY)] * len(args),
        out_specs=pl.BlockSpec(memory_space=pl.ANY),
        scratch_shapes=scratch,
        grid=(1,),
        compiler_params=pltpu.CompilerParams(vmem_limit_bytes=100 * 1024 * 1024, disable_semaphore_checks=True,
                                             disable_bounds_checks=True),
        name="adaln_h3_mixer",
    )(*args)
    return out.reshape(1, S, D)
```

```python
import numpy as np
import jax
import jax.numpy as jnp
import jax.experimental.pallas as pl
import jax.experimental.pallas.tpu as pltpu

F32 = jnp.float32
BF16 = jnp.bfloat16
U32 = jnp.uint32

S = 2048
D = 640
FF = 1728
NC = D // 128
R = 4
P = 128 * R
NA = S // P
TS = 256
NT = S // TS
LEAD = 16
EPS = 1e-5
NEST = (1, 4, 2, 3, 5)
NQ = len(NEST)
FT = (FF - 1536) // 2
FM = (FF // 128) * 128
FR = FF - FM
P1_ORDER = "t0 t1 t2 t3 k0 k1 k2 k3 u0 i0 u1 i1 u2 i2 u3 i3"


def _freq(row):
    t, part, s = row >> 4, (row >> 3) & 1, row & 7
    return 32 * (t & 7) + 4 * s + 2 * (t >> 3) + 1, P * part


def _cos(j, scale):
    jf = (j & (4 * P - 1)).astype(F32)
    u = 2.0 * np.pi / (4 * P)
    x = jnp.abs(jf * u - np.pi) - 0.5 * np.pi
    x2 = x * x
    poly = scale / 362880.0 - x2 * (scale / 39916800.0)
    for coef in (-1.0 / 5040.0, 1.0 / 120.0, -1.0 / 6.0, 1.0):
        poly = poly * x2 + coef * scale
    return poly * x


_DUR = {"t": 8, "u": 16, "k": 16, "i": 16, "m": 12, "g": 0, "c": 0, "j": 16}
_POST = {"t": 8.0, "u": 16.0, "k": 24.0, "i": 4.0, "j": 4.0, "m": 18.0}


def _plan_tokens(order, maxutil):
    lag, cap, pre, margin = 8, 60, 4, 3
    start, slots = {}, []
    for n in order:
        start[n] = len(slots)
        slots += [(n, r) for r in range(_DUR[n[0]])]
    nslot = len(slots) + lag
    free = [cap - (_POST[slots[i - lag][0][0]] if i >= lag else 0.0) for i in range(-pre, nslot)]
    units = []
    for n in order:
        kind, a, c = n
        if kind == "u":
            units += [(n + (g,), 94.0, start[n], -pre) for g in range(8)]
        elif kind == "g":
            units += [(n + (g,), 150.0, start[n], -pre) for g in range(8)]
        elif kind in "ic":
            src_ = [start[m] for m in (("u", a, c), ("k", a, c)) if m in start]
            for t in range(16):
                rel = max(max(src_) + 16, max(src_) + t + lag + 3) if src_ else -pre
                units.append((n + (t,), 32.0 * a + 48.0, nslot if kind == 'c' else start[n], rel))

    def simulate(util):
        left = [u[1] for u in units]
        done = [None] * len(units)
        for i in range(-pre, nslot):
            budget = util * free[i + pre]
            for j, u in enumerate(units):
                if budget <= 0.0:
                    break
                if done[j] is None and u[3] <= i:
                    use = min(budget, left[j])
                    left[j] -= use
                    budget -= use
                    if left[j] <= 1e-9:
                        done[j] = i + 1
        ok = all(u[2] < 8 or (d is not None and d <= max(u[2] - (1 if u[0][0] in 'cg' else margin), u[3] + 1))
                 for d, u in zip(done, units))
        return done, ok

    lo_, hi_ = 0.05, maxutil
    for _ in range(12):
        mid = 0.5 * (lo_ + hi_)
        if simulate(mid)[1]:
            hi_ = mid
        else:
            lo_ = mid
    done, _ = simulate(hi_)
    plan = {}
    for u, d in zip(units, done):
        if u[0][0] == "c":
            plan[u[0]] = slots[max((nslot - 1 if d is None else min(d, nslot - 1)) - lag, 0)]
        elif d is not None and 0 <= d < u[2]:
            plan.setdefault(slots[d], []).append(u[0])
    return plan


def _pack(x):
    return pltpu.bitcast(x.astype(BF16), U32)


def _unpack(w):
    return pltpu.bitcast(w, BF16)


def _dot(a, b):
    return jnp.dot(a.astype(BF16), b, preferred_element_type=F32)


def _dot_nt(a, b):
    return jax.lax.dot_general(a.astype(BF16), b, (((1,), (1,)), ((), ())), preferred_element_type=F32)


def _dot_fine(x, w, chunk, nt=False):
    if not chunk:
        return _dot_nt(x, w) if nt else _dot(x, w)
    n = w.shape[0] if nt else w.shape[1]
    head, last = (w[:n - 128], w[n - 128:]) if nt else (w[:, :n - 128], w[:, n - 128:])
    f = _dot_nt if nt else _dot
    parts = [f(x, head)] if n > 128 else []
    parts.append(jnp.concatenate([f(x[r:r + chunk], last) for r in range(0, x.shape[0], chunk)], axis=0))
    return jnp.concatenate(parts, axis=1)


def _rows2(x):
    n, c = x.shape
    x = x.reshape(n // 32, 2, 16, c)
    return x[:, 0].reshape(n // 2, c), x[:, 1].reshape(n // 2, c)


def _unrows2(top, bot):
    n, c = top.shape
    return jnp.stack([top.reshape(n // 16, 16, c), bot.reshape(n // 16, 16, c)], axis=1).reshape(2 * n, c)


def _sums_a(a11, a12, a21, a22):
    return [a11 + a22, a21 + a22, a11 + a12, a21 - a11, a12 - a22]


def _sums_b(b11, b12, b21, b22):
    return [b11 + b22, b12 - b22, b21 - b11, b11 + b12, b21 + b22]


_STRASSEN = ((0, 0), (1, 5), (5, 1), (6, 2), (2, 6), (3, 3), (4, 4))


_SUMS_A = ((0, 3, 1), (2, 3, 1), (0, 1, 1), (2, 0, -1), (1, 3, -1))
_SUMS_B = ((0, 3, 1), (1, 3, -1), (2, 0, -1), (0, 1, 1), (2, 3, 1))


def _combine(m1, m2, m3, m4, m5, m6, m7):
    return (m1 + m4) + (m7 - m5), m3 + m5, m2 + m4, (m1 - m2) + (m3 + m6)


def _lo(w):
    return pltpu.bitcast(w << 16, F32)


def _hi(w):
    return pltpu.bitcast(w & jnp.uint32(0xFFFF0000), F32)


def _ln(x, eps=EPS):
    m = jnp.sum(x, axis=-1, keepdims=True) * (1.0 / D)
    xc = x - m
    v = jnp.sum(xc * xc, axis=-1, keepdims=True) * (1.0 / D)
    return xc * jnp.exp(-0.5 * jnp.log(v + eps))


def _gelu2(x):
    c0 = 0.7978845608028654
    c1 = c0 * 0.044715
    return x + x * jnp.tanh(x * (c0 + c1 * (x * x)))


def _bfly(tr, ti, sign):
    s02r, s02i = tr[0] + tr[2], ti[0] + ti[2]
    d02r, d02i = tr[0] - tr[2], ti[0] - ti[2]
    s13r, s13i = tr[1] + tr[3], ti[1] + ti[3]
    d13r, d13i = tr[1] - tr[3], ti[1] - ti[3]
    x0r, x0i = s02r + s13r, s02i + s13i
    x2r, x2i = s02r - s13r, s02i - s13i
    ar, ai = d02r + d13i, d02i - d13r
    br, bi = d02r - d13i, d02i + d13r
    if sign < 0:
        return [x0r, ar, x2r, br], [x0i, ai, x2i, bi]
    return [x0r, br, x2r, ar], [x0i, bi, x2i, ai]


def _kernel(q_hbm, k_hbm, v_hbm, shift_hbm, ssmk_hbm, ssmd_hbm, w1_hbm, w2_hbm, w3t_hbm, w4_hbm,
            c_hbm, wmod_hbm,
            out_hbm,
            kbuf, vbuf, skbuf, fwdbuf, invbuf, permbuf,
            wmodbuf, w1buf, w2buf, w3buf, w4buf, qbuf,
            xs0, xs1, xs2, xs3, xs4, kraw, wbuf, zbuf, coefbuf, ybuf, modbuf, x2buf, hbuf, hhbuf, xnbuf, xsbuf,
             w1s, w2s, w3s, w3ts, w4s, hba, hbb, w4n, w4q, obuf, shiftbuf, dbuf, cbuf,
            zsm, sem_in, sem_out):
    cps = {}
    n_sem = [0]

    def start(name, src, dst):
        cp = pltpu.make_async_copy(src, dst, sem_in.at[n_sem[0]])
        n_sem[0] += 1
        cp.start()
        cps[name] = cp

    class Both:
        def __init__(self, a, b):
            self.cps = (a, b)

        def wait(self):
            for cp in self.cps:
                cp.wait()

    def start_w(name, src, dst, c0=0, n=NC):
        for e in range(2):
            start(name + str(e), src.at[:, e, pl.ds(c0, n)], dst.at[:, pl.ds(c0, n), pl.ds(8 * e, 8), :])
        cps[name] = Both(cps[name + "0"], cps[name + "1"])

    CH = P * NC
    HALO = 8 * NC

    def start_s(a):
        cols = pl.ds(a * P, P)
        start("s%d" % a, ssmk_hbm.at[:, cols], skbuf.at[:, cols])

    def start_kv(a):
        if a == 0:
            kbuf[0, pl.ds(0, HALO + 8), :] = jnp.zeros((HALO + 8, 128), BF16)
            start("k0", k_hbm.at[pl.ds(0, CH), :], kbuf.at[0, pl.ds(HALO, CH), :])
        else:
            start("k%d" % a, k_hbm.at[pl.ds(a * CH - HALO, CH + HALO), :], kbuf.at[a, pl.ds(0, CH + HALO), :])
        start("v%d" % a, v_hbm.at[pl.ds(a * CH, CH), :], vbuf.at[a, pl.ds(0, CH), :])

    for n in "s0 x0 s1 k0 k1 s2 k2 s3 k3".split():
        if n[0] == "s":
            start_s(int(n[1]))
        elif n[0] == "k":
            start_kv(int(n[1]))
        else:
            start("d", ssmd_hbm, dbuf)
            start("shift", shift_hbm, shiftbuf)
            start("c", c_hbm, cbuf)
    QA = TS + LEAD
    XA = 128
    QB = 2 * TS + LEAD
    W1A = 2

    def start_q(name, r0, n):
        start(name, q_hbm.at[pl.ds(r0, n), :], qbuf.at[pl.ds(r0, n), :])

    start_q("qa", 0, QA)
    start_w("wmoda", wmod_hbm, wmodbuf, 0, 3 * NC)
    start_w("wmodb", wmod_hbm, wmodbuf, 3 * NC, 2 * NC)
    start_q("qx", QA, XA)
    start_w("w1a", w1_hbm, w1buf, 0, W1A)
    start_w("w1b", w1_hbm, w1buf, W1A, NC - W1A)
    start_q("qb", QA + XA, QB - QA - XA)
    start_w("w2", w2_hbm, w2buf)
    start_w("w3", w3t_hbm, w3buf)
    start_w("w4", w4_hbm, w4buf)
    start_w("wmodg", wmod_hbm, wmodbuf, 5 * NC, NC)
    start_q("q1", QB, S - QB)

    kw = kbuf.bitcast(U32)
    vw = vbuf.bitcast(U32)
    zbuf[...] = jnp.zeros(zbuf.shape, U32)
    for j in range(64):
        zsm[j] = 0
    for c in range(NC):
        ybuf[c, pl.ds(S, LEAD), :] = jnp.zeros((LEAD, 128), F32)
        hhbuf[c, pl.ds(0, 8), :] = jnp.zeros((8, 128), F32)
    qbuf[pl.ds(S, LEAD), :] = jnp.zeros((LEAD, D), BF16)

    def tables(p, carry):
        i0 = jax.lax.broadcasted_iota(jnp.int32, (128, 128), 0)
        n = R * jax.lax.broadcasted_iota(jnp.int32, (128, 128), 1) + p
        f2, off = _freq(2 * i0)
        j = f2 * n + off
        fwdbuf[p] = pltpu.pack_elementwise([_cos(j, 1.0), _cos(j + 4 * n, 1.0)], packed_dtype=BF16)
        return carry

    jax.lax.fori_loop(0, R, tables, 0)

    def unit_g(kt, r):
        col = jax.lax.broadcasted_iota(jnp.int32, (8, 128), 1) + 128 * kt
        f2, off = _freq((col & ~15) + 8 * (col & 1) + ((col >> 1) & 7))
        m = 2 * jax.lax.broadcasted_iota(jnp.int32, (8, 128), 0) + 16 * r
        j0 = f2 * (R * m) + off
        out = []
        for p in range(R):
            j = j0 + p * f2
            out.append(pltpu.pack_elementwise([_cos(j, 1.0 / P), _cos(j + R * f2, 1.0 / P)], packed_dtype=BF16))
            invbuf[p, pl.ds(8 * r, 8), pl.ds(128 * kt, 128)] = out[-1]
        return out

    i0 = jax.lax.broadcasted_iota(jnp.int32, (128, 128), 0)
    i1 = jax.lax.broadcasted_iota(jnp.int32, (128, 128), 1)
    permbuf[...] = _pack(jnp.where(i0 == (128 // R) * (i1 & (R - 1)) + (i1 >> 2), 1.0, 0.0).astype(F32))

    def fill_coef():
        cv = cbuf[...].astype(F32)
        modbuf[6] = jnp.broadcast_to(cv * jax.nn.sigmoid(cv), (8, D))
        coef = shiftbuf[...].astype(F32)
        dval = dbuf[...].astype(F32)
        for c in range(NC):
            for j in range(4):
                coefbuf[c, j] = jnp.broadcast_to(coef[j:j + 1, c * 128:(c + 1) * 128], (8, 128))
            coefbuf[c, 4] = jnp.broadcast_to(dval[c:c + 1, :], (8, 128))

    xs = (xs0, xs1, xs2, xs3, xs4)
    wsbufs = dict(w1=w1s, w2=w2s, w3=w3s, w4=w4s, w3t=w3ts)
    def split_ri(t):
        t = t.reshape(16, 2, 8, 128)
        return t[:, 0], t[:, 1]

    def get_never():
        return zbuf[pl.ds(0, 8), :] != 0

    def pack2(x, y):
        return pltpu.pack_elementwise([x, y], packed_dtype=BF16)

    def words(ref, a, c, r):
        return ref[a, pl.ds((r // 4) * 4 * NC + 4 * c + r % 4, 8, stride=4 * NC), :]

    def unit_u(a, c, g):
        c0, c1, c2, c3 = (coefbuf[c, pl.ds(j, 1)] for j in range(4))
        kk = jnp.stack([words(kw, a, c, 4 + 32 * g + d) for d in range(-2, 4)])
        vv = jnp.stack([words(vw, a, c, 32 * g + d) for d in range(4)])
        lo, hi = _lo(kk), _hi(kk)
        k0, k1, k2 = lo[2:], hi[1:5], lo[1:5]
        even = (((k0 * c0 + k1 * c1) + (k2 * c2 + hi[:4] * c3)) * _lo(vv)).reshape(32, 128)
        odd = (((hi[2:] * c0 + k0 * c1) + (k1 * c2 + k2 * c3)) * _hi(vv)).reshape(32, 128)
        e, o = pack2(even[:16], even[16:]), pack2(odd[:16], odd[16:])
        return [e[:8], o[:8], e[8:], o[8:]]

    def unit_i(a, c, t, z):
        x_c = xs[c].at[pl.ds(z, NA)]
        yr = yi = None
        for j in range(a + 1):
            ur, ui = x_c[j, :, t, 0], x_c[j, :, t, 1]
            kr, ki = x_c[a - j, :, t, 2], x_c[a - j, :, t, 3]
            pr = ur * kr - ui * ki
            pi = ur * ki + ui * kr
            yr = pr if yr is None else yr + pr
            yi = pi if yi is None else yi + pi
        halves = lambda x: (x[:x.shape[0] // 2], x[x.shape[0] // 2:])
        (ra, rb), (ia, ib) = halves(yr.reshape(32, 128)), halves(yi.reshape(32, 128))
        (sr0, sr1), (si0, si1), (dr0, dr1), (di0, di1) = (halves(x) for x in (ra + rb, ia + ib, ra - rb, ia - ib))
        return [pack2(sr0 + sr1, si0 + si1), pack2(dr0 - di1, di0 + dr1),
                pack2(sr0 - sr1, si0 - si1), pack2(dr0 + di1, di0 - dr1)]

    def segment(spec, z, maxutil=1.0, mod_fn=None):
        order = [(n[0], int(n[1]), int(n[2])) for n in spec.split()]
        plan = _plan_tokens(order, maxutil) if maxutil > 0 else {}
        never = get_never()
        units, res = {}, {}

        def unit(key):
            if key not in units:
                kind, a, c, j = key
                if kind == "u":
                    units[key] = unit_u(a, c, j)
                elif kind == "g":
                    units[key] = unit_g(a, j)
                else:
                    fresh = ("u", a, c) in order or ("k", a, c) in order
                    units[key] = unit_i(a, c, j, z if fresh else 0)
            return units[key]

        def lhs(name, p, full, r0=0):
            out, last = [], 0
            for r in range(full.shape[0] // 8):
                keys = plan.get((name, r0 + r), ())
                if keys:
                    if 8 * r > last:
                        out.append(full[last:8 * r])
                    v = full[8 * r:8 * r + 8]
                    for key in keys:
                        v = jax.lax.select(never, unit(key)[p], v)
                    out.append(v)
                    last = 8 * r + 8
            if last < full.shape[0]:
                out.append(full[last:] if last else full)
            return out[0] if len(out) == 1 else jnp.concatenate(out, axis=0)

        def dft(name, rhs):
            tr, ti = [], []
            for p in range(R):
                f = lhs(name, p, fwdbuf[p])
                r_, i_ = split_ri(_dot(_unpack(f), rhs[p]))
                if p == 0:
                    res.update({(name, r): (lambda r=r, v=r_: v[r]) for r in range(16)})
                tr.append(r_)
                ti.append(i_)
            return _bfly(tr, ti, -1)

        st = {}
        for name in order:
            kind, a, c = name
            x_c = xs[c]
            if kind == "g":
                for r in range(8):
                    unit(name + (r,))
            elif kind == "c":
                for t in range(16):
                    after = pltpu.bitcast(res[plan[name + (t,)]](), U32)
                    for p in range(R):
                        wbuf[c, p, pl.ds(8 * t, 8), :] = jax.lax.select(never, after, unit(name + (t,))[p])
            elif kind == "m":
                toks = {}
                for r in range(_DUR["m"]):
                    for n_, key in enumerate(plan.get((name, r), ())):
                        toks.setdefault(2 * r + n_ % 2, []).extend(unit(key))
                mod_fn(a, toks)
            elif kind == "t":
                trs = []
                for b in range(R):
                    pm = lhs(name, b, permbuf[...])
                    trs.append(_dot_nt(_unpack(pm), skbuf[pl.ds(c * 128, 128), pl.ds(a * P + b * 128, 128)]))
                res.update({(name, r): (lambda r=r, v=trs[0]: v[16 * r:16 * r + 8]) for r in range(8)})
                g_ = 128 // R
                st[a, c] = [jnp.concatenate([trs[b][p * g_:(p + 1) * g_] for b in range(R)], axis=0).astype(BF16)
                            for p in range(R)]
            elif kind == "u":
                rhs = [_unpack(jnp.concatenate([unit(name + (g,))[p] for g in range(8)], axis=0)) for p in range(R)]
                xr, xi = dft(name, rhs)
                for q in range(R):
                    x_c[a, q, :, 0] = xr[q]
                    x_c[a, q, :, 1] = xi[q]
            elif kind == "k":
                xr, xi = dft(name, st[a, c])
                for q in range(R):
                    if a == 0:
                        x_c[a, q, :, 2] = xr[q] + coefbuf[c, 4]
                        x_c[a, q, :, 3] = xi[q]
                    else:
                        pr, pi = kraw[c, (a - 1) % 2, q, :, 0], kraw[c, (a - 1) % 2, q, :, 1]
                        x_c[a, q, pl.ds(0, 8), 2] = xr[q][:8] - pi[:8]
                        x_c[a, q, pl.ds(0, 8), 3] = xi[q][:8] + pr[:8]
                        x_c[a, q, pl.ds(8, 8), 2] = xr[q][8:] + pi[8:]
                        x_c[a, q, pl.ds(8, 8), 3] = xi[q][8:] - pr[8:]
                    if a + 1 < NA:
                        kraw[c, a % 2, q, :, 0] = xr[q]
                        kraw[c, a % 2, q, :, 1] = xi[q]
            else:
                for p in range(R):
                    cols = [lhs(name, 2 * (p % 2) + kt,
                                invbuf[p, :, pl.ds(128 * kt, 128)], 8 * (p // 2))
                            for kt in range(2)]
                    g = _unpack(jnp.concatenate(cols, axis=1))
                    if kind == "j":
                        wp = _unpack(wbuf[c, p])
                    else:
                        wp = _unpack(jnp.concatenate([unit(name + (t,))[p] for t in range(16)], axis=0))
                    yp = _dot(g, wp)
                    if p % 2 == 0:
                        res.update({(name, 4 * p + r): (lambda r=r, v=yp: v[16 * r:16 * r + 8]) for r in range(8)})
                    ybuf[c, pl.ds(a * P + p, 128, stride=R), :] = yp

    one = jnp.minimum(pl.program_id(0) + 1, 1)

    def once(fn):
        def body(z, carry):
            fn(z)
            return carry
        jax.lax.fori_loop(0, one, body, 0)

    default = "t00 t01 t02 k00 t03 k01 t04 k02 k03 k04 g00|t10 t11 t12 k10 k11 k12 g10|t13 t14 k13 u00 k14 u01 u02 u03 i00 u04 i01 c02 c03|j02 j03 u10 i04 u11 u12 u13 i10 u14 i11 c12|t20 t21 j12 t22 t23 t24 k20 u20 k21 u21 k22 i13 k23 u22 k24 i14 u23 i20 u24 i21 c22|t30 t31 j22 t32 t33 t34 k30 u30 k31 u31 k32 i23 k33 u32 k34 i24 u33 i30 u34 i31 c32|m00 j32 m10 m20 i33 i34"
    specs = default.split("|")
    G5B = specs[-1]
    segs = list(zip("s0 d shift c|s1|k0 v0|k1 v1|s2 k2 v2|s3 k3 v3".split("|"), specs[:-1]))
    MU = 1.5
    for i, (waits, spec) in enumerate(segs):
        with jax.named_scope("g%d" % i):
            for n in waits.split():
                cps[n].wait()
            if i == 0:
                fill_coef()
            once(lambda z: segment(spec, z, MU))

    def mod_cols(lo, n, toks=None):
        m = _dot(modbuf[6], weights(wmodbuf, lo * NC, (lo + n) * NC, toks=toks))
        return [m[:, j * D:(j + 1) * D] for j in range(n)]

    def mul_mod(x, j, cols=None):
        m = modbuf[j] if cols is None else modbuf[j, :, cols]
        return (x.reshape(-1, 8, x.shape[-1]) * m[None]).reshape(x.shape)

    def add_mod(x, j):
        return (x.reshape(-1, 8, x.shape[-1]) + modbuf[j][None]).reshape(x.shape)

    def slabs(ref, r0, n):
        return jnp.concatenate([ref[c, pl.ds(r0, n), :] for c in range(NC)], axis=1)

    def put(ref, rows, x):
        for c in range(NC):
            ref[c, rows, :] = x[:, c * 128:(c + 1) * 128]

    def parity(ref, r0, n, e):
        return jnp.concatenate([ref[c, pl.ds(r0 + e, n // 2, stride=2), :] for c in range(NC)], axis=1)

    def window(base, n, half):
        rows = pl.ds(base, n)
        return dict(xs=xsbuf,
                    q=qbuf.at[rows, :], y=ybuf.at[:, rows, :], x2=x2buf.at[rows, :], h=hbuf.at[:, rows, :],
                    hh=hhbuf.at[:, pl.ds(base, n + 8), :], xn=xnbuf,
                    o=obuf.at[pl.ds(base, n - LEAD), :])

    def weights(ref, c0=0, c1=NC, r0=0, r1=None, toks=None, raw=False, z=None):
        r1 = 16 * ref.shape[0] if r1 is None else r1
        view = ref.bitcast(U32)
        if z is not None:
            view = view.at[pl.ds(z, ref.shape[0])]
        never = get_never() if toks else None
        rt = -(-(r1 - r0) // 128)
        cols = []
        for j in range(c0, c1):
            wu = view[pl.ds(r0 // 16, (r1 - r0) // 16), j].reshape((r1 - r0) // 2, 128)
            if toks:
                parts, last = [], 0
                for i in range(rt):
                    for n_, t in enumerate(toks.get((j - c0) * rt + i, ())):
                        r = 64 * i + 8 * n_
                        if r > last:
                            parts.append(wu[last:r])
                        parts.append(jax.lax.select(never, t, wu[r:r + 8]))
                        last = r + 8
                parts.append(wu[last:])
                wu = jnp.concatenate(parts, axis=0)
            cols.append(wu)
        wu = jnp.concatenate(cols, axis=1)
        return wu if raw else _unpack(wu)

    def wblocks(name, j, z=None):
        if name == "w3":
            blk = lambda kh, nh: weights(w3buf, 2 * kh, 2 * kh + 2, 128 * (j + 6 * nh), 128 * (j + 6 * nh + 1), raw=True, z=z)
        elif name == "w4":
            def blk(kh, nh):
                c = j + 2 * nh
                parts = [weights(w4buf, c, c + 1, 768 * kh, 768 * (kh + 1), raw=True, z=z),
                         weights(w4buf, c, c + 1, 1536 + FT * kh, 1536 + FT * (kh + 1), raw=True, z=z),
                         jnp.zeros(((128 - FT) // 2, 128), U32)]
                return jnp.concatenate(parts, axis=0)
        elif name == "w3t":
            blk = lambda kh, nh: weights(w3buf, 2 * kh, 2 * kh + 2, 1536 + FT * nh, 1536 + FT * (nh + 1), raw=True, z=z)
        else:
            ref = w1buf if name == "w1" else w2buf
            blk = lambda kh, nh: weights(ref, j + 2 * nh, j + 2 * nh + 1, 256 * kh, 256 * (kh + 1), raw=True, z=z)
        return blk

    def wsum(name, j, k):
        blk = wblocks(name, j, zsm[k])
        p, q, sign = ((0, 3, 1), (1, 3, -1), (2, 0, -1), (0, 1, 1), (2, 3, 1))[k]
        x, y = blk(p // 2, p % 2), blk(q // 2, q % 2)
        if sign > 0:
            return pack2(_lo(x) + _lo(y), _hi(x) + _hi(y))
        return pack2(_lo(x) - _lo(y), _hi(x) - _hi(y))

    pending = []

    def attach(wv):
        if not pending:
            return wv
        never = get_never()
        rows = [wv[8 * i:8 * i + 8, :128] for i in range(8)]
        for i, t in enumerate(pending):
            rows[i % 8] = jax.lax.select(never, pltpu.bitcast(t, U32), rows[i % 8])
        pending.clear()
        first = jnp.concatenate(rows + ([wv[64:, :128]] if wv.shape[0] > 64 else []), axis=0)
        return first if wv.shape[1] == 128 else jnp.concatenate([first, wv[:, 128:]], axis=1)

    def sprods(name, j, lhs, k0=0, k1=7, prep=False):
        blk, buf = wblocks(name, j), wsbufs[name]
        if prep == "fresh":
            buf, prep = buf.at[pl.ds(zsm[6], 5)], False
        out = []
        for ia, ib in _STRASSEN[k0:k1]:
            wv = blk(ib - 5, ib - 5) if ib >= 5 else (wsum(name, j, ib) if prep else buf[ib, j])
            if name == "w3t":
                out.append(_dot_nt(_unpack(wv), lhs(ia)))
            else:
                out.append((_dot_nt if name == "w3" else _dot)(lhs(ia), _unpack(attach(wv))))
            if prep and ib < 5:
                buf[ib, j] = wv
        return out

    def spair(name, j, lhs, prep=False):
        return _combine(*sprods(name, j, lhs, prep=prep))

    def dd_rest(name, t, b):
        ref = w1buf if name == "w1" else w2buf
        m = t.shape[0]
        xb = jnp.concatenate([t, b], axis=0)
        last = _dot(xb, weights(ref, 4, 5))
        rem = _dot(xb[:, 512:], weights(ref, 0, 4, r0=512))
        return t, b, rem[:m], rem[m:], last[:m], last[m:]

    def dd_main(name, parts, prep=False):
        t, b, rt, rb, lt, lb = (jnp.concatenate(v, axis=0) for v in zip(*parts))
        ops = _sums_a(t[:, :256], t[:, 256:512], b[:, :256], b[:, 256:512]) + [t[:, :256], b[:, 256:512]]
        top, bot = [None] * 4, [None] * 4
        for j in range(2):
            top[j], top[j + 2], bot[j], bot[j + 2] = spair(name, j, lambda i: ops[i], prep)
        return (jnp.concatenate([jnp.concatenate(top, axis=1) + rt, lt], axis=1),
                jnp.concatenate([jnp.concatenate(bot, axis=1) + rb, lb], axis=1))

    def stage_a0(w, r0, n):
        rows = pl.ds(r0, n)
        x = w["q"][rows, :].astype(F32)
        x2 = x + add_mod(mul_mod(_ln(x), 1), 0) * slabs(w["y"], r0, n)
        w["x2"][rows, :] = x2
        return _ln(x2)

    def stage_a1(w, r0, n, n2=None, f32=False):
        if n2 is None:
            n2 = stage_a0(w, r0, n)
        h = add_mod(mul_mod(n2, 4), 3)
        put(w["h"], pl.ds(r0, n), h)
        n3 = _ln(h, 4 * EPS)
        return n3 if f32 else n3.astype(BF16)

    def stage_a2(w, n3, r0, n, last_valid=None, fine=0, c0=0, c1=NC, prep=False):
        hh = _gelu2(_unrows2(*dd_main("w1", n3, prep)) if isinstance(n3, list) else _dot_fine(n3, weights(w1buf, c0, c1), fine))
        for c in range(c0, c1):
            blk = hh[:, (c - c0) * 128:(c - c0 + 1) * 128]
            w["hh"][c, pl.ds(r0 + 8, n - LEAD), :] = blk[:n - LEAD]
            tail = blk[n - LEAD:]
            if last_valid is not None:
                tail = jnp.where(last_valid, tail, 0.0)
            w["hh"][c, pl.ds(r0 + 8 + n - LEAD, LEAD), :] = tail

    def stage_b1a(w, r0, n, fine=0, fast=False, prep=False):
        m = n // 2
        lane = jax.lax.broadcasted_iota(jnp.int32, (m, 128), 1)
        g = []
        for e in range(2):
            sh = lambda c, d: w["hh"][c, pl.ds(r0 + 8 + e + d, m, stride=2), :]
            g.append(jnp.concatenate([sh(0, -1),
                                      jnp.where(lane < 32, sh(1, -1), sh(1, 1)),
                                      jnp.where(lane < 64, sh(2, 1), sh(2, -2)),
                                      jnp.where(lane < 96, sh(3, -2), sh(3, 2)),
                                      sh(4, 2)], axis=1))
        if fast:
            hs = dd_main("w2", [dd_rest("w2", *g)], prep)
        else:
            hs = _dot_fine(jnp.concatenate(g, axis=0), weights(w2buf), fine)
            hs = hs[:m], hs[m:]
        x1 = [parity(w["h"], r0, n, e) + hs[e] for e in range(2)]
        for e in range(2):
            put(w["h"], pl.ds(r0 + e, m, stride=2), x1[e])
        return x1

    def stage_b1b(w, x1, r0, n):
        xn = jnp.stack([_ln(x, 4 * EPS).reshape(n // 16, 8, D) for x in x1], axis=1).reshape(n, D)
        t, b = _rows2(xn)
        w["xn"][0, pl.ds(r0 // 2, n // 2), :] = t.astype(BF16)
        w["xn"][1, pl.ds(r0 // 2, n // 2), :] = b.astype(BF16)
        sa = _sums_a(t[:, :256], t[:, 256:512], b[:, :256], b[:, 256:512])
        w["xs"][pl.ds(r0 // 2, n // 2), :] = jnp.concatenate(sa, axis=1).astype(BF16)

    def stage_b1(w, r0, n, fast=False, prep=False):
        stage_b1b(w, stage_b1a(w, r0, n, fast=fast, prep=prep), r0, n)

    def out_copy(r0, n):
        rows = pl.ds(r0, n)
        return pltpu.make_async_copy(obuf.at[rows, :], out_hbm.at[rows, :], sem_out.at[0])


    def opaque(ref, i):
        return ref.at[:, :, pl.ds(pl.multiple_of(zsm[i] * 32, 32), ref.shape[2]), :]

    def packrows(v):
        v = v.reshape(v.shape[0] // 16, 2, 8, 128)
        return pack2(v[:, 0], v[:, 1]).reshape(-1, 128)

    def emit(h3, j, left, right):
        m = left.shape[0] // 2
        g = [left[:m], right[:m], left[m:], right[m:]]
        for k, v in enumerate(_sums_a(*g) + g):
            h3[j, k, pl.ds(0, m // 2), :] = packrows(v)

    def load_xn(w, r0, n):
        return w["xn"][:, pl.ds(r0 // 2, n // 2), :].reshape(n, D)

    def w3_operands(w, r0, n):
        xn = load_xn(w, r0, n)
        xsum = w["xs"][pl.ds(r0 // 2, n // 2), :]
        m = n // 2
        return xn, [xsum[:, 256 * k:256 * (k + 1)] for k in range(5)] + [xn[:m, :256], xn[m:, 256:512]]

    def stage_b2h(w, h3, r0, n, prep=False):
        xn, ops = w3_operands(w, r0, n)
        m = n // 2
        rem = _dot_nt(weights(w3buf, 4, 5, r0=1536), xn[:, 512:])
        c11, c12, c21, c22 = spair("w3t", 0, lambda i: ops[i], prep)
        pad = jnp.zeros((128 - FT, m), F32)
        g11, g12, g21, g22 = (jnp.concatenate([_gelu2(c + r), pad], axis=0).T for c, r in (
            (c11, rem[:FT, :m]), (c12, rem[FT:, :m]), (c21, rem[:FT, m:]), (c22, rem[FT:, m:])))
        emit(h3, 6, jnp.concatenate([g11, g21], axis=0), jnp.concatenate([g12, g22], axis=0))

    def stage_b2a(w, h3, r0, n, lo=0, hi=6, prep=False):
        xn, ops = w3_operands(w, r0, n)
        for j in range(lo, hi):
            r1, r2 = (_dot_nt(xn[:, 512:], weights(w3buf, 4, 5, 128 * t, 128 * (t + 1))) for t in (j, j + 6))
            c11, c12, c21, c22 = spair("w3", j, lambda i: ops[i], prep)
            emit(h3, j, _gelu2(jnp.concatenate([c11, c21], axis=0) + r1), _gelu2(jnp.concatenate([c12, c22], axis=0) + r2))

    def finish(w, h2, r0, n, c):
        rows, cols = pl.ds(r0, n), pl.ds(c * 128, 128)
        w["o"][rows, cols] = (w["x2"][rows, cols] + mul_mod(w["h"][c, rows, :] + h2, 5, cols)).astype(BF16)

    def b2_done(w, done, r0, n, j):
        if len(done[j]) == 7:
            c11, c12, c21, c22 = _combine(*[done[j][k] for k in range(7)])
            finish(w, _unrows2(c11, c21), r0, n, j)
            finish(w, _unrows2(c12, c22), r0, n, j + 2)

    def stage_b2b(w, h3, r0, n, j, k0=0, k1=7, done=None, prep=False, fine=0, sub=0, marks=()):
        hv = opaque(h3, j)
        blk = lambda k: jnp.concatenate([hv[p, k, pl.ds(sub // 4, n // 4), :] for p in range(7)], axis=1)
        r0 += sub
        if j < 2:
            for k in range(k0, k1):
                if k not in NEST:
                    done[j][k] = sprods("w4", j, lambda i: _unpack(blk(8 if i == 6 else i)), k, k + 1, prep)[0]
                    b2_done(w, done, r0, n, j)
            return
        wb = wblocks("w4", 4)
        lhs = jnp.concatenate([jnp.concatenate([blk(5), blk(6)], axis=1),
                               jnp.concatenate([blk(7), blk(8)], axis=1)], axis=0)
        if marks:
            lo_, hi_ = 0, 48
            never, at = get_never(), {}
            for i, mk in enumerate(marks):
                s_ = lo_ + (hi_ - lo_) * i // len(marks)
                at[4 * (s_ // 16), s_ % 16] = mk
            cols = []
            for kt in range(14):
                col = lhs[:, 128 * kt:128 * (kt + 1)]
                if any(k_[0] == kt for k_ in at):
                    col = jnp.concatenate([jax.lax.select(never, at[kt, r], col[8 * r:8 * r + 8]) if (kt, r) in at
                                           else col[8 * r:8 * r + 8] for r in range(16)], axis=0)
                cols.append(col)
            lhs = jnp.concatenate(cols, axis=1)
        h2 = _dot_fine(_unpack(lhs), _unpack(jnp.concatenate([wb(0, 0), wb(1, 0)], axis=0)), fine)
        finish(w, _unrows2(h2[:n // 2], h2[n // 2:]), r0, n, 4)


    def psum(x, y, sign):
        if sign > 0:
            return pack2(_lo(x) + _lo(y), _hi(x) + _hi(y))
        return pack2(_lo(x) - _lo(y), _hi(x) - _hi(y))

    def prep_w4(nchunk):
        rows = 384 // nchunk
        marks = []
        for ch in [nchunk] + list(range(nchunk)):
            tail = ch == nchunk
            raw = {}
            for kh in range(2):
                for e in range(1 if tail else 2):
                    r0 = 1536 + FT * kh if tail else 768 * kh + 384 * e + rows * ch
                    x = weights(w4buf, 0, 4, r0, r0 + (FT if tail else rows), raw=True)
                    raw[kh, e] = jnp.stack([_lo(x), _hi(x)])
            blk = lambda i, e: raw[i // 2, e][:, :, 256 * (i % 2):256 * (i % 2 + 1)]
            for k, (ia, ib) in enumerate(_STRASSEN):
                if k not in NEST or ib >= 5:
                    continue
                half = {}
                for e in range(1 if tail else 2):
                    if ib >= 5:
                        half[e] = blk(3 * (ib - 5), e)
                    else:
                        p_, q_, sg = _SUMS_B[ib]
                        half[e] = blk(p_, e) + blk(q_, e) if sg > 0 else blk(p_, e) - blk(q_, e)
                quad = lambda i: half[i // 2][:, :, 128 * (i % 2):128 * (i % 2 + 1)]
                if tail or k not in NEST:
                    if ib < 5:
                        for e in half:
                            for j in range(2):
                                r = 384 if tail else 192 * e + rows // 2 * ch
                                v = quad(2 * e + j)
                                w4q[NEST.index(k), 7, pl.ds(64 * j, v.shape[1]), :] = pack2(v[0], v[1])
                                if tail:
                                    w4q[NEST.index(k), 7, pl.ds(64 * j + FT // 2, 64 - FT // 2), :] = jnp.zeros((64 - FT // 2, 128), U32)
                    continue
                ops = _sums_b(*[quad(i) for i in range(4)]) + ([quad(0), quad(3)] if ib < 5 else [])
                for jb, v in enumerate(ops):
                    w4q[NEST.index(k), jb, pl.ds(rows // 2 * ch, rows // 2), :] = pack2(v[0], v[1])
                first = NEST.index(k)
            if not tail:
                marks.append(w4q.at[pl.ds(zsm[32 + ch], NQ)][first, 0, pl.ds(0, 8), :])
        return marks

    def stage_b2n(*args, **kw):
        for _ in steps_b2n(*args, **kw):
            pass

    def steps_b2n(w, h3, r0, n, k, done, prep=False):
        ia, ib = _STRASSEN[k]
        ka, q, slot = (8 if ia == 6 else ia), n // 8, NEST.index(k)

        def lblk(i, z):
            hv = opaque(h3, z)
            return jnp.concatenate([hv[g + 3 * (i % 2), ka, pl.ds((i // 2) * q, q), :] for g in range(3)], axis=1)

        def wterms(j, lo, hi, z):
            blk = wblocks("w4", j, z)
            if ib >= 5:
                return [(1, blk(ib - 5, ib - 5)[lo:hi])]
            p_, q_, sg = _SUMS_B[ib]
            return [(1, blk(p_ // 2, p_ % 2)[lo:hi]), (sg, blk(q_ // 2, q_ % 2)[lo:hi])]

        def build(terms, dst):
            if len(terms) == 1:
                return terms[0][1]
            if not prep:
                return dst[...]
            acc = None
            for sg, x in terms:
                v = (_lo(x), _hi(x))
                acc = v if acc is None else tuple(a + b_ if sg > 0 else a - b_ for a, b_ in zip(acc, v))
            dst[...] = wv = pack2(*acc)
            return wv

        wq = w4n if ib >= 5 else w4q.at[pl.ds(zsm[6], NQ)] if prep else w4q
        prep = prep and ib >= 5
        quad = lambda i, z: wterms(i % 2, 192 * (i // 2), 192 * (i // 2 + 1), z)
        wt = [build(wterms(j, 384, 448, None), wq.at[slot, 7, pl.ds(64 * j, 64), :]) for j in range(2)]
        tail = _dot(_unpack(opaque(h3, 5)[6, ka, pl.ds(0, 2 * q), :]), _unpack(jnp.concatenate(wt, axis=1)))
        ms = []
        for ja, jb in _STRASSEN:
            if ja >= 5:
                lv = lblk(3 * (ja - 5), 5)
            else:
                p_, q_, sg = _SUMS_A[ja]
                lv = psum(lblk(p_, ja), lblk(q_, ja), sg)
            z = zsm[8 + 7 * slot + jb] if prep else None
            if jb >= 5:
                terms = quad(3 * (jb - 5), z)
            else:
                p_, q_, sg = _SUMS_B[jb]
                terms = quad(p_, z) + [(sg * s_, x) for s_, x in quad(q_, z)]
            ms.append(_dot(_unpack(lv), _unpack(build(terms, wq.at[slot, jb]))))
            if len(ms) < 7:
                yield
        c11, c12, c21, c22 = _combine(*ms)
        done[0][k] = jnp.concatenate([c11, c21], axis=0) + tail[:, :128]
        done[1][k] = jnp.concatenate([c12, c22], axis=0) + tail[:, 128:]
        for j in range(2):
            b2_done(w, done, r0, n, j)

    w = window(0, 2 * TS + LEAD, 0)
    H = TS // 2
    with jax.named_scope("t0a"):
        cps["qa"].wait()
        cps["wmoda"].wait()

        mv = {}

        def mod_fn(j, toks):
            mv[j] = mod_cols(j, 1, toks)[0]
            if len(mv) == 3:
                modbuf[0] = mv[2] * mv[0]
                modbuf[1] = mv[2] * (1.0 + mv[1])

        segment(G5B, 0, MU, mod_fn=mod_fn)
        put(w["h"], pl.ds(0, QA), stage_a0(w, 0, QA))
    with jax.named_scope("t0b"):
        cps["wmodb"].wait()
        sb, cb = mod_cols(3, 2)
        modbuf[3] = 2.0 * sb
        modbuf[4] = 2.0 + 2.0 * cb
        n3 = stage_a1(w, 0, QA, n2=slabs(w["h"], 0, QA))
    XB = TS - XA
    FN = 32
    F4 = 64
    P1B = "1" == "1"
    with jax.named_scope("t1a"):
        cps["w1a"].wait()
        cps["qx"].wait()
        put(w["h"], pl.ds(QA, XA), stage_a0(w, QA, XA))
        stage_a2(w, n3, 0, QA, c1=W1A, fine=80)
    with jax.named_scope("t1b"):
        cps["w1b"].wait()
        n3a = stage_a1(w, QA, XA, n2=slabs(w["h"], QA, XA), f32=True)
        stage_a2(w, n3, 0, QA, c0=W1A)
        if P1B:
            stage_a2(w, [dd_rest("w1", *_rows2(n3a))], QA, XA, prep=True)
        else:
            stage_a2(w, n3a, QA, XA, fine=FN)
    with jax.named_scope("t2"):
        cps["qb"].wait()
        cps["w2"].wait()
        n3b = stage_a1(w, QA + XA, XB, f32=True)
        x1 = {}
        for op in "2aP na 1 2bF nb 2cF".split():
            r, n = dict(a=(0, TS), b=(TS, XA), c=(TS + XA, XB), d=(0, H), e=(H, H), f=(H, TS), g=(TS, TS)).get(op[1:2], (0, 0))
            if op == "1":
                stage_a2(w, [dd_rest("w1", *_rows2(n3b))], QA + XA, XB, prep=not P1B)
            elif op[0] == "n":
                stage_b1b(w, x1[op[1]], r, n)
            else:
                x1[op[1]] = stage_b1a(w, r, n, fast=op[2] in "PF", prep=op[2] == "P", fine=FN if op[2] == "f" else 0)
    ha, hb = hba, hbb
    with jax.named_scope("t3"):
        cps["w3"].wait()
        r, n = (TS + XA, XB)
        stage_b1b(w, [parity(w["h"], r, n, e) for e in range(2)], r, n)
        for op in "ha 3a:0:6 hb 3b:0:6".split():
            op, *rng = op.split(":")
            rng = [int(x) for x in rng]
            hx, r = (ha, 0) if op[1] == "a" else (hb, TS)
            if op[0] == "h":
                stage_b2h(w, hx, r, TS, prep=op[1] == "a")
            else:
                stage_b2a(w, hx, r, TS, *rng, prep=op[1] == "a")
    with jax.named_scope("t4"):
        cps["w4"].wait()
        cps["wmodg"].wait()
        done, gens = {0: {}, 1: {}}, {}
        LC = 64
        for op in "m4 P m0 4:0:0:1 m2 8:1 m1 4:1:0:1 m3 8:2 4:0:6:7 8:3 8:4 4:1:6:7 8:5".split():
            op, *rng = op.split(":")
            rng = [int(x) for x in rng]
            if op[0] == "m":
                c = int(op[1])
                modbuf[5, :, pl.ds(c * 128, 128)] = 0.5 * _dot(modbuf[6], weights(wmodbuf, 5 * NC + c, 5 * NC + c + 1))
            elif op[0] == "8":
                g = gens.setdefault(rng[0], steps_b2n(w, ha, 0, TS, rng[0], done, prep=True))
                for _ in range(rng[1] if len(rng) > 1 else 7):
                    next(g, None)
            elif op[0] == "P":
                stage_b2b(w, ha, 0, TS, 2, marks=prep_w4(24))
            elif op[0] == "L":
                stage_b2b(w, ha, 0, LC, 2, sub=LC * int(op[1]))
            else:
                stage_b2b(w, ha, 0, TS, *rng, done=done, prep=True)
        out_copy(0, TS).start()
        cps["q1"].wait()

    CBS = (160, 96)
    PART = {"a": (TS, TS), "c": (TS, H), "d": (TS + H, H)}
    BODY = "4:2 8:5 8:1 8:4 r0 8:3 r1 1a 8:2 2c nc 2d nd 4:1:6:7 4:1:0:1 4:0:6:7 4:0:0:1 3a:0:1 ha 3a:1:6"

    def step(s, carry):
        r0 = pl.multiple_of(s * TS, TS)
        w = window(r0, 2 * TS + LEAD, pl.multiple_of(s * H, H))
        x1, rest, done = {}, {}, {0: {}, 1: {}}
        for op in BODY.split():
            op, *rng = op.split(":")
            rng = [int(x) for x in rng]
            if op[0] == "3":
                stage_b2a(w, hb, TS, TS, *rng)
            elif op[0] == "h":
                stage_b2h(w, hb, TS, TS)
            elif op[0] == "4":
                stage_b2b(w, hb, 0, TS, *rng, done=done)
            elif op[0] == "8":
                stage_b2n(w, hb, 0, TS, *rng, done)
            elif op[0] == "2":
                x1[op[1]] = stage_b1a(w, *PART[op[1]], fast=True)
            elif op[0] == "n":
                stage_b1b(w, x1[op[1]], *PART[op[1]])
            elif op[0] == "r":
                j = int(op[1])
                rest[j] = dd_rest("w1", *_rows2(stage_a1(w, TS + LEAD + sum(CBS[:j]), CBS[j], f32=True)))
            else:
                ra, n = PART[op[1]]
                parts = [rest[j] for j in range(len(CBS)) if ra - TS <= sum(CBS[:j]) < ra - TS + n]
                stage_a2(w, parts, ra + LEAD, n, last_valid=(s < NT - 2) if ra + n == 2 * TS else None)
        out_copy(r0, TS).start()
        return carry

    with jax.named_scope("p2main"):
        jax.lax.fori_loop(1, NT - 1, step, 0)
    with jax.named_scope("p2epi"):
        w = window(S - 2 * TS, 2 * TS + LEAD, S // 2 - TS)
        rows = pl.ds(S - TS, TS)
        pending.append(hhbuf[0, pl.ds(S, 8), :])
        def flush(rows, cols):
            pltpu.make_async_copy(obuf.at[rows, cols], out_hbm.at[rows, cols], sem_out.at[0]).start()

        done = {0: {}, 1: {}}
        stage_b2b(w, hb, TS, TS, 0, 0, 1, done=done)
        for k in NEST:
            stage_b2n(w, hb, TS, TS, k, done)
        stage_b2b(w, hb, TS, TS, 0, 1, done=done)
        stage_b2b(w, hb, TS, TS, 1, done=done)
        flush(rows, pl.ds(0, 512))
        sub = 0
        for n in (128, 64, 64):
            stage_b2b(w, hb, TS, n, 2, sub=sub)
            flush(pl.ds(S - TS + sub, n), pl.ds(512, 128))
            sub += n
        pltpu.make_async_copy(obuf, out_hbm, sem_out.at[0]).wait()


@jax.jit
def pallas_adaLN_cond__ssm_conv_h3__mixer_s_mlp__prompt_kernel(
    A_q: jax.Array,
    A_k: jax.Array,
    A_v: jax.Array,
    A_shift_k: jax.Array,
    A_ssm_k: jax.Array,
    A_ssm_D: jax.Array,
    B_x: jax.Array,
    B_w1: jax.Array,
    B_w2: jax.Array,
    B_w3: jax.Array,
    B_w4: jax.Array,
    c: jax.Array,
    w_mod: jax.Array,
):
    del B_x

    def tiles(x):
        return x.reshape(S // 8, 8, NC, 128).transpose(0, 2, 1, 3).reshape(S * NC, 128)

    def pairs(x):
        r, n = x.shape
        return x.reshape(r // 16, 2, 8, n // 128, 128).transpose(0, 1, 3, 2, 4)

    args = (
        A_q.reshape(S, D), tiles(A_k), tiles(A_v),
        A_shift_k.T, A_ssm_k, A_ssm_D.reshape(NC, 128),
        pairs(B_w1), pairs(B_w2), pairs(B_w3.T), pairs(B_w4), c, pairs(w_mod),
    )
    scratch = [
        pltpu.VMEM((NA, P * NC + 128, 128), BF16),
        pltpu.VMEM((NA, P * NC + 64, 128), BF16),
        pltpu.VMEM((D, S), BF16),
        pltpu.VMEM((R, 128, 128), U32),
        pltpu.VMEM((R, 64, 256), U32),
        pltpu.VMEM((64, 128), U32),
        pltpu.VMEM((D // 16, 6 * NC, 16, 128), BF16),
        pltpu.VMEM((D // 16, NC, 16, 128), BF16),
        pltpu.VMEM((D // 16, NC, 16, 128), BF16),
        pltpu.VMEM((FF // 16, NC, 16, 128), BF16),
        pltpu.VMEM((FF // 16, NC, 16, 128), BF16),
        pltpu.VMEM((S + 64, D), BF16),
        *[pltpu.VMEM((NA, R, 16, 4, 8, 128), F32) for _ in range(NC)],
        pltpu.VMEM((NC, 2, R, 16, 2, 8, 128), F32),
        pltpu.VMEM((NC, R, 128, 128), U32),
        pltpu.VMEM((32, 128), U32),
        pltpu.VMEM((NC, 8, 8, 128), F32),
        pltpu.VMEM((NC, S + 32, 128), F32),
        pltpu.VMEM((8, 8, D), F32),
        pltpu.VMEM((S + 32, D), F32),
        pltpu.VMEM((NC, S + 32, 128), F32),
        pltpu.VMEM((NC, S + 32, 128), F32),
        pltpu.VMEM((2, TS, D), BF16),
        pltpu.VMEM((TS, 5 * 256), BF16),
        pltpu.VMEM((5, 2, 128, 128), U32),
        pltpu.VMEM((5, 2, 128, 128), U32),
        pltpu.VMEM((5, 6, 64, 256), U32),
        pltpu.VMEM((5, 2, FT // 2, 256), U32),
        pltpu.VMEM((5, 2, 448, 128), U32),
        pltpu.VMEM((8, 9, 72, 128), U32),
        pltpu.VMEM((8, 9, 72, 128), U32),
        pltpu.VMEM((2, 8, 192, 128), U32),
        pltpu.VMEM((NQ, 8, 192, 128), U32),
        pltpu.VMEM((S, D), BF16),
        pltpu.VMEM((4, D), BF16),
        pltpu.VMEM((NC, 128), BF16),
        pltpu.VMEM((1, D), BF16),
        pltpu.SMEM((64,), jnp.int32),
        pltpu.SemaphoreType.DMA((40,)),
        pltpu.SemaphoreType.DMA((1,)),
    ]
    out = pl.pallas_call(
        _kernel,
        out_shape=jax.ShapeDtypeStruct((S, D), BF16),
        in_specs=[pl.BlockSpec(memory_space=pl.ANY)] * len(args),
        out_specs=pl.BlockSpec(memory_space=pl.ANY),
        scratch_shapes=scratch,
        grid=(1,),
        compiler_params=pltpu.CompilerParams(vmem_limit_bytes=108 * 1024 * 1024, disable_semaphore_checks=True,
                                             disable_bounds_checks=True),
        name="adaln_h3_mixer",
    )(*args)
    return out.reshape(1, S, D)
```

```python
import numpy as np
import jax
import jax.numpy as jnp
import jax.experimental.pallas as pl
import jax.experimental.pallas.tpu as pltpu

F32 = jnp.float32
BF16 = jnp.bfloat16
U32 = jnp.uint32

S = 2048
D = 640
FF = 1728
NC = D // 128
R = 4
P = 128 * R
NA = S // P
TS = 256
NT = S // TS
LEAD = 16
EPS = 1e-5
NEST = (1, 4, 2, 3, 5, 6)
NQ = len(NEST)
FT = (FF - 1536) // 2
FM = (FF // 128) * 128
FR = FF - FM
P1_ORDER = "t0 t1 t2 t3 k0 k1 k2 k3 u0 i0 u1 i1 u2 i2 u3 i3"


def _freq(row):
    t, part, s = row >> 4, (row >> 3) & 1, row & 7
    return 32 * (t & 7) + 4 * s + 2 * (t >> 3) + 1, P * part


def _cos(j, scale):
    jf = (j & (4 * P - 1)).astype(F32)
    u = 2.0 * np.pi / (4 * P)
    x = jnp.abs(jf * u - np.pi) - 0.5 * np.pi
    x2 = x * x
    poly = scale / 362880.0 - x2 * (scale / 39916800.0)
    for coef in (-1.0 / 5040.0, 1.0 / 120.0, -1.0 / 6.0, 1.0):
        poly = poly * x2 + coef * scale
    return poly * x


_DUR = {"t": 8, "u": 16, "k": 16, "i": 16, "m": 12, "g": 0, "c": 0, "j": 16}
_POST = {"t": 8.0, "u": 16.0, "k": 24.0, "i": 4.0, "j": 4.0, "m": 18.0}


def _plan_tokens(order, maxutil):
    lag, cap, pre, margin = 8, 60, 4, 3
    start, slots = {}, []
    for n in order:
        start[n] = len(slots)
        slots += [(n, r) for r in range(_DUR[n[0]])]
    nslot = len(slots) + lag
    free = [cap - (_POST[slots[i - lag][0][0]] if i >= lag else 0.0) for i in range(-pre, nslot)]
    units = []
    for n in order:
        kind, a, c = n
        if kind == "u":
            units += [(n + (g,), 94.0, start[n], -pre) for g in range(8)]
        elif kind == "g":
            units += [(n + (g,), 150.0, start[n], -pre) for g in range(8)]
        elif kind in "ic":
            src_ = [start[m] for m in (("u", a, c), ("k", a, c)) if m in start]
            for t in range(16):
                rel = max(max(src_) + 16, max(src_) + t + lag + 3) if src_ else -pre
                units.append((n + (t,), 32.0 * a + 48.0, nslot if kind == 'c' else start[n], rel))

    def simulate(util):
        left = [u[1] for u in units]
        done = [None] * len(units)
        for i in range(-pre, nslot):
            budget = util * free[i + pre]
            for j, u in enumerate(units):
                if budget <= 0.0:
                    break
                if done[j] is None and u[3] <= i:
                    use = min(budget, left[j])
                    left[j] -= use
                    budget -= use
                    if left[j] <= 1e-9:
                        done[j] = i + 1
        ok = all(u[2] < 8 or (d is not None and d <= max(u[2] - (1 if u[0][0] in 'cg' else margin), u[3] + 1))
                 for d, u in zip(done, units))
        return done, ok

    lo_, hi_ = 0.05, maxutil
    for _ in range(12):
        mid = 0.5 * (lo_ + hi_)
        if simulate(mid)[1]:
            hi_ = mid
        else:
            lo_ = mid
    done, _ = simulate(hi_)
    plan = {}
    for u, d in zip(units, done):
        if u[0][0] == "c":
            plan[u[0]] = slots[max((nslot - 1 if d is None else min(d, nslot - 1)) - lag, 0)]
        elif d is not None and 0 <= d < u[2]:
            plan.setdefault(slots[d], []).append(u[0])
    return plan


def _pack(x):
    return pltpu.bitcast(x.astype(BF16), U32)


def _unpack(w):
    return pltpu.bitcast(w, BF16)


def _dot(a, b):
    return jnp.dot(a.astype(BF16), b, preferred_element_type=F32)


def _dot_nt(a, b):
    return jax.lax.dot_general(a.astype(BF16), b, (((1,), (1,)), ((), ())), preferred_element_type=F32)


def _dot_fine(x, w, chunk, nt=False):
    if not chunk:
        return _dot_nt(x, w) if nt else _dot(x, w)
    n = w.shape[0] if nt else w.shape[1]
    head, last = (w[:n - 128], w[n - 128:]) if nt else (w[:, :n - 128], w[:, n - 128:])
    f = _dot_nt if nt else _dot
    parts = [f(x, head)] if n > 128 else []
    parts.append(jnp.concatenate([f(x[r:r + chunk], last) for r in range(0, x.shape[0], chunk)], axis=0))
    return jnp.concatenate(parts, axis=1)


def _rows2(x):
    n, c = x.shape
    x = x.reshape(n // 32, 2, 16, c)
    return x[:, 0].reshape(n // 2, c), x[:, 1].reshape(n // 2, c)


def _unrows2(top, bot):
    n, c = top.shape
    return jnp.stack([top.reshape(n // 16, 16, c), bot.reshape(n // 16, 16, c)], axis=1).reshape(2 * n, c)


def _sums_a(a11, a12, a21, a22):
    return [a11 + a22, a21 + a22, a11 + a12, a21 - a11, a12 - a22]


def _sums_b(b11, b12, b21, b22):
    return [b11 + b22, b12 - b22, b21 - b11, b11 + b12, b21 + b22]


_STRASSEN = ((0, 0), (1, 5), (5, 1), (6, 2), (2, 6), (3, 3), (4, 4))


_SUMS_A = ((0, 3, 1), (2, 3, 1), (0, 1, 1), (2, 0, -1), (1, 3, -1))
_SUMS_B = ((0, 3, 1), (1, 3, -1), (2, 0, -1), (0, 1, 1), (2, 3, 1))


def _combine(m1, m2, m3, m4, m5, m6, m7):
    return (m1 + m4) + (m7 - m5), m3 + m5, m2 + m4, (m1 - m2) + (m3 + m6)


def _lo(w):
    return pltpu.bitcast(w << 16, F32)


def _hi(w):
    return pltpu.bitcast(w & jnp.uint32(0xFFFF0000), F32)


def _ln(x, eps=EPS):
    m = jnp.sum(x, axis=-1, keepdims=True) * (1.0 / D)
    xc = x - m
    v = jnp.sum(xc * xc, axis=-1, keepdims=True) * (1.0 / D)
    return xc * jnp.exp(-0.5 * jnp.log(v + eps))


def _gelu2(x):
    c0 = 0.7978845608028654
    c1 = c0 * 0.044715
    return x + x * jnp.tanh(x * (c0 + c1 * (x * x)))


def _bfly(tr, ti, sign):
    s02r, s02i = tr[0] + tr[2], ti[0] + ti[2]
    d02r, d02i = tr[0] - tr[2], ti[0] - ti[2]
    s13r, s13i = tr[1] + tr[3], ti[1] + ti[3]
    d13r, d13i = tr[1] - tr[3], ti[1] - ti[3]
    x0r, x0i = s02r + s13r, s02i + s13i
    x2r, x2i = s02r - s13r, s02i - s13i
    ar, ai = d02r + d13i, d02i - d13r
    br, bi = d02r - d13i, d02i + d13r
    if sign < 0:
        return [x0r, ar, x2r, br], [x0i, ai, x2i, bi]
    return [x0r, br, x2r, ar], [x0i, bi, x2i, ai]


def _kernel(q_hbm, k_hbm, v_hbm, shift_hbm, ssmk_hbm, ssmd_hbm, w1_hbm, w2_hbm, w3t_hbm, w4_hbm,
            c_hbm, wmod_hbm,
            out_hbm,
            kbuf, vbuf, skbuf, fwdbuf, invbuf, permbuf,
            wmodbuf, w1buf, w2buf, w3buf, w4buf, qbuf,
            xs0, xs1, xs2, xs3, xs4, kraw, wbuf, zbuf, coefbuf, ybuf, modbuf, x2buf, hbuf, hhbuf, xnbuf, xsbuf,
             w1s, w2s, w3s, w3ts, w4s, hba, hbb, w4n, w4q, obuf, shiftbuf, dbuf, cbuf,
            zsm, sem_in, sem_out):
    cps = {}
    n_sem = [0]

    def start(name, src, dst):
        cp = pltpu.make_async_copy(src, dst, sem_in.at[n_sem[0]])
        n_sem[0] += 1
        cp.start()
        cps[name] = cp

    class Both:
        def __init__(self, a, b):
            self.cps = (a, b)

        def wait(self):
            for cp in self.cps:
                cp.wait()

    def start_w(name, src, dst, c0=0, n=NC):
        for e in range(2):
            start(name + str(e), src.at[:, e, pl.ds(c0, n)], dst.at[:, pl.ds(c0, n), pl.ds(8 * e, 8), :])
        cps[name] = Both(cps[name + "0"], cps[name + "1"])

    CH = P * NC
    HALO = 8 * NC

    def start_s(a):
        cols = pl.ds(a * P, P)
        start("s%d" % a, ssmk_hbm.at[:, cols], skbuf.at[:, cols])

    def start_kv(a):
        if a == 0:
            kbuf[0, pl.ds(0, HALO + 8), :] = jnp.zeros((HALO + 8, 128), BF16)
            start("k0", k_hbm.at[pl.ds(0, CH), :], kbuf.at[0, pl.ds(HALO, CH), :])
        else:
            start("k%d" % a, k_hbm.at[pl.ds(a * CH - HALO, CH + HALO), :], kbuf.at[a, pl.ds(0, CH + HALO), :])
        start("v%d" % a, v_hbm.at[pl.ds(a * CH, CH), :], vbuf.at[a, pl.ds(0, CH), :])

    for n in "s0 x0 s1 k0 k1 s2 k2 s3 k3".split():
        if n[0] == "s":
            start_s(int(n[1]))
        elif n[0] == "k":
            start_kv(int(n[1]))
        else:
            start("d", ssmd_hbm, dbuf)
            start("shift", shift_hbm, shiftbuf)
            start("c", c_hbm, cbuf)
    QA = TS + LEAD
    XA = 128
    QB = 2 * TS + LEAD
    W1A = 2

    def start_q(name, r0, n):
        start(name, q_hbm.at[pl.ds(r0, n), :], qbuf.at[pl.ds(r0, n), :])

    start_q("qa", 0, QA)
    start_w("wmoda", wmod_hbm, wmodbuf, 0, 3 * NC)
    start_w("wmodb", wmod_hbm, wmodbuf, 3 * NC, 2 * NC)
    start_q("qx", QA, XA)
    start_w("w1a", w1_hbm, w1buf, 0, W1A)
    start_w("w1b", w1_hbm, w1buf, W1A, NC - W1A)
    start_q("qb", QA + XA, QB - QA - XA)
    start_w("w2", w2_hbm, w2buf)
    start_w("w3", w3t_hbm, w3buf)
    start_w("w4", w4_hbm, w4buf)
    start_w("wmodg", wmod_hbm, wmodbuf, 5 * NC, NC)
    start_q("q1", QB, S - QB)

    kw = kbuf.bitcast(U32)
    vw = vbuf.bitcast(U32)
    zbuf[...] = jnp.zeros(zbuf.shape, U32)
    for j in range(64):
        zsm[j] = 0
    for c in range(NC):
        ybuf[c, pl.ds(S, LEAD), :] = jnp.zeros((LEAD, 128), F32)
        hhbuf[c, pl.ds(0, 8), :] = jnp.zeros((8, 128), F32)
    qbuf[pl.ds(S, LEAD), :] = jnp.zeros((LEAD, D), BF16)

    def tables(p, carry):
        i0 = jax.lax.broadcasted_iota(jnp.int32, (128, 128), 0)
        n = R * jax.lax.broadcasted_iota(jnp.int32, (128, 128), 1) + p
        f2, off = _freq(2 * i0)
        j = f2 * n + off
        fwdbuf[p] = pltpu.pack_elementwise([_cos(j, 1.0), _cos(j + 4 * n, 1.0)], packed_dtype=BF16)
        return carry

    jax.lax.fori_loop(0, R, tables, 0)

    def unit_g(kt, r):
        col = jax.lax.broadcasted_iota(jnp.int32, (8, 128), 1) + 128 * kt
        f2, off = _freq((col & ~15) + 8 * (col & 1) + ((col >> 1) & 7))
        m = 2 * jax.lax.broadcasted_iota(jnp.int32, (8, 128), 0) + 16 * r
        j0 = f2 * (R * m) + off
        out = []
        for p in range(R):
            j = j0 + p * f2
            out.append(pltpu.pack_elementwise([_cos(j, 1.0 / P), _cos(j + R * f2, 1.0 / P)], packed_dtype=BF16))
            invbuf[p, pl.ds(8 * r, 8), pl.ds(128 * kt, 128)] = out[-1]
        return out

    i0 = jax.lax.broadcasted_iota(jnp.int32, (128, 128), 0)
    i1 = jax.lax.broadcasted_iota(jnp.int32, (128, 128), 1)
    permbuf[...] = _pack(jnp.where(i0 == (128 // R) * (i1 & (R - 1)) + (i1 >> 2), 1.0, 0.0).astype(F32))

    def fill_coef():
        cv = cbuf[...].astype(F32)
        modbuf[6] = jnp.broadcast_to(cv * jax.nn.sigmoid(cv), (8, D))
        coef = shiftbuf[...].astype(F32)
        dval = dbuf[...].astype(F32)
        for c in range(NC):
            for j in range(4):
                coefbuf[c, j] = jnp.broadcast_to(coef[j:j + 1, c * 128:(c + 1) * 128], (8, 128))
            coefbuf[c, 4] = jnp.broadcast_to(dval[c:c + 1, :], (8, 128))

    xs = (xs0, xs1, xs2, xs3, xs4)
    wsbufs = dict(w1=w1s, w2=w2s, w3=w3s, w4=w4s, w3t=w3ts)
    def split_ri(t):
        t = t.reshape(16, 2, 8, 128)
        return t[:, 0], t[:, 1]

    def get_never():
        return zbuf[pl.ds(0, 8), :] != 0

    def pack2(x, y):
        return pltpu.pack_elementwise([x, y], packed_dtype=BF16)

    def words(ref, a, c, r):
        return ref[a, pl.ds((r // 4) * 4 * NC + 4 * c + r % 4, 8, stride=4 * NC), :]

    def unit_u(a, c, g):
        c0, c1, c2, c3 = (coefbuf[c, pl.ds(j, 1)] for j in range(4))
        kk = jnp.stack([words(kw, a, c, 4 + 32 * g + d) for d in range(-2, 4)])
        vv = jnp.stack([words(vw, a, c, 32 * g + d) for d in range(4)])
        lo, hi = _lo(kk), _hi(kk)
        k0, k1, k2 = lo[2:], hi[1:5], lo[1:5]
        even = (((k0 * c0 + k1 * c1) + (k2 * c2 + hi[:4] * c3)) * _lo(vv)).reshape(32, 128)
        odd = (((hi[2:] * c0 + k0 * c1) + (k1 * c2 + k2 * c3)) * _hi(vv)).reshape(32, 128)
        e, o = pack2(even[:16], even[16:]), pack2(odd[:16], odd[16:])
        return [e[:8], o[:8], e[8:], o[8:]]

    def unit_i(a, c, t, z):
        x_c = xs[c].at[pl.ds(z, NA)]
        yr = yi = None
        for j in range(a + 1):
            ur, ui = x_c[j, :, t, 0], x_c[j, :, t, 1]
            kr, ki = x_c[a - j, :, t, 2], x_c[a - j, :, t, 3]
            pr = ur * kr - ui * ki
            pi = ur * ki + ui * kr
            yr = pr if yr is None else yr + pr
            yi = pi if yi is None else yi + pi
        halves = lambda x: (x[:x.shape[0] // 2], x[x.shape[0] // 2:])
        (ra, rb), (ia, ib) = halves(yr.reshape(32, 128)), halves(yi.reshape(32, 128))
        (sr0, sr1), (si0, si1), (dr0, dr1), (di0, di1) = (halves(x) for x in (ra + rb, ia + ib, ra - rb, ia - ib))
        return [pack2(sr0 + sr1, si0 + si1), pack2(dr0 - di1, di0 + dr1),
                pack2(sr0 - sr1, si0 - si1), pack2(dr0 + di1, di0 - dr1)]

    def segment(spec, z, maxutil=1.0, mod_fn=None):
        order = [(n[0], int(n[1]), int(n[2])) for n in spec.split()]
        plan = _plan_tokens(order, maxutil) if maxutil > 0 else {}
        never = get_never()
        units, res = {}, {}

        def unit(key):
            if key not in units:
                kind, a, c, j = key
                if kind == "u":
                    units[key] = unit_u(a, c, j)
                elif kind == "g":
                    units[key] = unit_g(a, j)
                else:
                    fresh = ("u", a, c) in order or ("k", a, c) in order
                    units[key] = unit_i(a, c, j, z if fresh else 0)
            return units[key]

        def lhs(name, p, full, r0=0):
            out, last = [], 0
            for r in range(full.shape[0] // 8):
                keys = plan.get((name, r0 + r), ())
                if keys:
                    if 8 * r > last:
                        out.append(full[last:8 * r])
                    v = full[8 * r:8 * r + 8]
                    for key in keys:
                        v = jax.lax.select(never, unit(key)[p], v)
                    out.append(v)
                    last = 8 * r + 8
            if last < full.shape[0]:
                out.append(full[last:] if last else full)
            return out[0] if len(out) == 1 else jnp.concatenate(out, axis=0)

        def dft(name, rhs):
            tr, ti = [], []
            for p in range(R):
                f = lhs(name, p, fwdbuf[p])
                r_, i_ = split_ri(_dot(_unpack(f), rhs[p]))
                if p == 0:
                    res.update({(name, r): (lambda r=r, v=r_: v[r]) for r in range(16)})
                tr.append(r_)
                ti.append(i_)
            return _bfly(tr, ti, -1)

        st = {}
        for name in order:
            kind, a, c = name
            x_c = xs[c]
            if kind == "g":
                for r in range(8):
                    unit(name + (r,))
            elif kind == "c":
                for t in range(16):
                    after = pltpu.bitcast(res[plan[name + (t,)]](), U32)
                    for p in range(R):
                        wbuf[c, p, pl.ds(8 * t, 8), :] = jax.lax.select(never, after, unit(name + (t,))[p])
            elif kind == "m":
                toks = {}
                for r in range(_DUR["m"]):
                    for n_, key in enumerate(plan.get((name, r), ())):
                        toks.setdefault(2 * r + n_ % 2, []).extend(unit(key))
                mod_fn(a, toks)
            elif kind == "t":
                trs = []
                for b in range(R):
                    pm = lhs(name, b, permbuf[...])
                    trs.append(_dot_nt(_unpack(pm), skbuf[pl.ds(c * 128, 128), pl.ds(a * P + b * 128, 128)]))
                res.update({(name, r): (lambda r=r, v=trs[0]: v[16 * r:16 * r + 8]) for r in range(8)})
                g_ = 128 // R
                st[a, c] = [jnp.concatenate([trs[b][p * g_:(p + 1) * g_] for b in range(R)], axis=0).astype(BF16)
                            for p in range(R)]
            elif kind == "u":
                rhs = [_unpack(jnp.concatenate([unit(name + (g,))[p] for g in range(8)], axis=0)) for p in range(R)]
                xr, xi = dft(name, rhs)
                for q in range(R):
                    x_c[a, q, :, 0] = xr[q]
                    x_c[a, q, :, 1] = xi[q]
            elif kind == "k":
                xr, xi = dft(name, st[a, c])
                for q in range(R):
                    if a == 0:
                        x_c[a, q, :, 2] = xr[q] + coefbuf[c, 4]
                        x_c[a, q, :, 3] = xi[q]
                    else:
                        pr, pi = kraw[c, (a - 1) % 2, q, :, 0], kraw[c, (a - 1) % 2, q, :, 1]
                        x_c[a, q, pl.ds(0, 8), 2] = xr[q][:8] - pi[:8]
                        x_c[a, q, pl.ds(0, 8), 3] = xi[q][:8] + pr[:8]
                        x_c[a, q, pl.ds(8, 8), 2] = xr[q][8:] + pi[8:]
                        x_c[a, q, pl.ds(8, 8), 3] = xi[q][8:] - pr[8:]
                    if a + 1 < NA:
                        kraw[c, a % 2, q, :, 0] = xr[q]
                        kraw[c, a % 2, q, :, 1] = xi[q]
            else:
                for p in range(R):
                    cols = [lhs(name, 2 * (p % 2) + kt,
                                invbuf[p, :, pl.ds(128 * kt, 128)], 8 * (p // 2))
                            for kt in range(2)]
                    g = _unpack(jnp.concatenate(cols, axis=1))
                    if kind == "j":
                        wp = _unpack(wbuf[c, p])
                    else:
                        wp = _unpack(jnp.concatenate([unit(name + (t,))[p] for t in range(16)], axis=0))
                    yp = _dot(g, wp)
                    if p % 2 == 0:
                        res.update({(name, 4 * p + r): (lambda r=r, v=yp: v[16 * r:16 * r + 8]) for r in range(8)})
                    ybuf[c, pl.ds(a * P + p, 128, stride=R), :] = yp

    one = jnp.minimum(pl.program_id(0) + 1, 1)

    def once(fn):
        def body(z, carry):
            fn(z)
            return carry
        jax.lax.fori_loop(0, one, body, 0)

    default = "t00 t01 t02 k00 t03 k01 t04 k02 k03 k04 g00|t10 t11 t12 k10 k11 k12 g10|t13 t14 k13 u00 k14 u01 u02 u03 i00 u04 i01 c02 c03|j02 j03 u10 i04 u11 u12 u13 i10 u14 i11 c12|t20 t21 j12 t22 t23 t24 k20 u20 k21 u21 k22 i13 k23 u22 k24 i14 u23 i20 u24 i21 c22|t30 t31 j22 t32 t33 t34 k30 u30 k31 u31 k32 i23 k33 u32 k34 i24 u33 i30 u34 i31 c32|m00 j32 m10 m20 i33 i34"
    specs = default.split("|")
    G5B = specs[-1]
    segs = list(zip("s0 d shift c|s1|k0 v0|k1 v1|s2 k2 v2|s3 k3 v3".split("|"), specs[:-1]))
    MU = 1.5
    for i, (waits, spec) in enumerate(segs):
        with jax.named_scope("g%d" % i):
            for n in waits.split():
                cps[n].wait()
            if i == 0:
                fill_coef()
            once(lambda z: segment(spec, z, MU))

    def mod_cols(lo, n, toks=None):
        m = _dot(modbuf[6], weights(wmodbuf, lo * NC, (lo + n) * NC, toks=toks))
        return [m[:, j * D:(j + 1) * D] for j in range(n)]

    def mul_mod(x, j, cols=None):
        m = modbuf[j] if cols is None else modbuf[j, :, cols]
        return (x.reshape(-1, 8, x.shape[-1]) * m[None]).reshape(x.shape)

    def add_mod(x, j):
        return (x.reshape(-1, 8, x.shape[-1]) + modbuf[j][None]).reshape(x.shape)

    def slabs(ref, r0, n):
        return jnp.concatenate([ref[c, pl.ds(r0, n), :] for c in range(NC)], axis=1)

    def put(ref, rows, x):
        for c in range(NC):
            ref[c, rows, :] = x[:, c * 128:(c + 1) * 128]

    def parity(ref, r0, n, e):
        return jnp.concatenate([ref[c, pl.ds(r0 + e, n // 2, stride=2), :] for c in range(NC)], axis=1)

    def window(base, n, half):
        rows = pl.ds(base, n)
        return dict(xs=xsbuf,
                    q=qbuf.at[rows, :], y=ybuf.at[:, rows, :], x2=x2buf.at[rows, :], h=hbuf.at[:, rows, :],
                    hh=hhbuf.at[:, pl.ds(base, n + 8), :], xn=xnbuf,
                    o=obuf.at[pl.ds(base, n - LEAD), :])

    def weights(ref, c0=0, c1=NC, r0=0, r1=None, toks=None, raw=False, z=None):
        r1 = 16 * ref.shape[0] if r1 is None else r1
        view = ref.bitcast(U32)
        if z is not None:
            view = view.at[pl.ds(z, ref.shape[0])]
        never = get_never() if toks else None
        rt = -(-(r1 - r0) // 128)
        cols = []
        for j in range(c0, c1):
            wu = view[pl.ds(r0 // 16, (r1 - r0) // 16), j].reshape((r1 - r0) // 2, 128)
            if toks:
                parts, last = [], 0
                for i in range(rt):
                    for n_, t in enumerate(toks.get((j - c0) * rt + i, ())):
                        r = 64 * i + 8 * n_
                        if r > last:
                            parts.append(wu[last:r])
                        parts.append(jax.lax.select(never, t, wu[r:r + 8]))
                        last = r + 8
                parts.append(wu[last:])
                wu = jnp.concatenate(parts, axis=0)
            cols.append(wu)
        wu = jnp.concatenate(cols, axis=1)
        return wu if raw else _unpack(wu)

    def wblocks(name, j, z=None):
        if name == "w3":
            blk = lambda kh, nh: weights(w3buf, 2 * kh, 2 * kh + 2, 128 * (j + 6 * nh), 128 * (j + 6 * nh + 1), raw=True, z=z)
        elif name == "w4":
            def blk(kh, nh):
                c = j + 2 * nh
                parts = [weights(w4buf, c, c + 1, 768 * kh, 768 * (kh + 1), raw=True, z=z),
                         weights(w4buf, c, c + 1, 1536 + FT * kh, 1536 + FT * (kh + 1), raw=True, z=z),
                         jnp.zeros(((128 - FT) // 2, 128), U32)]
                return jnp.concatenate(parts, axis=0)
        elif name == "w3t":
            blk = lambda kh, nh: weights(w3buf, 2 * kh, 2 * kh + 2, 1536 + FT * nh, 1536 + FT * (nh + 1), raw=True, z=z)
        else:
            ref = w1buf if name == "w1" else w2buf
            blk = lambda kh, nh: weights(ref, j + 2 * nh, j + 2 * nh + 1, 256 * kh, 256 * (kh + 1), raw=True, z=z)
        return blk

    def wsum(name, j, k):
        blk = wblocks(name, j, zsm[k])
        p, q, sign = ((0, 3, 1), (1, 3, -1), (2, 0, -1), (0, 1, 1), (2, 3, 1))[k]
        x, y = blk(p // 2, p % 2), blk(q // 2, q % 2)
        if sign > 0:
            return pack2(_lo(x) + _lo(y), _hi(x) + _hi(y))
        return pack2(_lo(x) - _lo(y), _hi(x) - _hi(y))

    pending = []

    def attach(wv):
        if not pending:
            return wv
        never = get_never()
        rows = [wv[8 * i:8 * i + 8, :128] for i in range(8)]
        for i, t in enumerate(pending):
            rows[i % 8] = jax.lax.select(never, pltpu.bitcast(t, U32), rows[i % 8])
        pending.clear()
        first = jnp.concatenate(rows + ([wv[64:, :128]] if wv.shape[0] > 64 else []), axis=0)
        return first if wv.shape[1] == 128 else jnp.concatenate([first, wv[:, 128:]], axis=1)

    def sprods(name, j, lhs, k0=0, k1=7, prep=False):
        blk, buf = wblocks(name, j), wsbufs[name]
        if prep == "fresh":
            buf, prep = buf.at[pl.ds(zsm[6], 5)], False
        out = []
        for ia, ib in _STRASSEN[k0:k1]:
            wv = blk(ib - 5, ib - 5) if ib >= 5 else (wsum(name, j, ib) if prep else buf[ib, j])
            if name == "w3t":
                out.append(_dot_nt(_unpack(wv), lhs(ia)))
            else:
                out.append((_dot_nt if name == "w3" else _dot)(lhs(ia), _unpack(attach(wv))))
            if prep and ib < 5:
                buf[ib, j] = wv
        return out

    def spair(name, j, lhs, prep=False):
        return _combine(*sprods(name, j, lhs, prep=prep))

    def dd_rest(name, t, b):
        ref = w1buf if name == "w1" else w2buf
        m = t.shape[0]
        xb = jnp.concatenate([t, b], axis=0)
        last = _dot(xb, weights(ref, 4, 5))
        rem = _dot(xb[:, 512:], weights(ref, 0, 4, r0=512))
        return t, b, rem[:m], rem[m:], last[:m], last[m:]

    def dd_main(name, parts, prep=False):
        t, b, rt, rb, lt, lb = (jnp.concatenate(v, axis=0) for v in zip(*parts))
        ops = _sums_a(t[:, :256], t[:, 256:512], b[:, :256], b[:, 256:512]) + [t[:, :256], b[:, 256:512]]
        top, bot = [None] * 4, [None] * 4
        for j in range(2):
            top[j], top[j + 2], bot[j], bot[j + 2] = spair(name, j, lambda i: ops[i], prep)
        return (jnp.concatenate([jnp.concatenate(top, axis=1) + rt, lt], axis=1),
                jnp.concatenate([jnp.concatenate(bot, axis=1) + rb, lb], axis=1))

    def stage_a0(w, r0, n):
        rows = pl.ds(r0, n)
        x = w["q"][rows, :].astype(F32)
        x2 = x + add_mod(mul_mod(_ln(x), 1), 0) * slabs(w["y"], r0, n)
        w["x2"][rows, :] = x2
        return _ln(x2)

    def stage_a1(w, r0, n, n2=None, f32=False):
        if n2 is None:
            n2 = stage_a0(w, r0, n)
        h = add_mod(mul_mod(n2, 4), 3)
        put(w["h"], pl.ds(r0, n), h)
        n3 = _ln(h, 4 * EPS)
        return n3 if f32 else n3.astype(BF16)

    def stage_a2(w, n3, r0, n, last_valid=None, fine=0, c0=0, c1=NC, prep=False):
        hh = _gelu2(_unrows2(*dd_main("w1", n3, prep)) if isinstance(n3, list) else _dot_fine(n3, weights(w1buf, c0, c1), fine))
        for c in range(c0, c1):
            blk = hh[:, (c - c0) * 128:(c - c0 + 1) * 128]
            w["hh"][c, pl.ds(r0 + 8, n - LEAD), :] = blk[:n - LEAD]
            tail = blk[n - LEAD:]
            if last_valid is not None:
                tail = jnp.where(last_valid, tail, 0.0)
            w["hh"][c, pl.ds(r0 + 8 + n - LEAD, LEAD), :] = tail

    def stage_b1a(w, r0, n, fine=0, fast=False, prep=False):
        m = n // 2
        lane = jax.lax.broadcasted_iota(jnp.int32, (m, 128), 1)
        g = []
        for e in range(2):
            sh = lambda c, d: w["hh"][c, pl.ds(r0 + 8 + e + d, m, stride=2), :]
            g.append(jnp.concatenate([sh(0, -1),
                                      jnp.where(lane < 32, sh(1, -1), sh(1, 1)),
                                      jnp.where(lane < 64, sh(2, 1), sh(2, -2)),
                                      jnp.where(lane < 96, sh(3, -2), sh(3, 2)),
                                      sh(4, 2)], axis=1))
        if fast:
            hs = dd_main("w2", [dd_rest("w2", *g)], prep)
        else:
            hs = _dot_fine(jnp.concatenate(g, axis=0), weights(w2buf), fine)
            hs = hs[:m], hs[m:]
        x1 = [parity(w["h"], r0, n, e) + hs[e] for e in range(2)]
        for e in range(2):
            put(w["h"], pl.ds(r0 + e, m, stride=2), x1[e])
        return x1

    def stage_b1b(w, x1, r0, n):
        xn = jnp.stack([_ln(x, 4 * EPS).reshape(n // 16, 8, D) for x in x1], axis=1).reshape(n, D)
        t, b = _rows2(xn)
        w["xn"][0, pl.ds(r0 // 2, n // 2), :] = t.astype(BF16)
        w["xn"][1, pl.ds(r0 // 2, n // 2), :] = b.astype(BF16)
        sa = _sums_a(t[:, :256], t[:, 256:512], b[:, :256], b[:, 256:512])
        w["xs"][pl.ds(r0 // 2, n // 2), :] = jnp.concatenate(sa, axis=1).astype(BF16)

    def stage_b1(w, r0, n, fast=False, prep=False):
        stage_b1b(w, stage_b1a(w, r0, n, fast=fast, prep=prep), r0, n)

    def out_copy(r0, n):
        rows = pl.ds(r0, n)
        return pltpu.make_async_copy(obuf.at[rows, :], out_hbm.at[rows, :], sem_out.at[0])


    def opaque(ref, i):
        return ref.at[:, :, pl.ds(pl.multiple_of(zsm[i] * 32, 32), ref.shape[2]), :]

    def packrows(v):
        v = v.reshape(v.shape[0] // 16, 2, 8, 128)
        return pack2(v[:, 0], v[:, 1]).reshape(-1, 128)

    def emit(h3, j, left, right):
        m = left.shape[0] // 2
        g = [left[:m], right[:m], left[m:], right[m:]]
        for k, v in enumerate(_sums_a(*g) + g):
            h3[j, k, pl.ds(0, m // 2), :] = packrows(v)

    def load_xn(w, r0, n):
        return w["xn"][:, pl.ds(r0 // 2, n // 2), :].reshape(n, D)

    def w3_operands(w, r0, n):
        xn = load_xn(w, r0, n)
        xsum = w["xs"][pl.ds(r0 // 2, n // 2), :]
        m = n // 2
        return xn, [xsum[:, 256 * k:256 * (k + 1)] for k in range(5)] + [xn[:m, :256], xn[m:, 256:512]]

    def stage_b2h(w, h3, r0, n, prep=False):
        xn, ops = w3_operands(w, r0, n)
        m = n // 2
        rem = _dot_nt(weights(w3buf, 4, 5, r0=1536), xn[:, 512:])
        c11, c12, c21, c22 = spair("w3t", 0, lambda i: ops[i], prep)
        pad = jnp.zeros((128 - FT, m), F32)
        g11, g12, g21, g22 = (jnp.concatenate([_gelu2(c + r), pad], axis=0).T for c, r in (
            (c11, rem[:FT, :m]), (c12, rem[FT:, :m]), (c21, rem[:FT, m:]), (c22, rem[FT:, m:])))
        emit(h3, 6, jnp.concatenate([g11, g21], axis=0), jnp.concatenate([g12, g22], axis=0))

    def stage_b2a(w, h3, r0, n, lo=0, hi=6, prep=False):
        xn, ops = w3_operands(w, r0, n)
        for j in range(lo, hi):
            r1, r2 = (_dot_nt(xn[:, 512:], weights(w3buf, 4, 5, 128 * t, 128 * (t + 1))) for t in (j, j + 6))
            c11, c12, c21, c22 = spair("w3", j, lambda i: ops[i], prep)
            emit(h3, j, _gelu2(jnp.concatenate([c11, c21], axis=0) + r1), _gelu2(jnp.concatenate([c12, c22], axis=0) + r2))

    def finish(w, h2, r0, n, c):
        rows, cols = pl.ds(r0, n), pl.ds(c * 128, 128)
        w["o"][rows, cols] = (w["x2"][rows, cols] + mul_mod(w["h"][c, rows, :] + h2, 5, cols)).astype(BF16)

    def b2_done(w, done, r0, n, j):
        if len(done[j]) == 7:
            c11, c12, c21, c22 = _combine(*[done[j][k] for k in range(7)])
            finish(w, _unrows2(c11, c21), r0, n, j)
            finish(w, _unrows2(c12, c22), r0, n, j + 2)

    def stage_b2b(w, h3, r0, n, j, k0=0, k1=7, done=None, prep=False, fine=0, sub=0, marks=()):
        hv = opaque(h3, j)
        blk = lambda k: jnp.concatenate([hv[p, k, pl.ds(sub // 4, n // 4), :] for p in range(7)], axis=1)
        r0 += sub
        if j < 2:
            for k in range(k0, k1):
                if k not in NEST:
                    done[j][k] = sprods("w4", j, lambda i: _unpack(blk(8 if i == 6 else i)), k, k + 1, prep)[0]
                    b2_done(w, done, r0, n, j)
            return
        wb = wblocks("w4", 4)
        lhs = jnp.concatenate([jnp.concatenate([blk(5), blk(6)], axis=1),
                               jnp.concatenate([blk(7), blk(8)], axis=1)], axis=0)
        if marks:
            lo_, hi_ = 0, 52
            never, at = get_never(), {}
            for i, mk in enumerate(marks):
                s_ = lo_ + (hi_ - lo_) * i // len(marks)
                at[4 * (s_ // 16), s_ % 16] = mk
            cols = []
            for kt in range(14):
                col = lhs[:, 128 * kt:128 * (kt + 1)]
                if any(k_[0] == kt for k_ in at):
                    col = jnp.concatenate([jax.lax.select(never, at[kt, r], col[8 * r:8 * r + 8]) if (kt, r) in at
                                           else col[8 * r:8 * r + 8] for r in range(16)], axis=0)
                cols.append(col)
            lhs = jnp.concatenate(cols, axis=1)
        h2 = _dot_fine(_unpack(lhs), _unpack(jnp.concatenate([wb(0, 0), wb(1, 0)], axis=0)), fine)
        finish(w, _unrows2(h2[:n // 2], h2[n // 2:]), r0, n, 4)


    def psum(x, y, sign):
        if sign > 0:
            return pack2(_lo(x) + _lo(y), _hi(x) + _hi(y))
        return pack2(_lo(x) - _lo(y), _hi(x) - _hi(y))

    def prep_w4(nchunk):
        rows = 384 // nchunk
        marks = []
        for ch in [nchunk] + list(range(nchunk)):
            tail = ch == nchunk
            raw = {}
            for kh in range(2):
                for e in range(1 if tail else 2):
                    r0 = 1536 + FT * kh if tail else 768 * kh + 384 * e + rows * ch
                    x = weights(w4buf, 0, 4, r0, r0 + (FT if tail else rows), raw=True)
                    raw[kh, e] = jnp.stack([_lo(x), _hi(x)])
            blk = lambda i, e: raw[i // 2, e][:, :, 256 * (i % 2):256 * (i % 2 + 1)]
            for k, (ia, ib) in enumerate(_STRASSEN):
                if k not in NEST or ib >= 5:
                    continue
                half = {}
                for e in range(1 if tail else 2):
                    if ib >= 5:
                        half[e] = blk(3 * (ib - 5), e)
                    else:
                        p_, q_, sg = _SUMS_B[ib]
                        half[e] = blk(p_, e) + blk(q_, e) if sg > 0 else blk(p_, e) - blk(q_, e)
                quad = lambda i: half[i // 2][:, :, 128 * (i % 2):128 * (i % 2 + 1)]
                if tail or k not in NEST:
                    if ib < 5:
                        for e in half:
                            for j in range(2):
                                r = 384 if tail else 192 * e + rows // 2 * ch
                                v = quad(2 * e + j)
                                w4q[NEST.index(k), 7, pl.ds(64 * j, v.shape[1]), :] = pack2(v[0], v[1])
                                if tail:
                                    w4q[NEST.index(k), 7, pl.ds(64 * j + FT // 2, 64 - FT // 2), :] = jnp.zeros((64 - FT // 2, 128), U32)
                    continue
                ops = _sums_b(*[quad(i) for i in range(4)]) + ([quad(0), quad(3)] if ib < 5 else [])
                for jb, v in enumerate(ops):
                    w4q[NEST.index(k), jb, pl.ds(rows // 2 * ch, rows // 2), :] = pack2(v[0], v[1])
                first = NEST.index(k)
            if not tail:
                marks.append(w4q.at[pl.ds(zsm[32 + ch], NQ)][first, 0, pl.ds(0, 8), :])
        return marks

    def stage_b2n(*args, **kw):
        for _ in steps_b2n(*args, **kw):
            pass

    def steps_b2n(w, h3, r0, n, k, done, prep=False):
        ia, ib = _STRASSEN[k]
        ka, q, slot = (8 if ia == 6 else ia), n // 8, NEST.index(k)

        def lblk(i, z):
            hv = opaque(h3, z)
            return jnp.concatenate([hv[g + 3 * (i % 2), ka, pl.ds((i // 2) * q, q), :] for g in range(3)], axis=1)

        def wterms(j, lo, hi, z):
            blk = wblocks("w4", j, z)
            if ib >= 5:
                return [(1, blk(ib - 5, ib - 5)[lo:hi])]
            p_, q_, sg = _SUMS_B[ib]
            return [(1, blk(p_ // 2, p_ % 2)[lo:hi]), (sg, blk(q_ // 2, q_ % 2)[lo:hi])]

        def build(terms, dst):
            if len(terms) == 1:
                return terms[0][1]
            if not prep:
                return dst[...]
            acc = None
            for sg, x in terms:
                v = (_lo(x), _hi(x))
                acc = v if acc is None else tuple(a + b_ if sg > 0 else a - b_ for a, b_ in zip(acc, v))
            dst[...] = wv = pack2(*acc)
            return wv

        wq = w4n if ib >= 5 else w4q.at[pl.ds(zsm[6], NQ)] if prep else w4q
        prep = prep and ib >= 5
        quad = lambda i, z: wterms(i % 2, 192 * (i // 2), 192 * (i // 2 + 1), z)
        wt = [build(wterms(j, 384, 448, None), wq.at[slot, 7, pl.ds(64 * j, 64), :]) for j in range(2)]
        tail = _dot(_unpack(opaque(h3, 5)[6, ka, pl.ds(0, 2 * q), :]), _unpack(jnp.concatenate(wt, axis=1)))
        ms = []
        for ja, jb in _STRASSEN:
            if ja >= 5:
                lv = lblk(3 * (ja - 5), 5)
            else:
                p_, q_, sg = _SUMS_A[ja]
                lv = psum(lblk(p_, ja), lblk(q_, ja), sg)
            z = zsm[8 + 7 * slot + jb] if prep else None
            if jb >= 5:
                terms = quad(3 * (jb - 5), z)
            else:
                p_, q_, sg = _SUMS_B[jb]
                terms = quad(p_, z) + [(sg * s_, x) for s_, x in quad(q_, z)]
            ms.append(_dot(_unpack(lv), _unpack(build(terms, wq.at[slot, jb]))))
            if len(ms) < 7:
                yield
        c11, c12, c21, c22 = _combine(*ms)
        done[0][k] = jnp.concatenate([c11, c21], axis=0) + tail[:, :128]
        done[1][k] = jnp.concatenate([c12, c22], axis=0) + tail[:, 128:]
        for j in range(2):
            b2_done(w, done, r0, n, j)

    w = window(0, 2 * TS + LEAD, 0)
    H = TS // 2
    with jax.named_scope("t0a"):
        cps["qa"].wait()
        cps["wmoda"].wait()

        mv = {}

        def mod_fn(j, toks):
            mv[j] = mod_cols(j, 1, toks)[0]
            if len(mv) == 3:
                modbuf[0] = mv[2] * mv[0]
                modbuf[1] = mv[2] * (1.0 + mv[1])

        segment(G5B, 0, MU, mod_fn=mod_fn)
        put(w["h"], pl.ds(0, QA), stage_a0(w, 0, QA))
    with jax.named_scope("t0b"):
        cps["wmodb"].wait()
        sb, cb = mod_cols(3, 2)
        modbuf[3] = 2.0 * sb
        modbuf[4] = 2.0 + 2.0 * cb
        n3 = stage_a1(w, 0, QA, n2=slabs(w["h"], 0, QA))
    XB = TS - XA
    FN = 32
    F4 = 64
    P1B = "1" == "1"
    with jax.named_scope("t1a"):
        cps["w1a"].wait()
        cps["qx"].wait()
        put(w["h"], pl.ds(QA, XA), stage_a0(w, QA, XA))
        stage_a2(w, n3, 0, QA, c1=W1A, fine=80)
    with jax.named_scope("t1b"):
        cps["w1b"].wait()
        n3a = stage_a1(w, QA, XA, n2=slabs(w["h"], QA, XA), f32=True)
        stage_a2(w, n3, 0, QA, c0=W1A)
        if P1B:
            stage_a2(w, [dd_rest("w1", *_rows2(n3a))], QA, XA, prep=True)
        else:
            stage_a2(w, n3a, QA, XA, fine=FN)
    with jax.named_scope("t2"):
        cps["qb"].wait()
        cps["w2"].wait()
        n3b = stage_a1(w, QA + XA, XB, f32=True)
        x1 = {}
        for op in "2aP na 1 2bF nb 2cF".split():
            r, n = dict(a=(0, TS), b=(TS, XA), c=(TS + XA, XB), d=(0, H), e=(H, H), f=(H, TS), g=(TS, TS)).get(op[1:2], (0, 0))
            if op == "1":
                stage_a2(w, [dd_rest("w1", *_rows2(n3b))], QA + XA, XB, prep=not P1B)
            elif op[0] == "n":
                stage_b1b(w, x1[op[1]], r, n)
            else:
                x1[op[1]] = stage_b1a(w, r, n, fast=op[2] in "PF", prep=op[2] == "P", fine=FN if op[2] == "f" else 0)
    ha, hb = hba, hbb
    with jax.named_scope("t3"):
        cps["w3"].wait()
        r, n = (TS + XA, XB)
        stage_b1b(w, [parity(w["h"], r, n, e) for e in range(2)], r, n)
        for op in "ha 3a:0:6 hb 3b:0:6".split():
            op, *rng = op.split(":")
            rng = [int(x) for x in rng]
            hx, r = (ha, 0) if op[1] == "a" else (hb, TS)
            if op[0] == "h":
                stage_b2h(w, hx, r, TS, prep=op[1] == "a")
            else:
                stage_b2a(w, hx, r, TS, *rng, prep=op[1] == "a")
    with jax.named_scope("t4"):
        cps["w4"].wait()
        cps["wmodg"].wait()
        done, gens = {0: {}, 1: {}}, {}
        LC = 64
        for op in "m4 P m0 4:0:0:1 m2 8:2 m1 8:1 m3 8:3 4:1:0:1 8:6 8:4 8:5".split():
            op, *rng = op.split(":")
            rng = [int(x) for x in rng]
            if op[0] == "m":
                c = int(op[1])
                modbuf[5, :, pl.ds(c * 128, 128)] = 0.5 * _dot(modbuf[6], weights(wmodbuf, 5 * NC + c, 5 * NC + c + 1))
            elif op[0] == "8":
                g = gens.setdefault(rng[0], steps_b2n(w, ha, 0, TS, rng[0], done, prep=True))
                for _ in range(rng[1] if len(rng) > 1 else 7):
                    next(g, None)
            elif op[0] == "P":
                stage_b2b(w, ha, 0, TS, 2, marks=prep_w4(24))
            elif op[0] == "L":
                stage_b2b(w, ha, 0, LC, 2, sub=LC * int(op[1]))
            else:
                stage_b2b(w, ha, 0, TS, *rng, done=done, prep=True)
        out_copy(0, TS).start()
        cps["q1"].wait()

    CBS = (128, 128)
    PART = {"a": (TS, TS), "c": (TS, H), "d": (TS + H, H)}
    BODY = "4:2 4:0:0:1 4:1:0:1 8:1 8:4 r0 r1 1a 8:2 2c nc 2d nd 8:6 8:5 8:3 3a:0:2 ha 3a:2:6"

    def step(s, carry):
        r0 = pl.multiple_of(s * TS, TS)
        w = window(r0, 2 * TS + LEAD, pl.multiple_of(s * H, H))
        x1, rest, done = {}, {}, {0: {}, 1: {}}
        for op in BODY.split():
            op, *rng = op.split(":")
            rng = [int(x) for x in rng]
            if op[0] == "3":
                stage_b2a(w, hb, TS, TS, *rng)
            elif op[0] == "h":
                stage_b2h(w, hb, TS, TS)
            elif op[0] == "4":
                stage_b2b(w, hb, 0, TS, *rng, done=done)
            elif op[0] == "8":
                stage_b2n(w, hb, 0, TS, *rng, done)
            elif op[0] == "2":
                x1[op[1]] = stage_b1a(w, *PART[op[1]], fast=True)
            elif op[0] == "n":
                stage_b1b(w, x1[op[1]], *PART[op[1]])
            elif op[0] == "r":
                j = int(op[1])
                rest[j] = dd_rest("w1", *_rows2(stage_a1(w, TS + LEAD + sum(CBS[:j]), CBS[j], f32=True)))
            else:
                ra, n = PART[op[1]]
                parts = [rest[j] for j in range(len(CBS)) if ra - TS <= sum(CBS[:j]) < ra - TS + n]
                stage_a2(w, parts, ra + LEAD, n, last_valid=(s < NT - 2) if ra + n == 2 * TS else None)
        out_copy(r0, TS).start()
        return carry

    with jax.named_scope("p2main"):
        jax.lax.fori_loop(1, NT - 1, step, 0)
    with jax.named_scope("p2epi"):
        w = window(S - 2 * TS, 2 * TS + LEAD, S // 2 - TS)
        rows = pl.ds(S - TS, TS)
        pending.append(hhbuf[0, pl.ds(S, 8), :])
        def flush(rows, cols):
            pltpu.make_async_copy(obuf.at[rows, cols], out_hbm.at[rows, cols], sem_out.at[0]).start()

        done = {0: {}, 1: {}}
        stage_b2b(w, hb, TS, TS, 0, 0, 1, done=done)
        for k in NEST:
            stage_b2n(w, hb, TS, TS, k, done)
        stage_b2b(w, hb, TS, TS, 0, 1, done=done)
        stage_b2b(w, hb, TS, TS, 1, done=done)
        flush(rows, pl.ds(0, 512))
        sub = 0
        for n in (128, 64, 64):
            stage_b2b(w, hb, TS, n, 2, sub=sub)
            flush(pl.ds(S - TS + sub, n), pl.ds(512, 128))
            sub += n
        pltpu.make_async_copy(obuf, out_hbm, sem_out.at[0]).wait()


@jax.jit
def pallas_adaLN_cond__ssm_conv_h3__mixer_s_mlp__prompt_kernel(
    A_q: jax.Array,
    A_k: jax.Array,
    A_v: jax.Array,
    A_shift_k: jax.Array,
    A_ssm_k: jax.Array,
    A_ssm_D: jax.Array,
    B_x: jax.Array,
    B_w1: jax.Array,
    B_w2: jax.Array,
    B_w3: jax.Array,
    B_w4: jax.Array,
    c: jax.Array,
    w_mod: jax.Array,
):
    del B_x

    def tiles(x):
        return x.reshape(S // 8, 8, NC, 128).transpose(0, 2, 1, 3).reshape(S * NC, 128)

    def pairs(x):
        r, n = x.shape
        return x.reshape(r // 16, 2, 8, n // 128, 128).transpose(0, 1, 3, 2, 4)

    args = (
        A_q.reshape(S, D), tiles(A_k), tiles(A_v),
        A_shift_k.T, A_ssm_k, A_ssm_D.reshape(NC, 128),
        pairs(B_w1), pairs(B_w2), pairs(B_w3.T), pairs(B_w4), c, pairs(w_mod),
    )
    scratch = [
        pltpu.VMEM((NA, P * NC + 128, 128), BF16),
        pltpu.VMEM((NA, P * NC + 64, 128), BF16),
        pltpu.VMEM((D, S), BF16),
        pltpu.VMEM((R, 128, 128), U32),
        pltpu.VMEM((R, 64, 256), U32),
        pltpu.VMEM((64, 128), U32),
        pltpu.VMEM((D // 16, 6 * NC, 16, 128), BF16),
        pltpu.VMEM((D // 16, NC, 16, 128), BF16),
        pltpu.VMEM((D // 16, NC, 16, 128), BF16),
        pltpu.VMEM((FF // 16, NC, 16, 128), BF16),
        pltpu.VMEM((FF // 16, NC, 16, 128), BF16),
        pltpu.VMEM((S + 64, D), BF16),
        *[pltpu.VMEM((NA, R, 16, 4, 8, 128), F32) for _ in range(NC)],
        pltpu.VMEM((NC, 2, R, 16, 2, 8, 128), F32),
        pltpu.VMEM((NC, R, 128, 128), U32),
        pltpu.VMEM((32, 128), U32),
        pltpu.VMEM((NC, 8, 8, 128), F32),
        pltpu.VMEM((NC, S + 32, 128), F32),
        pltpu.VMEM((8, 8, D), F32),
        pltpu.VMEM((S + 32, D), F32),
        pltpu.VMEM((NC, S + 32, 128), F32),
        pltpu.VMEM((NC, S + 32, 128), F32),
        pltpu.VMEM((2, TS, D), BF16),
        pltpu.VMEM((TS, 5 * 256), BF16),
        pltpu.VMEM((5, 2, 128, 128), U32),
        pltpu.VMEM((5, 2, 128, 128), U32),
        pltpu.VMEM((5, 6, 64, 256), U32),
        pltpu.VMEM((5, 2, FT // 2, 256), U32),
        pltpu.VMEM((5, 2, 448, 128), U32),
        pltpu.VMEM((8, 9, 72, 128), U32),
        pltpu.VMEM((8, 9, 72, 128), U32),
        pltpu.VMEM((2, 8, 192, 128), U32),
        pltpu.VMEM((NQ, 8, 192, 128), U32),
        pltpu.VMEM((S, D), BF16),
        pltpu.VMEM((4, D), BF16),
        pltpu.VMEM((NC, 128), BF16),
        pltpu.VMEM((1, D), BF16),
        pltpu.SMEM((64,), jnp.int32),
        pltpu.SemaphoreType.DMA((40,)),
        pltpu.SemaphoreType.DMA((1,)),
    ]
    out = pl.pallas_call(
        _kernel,
        out_shape=jax.ShapeDtypeStruct((S, D), BF16),
        in_specs=[pl.BlockSpec(memory_space=pl.ANY)] * len(args),
        out_specs=pl.BlockSpec(memory_space=pl.ANY),
        scratch_shapes=scratch,
        grid=(1,),
        compiler_params=pltpu.CompilerParams(vmem_limit_bytes=108 * 1024 * 1024, disable_semaphore_checks=True,
                                             disable_bounds_checks=True),
        name="adaln_h3_mixer",
    )(*args)
    return out.reshape(1, S, D)
```

```python
import numpy as np
import jax
import jax.numpy as jnp
import jax.experimental.pallas as pl
import jax.experimental.pallas.tpu as pltpu

F32 = jnp.float32
BF16 = jnp.bfloat16
U32 = jnp.uint32

S = 2048
D = 640
FF = 1728
NC = D // 128
R = 4
P = 128 * R
NA = S // P
TS = 256
NT = S // TS
LEAD = 16
EPS = 1e-5
NEST = (1, 4, 0, 3, 5, 6)
NQ = len(NEST)
FT = (FF - 1536) // 2


def _freq(row):
    t, part, s = row >> 4, (row >> 3) & 1, row & 7
    return 32 * (t & 7) + 4 * s + 2 * (t >> 3) + 1, P * part


def _cos(j, scale):
    jf = (j & (4 * P - 1)).astype(F32)
    u = 2.0 * np.pi / (4 * P)
    x = jnp.abs(jf * u - np.pi) - 0.5 * np.pi
    x2 = x * x
    poly = scale / 362880.0 - x2 * (scale / 39916800.0)
    for coef in (-1.0 / 5040.0, 1.0 / 120.0, -1.0 / 6.0, 1.0):
        poly = poly * x2 + coef * scale
    return poly * x


_DUR = {"t": 8, "u": 16, "k": 16, "i": 16, "m": 12, "g": 0, "c": 0, "j": 16}
_POST = {"t": 8.0, "u": 16.0, "k": 24.0, "i": 4.0, "j": 4.0, "m": 18.0}


def _plan_tokens(order, maxutil):
    lag, cap, pre, margin = 8, 60, 4, 3
    start, slots = {}, []
    for n in order:
        start[n] = len(slots)
        slots += [(n, r) for r in range(_DUR[n[0]])]
    nslot = len(slots) + lag
    free = [cap - (_POST[slots[i - lag][0][0]] if i >= lag else 0.0) for i in range(-pre, nslot)]
    units = []
    for n in order:
        kind, a, c = n
        if kind == "u":
            units += [(n + (g,), 94.0, start[n], -pre) for g in range(8)]
        elif kind == "g":
            units += [(n + (g,), 150.0, start[n], -pre) for g in range(8)]
        elif kind in "ic":
            src_ = [start[m] for m in (("u", a, c), ("k", a, c)) if m in start]
            for t in range(16):
                rel = max(max(src_) + 16, max(src_) + t + lag + 3) if src_ else -pre
                units.append((n + (t,), 32.0 * a + 48.0, nslot if kind == 'c' else start[n], rel))

    def simulate(util):
        left = [u[1] for u in units]
        done = [None] * len(units)
        for i in range(-pre, nslot):
            budget = util * free[i + pre]
            for j, u in enumerate(units):
                if budget <= 0.0:
                    break
                if done[j] is None and u[3] <= i:
                    use = min(budget, left[j])
                    left[j] -= use
                    budget -= use
                    if left[j] <= 1e-9:
                        done[j] = i + 1
        ok = all(u[2] < 8 or (d is not None and d <= max(u[2] - (1 if u[0][0] in 'cg' else margin), u[3] + 1))
                 for d, u in zip(done, units))
        return done, ok

    lo_, hi_ = 0.05, maxutil
    for _ in range(12):
        mid = 0.5 * (lo_ + hi_)
        if simulate(mid)[1]:
            hi_ = mid
        else:
            lo_ = mid
    done, _ = simulate(hi_)
    plan = {}
    for u, d in zip(units, done):
        if u[0][0] == "c":
            plan[u[0]] = slots[max((nslot - 1 if d is None else min(d, nslot - 1)) - lag, 0)]
        elif d is not None and 0 <= d < u[2]:
            plan.setdefault(slots[d], []).append(u[0])
    return plan


def _pack(x):
    return pltpu.bitcast(x.astype(BF16), U32)


def _unpack(w):
    return pltpu.bitcast(w, BF16)


def _dot(a, b):
    return jnp.dot(a.astype(BF16), b, preferred_element_type=F32)


def _dot_nt(a, b):
    return jax.lax.dot_general(a.astype(BF16), b, (((1,), (1,)), ((), ())), preferred_element_type=F32)


def _dot_fine(x, w, chunk):
    if not chunk:
        return _dot(x, w)
    n = w.shape[1]
    head = _dot(x, w[:, :n - 128])
    last = jnp.concatenate([_dot(x[r:r + chunk], w[:, n - 128:]) for r in range(0, x.shape[0], chunk)], axis=0)
    return jnp.concatenate([head, last], axis=1)


def _rows2(x):
    n, c = x.shape
    x = x.reshape(n // 32, 2, 16, c)
    return x[:, 0].reshape(n // 2, c), x[:, 1].reshape(n // 2, c)


def _unrows2(top, bot):
    n, c = top.shape
    return jnp.stack([top.reshape(n // 16, 16, c), bot.reshape(n // 16, 16, c)], axis=1).reshape(2 * n, c)


def _sums_a(a11, a12, a21, a22):
    return [a11 + a22, a21 + a22, a11 + a12, a21 - a11, a12 - a22]


def _sums_b(b11, b12, b21, b22):
    return [b11 + b22, b12 - b22, b21 - b11, b11 + b12, b21 + b22]


_STRASSEN = ((0, 0), (1, 5), (5, 1), (6, 2), (2, 6), (3, 3), (4, 4))


_SUMS_A = ((0, 3, 1), (2, 3, 1), (0, 1, 1), (2, 0, -1), (1, 3, -1))
_SUMS_B = ((0, 3, 1), (1, 3, -1), (2, 0, -1), (0, 1, 1), (2, 3, 1))


def _combine(m1, m2, m3, m4, m5, m6, m7):
    return (m1 + m4) + (m7 - m5), m3 + m5, m2 + m4, (m1 - m2) + (m3 + m6)


def _lo(w):
    return pltpu.bitcast(w << 16, F32)


def _hi(w):
    return pltpu.bitcast(w & jnp.uint32(0xFFFF0000), F32)


def _ln(x, eps=EPS):
    m = jnp.sum(x, axis=-1, keepdims=True) * (1.0 / D)
    xc = x - m
    v = jnp.sum(xc * xc, axis=-1, keepdims=True) * (1.0 / D)
    return xc * jnp.exp(-0.5 * jnp.log(v + eps))


def _gelu2(x):
    c0 = 0.7978845608028654
    c1 = c0 * 0.044715
    return x + x * jnp.tanh(x * (c0 + c1 * (x * x)))


def _bfly(tr, ti):
    s02r, s02i = tr[0] + tr[2], ti[0] + ti[2]
    d02r, d02i = tr[0] - tr[2], ti[0] - ti[2]
    s13r, s13i = tr[1] + tr[3], ti[1] + ti[3]
    d13r, d13i = tr[1] - tr[3], ti[1] - ti[3]
    x0r, x0i = s02r + s13r, s02i + s13i
    x2r, x2i = s02r - s13r, s02i - s13i
    return [x0r, d02r + d13i, x2r, d02r - d13i], [x0i, d02i - d13r, x2i, d02i + d13r]


def _kernel(q_hbm, k_hbm, v_hbm, shift_hbm, ssmk_hbm, ssmd_hbm, w1_hbm, w2_hbm, w3t_hbm, w4_hbm,
            c_hbm, wmod_hbm,
            out_hbm,
            kbuf, vbuf, skbuf, fwdbuf, invbuf, permbuf,
            wmodbuf, w1buf, w2buf, w3buf, w4buf, qbuf,
            xs0, xs1, xs2, xs3, xs4, kraw, wbuf, zbuf, coefbuf, ybuf, modbuf, x2buf, hbuf, hhbuf, xnbuf, xsbuf,
             w1s, w2s, w3s, w3ts, w4s, hba, hbb, w4n, w4q, obuf, shiftbuf, dbuf, cbuf,
            zsm, sem_in, sem_out):
    cps = {}
    n_sem = [0]

    def start(name, src, dst):
        cp = pltpu.make_async_copy(src, dst, sem_in.at[n_sem[0]])
        n_sem[0] += 1
        cp.start()
        cps[name] = cp

    class Both:
        def __init__(self, a, b):
            self.cps = (a, b)

        def wait(self):
            for cp in self.cps:
                cp.wait()

    def start_w(name, src, dst, c0=0, n=NC):
        for e in range(2):
            start(name + str(e), src.at[:, e, pl.ds(c0, n)], dst.at[:, pl.ds(c0, n), pl.ds(8 * e, 8), :])
        cps[name] = Both(cps[name + "0"], cps[name + "1"])

    CH = P * NC
    HALO = 8 * NC

    def start_s(a):
        cols = pl.ds(a * P, P)
        start("s%d" % a, ssmk_hbm.at[:, cols], skbuf.at[:, cols])

    def start_kv(a):
        if a == 0:
            kbuf[0, pl.ds(0, HALO + 8), :] = jnp.zeros((HALO + 8, 128), BF16)
            start("k0", k_hbm.at[pl.ds(0, CH), :], kbuf.at[0, pl.ds(HALO, CH), :])
        else:
            start("k%d" % a, k_hbm.at[pl.ds(a * CH - HALO, CH + HALO), :], kbuf.at[a, pl.ds(0, CH + HALO), :])
        start("v%d" % a, v_hbm.at[pl.ds(a * CH, CH), :], vbuf.at[a, pl.ds(0, CH), :])

    for n in "s0 x0 s1 k0 k1 s2 k2 s3 k3".split():
        if n[0] == "s":
            start_s(int(n[1]))
        elif n[0] == "k":
            start_kv(int(n[1]))
        else:
            start("d", ssmd_hbm, dbuf)
            start("shift", shift_hbm, shiftbuf)
            start("c", c_hbm, cbuf)
    QA = TS + LEAD
    XA = 128
    QB = 2 * TS + LEAD
    W1A = 2

    def start_q(name, r0, n):
        start(name, q_hbm.at[pl.ds(r0, n), :], qbuf.at[pl.ds(r0, n), :])

    start_q("qa", 0, QA)
    start_w("wmoda", wmod_hbm, wmodbuf, 0, 3 * NC)
    start_w("wmodb", wmod_hbm, wmodbuf, 3 * NC, 2 * NC)
    start_q("qx", QA, XA)
    start_w("w1a", w1_hbm, w1buf, 0, W1A)
    start_w("w1b", w1_hbm, w1buf, W1A, NC - W1A)
    start_q("qb", QA + XA, QB - QA - XA)
    start_w("w2", w2_hbm, w2buf)
    start_w("w3", w3t_hbm, w3buf)
    start_w("w4", w4_hbm, w4buf)
    start_w("wmodg", wmod_hbm, wmodbuf, 5 * NC, NC)
    start_q("q1", QB, S - QB)

    kw = kbuf.bitcast(U32)
    vw = vbuf.bitcast(U32)
    zbuf[...] = jnp.zeros(zbuf.shape, U32)
    for j in range(64):
        zsm[j] = 0
    for c in range(NC):
        ybuf[c, pl.ds(S, LEAD), :] = jnp.zeros((LEAD, 128), F32)
        hhbuf[c, pl.ds(0, 8), :] = jnp.zeros((8, 128), F32)
    qbuf[pl.ds(S, LEAD), :] = jnp.zeros((LEAD, D), BF16)

    def tables(p, carry):
        i0 = jax.lax.broadcasted_iota(jnp.int32, (128, 128), 0)
        n = R * jax.lax.broadcasted_iota(jnp.int32, (128, 128), 1) + p
        f2, off = _freq(2 * i0)
        j = f2 * n + off
        fwdbuf[p] = pltpu.pack_elementwise([_cos(j, 1.0), _cos(j + 4 * n, 1.0)], packed_dtype=BF16)
        return carry

    jax.lax.fori_loop(0, R, tables, 0)

    def unit_g(kt, r):
        col = jax.lax.broadcasted_iota(jnp.int32, (8, 128), 1) + 128 * kt
        f2, off = _freq((col & ~15) + 8 * (col & 1) + ((col >> 1) & 7))
        m = 2 * jax.lax.broadcasted_iota(jnp.int32, (8, 128), 0) + 16 * r
        j0 = f2 * (R * m) + off
        out = []
        for p in range(R):
            j = j0 + p * f2
            out.append(pltpu.pack_elementwise([_cos(j, 1.0 / P), _cos(j + R * f2, 1.0 / P)], packed_dtype=BF16))
            invbuf[p, pl.ds(8 * r, 8), pl.ds(128 * kt, 128)] = out[-1]
        return out

    i0 = jax.lax.broadcasted_iota(jnp.int32, (128, 128), 0)
    i1 = jax.lax.broadcasted_iota(jnp.int32, (128, 128), 1)
    permbuf[...] = _pack(jnp.where(i0 == (128 // R) * (i1 & (R - 1)) + (i1 >> 2), 1.0, 0.0).astype(F32))

    def fill_coef():
        cv = cbuf[...].astype(F32)
        modbuf[6] = jnp.broadcast_to(cv * jax.nn.sigmoid(cv), (8, D))
        coef = shiftbuf[...].astype(F32)
        dval = dbuf[...].astype(F32)
        for c in range(NC):
            for j in range(4):
                coefbuf[c, j] = jnp.broadcast_to(coef[j:j + 1, c * 128:(c + 1) * 128], (8, 128))
            coefbuf[c, 4] = jnp.broadcast_to(dval[c:c + 1, :], (8, 128))

    xs = (xs0, xs1, xs2, xs3, xs4)
    wsbufs = dict(w1=w1s, w2=w2s, w3=w3s, w4=w4s, w3t=w3ts)
    def split_ri(t):
        t = t.reshape(16, 2, 8, 128)
        return t[:, 0], t[:, 1]

    def get_never():
        return zbuf[pl.ds(0, 8), :] != 0

    def pack2(x, y):
        return pltpu.pack_elementwise([x, y], packed_dtype=BF16)

    def words(ref, a, c, r):
        return ref[a, pl.ds((r // 4) * 4 * NC + 4 * c + r % 4, 8, stride=4 * NC), :]

    def unit_u(a, c, g):
        c0, c1, c2, c3 = (coefbuf[c, pl.ds(j, 1)] for j in range(4))
        kk = jnp.stack([words(kw, a, c, 4 + 32 * g + d) for d in range(-2, 4)])
        vv = jnp.stack([words(vw, a, c, 32 * g + d) for d in range(4)])
        lo, hi = _lo(kk), _hi(kk)
        k0, k1, k2 = lo[2:], hi[1:5], lo[1:5]
        even = (((k0 * c0 + k1 * c1) + (k2 * c2 + hi[:4] * c3)) * _lo(vv)).reshape(32, 128)
        odd = (((hi[2:] * c0 + k0 * c1) + (k1 * c2 + k2 * c3)) * _hi(vv)).reshape(32, 128)
        e, o = pack2(even[:16], even[16:]), pack2(odd[:16], odd[16:])
        return [e[:8], o[:8], e[8:], o[8:]]

    def unit_i(a, c, t, z):
        x_c = xs[c].at[pl.ds(z, NA)]
        yr = yi = None
        for j in range(a + 1):
            ur, ui = x_c[j, :, t, 0], x_c[j, :, t, 1]
            kr, ki = x_c[a - j, :, t, 2], x_c[a - j, :, t, 3]
            pr = ur * kr - ui * ki
            pi = ur * ki + ui * kr
            yr = pr if yr is None else yr + pr
            yi = pi if yi is None else yi + pi
        halves = lambda x: (x[:x.shape[0] // 2], x[x.shape[0] // 2:])
        (ra, rb), (ia, ib) = halves(yr.reshape(32, 128)), halves(yi.reshape(32, 128))
        (sr0, sr1), (si0, si1), (dr0, dr1), (di0, di1) = (halves(x) for x in (ra + rb, ia + ib, ra - rb, ia - ib))
        return [pack2(sr0 + sr1, si0 + si1), pack2(dr0 - di1, di0 + dr1),
                pack2(sr0 - sr1, si0 - si1), pack2(dr0 + di1, di0 - dr1)]

    def segment(spec, z, maxutil=1.0, mod_fn=None):
        order = [(n[0], int(n[1]), int(n[2])) for n in spec.split()]
        plan = _plan_tokens(order, maxutil) if maxutil > 0 else {}
        never = get_never()
        units, res = {}, {}

        def unit(key):
            if key not in units:
                kind, a, c, j = key
                if kind == "u":
                    units[key] = unit_u(a, c, j)
                elif kind == "g":
                    units[key] = unit_g(a, j)
                else:
                    fresh = ("u", a, c) in order or ("k", a, c) in order
                    units[key] = unit_i(a, c, j, z if fresh else 0)
            return units[key]

        def lhs(name, p, full, r0=0):
            out, last = [], 0
            for r in range(full.shape[0] // 8):
                keys = plan.get((name, r0 + r), ())
                if keys:
                    if 8 * r > last:
                        out.append(full[last:8 * r])
                    v = full[8 * r:8 * r + 8]
                    for key in keys:
                        v = jax.lax.select(never, unit(key)[p], v)
                    out.append(v)
                    last = 8 * r + 8
            if last < full.shape[0]:
                out.append(full[last:] if last else full)
            return out[0] if len(out) == 1 else jnp.concatenate(out, axis=0)

        def dft(name, rhs):
            tr, ti = [], []
            for p in range(R):
                f = lhs(name, p, fwdbuf[p])
                r_, i_ = split_ri(_dot(_unpack(f), rhs[p]))
                if p == 0:
                    res.update({(name, r): (lambda r=r, v=r_: v[r]) for r in range(16)})
                tr.append(r_)
                ti.append(i_)
            return _bfly(tr, ti)

        st = {}
        for name in order:
            kind, a, c = name
            x_c = xs[c]
            if kind == "g":
                for r in range(8):
                    unit(name + (r,))
            elif kind == "c":
                for t in range(16):
                    after = pltpu.bitcast(res[plan[name + (t,)]](), U32)
                    for p in range(R):
                        wbuf[c, p, pl.ds(8 * t, 8), :] = jax.lax.select(never, after, unit(name + (t,))[p])
            elif kind == "m":
                toks = {}
                for r in range(_DUR["m"]):
                    for n_, key in enumerate(plan.get((name, r), ())):
                        toks.setdefault(2 * r + n_ % 2, []).extend(unit(key))
                mod_fn(a, toks)
            elif kind == "t":
                trs = []
                for b in range(R):
                    pm = lhs(name, b, permbuf[...])
                    trs.append(_dot_nt(_unpack(pm), skbuf[pl.ds(c * 128, 128), pl.ds(a * P + b * 128, 128)]))
                res.update({(name, r): (lambda r=r, v=trs[0]: v[16 * r:16 * r + 8]) for r in range(8)})
                g_ = 128 // R
                st[a, c] = [jnp.concatenate([trs[b][p * g_:(p + 1) * g_] for b in range(R)], axis=0).astype(BF16)
                            for p in range(R)]
            elif kind == "u":
                rhs = [_unpack(jnp.concatenate([unit(name + (g,))[p] for g in range(8)], axis=0)) for p in range(R)]
                xr, xi = dft(name, rhs)
                for q in range(R):
                    x_c[a, q, :, 0] = xr[q]
                    x_c[a, q, :, 1] = xi[q]
            elif kind == "k":
                xr, xi = dft(name, st[a, c])
                for q in range(R):
                    if a == 0:
                        x_c[a, q, :, 2] = xr[q] + coefbuf[c, 4]
                        x_c[a, q, :, 3] = xi[q]
                    else:
                        pr, pi = kraw[c, (a - 1) % 2, q, :, 0], kraw[c, (a - 1) % 2, q, :, 1]
                        x_c[a, q, pl.ds(0, 8), 2] = xr[q][:8] - pi[:8]
                        x_c[a, q, pl.ds(0, 8), 3] = xi[q][:8] + pr[:8]
                        x_c[a, q, pl.ds(8, 8), 2] = xr[q][8:] + pi[8:]
                        x_c[a, q, pl.ds(8, 8), 3] = xi[q][8:] - pr[8:]
                    if a + 1 < NA:
                        kraw[c, a % 2, q, :, 0] = xr[q]
                        kraw[c, a % 2, q, :, 1] = xi[q]
            else:
                for p in range(R):
                    cols = [lhs(name, 2 * (p % 2) + kt,
                                invbuf[p, :, pl.ds(128 * kt, 128)], 8 * (p // 2))
                            for kt in range(2)]
                    g = _unpack(jnp.concatenate(cols, axis=1))
                    if kind == "j":
                        wp = _unpack(wbuf[c, p])
                    else:
                        wp = _unpack(jnp.concatenate([unit(name + (t,))[p] for t in range(16)], axis=0))
                    yp = _dot(g, wp)
                    if p % 2 == 0:
                        res.update({(name, 4 * p + r): (lambda r=r, v=yp: v[16 * r:16 * r + 8]) for r in range(8)})
                    ybuf[c, pl.ds(a * P + p, 128, stride=R), :] = yp

    one = jnp.minimum(pl.program_id(0) + 1, 1)

    def once(fn):
        def body(z, carry):
            fn(z)
            return carry
        jax.lax.fori_loop(0, one, body, 0)

    default = "t00 t01 t02 k00 t03 k01 t04 k02 k03 k04 g00|t10 t11 t12 k10 k11 k12 g10|t13 t14 k13 u00 k14 u01 u02 u03 i00 u04 i01 c02 c03|j02 j03 u10 i04 u11 u12 u13 i10 u14 i11 c12|t20 t21 j12 t22 t23 t24 k20 u20 k21 u21 k22 i13 k23 u22 k24 i14 u23 i20 u24 i21 c22|t30 t31 j22 t32 t33 t34 k30 u30 k31 u31 k32 i23 k33 u32 k34 i24 u33 i30 u34 i31 c32|m00 j32 m10 m20 i33 i34"
    specs = default.split("|")
    G5B = specs[-1]
    segs = list(zip("s0 d shift c|s1|k0 v0|k1 v1|s2 k2 v2|s3 k3 v3".split("|"), specs[:-1]))
    MU = 1.5
    for i, (waits, spec) in enumerate(segs):
        with jax.named_scope("g%d" % i):
            for n in waits.split():
                cps[n].wait()
            if i == 0:
                fill_coef()
            once(lambda z: segment(spec, z, MU))

    def mod_cols(lo, n, toks=None):
        m = _dot(modbuf[6], weights(wmodbuf, lo * NC, (lo + n) * NC, toks=toks))
        return [m[:, j * D:(j + 1) * D] for j in range(n)]

    def mul_mod(x, j, cols=None):
        m = modbuf[j] if cols is None else modbuf[j, :, cols]
        return (x.reshape(-1, 8, x.shape[-1]) * m[None]).reshape(x.shape)

    def add_mod(x, j):
        return (x.reshape(-1, 8, x.shape[-1]) + modbuf[j][None]).reshape(x.shape)

    def slabs(ref, r0, n):
        return jnp.concatenate([ref[c, pl.ds(r0, n), :] for c in range(NC)], axis=1)

    def put(ref, rows, x):
        for c in range(NC):
            ref[c, rows, :] = x[:, c * 128:(c + 1) * 128]

    def parity(ref, r0, n, e):
        return jnp.concatenate([ref[c, pl.ds(r0 + e, n // 2, stride=2), :] for c in range(NC)], axis=1)

    def window(base, n):
        rows = pl.ds(base, n)
        return dict(q=qbuf.at[rows, :], y=ybuf.at[:, rows, :], x2=x2buf.at[rows, :], h=hbuf.at[:, rows, :],
                    hh=hhbuf.at[:, pl.ds(base, n + 8), :],
                    o=obuf.at[pl.ds(base, n - LEAD), :])

    def weights(ref, c0=0, c1=NC, r0=0, r1=None, toks=None, raw=False, z=None):
        r1 = 16 * ref.shape[0] if r1 is None else r1
        view = ref.bitcast(U32)
        if z is not None:
            view = view.at[pl.ds(z, ref.shape[0])]
        never = get_never() if toks else None
        rt = -(-(r1 - r0) // 128)
        cols = []
        for j in range(c0, c1):
            wu = view[pl.ds(r0 // 16, (r1 - r0) // 16), j].reshape((r1 - r0) // 2, 128)
            if toks:
                parts, last = [], 0
                for i in range(rt):
                    for n_, t in enumerate(toks.get((j - c0) * rt + i, ())):
                        r = 64 * i + 8 * n_
                        if r > last:
                            parts.append(wu[last:r])
                        parts.append(jax.lax.select(never, t, wu[r:r + 8]))
                        last = r + 8
                parts.append(wu[last:])
                wu = jnp.concatenate(parts, axis=0)
            cols.append(wu)
        wu = jnp.concatenate(cols, axis=1)
        return wu if raw else _unpack(wu)

    def wblocks(name, j, z=None):
        if name == "w3":
            blk = lambda kh, nh: weights(w3buf, 2 * kh, 2 * kh + 2, 128 * (j + 6 * nh), 128 * (j + 6 * nh + 1), raw=True, z=z)
        elif name == "w4":
            def blk(kh, nh):
                c = j + 2 * nh
                parts = [weights(w4buf, c, c + 1, 768 * kh, 768 * (kh + 1), raw=True, z=z),
                         weights(w4buf, c, c + 1, 1536 + FT * kh, 1536 + FT * (kh + 1), raw=True, z=z),
                         jnp.zeros(((128 - FT) // 2, 128), U32)]
                return jnp.concatenate(parts, axis=0)
        elif name == "w3t":
            blk = lambda kh, nh: weights(w3buf, 2 * kh, 2 * kh + 2, 1536 + FT * nh, 1536 + FT * (nh + 1), raw=True, z=z)
        else:
            ref = w1buf if name == "w1" else w2buf
            blk = lambda kh, nh: weights(ref, j + 2 * nh, j + 2 * nh + 1, 256 * kh, 256 * (kh + 1), raw=True, z=z)
        return blk

    def wsum(name, j, k):
        blk = wblocks(name, j, zsm[k])
        p, q, sign = _SUMS_B[k]
        return psum(blk(p // 2, p % 2), blk(q // 2, q % 2), sign)

    pending = []

    def attach(wv):
        if not pending:
            return wv
        never = get_never()
        rows = [wv[8 * i:8 * i + 8, :128] for i in range(8)]
        for i, t in enumerate(pending):
            rows[i % 8] = jax.lax.select(never, pltpu.bitcast(t, U32), rows[i % 8])
        pending.clear()
        first = jnp.concatenate(rows + ([wv[64:, :128]] if wv.shape[0] > 64 else []), axis=0)
        return first if wv.shape[1] == 128 else jnp.concatenate([first, wv[:, 128:]], axis=1)

    def sprods(name, j, lhs, k0=0, k1=7, prep=False):
        blk, buf = wblocks(name, j), wsbufs[name]
        out = []
        for ia, ib in _STRASSEN[k0:k1]:
            wv = blk(ib - 5, ib - 5) if ib >= 5 else (wsum(name, j, ib) if prep else buf[ib, j])
            if name == "w3t":
                out.append(_dot_nt(_unpack(wv), lhs(ia)))
            else:
                out.append((_dot_nt if name == "w3" else _dot)(lhs(ia), _unpack(attach(wv))))
            if prep and ib < 5:
                buf[ib, j] = wv
        return out

    def spair(name, j, lhs, prep=False):
        return _combine(*sprods(name, j, lhs, prep=prep))

    def dd_rest(name, t, b):
        ref = w1buf if name == "w1" else w2buf
        m = t.shape[0]
        xb = jnp.concatenate([t, b], axis=0)
        last = _dot(xb, weights(ref, 4, 5))
        rem = _dot(xb[:, 512:], weights(ref, 0, 4, r0=512))
        return t, b, rem[:m], rem[m:], last[:m], last[m:]

    def dd_main(name, parts, prep=False):
        t, b, rt, rb, lt, lb = (jnp.concatenate(v, axis=0) for v in zip(*parts))
        ops = _sums_a(t[:, :256], t[:, 256:512], b[:, :256], b[:, 256:512]) + [t[:, :256], b[:, 256:512]]
        top, bot = [None] * 4, [None] * 4
        for j in range(2):
            top[j], top[j + 2], bot[j], bot[j + 2] = spair(name, j, lambda i: ops[i], prep)
        return (jnp.concatenate([jnp.concatenate(top, axis=1) + rt, lt], axis=1),
                jnp.concatenate([jnp.concatenate(bot, axis=1) + rb, lb], axis=1))

    def stage_a0(w, r0, n):
        rows = pl.ds(r0, n)
        x = w["q"][rows, :].astype(F32)
        x2 = x + add_mod(mul_mod(_ln(x), 1), 0) * slabs(w["y"], r0, n)
        w["x2"][rows, :] = x2
        return _ln(x2)

    def stage_a1(w, r0, n, n2=None, f32=False):
        if n2 is None:
            n2 = stage_a0(w, r0, n)
        h = add_mod(mul_mod(n2, 4), 3)
        put(w["h"], pl.ds(r0, n), h)
        n3 = _ln(h, 4 * EPS)
        return n3 if f32 else n3.astype(BF16)

    def stage_a2(w, n3, r0, n, last_valid=None, fine=0, c0=0, c1=NC, prep=False):
        hh = _gelu2(_unrows2(*dd_main("w1", n3, prep)) if isinstance(n3, list) else _dot_fine(n3, weights(w1buf, c0, c1), fine))
        for c in range(c0, c1):
            blk = hh[:, (c - c0) * 128:(c - c0 + 1) * 128]
            w["hh"][c, pl.ds(r0 + 8, n - LEAD), :] = blk[:n - LEAD]
            tail = blk[n - LEAD:]
            if last_valid is not None:
                tail = jnp.where(last_valid, tail, 0.0)
            w["hh"][c, pl.ds(r0 + 8 + n - LEAD, LEAD), :] = tail

    def stage_b1a(w, r0, n, prep=False):
        m = n // 2
        lane = jax.lax.broadcasted_iota(jnp.int32, (m, 128), 1)
        g = []
        for e in range(2):
            sh = lambda c, d: w["hh"][c, pl.ds(r0 + 8 + e + d, m, stride=2), :]
            g.append(jnp.concatenate([sh(0, -1),
                                      jnp.where(lane < 32, sh(1, -1), sh(1, 1)),
                                      jnp.where(lane < 64, sh(2, 1), sh(2, -2)),
                                      jnp.where(lane < 96, sh(3, -2), sh(3, 2)),
                                      sh(4, 2)], axis=1))
        hs = dd_main("w2", [dd_rest("w2", *g)], prep)
        x1 = [parity(w["h"], r0, n, e) + hs[e] for e in range(2)]
        for e in range(2):
            put(w["h"], pl.ds(r0 + e, m, stride=2), x1[e])
        return x1

    def stage_b1b(w, x1, r0, n):
        xn = jnp.stack([_ln(x, 4 * EPS).reshape(n // 16, 8, D) for x in x1], axis=1).reshape(n, D)
        t, b = _rows2(xn)
        xnbuf[0, pl.ds(r0 // 2, n // 2), :] = t.astype(BF16)
        xnbuf[1, pl.ds(r0 // 2, n // 2), :] = b.astype(BF16)
        sa = _sums_a(t[:, :256], t[:, 256:512], b[:, :256], b[:, 256:512])
        xsbuf[pl.ds(r0 // 2, n // 2), :] = jnp.concatenate(sa, axis=1).astype(BF16)

    def out_copy(r0, n):
        rows = pl.ds(r0, n)
        return pltpu.make_async_copy(obuf.at[rows, :], out_hbm.at[rows, :], sem_out.at[0])


    def opaque(ref, i):
        return ref.at[:, :, pl.ds(pl.multiple_of(zsm[i] * 32, 32), ref.shape[2]), :]

    def packrows(v):
        v = v.reshape(v.shape[0] // 16, 2, 8, 128)
        return pack2(v[:, 0], v[:, 1]).reshape(-1, 128)

    def emit(h3, j, left, right):
        m = left.shape[0] // 2
        g = [left[:m], right[:m], left[m:], right[m:]]
        for k, v in enumerate(_sums_a(*g) + g):
            h3[j, k, pl.ds(0, m // 2), :] = packrows(v)

    def load_xn(w, r0, n):
        return xnbuf[:, pl.ds(r0 // 2, n // 2), :].reshape(n, D)

    def w3_operands(w, r0, n):
        xn = load_xn(w, r0, n)
        xsum = xsbuf[pl.ds(r0 // 2, n // 2), :]
        m = n // 2
        return xn, [xsum[:, 256 * k:256 * (k + 1)] for k in range(5)] + [xn[:m, :256], xn[m:, 256:512]]

    def stage_b2h(w, h3, r0, n, prep=False):
        xn, ops = w3_operands(w, r0, n)
        m = n // 2
        rem = _dot_nt(weights(w3buf, 4, 5, r0=1536), xn[:, 512:])
        c11, c12, c21, c22 = spair("w3t", 0, lambda i: ops[i], prep)
        pad = jnp.zeros((128 - FT, m), F32)
        g11, g12, g21, g22 = (jnp.concatenate([_gelu2(c + r), pad], axis=0).T for c, r in (
            (c11, rem[:FT, :m]), (c12, rem[FT:, :m]), (c21, rem[:FT, m:]), (c22, rem[FT:, m:])))
        emit(h3, 6, jnp.concatenate([g11, g21], axis=0), jnp.concatenate([g12, g22], axis=0))

    def stage_b2a(w, h3, r0, n, lo=0, hi=6, prep=False):
        xn, ops = w3_operands(w, r0, n)
        for j in range(lo, hi):
            r1, r2 = (_dot_nt(xn[:, 512:], weights(w3buf, 4, 5, 128 * t, 128 * (t + 1))) for t in (j, j + 6))
            c11, c12, c21, c22 = spair("w3", j, lambda i: ops[i], prep)
            emit(h3, j, _gelu2(jnp.concatenate([c11, c21], axis=0) + r1), _gelu2(jnp.concatenate([c12, c22], axis=0) + r2))

    def finish(w, h2, r0, n, c):
        nc = h2.shape[1] // 128
        rows, cols = pl.ds(r0, n), pl.ds(c * 128, nc * 128)
        x1 = jnp.concatenate([w["h"][c + i, rows, :] for i in range(nc)], axis=1)
        w["o"][rows, cols] = (w["x2"][rows, cols] + mul_mod(x1 + h2, 5, cols)).astype(BF16)

    def b2_done(w, done, r0, n):
        if len(done[0]) == len(done[1]) == 7:
            c11, c12, c21, c22 = _combine(*[jnp.concatenate([done[0][k], done[1][k]], axis=1) for k in range(7)])
            finish(w, _unrows2(c11, c21), r0, n, 0)
            finish(w, _unrows2(c12, c22), r0, n, 2)

    def stage_b2b(w, h3, r0, n, j, k0=0, k1=7, done=None, prep=False, sub=0, marks=()):
        hv = opaque(h3, j)
        blk = lambda k: jnp.concatenate([hv[p, k, pl.ds(sub // 4, n // 4), :] for p in range(7)], axis=1)
        r0 += sub
        if j < 2:
            for k in range(k0, k1):
                if k not in NEST:
                    done[j][k] = sprods("w4", j, lambda i: _unpack(blk(8 if i == 6 else i)), k, k + 1, prep)[0]
                    b2_done(w, done, r0, n)
            return
        wb = wblocks("w4", 4)
        lhs = jnp.concatenate([jnp.concatenate([blk(5), blk(6)], axis=1),
                               jnp.concatenate([blk(7), blk(8)], axis=1)], axis=0)
        if marks:
            lo_, hi_ = 0, 52
            never, at = get_never(), {}
            for i, mk in enumerate(marks):
                s_ = lo_ + (hi_ - lo_) * i // len(marks)
                at[4 * (s_ // 16), s_ % 16] = mk
            cols = []
            for kt in range(14):
                col = lhs[:, 128 * kt:128 * (kt + 1)]
                if any(k_[0] == kt for k_ in at):
                    col = jnp.concatenate([jax.lax.select(never, at[kt, r], col[8 * r:8 * r + 8]) if (kt, r) in at
                                           else col[8 * r:8 * r + 8] for r in range(16)], axis=0)
                cols.append(col)
            lhs = jnp.concatenate(cols, axis=1)
        h2 = _dot(_unpack(lhs), _unpack(jnp.concatenate([wb(0, 0), wb(1, 0)], axis=0)))
        finish(w, _unrows2(h2[:n // 2], h2[n // 2:]), r0, n, 4)


    def psum(x, y, sign):
        if sign > 0:
            return pack2(_lo(x) + _lo(y), _hi(x) + _hi(y))
        return pack2(_lo(x) - _lo(y), _hi(x) - _hi(y))

    def prep_w4(nchunk):
        rows = 384 // nchunk
        marks = []
        for ch in [nchunk] + list(range(nchunk)):
            tail = ch == nchunk
            raw = {}
            for kh in range(2):
                for e in range(1 if tail else 2):
                    r0 = 1536 + FT * kh if tail else 768 * kh + 384 * e + rows * ch
                    x = weights(w4buf, 0, 4, r0, r0 + (FT if tail else rows), raw=True)
                    raw[kh, e] = jnp.stack([_lo(x), _hi(x)])
            blk = lambda i, e: raw[i // 2, e][:, :, 256 * (i % 2):256 * (i % 2 + 1)]
            for k, (ia, ib) in enumerate(_STRASSEN):
                if k not in NEST or ib >= 5:
                    continue
                p_, q_, sg = _SUMS_B[ib]
                half = [blk(p_, e) + blk(q_, e) if sg > 0 else blk(p_, e) - blk(q_, e) for e in range(1 if tail else 2)]
                quad = lambda i: half[i // 2][:, :, 128 * (i % 2):128 * (i % 2 + 1)]
                first = NEST.index(k)
                if tail:
                    for j in range(2):
                        w4q[first, 7, pl.ds(64 * j, FT // 2), :] = pack2(quad(j)[0], quad(j)[1])
                        w4q[first, 7, pl.ds(64 * j + FT // 2, 64 - FT // 2), :] = jnp.zeros((64 - FT // 2, 128), U32)
                    continue
                for jb, v in enumerate(_sums_b(*[quad(i) for i in range(4)]) + [quad(0), quad(3)]):
                    w4q[first, jb, pl.ds(rows // 2 * ch, rows // 2), :] = pack2(v[0], v[1])
            if not tail:
                marks.append(w4q.at[pl.ds(zsm[32 + ch], NQ)][first, 0, pl.ds(0, 8), :])
        return marks

    def stage_b2n(w, h3, r0, n, k, done, prep=False):
        ia, ib = _STRASSEN[k]
        ka, q, slot = (8 if ia == 6 else ia), n // 8, NEST.index(k)

        def lblk(i, z):
            hv = opaque(h3, z)
            return jnp.concatenate([hv[g + 3 * (i % 2), ka, pl.ds((i // 2) * q, q), :] for g in range(3)], axis=1)

        def raw(j, lo, hi, z=None):
            return wblocks("w4", j, z)(ib - 5, ib - 5)[lo:hi]

        quad = lambda i, z=None: raw(i % 2, 192 * (i // 2), 192 * (i // 2 + 1), z)
        if ib >= 5:
            wt = [raw(j, 384, 448) for j in range(2)]
        else:
            wq = w4q.at[pl.ds(zsm[6], NQ)] if prep else w4q
            wt = [wq[slot, 7, pl.ds(64 * j, 64), :] for j in range(2)]
        tail = _dot(_unpack(opaque(h3, 5)[6, ka, pl.ds(0, 2 * q), :]), _unpack(jnp.concatenate(wt, axis=1)))
        ms = []
        for ja, jb in _STRASSEN:
            if ja >= 5:
                lv = lblk(3 * (ja - 5), 5)
            else:
                p_, q_, sg = _SUMS_A[ja]
                lv = psum(lblk(p_, ja), lblk(q_, ja), sg)
            z = zsm[8 + 7 * slot + jb] if prep and ib >= 5 else None
            if ib < 5:
                wv = wq[slot, jb]
            elif jb >= 5:
                wv = quad(3 * (jb - 5), z)
            elif prep:
                p_, q_, sg = _SUMS_B[jb]
                w4n[slot, jb] = wv = psum(quad(p_, z), quad(q_, z), sg)
            else:
                wv = w4n[slot, jb]
            ms.append(_dot(_unpack(lv), _unpack(wv)))
        c11, c12, c21, c22 = _combine(*ms)
        done[0][k] = jnp.concatenate([c11, c21], axis=0) + tail[:, :128]
        done[1][k] = jnp.concatenate([c12, c22], axis=0) + tail[:, 128:]
        b2_done(w, done, r0, n)

    w = window(0, 2 * TS + LEAD)
    H = TS // 2
    with jax.named_scope("t0a"):
        cps["qa"].wait()
        cps["wmoda"].wait()

        mv = {}

        def mod_fn(j, toks):
            mv[j] = mod_cols(j, 1, toks)[0]
            if len(mv) == 3:
                modbuf[0] = mv[2] * mv[0]
                modbuf[1] = mv[2] * (1.0 + mv[1])

        segment(G5B, 0, MU, mod_fn=mod_fn)
        put(w["h"], pl.ds(0, QA), stage_a0(w, 0, QA))
    with jax.named_scope("t0b"):
        cps["wmodb"].wait()
        sb, cb = mod_cols(3, 2)
        modbuf[3] = 2.0 * sb
        modbuf[4] = 2.0 + 2.0 * cb
        n3 = stage_a1(w, 0, QA, n2=slabs(w["h"], 0, QA))
    XB = TS - XA
    with jax.named_scope("t1a"):
        cps["w1a"].wait()
        cps["qx"].wait()
        put(w["h"], pl.ds(QA, XA), stage_a0(w, QA, XA))
        stage_a2(w, n3, 0, QA, c1=W1A, fine=80)
    with jax.named_scope("t1b"):
        cps["w1b"].wait()
        n3a = stage_a1(w, QA, XA, n2=slabs(w["h"], QA, XA), f32=True)
        stage_a2(w, n3, 0, QA, c0=W1A)
        stage_a2(w, [dd_rest("w1", *_rows2(n3a))], QA, XA, prep=True)
    with jax.named_scope("t2"):
        cps["qb"].wait()
        cps["w2"].wait()
        n3b = stage_a1(w, QA + XA, XB, f32=True)
        stage_b1b(w, stage_b1a(w, 0, TS, prep=True), 0, TS)
        stage_a2(w, [dd_rest("w1", *_rows2(n3b))], QA + XA, XB)
        stage_b1b(w, stage_b1a(w, TS, XA), TS, XA)
        stage_b1a(w, TS + XA, XB)
    with jax.named_scope("t3"):
        cps["w3"].wait()
        stage_b1b(w, [parity(w["h"], TS + XA, XB, e) for e in range(2)], TS + XA, XB)
        stage_b2h(w, hba, 0, TS, prep=True)
        stage_b2a(w, hba, 0, TS, prep=True)
        stage_b2h(w, hbb, TS, TS)
        stage_b2a(w, hbb, TS, TS)
    with jax.named_scope("t4"):
        cps["w4"].wait()
        cps["wmodg"].wait()
        done = {0: {}, 1: {}}
        for op in "m4 P m0 4:0:2:3 m2 8:0 m1 8:1 m3 8:3 4:1:2:3 8:6 8:4 8:5".split():
            op, *rng = op.split(":")
            rng = [int(x) for x in rng]
            if op[0] == "m":
                c = int(op[1])
                modbuf[5, :, pl.ds(c * 128, 128)] = 0.5 * _dot(modbuf[6], weights(wmodbuf, 5 * NC + c, 5 * NC + c + 1))
            elif op[0] == "8":
                stage_b2n(w, hba, 0, TS, *rng, done, prep=True)
            elif op[0] == "P":
                stage_b2b(w, hba, 0, TS, 2, marks=prep_w4(24))
            else:
                stage_b2b(w, hba, 0, TS, *rng, done=done, prep=True)
        out_copy(0, TS).start()
        cps["q1"].wait()

    CBS = (128, 128)
    PART = {"a": (TS, TS), "c": (TS, H), "d": (TS + H, H)}
    BODY = "4:2 4:0:2:3 4:1:2:3 8:3 8:0 r0 r1 1a 8:1 2c nc 2d nd 8:6 8:5 8:4 3a:0:2 ha 3a:2:6"

    def step(s, carry):
        r0 = pl.multiple_of(s * TS, TS)
        w = window(r0, 2 * TS + LEAD)
        x1, rest, done = {}, {}, {0: {}, 1: {}}
        for op in BODY.split():
            op, *rng = op.split(":")
            rng = [int(x) for x in rng]
            if op[0] == "3":
                stage_b2a(w, hbb, TS, TS, *rng)
            elif op[0] == "h":
                stage_b2h(w, hbb, TS, TS)
            elif op[0] == "4":
                stage_b2b(w, hbb, 0, TS, *rng, done=done)
            elif op[0] == "8":
                stage_b2n(w, hbb, 0, TS, *rng, done)
            elif op[0] == "2":
                x1[op[1]] = stage_b1a(w, *PART[op[1]])
            elif op[0] == "n":
                stage_b1b(w, x1[op[1]], *PART[op[1]])
            elif op[0] == "r":
                j = int(op[1])
                rest[j] = dd_rest("w1", *_rows2(stage_a1(w, TS + LEAD + sum(CBS[:j]), CBS[j], f32=True)))
            else:
                ra, n = PART[op[1]]
                parts = [rest[j] for j in range(len(CBS)) if ra - TS <= sum(CBS[:j]) < ra - TS + n]
                stage_a2(w, parts, ra + LEAD, n, last_valid=(s < NT - 2) if ra + n == 2 * TS else None)
        out_copy(r0, TS).start()
        return carry

    with jax.named_scope("p2main"):
        jax.lax.fori_loop(1, NT - 1, step, 0)
    with jax.named_scope("p2epi"):
        w = window(S - 2 * TS, 2 * TS + LEAD)
        rows = pl.ds(S - TS, TS)
        pending.append(hhbuf[0, pl.ds(S, 8), :])
        def flush(rows, cols):
            pltpu.make_async_copy(obuf.at[rows, cols], out_hbm.at[rows, cols], sem_out.at[0]).start()

        done = {0: {}, 1: {}}
        for j in range(2):
            stage_b2b(w, hbb, TS, TS, j, done=done)
        for k in NEST:
            stage_b2n(w, hbb, TS, TS, k, done)
        flush(rows, pl.ds(0, 512))
        sub = 0
        for n in (128, 64, 64):
            stage_b2b(w, hbb, TS, n, 2, sub=sub)
            flush(pl.ds(S - TS + sub, n), pl.ds(512, 128))
            sub += n
        pltpu.make_async_copy(obuf, out_hbm, sem_out.at[0]).wait()


@jax.jit
def pallas_adaLN_cond__ssm_conv_h3__mixer_s_mlp__prompt_kernel(
    A_q: jax.Array,
    A_k: jax.Array,
    A_v: jax.Array,
    A_shift_k: jax.Array,
    A_ssm_k: jax.Array,
    A_ssm_D: jax.Array,
    B_x: jax.Array,
    B_w1: jax.Array,
    B_w2: jax.Array,
    B_w3: jax.Array,
    B_w4: jax.Array,
    c: jax.Array,
    w_mod: jax.Array,
):
    del B_x

    def tiles(x):
        return x.reshape(S // 8, 8, NC, 128).transpose(0, 2, 1, 3).reshape(S * NC, 128)

    def pairs(x):
        r, n = x.shape
        return x.reshape(r // 16, 2, 8, n // 128, 128).transpose(0, 1, 3, 2, 4)

    args = (
        A_q.reshape(S, D), tiles(A_k), tiles(A_v),
        A_shift_k.T, A_ssm_k, A_ssm_D.reshape(NC, 128),
        pairs(B_w1), pairs(B_w2), pairs(B_w3.T), pairs(B_w4), c, pairs(w_mod),
    )
    scratch = [
        pltpu.VMEM((NA, P * NC + 128, 128), BF16),
        pltpu.VMEM((NA, P * NC + 64, 128), BF16),
        pltpu.VMEM((D, S), BF16),
        pltpu.VMEM((R, 128, 128), U32),
        pltpu.VMEM((R, 64, 256), U32),
        pltpu.VMEM((64, 128), U32),
        pltpu.VMEM((D // 16, 6 * NC, 16, 128), BF16),
        pltpu.VMEM((D // 16, NC, 16, 128), BF16),
        pltpu.VMEM((D // 16, NC, 16, 128), BF16),
        pltpu.VMEM((FF // 16, NC, 16, 128), BF16),
        pltpu.VMEM((FF // 16, NC, 16, 128), BF16),
        pltpu.VMEM((S + 64, D), BF16),
        *[pltpu.VMEM((NA, R, 16, 4, 8, 128), F32) for _ in range(NC)],
        pltpu.VMEM((NC, 2, R, 16, 2, 8, 128), F32),
        pltpu.VMEM((NC, R, 128, 128), U32),
        pltpu.VMEM((32, 128), U32),
        pltpu.VMEM((NC, 8, 8, 128), F32),
        pltpu.VMEM((NC, S + 32, 128), F32),
        pltpu.VMEM((8, 8, D), F32),
        pltpu.VMEM((S + 32, D), F32),
        pltpu.VMEM((NC, S + 32, 128), F32),
        pltpu.VMEM((NC, S + 32, 128), F32),
        pltpu.VMEM((2, TS, D), BF16),
        pltpu.VMEM((TS, 5 * 256), BF16),
        pltpu.VMEM((5, 2, 128, 128), U32),
        pltpu.VMEM((5, 2, 128, 128), U32),
        pltpu.VMEM((5, 6, 64, 256), U32),
        pltpu.VMEM((5, 2, FT // 2, 256), U32),
        pltpu.VMEM((5, 2, 448, 128), U32),
        pltpu.VMEM((8, 9, 72, 128), U32),
        pltpu.VMEM((8, 9, 72, 128), U32),
        pltpu.VMEM((2, 8, 192, 128), U32),
        pltpu.VMEM((NQ, 8, 192, 128), U32),
        pltpu.VMEM((S, D), BF16),
        pltpu.VMEM((4, D), BF16),
        pltpu.VMEM((NC, 128), BF16),
        pltpu.VMEM((1, D), BF16),
        pltpu.SMEM((64,), jnp.int32),
        pltpu.SemaphoreType.DMA((40,)),
        pltpu.SemaphoreType.DMA((1,)),
    ]
    out = pl.pallas_call(
        _kernel,
        out_shape=jax.ShapeDtypeStruct((S, D), BF16),
        in_specs=[pl.BlockSpec(memory_space=pl.ANY)] * len(args),
        out_specs=pl.BlockSpec(memory_space=pl.ANY),
        scratch_shapes=scratch,
        grid=(1,),
        compiler_params=pltpu.CompilerParams(vmem_limit_bytes=108 * 1024 * 1024, disable_semaphore_checks=True,
                                             disable_bounds_checks=True),
        name="adaln_h3_mixer",
    )(*args)
    return out.reshape(1, S, D)
```

```python
import numpy as np
import jax
import jax.numpy as jnp
import jax.experimental.pallas as pl
import jax.experimental.pallas.tpu as pltpu

F32 = jnp.float32
BF16 = jnp.bfloat16
U32 = jnp.uint32

S = 2048
D = 640
FF = 1728
NC = D // 128
R = 4
P = 128 * R
NA = S // P
TS = 256
NT = S // TS
LEAD = 16
EPS = 1e-5
NEST = (1, 4, 0, 3, 5, 6)
NQ = len(NEST)
FT = (FF - 1536) // 2


def _freq(row):
    t, part, s = row >> 4, (row >> 3) & 1, row & 7
    return 32 * (t & 7) + 4 * s + 2 * (t >> 3) + 1, P * part


def _cos(j, scale):
    jf = (j & (4 * P - 1)).astype(F32)
    u = 2.0 * np.pi / (4 * P)
    x = jnp.abs(jf * u - np.pi) - 0.5 * np.pi
    x2 = x * x
    poly = scale / 362880.0 - x2 * (scale / 39916800.0)
    for coef in (-1.0 / 5040.0, 1.0 / 120.0, -1.0 / 6.0, 1.0):
        poly = poly * x2 + coef * scale
    return poly * x


_DUR = {"t": 8, "u": 16, "k": 16, "i": 16, "m": 12, "g": 0, "c": 0, "j": 16}
_POST = {"t": 8.0, "u": 16.0, "k": 24.0, "i": 4.0, "j": 4.0, "m": 18.0}


def _plan_tokens(order, maxutil):
    lag, cap, pre, margin = 8, 62, 4, 3
    start, slots = {}, []
    for n in order:
        start[n] = len(slots)
        slots += [(n, r) for r in range(_DUR[n[0]])]
    nslot = len(slots) + lag
    free = [cap - (_POST[slots[i - lag][0][0]] if i >= lag else 0.0) for i in range(-pre, nslot)]
    units = []
    for n in order:
        kind, a, c = n
        if kind == "u":
            units += [(n + (g,), 94.0, start[n], -pre) for g in range(8)]
        elif kind == "g":
            units += [(n + (g,), 150.0, start[n], -pre) for g in range(8)]
        elif kind in "ic":
            src_ = [start[m] for m in (("u", a, c), ("k", a, c)) if m in start]
            for t in range(16):
                rel = max(max(src_) + 16, max(src_) + t + lag + 3) if src_ else -pre
                units.append((n + (t,), 32.0 * a + 48.0, nslot if kind == 'c' else start[n], rel))

    def simulate(util):
        left = [u[1] for u in units]
        done = [None] * len(units)
        for i in range(-pre, nslot):
            budget = util * free[i + pre]
            for j, u in enumerate(units):
                if budget <= 0.0:
                    break
                if done[j] is None and u[3] <= i:
                    use = min(budget, left[j])
                    left[j] -= use
                    budget -= use
                    if left[j] <= 1e-9:
                        done[j] = i + 1
        ok = all(u[2] < 8 or (d is not None and d <= max(u[2] - (1 if u[0][0] in 'cg' else margin), u[3] + 1))
                 for d, u in zip(done, units))
        return done, ok

    lo_, hi_ = 0.05, maxutil
    for _ in range(12):
        mid = 0.5 * (lo_ + hi_)
        if simulate(mid)[1]:
            hi_ = mid
        else:
            lo_ = mid
    done, _ = simulate(hi_)
    plan = {}
    for u, d in zip(units, done):
        if u[0][0] == "c":
            plan[u[0]] = slots[max((nslot - 1 if d is None else min(d, nslot - 1)) - lag, 0)]
        elif d is not None and 0 <= d < u[2]:
            plan.setdefault(slots[d], []).append(u[0])
    return plan


def _pack(x):
    return pltpu.bitcast(x.astype(BF16), U32)


def _unpack(w):
    return pltpu.bitcast(w, BF16)


def _dot(a, b):
    return jnp.dot(a.astype(BF16), b, preferred_element_type=F32)


def _dot_nt(a, b):
    return jax.lax.dot_general(a.astype(BF16), b, (((1,), (1,)), ((), ())), preferred_element_type=F32)


def _dot_fine(x, w, chunk):
    if not chunk:
        return _dot(x, w)
    n = w.shape[1]
    head = _dot(x, w[:, :n - 128])
    last = jnp.concatenate([_dot(x[r:r + chunk], w[:, n - 128:]) for r in range(0, x.shape[0], chunk)], axis=0)
    return jnp.concatenate([head, last], axis=1)


def _rows2(x):
    n, c = x.shape
    x = x.reshape(n // 32, 2, 16, c)
    return x[:, 0].reshape(n // 2, c), x[:, 1].reshape(n // 2, c)


def _unrows2(top, bot):
    n, c = top.shape
    return jnp.stack([top.reshape(n // 16, 16, c), bot.reshape(n // 16, 16, c)], axis=1).reshape(2 * n, c)


def _sums_a(a11, a12, a21, a22):
    return [a11 + a22, a21 + a22, a11 + a12, a21 - a11, a12 - a22]


def _sums_b(b11, b12, b21, b22):
    return [b11 + b22, b12 - b22, b21 - b11, b11 + b12, b21 + b22]


_STRASSEN = ((0, 0), (1, 5), (5, 1), (6, 2), (2, 6), (3, 3), (4, 4))


_SUMS_A = ((0, 3, 1), (2, 3, 1), (0, 1, 1), (2, 0, -1), (1, 3, -1))
_SUMS_B = ((0, 3, 1), (1, 3, -1), (2, 0, -1), (0, 1, 1), (2, 3, 1))


def _combine(m1, m2, m3, m4, m5, m6, m7):
    return (m1 + m4) + (m7 - m5), m3 + m5, m2 + m4, (m1 - m2) + (m3 + m6)


def _lo(w):
    return pltpu.bitcast(w << 16, F32)


def _hi(w):
    return pltpu.bitcast(w & jnp.uint32(0xFFFF0000), F32)


def _ln(x, eps=EPS):
    m = jnp.sum(x, axis=-1, keepdims=True) * (1.0 / D)
    xc = x - m
    v = jnp.sum(xc * xc, axis=-1, keepdims=True) * (1.0 / D)
    return xc * jnp.exp(-0.5 * jnp.log(v + eps))


def _gelu2(x):
    c0 = 0.7978845608028654
    c1 = c0 * 0.044715
    return x + x * jnp.tanh(x * (c0 + c1 * (x * x)))


def _bfly(tr, ti):
    s02r, s02i = tr[0] + tr[2], ti[0] + ti[2]
    d02r, d02i = tr[0] - tr[2], ti[0] - ti[2]
    s13r, s13i = tr[1] + tr[3], ti[1] + ti[3]
    d13r, d13i = tr[1] - tr[3], ti[1] - ti[3]
    x0r, x0i = s02r + s13r, s02i + s13i
    x2r, x2i = s02r - s13r, s02i - s13i
    return [x0r, d02r + d13i, x2r, d02r - d13i], [x0i, d02i - d13r, x2i, d02i + d13r]


def _kernel(q_hbm, k_hbm, v_hbm, shift_hbm, ssmk_hbm, ssmd_hbm, w1_hbm, w2_hbm, w3t_hbm, w4_hbm,
            c_hbm, wmod_hbm,
            out_hbm,
            kbuf, vbuf, skbuf, fwdbuf, invbuf, permbuf,
            wmodbuf, w1buf, w2buf, w3buf, w4buf, qbuf,
            xs0, xs1, xs2, xs3, xs4, kraw, wbuf, zbuf, coefbuf, ybuf, modbuf, x2buf, hbuf, hhbuf, xnbuf, xsbuf,
             w1s, w2s, w3s, w3ts, w4s, hba, hbb, w4n, w4q, obuf, shiftbuf, dbuf, cbuf,
            zsm, sem_in, sem_out):
    cps = {}
    n_sem = [0]

    def start(name, src, dst):
        cp = pltpu.make_async_copy(src, dst, sem_in.at[n_sem[0]])
        n_sem[0] += 1
        cp.start()
        cps[name] = cp

    class Both:
        def __init__(self, a, b):
            self.cps = (a, b)

        def wait(self):
            for cp in self.cps:
                cp.wait()

    def start_w(name, src, dst, c0=0, n=NC):
        for e in range(2):
            start(name + str(e), src.at[:, e, pl.ds(c0, n)], dst.at[:, pl.ds(c0, n), pl.ds(8 * e, 8), :])
        cps[name] = Both(cps[name + "0"], cps[name + "1"])

    CH = P * NC
    HALO = 8 * NC

    def start_s(a):
        cols = pl.ds(a * P, P)
        start("s%d" % a, ssmk_hbm.at[:, cols], skbuf.at[:, cols])

    def start_kv(a):
        if a == 0:
            kbuf[0, pl.ds(0, HALO + 8), :] = jnp.zeros((HALO + 8, 128), BF16)
            start("k0", k_hbm.at[pl.ds(0, CH), :], kbuf.at[0, pl.ds(HALO, CH), :])
        else:
            start("k%d" % a, k_hbm.at[pl.ds(a * CH - HALO, CH + HALO), :], kbuf.at[a, pl.ds(0, CH + HALO), :])
        start("v%d" % a, v_hbm.at[pl.ds(a * CH, CH), :], vbuf.at[a, pl.ds(0, CH), :])

    for n in "s0 x0 s1 k0 k1 s2 k2 s3 k3".split():
        if n[0] == "s":
            start_s(int(n[1]))
        elif n[0] == "k":
            start_kv(int(n[1]))
        else:
            start("d", ssmd_hbm, dbuf)
            start("shift", shift_hbm, shiftbuf)
            start("c", c_hbm, cbuf)
    QA = TS + LEAD
    XA = 128
    QB = 2 * TS + LEAD
    W1A = 2

    def start_q(name, r0, n):
        start(name, q_hbm.at[pl.ds(r0, n), :], qbuf.at[pl.ds(r0, n), :])

    start_q("qa", 0, QA)
    start_w("wmoda", wmod_hbm, wmodbuf, 0, 3 * NC)
    start_w("wmodb", wmod_hbm, wmodbuf, 3 * NC, 2 * NC)
    start_q("qx", QA, XA)
    start_w("w1a", w1_hbm, w1buf, 0, W1A)
    start_w("w1b", w1_hbm, w1buf, W1A, NC - W1A)
    start_q("qb", QA + XA, QB - QA - XA)
    start_w("w2", w2_hbm, w2buf)
    start_w("w3", w3t_hbm, w3buf)
    start_w("w4", w4_hbm, w4buf)
    start_w("wmodg", wmod_hbm, wmodbuf, 5 * NC, NC)
    start_q("q1", QB, S - QB)

    kw = kbuf.bitcast(U32)
    vw = vbuf.bitcast(U32)
    zbuf[...] = jnp.zeros(zbuf.shape, U32)
    for j in range(64):
        zsm[j] = 0
    for c in range(NC):
        ybuf[c, pl.ds(S, LEAD), :] = jnp.zeros((LEAD, 128), F32)
        hhbuf[c, pl.ds(0, 8), :] = jnp.zeros((8, 128), F32)
    qbuf[pl.ds(S, LEAD), :] = jnp.zeros((LEAD, D), BF16)

    def tables(p, carry):
        i0 = jax.lax.broadcasted_iota(jnp.int32, (128, 128), 0)
        n = R * jax.lax.broadcasted_iota(jnp.int32, (128, 128), 1) + p
        f2, off = _freq(2 * i0)
        j = f2 * n + off
        fwdbuf[p] = pltpu.pack_elementwise([_cos(j, 1.0), _cos(j + 4 * n, 1.0)], packed_dtype=BF16)
        return carry

    jax.lax.fori_loop(0, R, tables, 0)

    def unit_g(kt, r):
        col = jax.lax.broadcasted_iota(jnp.int32, (8, 128), 1) + 128 * kt
        f2, off = _freq((col & ~15) + 8 * (col & 1) + ((col >> 1) & 7))
        m = 2 * jax.lax.broadcasted_iota(jnp.int32, (8, 128), 0) + 16 * r
        j0 = f2 * (R * m) + off
        out = []
        for p in range(R):
            j = j0 + p * f2
            out.append(pltpu.pack_elementwise([_cos(j, 1.0 / P), _cos(j + R * f2, 1.0 / P)], packed_dtype=BF16))
            invbuf[p, pl.ds(8 * r, 8), pl.ds(128 * kt, 128)] = out[-1]
        return out

    i0 = jax.lax.broadcasted_iota(jnp.int32, (128, 128), 0)
    i1 = jax.lax.broadcasted_iota(jnp.int32, (128, 128), 1)
    permbuf[...] = _pack(jnp.where(i0 == (128 // R) * (i1 & (R - 1)) + (i1 >> 2), 1.0, 0.0).astype(F32))

    def fill_coef():
        cv = cbuf[...].astype(F32)
        modbuf[6] = jnp.broadcast_to(cv * jax.nn.sigmoid(cv), (8, D))
        coef = shiftbuf[...].astype(F32)
        dval = dbuf[...].astype(F32)
        for c in range(NC):
            for j in range(4):
                coefbuf[c, j] = jnp.broadcast_to(coef[j:j + 1, c * 128:(c + 1) * 128], (8, 128))
            coefbuf[c, 4] = jnp.broadcast_to(dval[c:c + 1, :], (8, 128))

    xs = (xs0, xs1, xs2, xs3, xs4)
    wsbufs = dict(w1=w1s, w2=w2s, w3=w3s, w4=w4s, w3t=w3ts)
    def split_ri(t):
        t = t.reshape(16, 2, 8, 128)
        return t[:, 0], t[:, 1]

    def get_never():
        return zbuf[pl.ds(0, 8), :] != 0

    def pack2(x, y):
        return pltpu.pack_elementwise([x, y], packed_dtype=BF16)

    UG = 8

    def unit_u(a, c, g0):
        c0, c1, c2, c3 = (coefbuf[c, pl.ds(j, 1)][None] for j in range(4))
        rows = lambda ref, r: ref[a, pl.ds((r // 4) * 4 * NC + 4 * c + r % 4, 8 * UG, stride=4 * NC), :]
        kk = jnp.stack([rows(kw, 4 + 32 * g0 + d) for d in range(-2, 4)]).reshape(6, UG, 8, 128)
        vv = jnp.stack([rows(vw, 32 * g0 + d) for d in range(4)]).reshape(4, UG, 8, 128)
        lo, hi = _lo(kk), _hi(kk)
        k0, k1, k2 = lo[2:], hi[1:5], lo[1:5]
        even = ((k0 * c0 + k1 * c1) + (k2 * c2 + hi[:4] * c3)) * _lo(vv)
        odd = ((hi[2:] * c0 + k0 * c1) + (k1 * c2 + k2 * c3)) * _hi(vv)
        e, o = pack2(even[:2], even[2:]).reshape(-1, 128), pack2(odd[:2], odd[2:]).reshape(-1, 128)
        n = 8 * UG
        return [e[:n], o[:n], e[n:], o[n:]]

    def unit_i(a, c, t0, z):
        x_c = xs[c].at[pl.ds(z, NA)]
        ts = pl.ds(t0, UG)
        yr = yi = None
        for j in range(a + 1):
            ur, ui = x_c[j, :, ts, 0], x_c[j, :, ts, 1]
            kr, ki = x_c[a - j, :, ts, 2], x_c[a - j, :, ts, 3]
            pr = ur * kr - ui * ki
            pi = ur * ki + ui * kr
            yr = pr if yr is None else yr + pr
            yi = pi if yi is None else yi + pi
        halves = lambda x: (x[:x.shape[0] // 2], x[x.shape[0] // 2:])
        (ra, rb), (ia, ib) = halves(yr.reshape(-1, 128)), halves(yi.reshape(-1, 128))
        (sr0, sr1), (si0, si1), (dr0, dr1), (di0, di1) = (halves(x) for x in (ra + rb, ia + ib, ra - rb, ia - ib))
        return [pack2(sr0 + sr1, si0 + si1), pack2(dr0 - di1, di0 + dr1),
                pack2(sr0 - sr1, si0 - si1), pack2(dr0 + di1, di0 - dr1)]

    def segment(spec, z, maxutil=1.0, mod_fn=None):
        order = [(n[0], int(n[1]), int(n[2])) for n in spec.split()]
        plan = _plan_tokens(order, maxutil) if maxutil > 0 else {}
        never = get_never()
        units, groups, res = {}, {}, {}

        def group(key):
            kind, a, c, j = key
            key = (kind, a, c, j - j % UG)
            if key not in groups:
                if kind == "u":
                    groups[key] = unit_u(a, c, key[3])
                else:
                    fresh = ("u", a, c) in order or ("k", a, c) in order
                    groups[key] = unit_i(a, c, key[3], z if fresh else 0)
            return groups[key]

        def unit(key):
            if key not in units:
                r = 8 * (key[3] % UG)
                units[key] = unit_g(key[1], key[3]) if key[0] == "g" else [v[r:r + 8] for v in group(key)]
            return units[key]

        def lhs(name, p, full, r0=0):
            out, last = [], 0
            for r in range(full.shape[0] // 8):
                keys = plan.get((name, r0 + r), ())
                if keys:
                    if 8 * r > last:
                        out.append(full[last:8 * r])
                    v = full[8 * r:8 * r + 8]
                    for key in keys:
                        v = jax.lax.select(never, unit(key)[p], v)
                    out.append(v)
                    last = 8 * r + 8
            if last < full.shape[0]:
                out.append(full[last:] if last else full)
            return out[0] if len(out) == 1 else jnp.concatenate(out, axis=0)

        def dft(name, rhs):
            tr, ti = [], []
            for p in range(R):
                f = lhs(name, p, fwdbuf[p])
                r_, i_ = split_ri(_dot(_unpack(f), rhs[p]))
                if p == 0:
                    res.update({(name, r): (lambda r=r, v=r_: v[r]) for r in range(16)})
                tr.append(r_)
                ti.append(i_)
            return _bfly(tr, ti)

        st = {}
        for name in order:
            kind, a, c = name
            x_c = xs[c]
            if kind == "g":
                for r in range(8):
                    unit(name + (r,))
            elif kind == "c":
                for t in range(16):
                    after = pltpu.bitcast(res[plan[name + (t,)]](), U32)
                    for p in range(R):
                        wbuf[c, p, pl.ds(8 * t, 8), :] = jax.lax.select(never, after, unit(name + (t,))[p])
            elif kind == "m":
                toks = {}
                for r in range(_DUR["m"]):
                    for n_, key in enumerate(plan.get((name, r), ())):
                        toks.setdefault(2 * r + n_ % 2, []).extend(unit(key))
                mod_fn(a, toks)
            elif kind == "t":
                trs = []
                for b in range(R):
                    pm = lhs(name, b, permbuf[...])
                    trs.append(_dot_nt(_unpack(pm), skbuf[pl.ds(c * 128, 128), pl.ds(a * P + b * 128, 128)]))
                res.update({(name, r): (lambda r=r, v=trs[0]: v[16 * r:16 * r + 8]) for r in range(8)})
                g_ = 128 // R
                st[a, c] = [jnp.concatenate([trs[b][p * g_:(p + 1) * g_] for b in range(R)], axis=0).astype(BF16)
                            for p in range(R)]
            elif kind == "u":
                rhs = [_unpack(jnp.concatenate([group(name + (g,))[p] for g in range(0, 8, UG)], axis=0)) for p in range(R)]
                xr, xi = dft(name, rhs)
                for q in range(R):
                    x_c[a, q, :, 0] = xr[q]
                    x_c[a, q, :, 1] = xi[q]
            elif kind == "k":
                xr, xi = dft(name, st[a, c])
                for q in range(R):
                    if a == 0:
                        x_c[a, q, :, 2] = xr[q] + coefbuf[c, 4]
                        x_c[a, q, :, 3] = xi[q]
                    else:
                        pr, pi = kraw[c, (a - 1) % 2, q, :, 0], kraw[c, (a - 1) % 2, q, :, 1]
                        x_c[a, q, pl.ds(0, 8), 2] = xr[q][:8] - pi[:8]
                        x_c[a, q, pl.ds(0, 8), 3] = xi[q][:8] + pr[:8]
                        x_c[a, q, pl.ds(8, 8), 2] = xr[q][8:] + pi[8:]
                        x_c[a, q, pl.ds(8, 8), 3] = xi[q][8:] - pr[8:]
                    if a + 1 < NA:
                        kraw[c, a % 2, q, :, 0] = xr[q]
                        kraw[c, a % 2, q, :, 1] = xi[q]
            else:
                for p in range(R):
                    cols = [lhs(name, 2 * (p % 2) + kt,
                                invbuf[p, :, pl.ds(128 * kt, 128)], 8 * (p // 2))
                            for kt in range(2)]
                    g = _unpack(jnp.concatenate(cols, axis=1))
                    if kind == "j":
                        wp = _unpack(wbuf[c, p])
                    else:
                        wp = _unpack(jnp.concatenate([group(name + (t,))[p] for t in range(0, 16, UG)], axis=0))
                    yp = _dot(g, wp)
                    if p % 2 == 0:
                        res.update({(name, 4 * p + r): (lambda r=r, v=yp: v[16 * r:16 * r + 8]) for r in range(8)})
                    ybuf[c, pl.ds(a * P + p, 128, stride=R), :] = yp

    one = jnp.minimum(pl.program_id(0) + 1, 1)

    def once(fn):
        def body(z, carry):
            fn(z)
            return carry
        jax.lax.fori_loop(0, one, body, 0)

    default = ("t00 t01 t02 k00 t03 k01 t04 k02 k03 k04 g00|"
               "t10 t11 t12 k10 k11 k12 g10|"
               "t13 t14 k13 u00 k14 u01 u02 u03 i00 u04 i01 c02 c03|"
               "j02 j03 u10 i04 u11 u12 u13 i10 u14 i11 c12 c13|"
               "t20 t21 j12 t22 j13 t23 t24 k20 u20 k21 u21 k22 i14 k23 u22 k24 u23 i20 u24 i21 c22|"
               "t30 t31 j22 t32 t33 t34 k30 u30 k31 u31 k32 i23 k33 u32 k34 i24 u33 i30 u34 i31 c32|"
               "m00 j32 m10 i33 m20 i34")
    specs = default.split("|")
    G5B = specs[-1]
    segs = list(zip("s0 d shift c|s1|k0 v0|k1 v1|s2 k2 v2|s3 k3 v3".split("|"), specs[:-1]))
    MU = 1.5
    for i, (waits, spec) in enumerate(segs):
        with jax.named_scope("g%d" % i):
            for n in waits.split():
                cps[n].wait()
            if i == 0:
                fill_coef()
            once(lambda z: segment(spec, z, MU))

    def mod_cols(lo, n, toks=None):
        m = _dot(modbuf[6], weights(wmodbuf, lo * NC, (lo + n) * NC, toks=toks))
        return [m[:, j * D:(j + 1) * D] for j in range(n)]

    def mul_mod(x, j, cols=None):
        m = modbuf[j] if cols is None else modbuf[j, :, cols]
        return (x.reshape(-1, 8, x.shape[-1]) * m[None]).reshape(x.shape)

    def add_mod(x, j):
        return (x.reshape(-1, 8, x.shape[-1]) + modbuf[j][None]).reshape(x.shape)

    def slabs(ref, r0, n):
        return jnp.concatenate([ref[c, pl.ds(r0, n), :] for c in range(NC)], axis=1)

    def put(ref, rows, x):
        for c in range(NC):
            ref[c, rows, :] = x[:, c * 128:(c + 1) * 128]

    def parity(ref, r0, n, e):
        return jnp.concatenate([ref[c, pl.ds(r0 + e, n // 2, stride=2), :] for c in range(NC)], axis=1)

    def window(base, n):
        rows = pl.ds(base, n)
        return dict(q=qbuf.at[rows, :], y=ybuf.at[:, rows, :], x2=x2buf.at[rows, :], h=hbuf.at[:, rows, :],
                    hh=hhbuf.at[:, pl.ds(base, n + 8), :],
                    o=obuf.at[pl.ds(base, n - LEAD), :])

    def weights(ref, c0=0, c1=NC, r0=0, r1=None, toks=None, raw=False, z=None):
        r1 = 16 * ref.shape[0] if r1 is None else r1
        view = ref.bitcast(U32)
        if z is not None:
            view = view.at[pl.ds(z, ref.shape[0])]
        never = get_never() if toks else None
        rt = -(-(r1 - r0) // 128)
        cols = []
        for j in range(c0, c1):
            wu = view[pl.ds(r0 // 16, (r1 - r0) // 16), j].reshape((r1 - r0) // 2, 128)
            if toks:
                parts, last = [], 0
                for i in range(rt):
                    for n_, t in enumerate(toks.get((j - c0) * rt + i, ())):
                        r = 64 * i + 8 * n_
                        if r > last:
                            parts.append(wu[last:r])
                        parts.append(jax.lax.select(never, t, wu[r:r + 8]))
                        last = r + 8
                parts.append(wu[last:])
                wu = jnp.concatenate(parts, axis=0)
            cols.append(wu)
        wu = jnp.concatenate(cols, axis=1)
        return wu if raw else _unpack(wu)

    def wblocks(name, j, z=None):
        if name == "w3":
            blk = lambda kh, nh: weights(w3buf, 2 * kh, 2 * kh + 2, 128 * (j + 6 * nh), 128 * (j + 6 * nh + 1), raw=True, z=z)
        elif name == "w4":
            def blk(kh, nh):
                c = j + 2 * nh
                parts = [weights(w4buf, c, c + 1, 768 * kh, 768 * (kh + 1), raw=True, z=z),
                         weights(w4buf, c, c + 1, 1536 + FT * kh, 1536 + FT * (kh + 1), raw=True, z=z),
                         jnp.zeros(((128 - FT) // 2, 128), U32)]
                return jnp.concatenate(parts, axis=0)
        elif name == "w3t":
            blk = lambda kh, nh: weights(w3buf, 2 * kh, 2 * kh + 2, 1536 + FT * nh, 1536 + FT * (nh + 1), raw=True, z=z)
        else:
            ref = w1buf if name == "w1" else w2buf
            blk = lambda kh, nh: weights(ref, j + 2 * nh, j + 2 * nh + 1, 256 * kh, 256 * (kh + 1), raw=True, z=z)
        return blk

    def wsum(name, j, k):
        blk = wblocks(name, j, zsm[k])
        p, q, sign = _SUMS_B[k]
        return psum(blk(p // 2, p % 2), blk(q // 2, q % 2), sign)

    pending = []

    def attach(wv):
        if not pending:
            return wv
        never = get_never()
        rows = [wv[8 * i:8 * i + 8, :128] for i in range(8)]
        for i, t in enumerate(pending):
            rows[i % 8] = jax.lax.select(never, pltpu.bitcast(t, U32), rows[i % 8])
        pending.clear()
        first = jnp.concatenate(rows + ([wv[64:, :128]] if wv.shape[0] > 64 else []), axis=0)
        return first if wv.shape[1] == 128 else jnp.concatenate([first, wv[:, 128:]], axis=1)

    def sprods(name, j, lhs, k0=0, k1=7, prep=False):
        blk, buf = wblocks(name, j), wsbufs[name]
        out = []
        for ia, ib in _STRASSEN[k0:k1]:
            wv = blk(ib - 5, ib - 5) if ib >= 5 else (wsum(name, j, ib) if prep else buf[ib, j])
            if name == "w3t":
                out.append(_dot_nt(_unpack(wv), lhs(ia)))
            else:
                out.append((_dot_nt if name == "w3" else _dot)(lhs(ia), _unpack(attach(wv))))
            if prep and ib < 5:
                buf[ib, j] = wv
        return out

    def spair(name, j, lhs, prep=False):
        return _combine(*sprods(name, j, lhs, prep=prep))

    def dd_rest(name, t, b):
        ref = w1buf if name == "w1" else w2buf
        m = t.shape[0]
        xb = jnp.concatenate([t, b], axis=0)
        last = _dot(xb, weights(ref, 4, 5))
        rem = _dot(xb[:, 512:], weights(ref, 0, 4, r0=512))
        return t, b, rem[:m], rem[m:], last[:m], last[m:]

    def dd_main(name, parts, prep=False):
        t, b, rt, rb, lt, lb = (jnp.concatenate(v, axis=0) for v in zip(*parts))
        ops = _sums_a(t[:, :256], t[:, 256:512], b[:, :256], b[:, 256:512]) + [t[:, :256], b[:, 256:512]]
        top, bot = [None] * 4, [None] * 4
        for j in range(2):
            top[j], top[j + 2], bot[j], bot[j + 2] = spair(name, j, lambda i: ops[i], prep)
        return (jnp.concatenate([jnp.concatenate(top, axis=1) + rt, lt], axis=1),
                jnp.concatenate([jnp.concatenate(bot, axis=1) + rb, lb], axis=1))

    def stage_a0(w, r0, n):
        rows = pl.ds(r0, n)
        x = w["q"][rows, :].astype(F32)
        x2 = x + add_mod(mul_mod(_ln(x), 1), 0) * slabs(w["y"], r0, n)
        w["x2"][rows, :] = x2
        return _ln(x2)

    def stage_a1(w, r0, n, n2=None, f32=False):
        if n2 is None:
            n2 = stage_a0(w, r0, n)
        h = add_mod(mul_mod(n2, 4), 3)
        put(w["h"], pl.ds(r0, n), h)
        n3 = _ln(h, 4 * EPS)
        return n3 if f32 else n3.astype(BF16)

    def stage_a2(w, n3, r0, n, last_valid=None, fine=0, c0=0, c1=NC, prep=False):
        hh = _gelu2(_unrows2(*dd_main("w1", n3, prep)) if isinstance(n3, list) else _dot_fine(n3, weights(w1buf, c0, c1), fine))
        for c in range(c0, c1):
            blk = hh[:, (c - c0) * 128:(c - c0 + 1) * 128]
            w["hh"][c, pl.ds(r0 + 8, n - LEAD), :] = blk[:n - LEAD]
            tail = blk[n - LEAD:]
            if last_valid is not None:
                tail = jnp.where(last_valid, tail, 0.0)
            w["hh"][c, pl.ds(r0 + 8 + n - LEAD, LEAD), :] = tail

    def stage_b1a(w, r0, n, prep=False):
        m = n // 2
        lane = jax.lax.broadcasted_iota(jnp.int32, (m, 128), 1)
        g = []
        for e in range(2):
            sh = lambda c, d: w["hh"][c, pl.ds(r0 + 8 + e + d, m, stride=2), :]
            g.append(jnp.concatenate([sh(0, -1),
                                      jnp.where(lane < 32, sh(1, -1), sh(1, 1)),
                                      jnp.where(lane < 64, sh(2, 1), sh(2, -2)),
                                      jnp.where(lane < 96, sh(3, -2), sh(3, 2)),
                                      sh(4, 2)], axis=1))
        hs = dd_main("w2", [dd_rest("w2", *g)], prep)
        x1 = [parity(w["h"], r0, n, e) + hs[e] for e in range(2)]
        for e in range(2):
            put(w["h"], pl.ds(r0 + e, m, stride=2), x1[e])
        return x1

    def stage_b1b(w, x1, r0, n):
        xn = jnp.stack([_ln(x, 4 * EPS).reshape(n // 16, 8, D) for x in x1], axis=1).reshape(n, D)
        t, b = _rows2(xn)
        xnbuf[0, pl.ds(r0 // 2, n // 2), :] = t.astype(BF16)
        xnbuf[1, pl.ds(r0 // 2, n // 2), :] = b.astype(BF16)
        sa = _sums_a(t[:, :256], t[:, 256:512], b[:, :256], b[:, 256:512])
        xsbuf[pl.ds(r0 // 2, n // 2), :] = jnp.concatenate(sa, axis=1).astype(BF16)

    def out_copy(r0, n):
        rows = pl.ds(r0, n)
        return pltpu.make_async_copy(obuf.at[rows, :], out_hbm.at[rows, :], sem_out.at[0])


    def opaque(ref, i):
        return ref.at[:, :, pl.ds(pl.multiple_of(zsm[i] * 32, 32), ref.shape[2]), :]

    def packrows(v):
        v = v.reshape(v.shape[0] // 16, 2, 8, 128)
        return pack2(v[:, 0], v[:, 1]).reshape(-1, 128)

    def emit(h3, j, left, right):
        m = left.shape[0] // 2
        g = [left[:m], right[:m], left[m:], right[m:]]
        for k, v in enumerate(_sums_a(*g) + g):
            h3[j, k, pl.ds(0, m // 2), :] = packrows(v)

    def load_xn(w, r0, n):
        return xnbuf[:, pl.ds(r0 // 2, n // 2), :].reshape(n, D)

    def w3_operands(w, r0, n):
        xn = load_xn(w, r0, n)
        xsum = xsbuf[pl.ds(r0 // 2, n // 2), :]
        m = n // 2
        return xn, [xsum[:, 256 * k:256 * (k + 1)] for k in range(5)] + [xn[:m, :256], xn[m:, 256:512]]

    def stage_b2h(w, h3, r0, n, prep=False):
        xn, ops = w3_operands(w, r0, n)
        m = n // 2
        rem = _dot_nt(weights(w3buf, 4, 5, r0=1536), xn[:, 512:])
        c11, c12, c21, c22 = spair("w3t", 0, lambda i: ops[i], prep)
        pad = jnp.zeros((128 - FT, m), F32)
        g11, g12, g21, g22 = (jnp.concatenate([_gelu2(c + r), pad], axis=0).T for c, r in (
            (c11, rem[:FT, :m]), (c12, rem[FT:, :m]), (c21, rem[:FT, m:]), (c22, rem[FT:, m:])))
        emit(h3, 6, jnp.concatenate([g11, g21], axis=0), jnp.concatenate([g12, g22], axis=0))

    def stage_b2a(w, h3, r0, n, lo=0, hi=6, prep=False):
        xn, ops = w3_operands(w, r0, n)
        for j in range(lo, hi):
            r1, r2 = (_dot_nt(xn[:, 512:], weights(w3buf, 4, 5, 128 * t, 128 * (t + 1))) for t in (j, j + 6))
            c11, c12, c21, c22 = spair("w3", j, lambda i: ops[i], prep)
            emit(h3, j, _gelu2(jnp.concatenate([c11, c21], axis=0) + r1), _gelu2(jnp.concatenate([c12, c22], axis=0) + r2))

    def finish(w, h2, r0, n, c):
        nc = h2.shape[1] // 128
        rows, cols = pl.ds(r0, n), pl.ds(c * 128, nc * 128)
        x1 = jnp.concatenate([w["h"][c + i, rows, :] for i in range(nc)], axis=1)
        w["o"][rows, cols] = (w["x2"][rows, cols] + mul_mod(x1 + h2, 5, cols)).astype(BF16)

    def b2_done(w, done, r0, n):
        if len(done[0]) == len(done[1]) == 7:
            c11, c12, c21, c22 = _combine(*[jnp.concatenate([done[0][k], done[1][k]], axis=1) for k in range(7)])
            finish(w, _unrows2(c11, c21), r0, n, 0)
            finish(w, _unrows2(c12, c22), r0, n, 2)

    def stage_b2b(w, h3, r0, n, j, k0=0, k1=7, done=None, prep=False, sub=0, marks=()):
        hv = opaque(h3, j)
        blk = lambda k: jnp.concatenate([hv[p, k, pl.ds(sub // 4, n // 4), :] for p in range(7)], axis=1)
        r0 += sub
        if j < 2:
            for k in range(k0, k1):
                if k not in NEST:
                    done[j][k] = sprods("w4", j, lambda i: _unpack(blk(8 if i == 6 else i)), k, k + 1, prep)[0]
                    b2_done(w, done, r0, n)
            return
        wb = wblocks("w4", 4)
        lhs = jnp.concatenate([jnp.concatenate([blk(5), blk(6)], axis=1),
                               jnp.concatenate([blk(7), blk(8)], axis=1)], axis=0)
        if marks:
            lo_, hi_ = 0, 52
            never, at = get_never(), {}
            for i, mk in enumerate(marks):
                s_ = lo_ + (hi_ - lo_) * i // len(marks)
                at[4 * (s_ // 16), s_ % 16] = mk
            cols = []
            for kt in range(14):
                col = lhs[:, 128 * kt:128 * (kt + 1)]
                if any(k_[0] == kt for k_ in at):
                    col = jnp.concatenate([jax.lax.select(never, at[kt, r], col[8 * r:8 * r + 8]) if (kt, r) in at
                                           else col[8 * r:8 * r + 8] for r in range(16)], axis=0)
                cols.append(col)
            lhs = jnp.concatenate(cols, axis=1)
        h2 = _dot(_unpack(lhs), _unpack(jnp.concatenate([wb(0, 0), wb(1, 0)], axis=0)))
        finish(w, _unrows2(h2[:n // 2], h2[n // 2:]), r0, n, 4)


    def psum(x, y, sign):
        if sign > 0:
            return pack2(_lo(x) + _lo(y), _hi(x) + _hi(y))
        return pack2(_lo(x) - _lo(y), _hi(x) - _hi(y))

    def prep_w4(nchunk):
        rows = 384 // nchunk
        marks = []
        for ch in [nchunk] + list(range(nchunk)):
            tail = ch == nchunk
            raw = {}
            for kh in range(2):
                for e in range(1 if tail else 2):
                    r0 = 1536 + FT * kh if tail else 768 * kh + 384 * e + rows * ch
                    x = weights(w4buf, 0, 4, r0, r0 + (FT if tail else rows), raw=True)
                    raw[kh, e] = jnp.stack([_lo(x), _hi(x)])
            blk = lambda i, e: raw[i // 2, e][:, :, 256 * (i % 2):256 * (i % 2 + 1)]
            for k, (ia, ib) in enumerate(_STRASSEN):
                if k not in NEST or ib >= 5:
                    continue
                p_, q_, sg = _SUMS_B[ib]
                half = [blk(p_, e) + blk(q_, e) if sg > 0 else blk(p_, e) - blk(q_, e) for e in range(1 if tail else 2)]
                quad = lambda i: half[i // 2][:, :, 128 * (i % 2):128 * (i % 2 + 1)]
                first = NEST.index(k)
                if tail:
                    for j in range(2):
                        w4q[first, 7, pl.ds(64 * j, FT // 2), :] = pack2(quad(j)[0], quad(j)[1])
                        w4q[first, 7, pl.ds(64 * j + FT // 2, 64 - FT // 2), :] = jnp.zeros((64 - FT // 2, 128), U32)
                    continue
                for jb, v in enumerate(_sums_b(*[quad(i) for i in range(4)]) + [quad(0), quad(3)]):
                    w4q[first, jb, pl.ds(rows // 2 * ch, rows // 2), :] = pack2(v[0], v[1])
            if not tail:
                marks.append(w4q.at[pl.ds(zsm[32 + ch], NQ)][first, 0, pl.ds(0, 8), :])
        return marks

    def stage_b2n(w, h3, r0, n, k, done, prep=False):
        ia, ib = _STRASSEN[k]
        ka, q, slot = (8 if ia == 6 else ia), n // 8, NEST.index(k)

        def lblk(i, z):
            hv = opaque(h3, z)
            return jnp.concatenate([hv[g + 3 * (i % 2), ka, pl.ds((i // 2) * q, q), :] for g in range(3)], axis=1)

        def raw(j, lo, hi, z=None):
            return wblocks("w4", j, z)(ib - 5, ib - 5)[lo:hi]

        quad = lambda i, z=None: raw(i % 2, 192 * (i // 2), 192 * (i // 2 + 1), z)
        if ib >= 5:
            wt = [raw(j, 384, 448) for j in range(2)]
        else:
            wq = w4q.at[pl.ds(zsm[6], NQ)] if prep else w4q
            wt = [wq[slot, 7, pl.ds(64 * j, 64), :] for j in range(2)]
        tail = _dot(_unpack(opaque(h3, 5)[6, ka, pl.ds(0, 2 * q), :]), _unpack(jnp.concatenate(wt, axis=1)))
        ms = []
        for ja, jb in _STRASSEN:
            if ja >= 5:
                lv = lblk(3 * (ja - 5), 5)
            else:
                p_, q_, sg = _SUMS_A[ja]
                lv = psum(lblk(p_, ja), lblk(q_, ja), sg)
            z = zsm[8 + 7 * slot + jb] if prep and ib >= 5 else None
            if ib < 5:
                wv = wq[slot, jb]
            elif jb >= 5:
                wv = quad(3 * (jb - 5), z)
            elif prep:
                p_, q_, sg = _SUMS_B[jb]
                w4n[slot, jb] = wv = psum(quad(p_, z), quad(q_, z), sg)
            else:
                wv = w4n[slot, jb]
            ms.append(_dot(_unpack(lv), _unpack(wv)))
        c11, c12, c21, c22 = _combine(*ms)
        done[0][k] = jnp.concatenate([c11, c21], axis=0) + tail[:, :128]
        done[1][k] = jnp.concatenate([c12, c22], axis=0) + tail[:, 128:]
        b2_done(w, done, r0, n)

    w = window(0, 2 * TS + LEAD)
    H = TS // 2
    with jax.named_scope("t0a"):
        cps["qa"].wait()
        cps["wmoda"].wait()

        mv = {}

        def mod_fn(j, toks):
            mv[j] = mod_cols(j, 1, toks)[0]
            if len(mv) == 3:
                modbuf[0] = mv[2] * mv[0]
                modbuf[1] = mv[2] * (1.0 + mv[1])

        segment(G5B, 0, MU, mod_fn=mod_fn)
        put(w["h"], pl.ds(0, QA), stage_a0(w, 0, QA))
    with jax.named_scope("t0b"):
        cps["wmodb"].wait()
        sb, cb = mod_cols(3, 2)
        modbuf[3] = 2.0 * sb
        modbuf[4] = 2.0 + 2.0 * cb
        n3 = stage_a1(w, 0, QA, n2=slabs(w["h"], 0, QA))
    XB = TS - XA
    with jax.named_scope("t1a"):
        cps["w1a"].wait()
        cps["qx"].wait()
        put(w["h"], pl.ds(QA, XA), stage_a0(w, QA, XA))
        stage_a2(w, n3, 0, QA, c1=W1A, fine=80)
    with jax.named_scope("t1b"):
        cps["w1b"].wait()
        n3a = stage_a1(w, QA, XA, n2=slabs(w["h"], QA, XA), f32=True)
        stage_a2(w, n3, 0, QA, c0=W1A)
        stage_a2(w, [dd_rest("w1", *_rows2(n3a))], QA, XA, prep=True)
    with jax.named_scope("t2"):
        cps["qb"].wait()
        cps["w2"].wait()
        n3b = stage_a1(w, QA + XA, XB, f32=True)
        stage_b1b(w, stage_b1a(w, 0, TS, prep=True), 0, TS)
        stage_a2(w, [dd_rest("w1", *_rows2(n3b))], QA + XA, XB)
        stage_b1b(w, stage_b1a(w, TS, XA), TS, XA)
        stage_b1a(w, TS + XA, XB)
    with jax.named_scope("t3"):
        cps["w3"].wait()
        stage_b1b(w, [parity(w["h"], TS + XA, XB, e) for e in range(2)], TS + XA, XB)
        stage_b2h(w, hba, 0, TS, prep=True)
        stage_b2a(w, hba, 0, TS, prep=True)
        stage_b2h(w, hbb, TS, TS)
        stage_b2a(w, hbb, TS, TS)
    with jax.named_scope("t4"):
        cps["w4"].wait()
        cps["wmodg"].wait()
        done = {0: {}, 1: {}}
        for op in "m4 P m0 4:0:2:3 m2 8:0 m1 8:1 m3 8:3 4:1:2:3 8:6 8:4 8:5".split():
            op, *rng = op.split(":")
            rng = [int(x) for x in rng]
            if op[0] == "m":
                c = int(op[1])
                modbuf[5, :, pl.ds(c * 128, 128)] = 0.5 * _dot(modbuf[6], weights(wmodbuf, 5 * NC + c, 5 * NC + c + 1))
            elif op[0] == "8":
                stage_b2n(w, hba, 0, TS, *rng, done, prep=True)
            elif op[0] == "P":
                stage_b2b(w, hba, 0, TS, 2, marks=prep_w4(24))
            else:
                stage_b2b(w, hba, 0, TS, *rng, done=done, prep=True)
        out_copy(0, TS).start()
        cps["q1"].wait()

    CBS = (128, 128)
    PART = {"a": (TS, TS), "c": (TS, H), "d": (TS + H, H)}
    BODY = "4:2 4:0:2:3 4:1:2:3 8:3 8:0 r0 r1 1a 8:1 2c nc 2d nd 8:6 8:5 8:4 3a:0:2 ha 3a:2:6"

    def step(s, carry):
        r0 = pl.multiple_of(s * TS, TS)
        w = window(r0, 2 * TS + LEAD)
        x1, rest, done = {}, {}, {0: {}, 1: {}}
        for op in BODY.split():
            op, *rng = op.split(":")
            rng = [int(x) for x in rng]
            if op[0] == "3":
                stage_b2a(w, hbb, TS, TS, *rng)
            elif op[0] == "h":
                stage_b2h(w, hbb, TS, TS)
            elif op[0] == "4":
                stage_b2b(w, hbb, 0, TS, *rng, done=done)
            elif op[0] == "8":
                stage_b2n(w, hbb, 0, TS, *rng, done)
            elif op[0] == "2":
                x1[op[1]] = stage_b1a(w, *PART[op[1]])
            elif op[0] == "n":
                stage_b1b(w, x1[op[1]], *PART[op[1]])
            elif op[0] == "r":
                j = int(op[1])
                rest[j] = dd_rest("w1", *_rows2(stage_a1(w, TS + LEAD + sum(CBS[:j]), CBS[j], f32=True)))
            else:
                ra, n = PART[op[1]]
                parts = [rest[j] for j in range(len(CBS)) if ra - TS <= sum(CBS[:j]) < ra - TS + n]
                stage_a2(w, parts, ra + LEAD, n, last_valid=(s < NT - 2) if ra + n == 2 * TS else None)
        out_copy(r0, TS).start()
        return carry

    with jax.named_scope("p2main"):
        jax.lax.fori_loop(1, NT - 1, step, 0)
    with jax.named_scope("p2epi"):
        w = window(S - 2 * TS, 2 * TS + LEAD)
        rows = pl.ds(S - TS, TS)
        pending.append(hhbuf[0, pl.ds(S, 8), :])
        def flush(rows, cols):
            pltpu.make_async_copy(obuf.at[rows, cols], out_hbm.at[rows, cols], sem_out.at[0]).start()

        done = {0: {}, 1: {}}
        for j in range(2):
            stage_b2b(w, hbb, TS, TS, j, done=done)
        for k in NEST:
            stage_b2n(w, hbb, TS, TS, k, done)
        flush(rows, pl.ds(0, 512))
        sub = 0
        for n in (128, 64, 64):
            stage_b2b(w, hbb, TS, n, 2, sub=sub)
            flush(pl.ds(S - TS + sub, n), pl.ds(512, 128))
            sub += n
        pltpu.make_async_copy(obuf, out_hbm, sem_out.at[0]).wait()


@jax.jit
def pallas_adaLN_cond__ssm_conv_h3__mixer_s_mlp__prompt_kernel(
    A_q: jax.Array,
    A_k: jax.Array,
    A_v: jax.Array,
    A_shift_k: jax.Array,
    A_ssm_k: jax.Array,
    A_ssm_D: jax.Array,
    B_x: jax.Array,
    B_w1: jax.Array,
    B_w2: jax.Array,
    B_w3: jax.Array,
    B_w4: jax.Array,
    c: jax.Array,
    w_mod: jax.Array,
):
    del B_x

    def tiles(x):
        return x.reshape(S // 8, 8, NC, 128).transpose(0, 2, 1, 3).reshape(S * NC, 128)

    def pairs(x):
        r, n = x.shape
        return x.reshape(r // 16, 2, 8, n // 128, 128).transpose(0, 1, 3, 2, 4)

    args = (
        A_q.reshape(S, D), tiles(A_k), tiles(A_v),
        A_shift_k.T, A_ssm_k, A_ssm_D.reshape(NC, 128),
        pairs(B_w1), pairs(B_w2), pairs(B_w3.T), pairs(B_w4), c, pairs(w_mod),
    )
    scratch = [
        pltpu.VMEM((NA, P * NC + 128, 128), BF16),
        pltpu.VMEM((NA, P * NC + 64, 128), BF16),
        pltpu.VMEM((D, S), BF16),
        pltpu.VMEM((R, 128, 128), U32),
        pltpu.VMEM((R, 64, 256), U32),
        pltpu.VMEM((64, 128), U32),
        pltpu.VMEM((D // 16, 6 * NC, 16, 128), BF16),
        pltpu.VMEM((D // 16, NC, 16, 128), BF16),
        pltpu.VMEM((D // 16, NC, 16, 128), BF16),
        pltpu.VMEM((FF // 16, NC, 16, 128), BF16),
        pltpu.VMEM((FF // 16, NC, 16, 128), BF16),
        pltpu.VMEM((S + 64, D), BF16),
        *[pltpu.VMEM((NA, R, 16, 4, 8, 128), F32) for _ in range(NC)],
        pltpu.VMEM((NC, 2, R, 16, 2, 8, 128), F32),
        pltpu.VMEM((NC, R, 128, 128), U32),
        pltpu.VMEM((32, 128), U32),
        pltpu.VMEM((NC, 8, 8, 128), F32),
        pltpu.VMEM((NC, S + 32, 128), F32),
        pltpu.VMEM((8, 8, D), F32),
        pltpu.VMEM((S + 32, D), F32),
        pltpu.VMEM((NC, S + 32, 128), F32),
        pltpu.VMEM((NC, S + 32, 128), F32),
        pltpu.VMEM((2, TS, D), BF16),
        pltpu.VMEM((TS, 5 * 256), BF16),
        pltpu.VMEM((5, 2, 128, 128), U32),
        pltpu.VMEM((5, 2, 128, 128), U32),
        pltpu.VMEM((5, 6, 64, 256), U32),
        pltpu.VMEM((5, 2, FT // 2, 256), U32),
        pltpu.VMEM((5, 2, 448, 128), U32),
        pltpu.VMEM((8, 9, 72, 128), U32),
        pltpu.VMEM((8, 9, 72, 128), U32),
        pltpu.VMEM((2, 8, 192, 128), U32),
        pltpu.VMEM((NQ, 8, 192, 128), U32),
        pltpu.VMEM((S, D), BF16),
        pltpu.VMEM((4, D), BF16),
        pltpu.VMEM((NC, 128), BF16),
        pltpu.VMEM((1, D), BF16),
        pltpu.SMEM((64,), jnp.int32),
        pltpu.SemaphoreType.DMA((40,)),
        pltpu.SemaphoreType.DMA((1,)),
    ]
    out = pl.pallas_call(
        _kernel,
        out_shape=jax.ShapeDtypeStruct((S, D), BF16),
        in_specs=[pl.BlockSpec(memory_space=pl.ANY)] * len(args),
        out_specs=pl.BlockSpec(memory_space=pl.ANY),
        scratch_shapes=scratch,
        grid=(1,),
        compiler_params=pltpu.CompilerParams(vmem_limit_bytes=108 * 1024 * 1024, disable_semaphore_checks=True,
                                             disable_bounds_checks=True),
        name="adaln_h3_mixer",
    )(*args)
    return out.reshape(1, S, D)
```

```python
import numpy as np
import jax
import jax.numpy as jnp
import jax.experimental.pallas as pl
import jax.experimental.pallas.tpu as pltpu

F32 = jnp.float32
BF16 = jnp.bfloat16
U32 = jnp.uint32

S = 2048
D = 640
FF = 1728
NC = D // 128
R = 4
P = 128 * R
NA = S // P
TS = 256
NT = S // TS
LEAD = 16
EPS = 1e-5
NEST = (1, 4, 0, 3, 5, 6)
NQ = len(NEST)
FT = (FF - 1536) // 2


def _freq(row):
    t, part, s = row >> 4, (row >> 3) & 1, row & 7
    return 32 * (t & 7) + 4 * s + 2 * (t >> 3) + 1, P * part


def _cos(j, scale):
    jf = (j & (4 * P - 1)).astype(F32)
    u = 2.0 * np.pi / (4 * P)
    x = jnp.abs(jf * u - np.pi) - 0.5 * np.pi
    x2 = x * x
    poly = scale / 362880.0 - x2 * (scale / 39916800.0)
    for coef in (-1.0 / 5040.0, 1.0 / 120.0, -1.0 / 6.0, 1.0):
        poly = poly * x2 + coef * scale
    return poly * x


_DUR = {"t": 8, "u": 16, "k": 16, "i": 16, "m": 12, "g": 0, "c": 0, "j": 16}
_POST = {"t": 8.0, "u": 16.0, "k": 24.0, "i": 4.0, "j": 4.0, "m": 18.0}


def _plan_tokens(order, maxutil):
    lag, cap, pre, margin = 8, 62, 4, 3
    start, slots = {}, []
    for n in order:
        start[n] = len(slots)
        slots += [(n, r) for r in range(_DUR[n[0]])]
    nslot = len(slots) + lag
    free = [cap - (_POST[slots[i - lag][0][0]] if i >= lag else 0.0) for i in range(-pre, nslot)]
    units = []
    for n in order:
        kind, a, c = n
        if kind == "u":
            units += [(n + (g,), 94.0, start[n], -pre) for g in range(8)]
        elif kind == "g":
            units += [(n + (g,), 150.0, start[n], -pre) for g in range(8)]
        elif kind in "ic":
            src_ = [start[m] for m in (("u", a, c), ("k", a, c)) if m in start]
            for t in range(16):
                rel = max(max(src_) + 16, max(src_) + t + lag + 3) if src_ else -pre
                units.append((n + (t,), 32.0 * a + 48.0, nslot if kind == 'c' else start[n], rel))

    def simulate(util):
        left = [u[1] for u in units]
        done = [None] * len(units)
        for i in range(-pre, nslot):
            budget = util * free[i + pre]
            for j, u in enumerate(units):
                if budget <= 0.0:
                    break
                if done[j] is None and u[3] <= i:
                    use = min(budget, left[j])
                    left[j] -= use
                    budget -= use
                    if left[j] <= 1e-9:
                        done[j] = i + 1
        ok = all(u[2] < 8 or (d is not None and d <= max(u[2] - (1 if u[0][0] in 'cg' else margin), u[3] + 1))
                 for d, u in zip(done, units))
        return done, ok

    lo_, hi_ = 0.05, maxutil
    for _ in range(12):
        mid = 0.5 * (lo_ + hi_)
        if simulate(mid)[1]:
            hi_ = mid
        else:
            lo_ = mid
    done, _ = simulate(hi_)
    plan = {}
    for u, d in zip(units, done):
        if u[0][0] == "c":
            plan[u[0]] = slots[max((nslot - 1 if d is None else min(d, nslot - 1)) - lag, 0)]
        elif d is not None and 0 <= d < u[2]:
            plan.setdefault(slots[d], []).append(u[0])
    return plan


def _unpack(w):
    return pltpu.bitcast(w, BF16)


def _dot(a, b):
    return jnp.dot(a.astype(BF16), b, preferred_element_type=F32)


def _dot_nt(a, b):
    return jax.lax.dot_general(a.astype(BF16), b, (((1,), (1,)), ((), ())), preferred_element_type=F32)


def _dot_fine(x, w, chunk):
    if not chunk:
        return _dot(x, w)
    n = w.shape[1]
    head = _dot(x, w[:, :n - 128])
    last = jnp.concatenate([_dot(x[r:r + chunk], w[:, n - 128:]) for r in range(0, x.shape[0], chunk)], axis=0)
    return jnp.concatenate([head, last], axis=1)


def _rows2(x):
    n, c = x.shape
    x = x.reshape(n // 32, 2, 16, c)
    return x[:, 0].reshape(n // 2, c), x[:, 1].reshape(n // 2, c)


def _unrows2(top, bot):
    n, c = top.shape
    return jnp.stack([top.reshape(n // 16, 16, c), bot.reshape(n // 16, 16, c)], axis=1).reshape(2 * n, c)


def _sums_a(a11, a12, a21, a22):
    return [a11 + a22, a21 + a22, a11 + a12, a21 - a11, a12 - a22]


def _sums_b(b11, b12, b21, b22):
    return [b11 + b22, b12 - b22, b21 - b11, b11 + b12, b21 + b22]


_STRASSEN = ((0, 0), (1, 5), (5, 1), (6, 2), (2, 6), (3, 3), (4, 4))


_SUMS_A = ((0, 3, 1), (2, 3, 1), (0, 1, 1), (2, 0, -1), (1, 3, -1))
_SUMS_B = ((0, 3, 1), (1, 3, -1), (2, 0, -1), (0, 1, 1), (2, 3, 1))


def _combine(m1, m2, m3, m4, m5, m6, m7):
    return (m1 + m4) + (m7 - m5), m3 + m5, m2 + m4, (m1 - m2) + (m3 + m6)


def _lo(w):
    return pltpu.bitcast(w << 16, F32)


def _hi(w):
    return pltpu.bitcast(w & jnp.uint32(0xFFFF0000), F32)


def _ln(x, eps=EPS):
    m = jnp.sum(x, axis=-1, keepdims=True) * (1.0 / D)
    xc = x - m
    v = jnp.sum(xc * xc, axis=-1, keepdims=True) * (1.0 / D)
    return xc * jnp.exp(-0.5 * jnp.log(v + eps))


def _gelu2(x):
    c0 = 0.7978845608028654
    c1 = c0 * 0.044715
    return x + x * jnp.tanh(x * (c0 + c1 * (x * x)))


def _bfly(tr, ti):
    s02r, s02i = tr[0] + tr[2], ti[0] + ti[2]
    d02r, d02i = tr[0] - tr[2], ti[0] - ti[2]
    s13r, s13i = tr[1] + tr[3], ti[1] + ti[3]
    d13r, d13i = tr[1] - tr[3], ti[1] - ti[3]
    x0r, x0i = s02r + s13r, s02i + s13i
    x2r, x2i = s02r - s13r, s02i - s13i
    return [x0r, d02r + d13i, x2r, d02r - d13i], [x0i, d02i - d13r, x2i, d02i + d13r]


def _kernel(q_hbm, k_hbm, v_hbm, shift_hbm, ssmk_hbm, ssmd_hbm, w1_hbm, w2_hbm, w3t_hbm, w4_hbm,
            c_hbm, wmod_hbm,
            out_hbm,
            kbuf, vbuf, skbuf, fwdbuf, invbuf, permbuf,
            wmodbuf, w1buf, w2buf, w3buf, w4buf, qbuf,
            xs0, xs1, xs2, xs3, xs4, kraw, stg, zbuf, coefbuf, ybuf, modbuf, x2buf, hbuf, hhbuf, xobuf,
             w1s, w2s, w3s, w3ts, w4s, hba, hbb, w4n, w4q, obuf, shiftbuf, dbuf, cbuf,
            zsm, sem_in, sem_out):
    cps = {}
    n_sem = [0]

    def start(name, src, dst):
        cp = pltpu.make_async_copy(src, dst, sem_in.at[n_sem[0]])
        n_sem[0] += 1
        cp.start()
        cps[name] = cp

    class Both:
        def __init__(self, a, b):
            self.cps = (a, b)

        def wait(self):
            for cp in self.cps:
                cp.wait()

    def start_w(name, src, dst, c0=0, n=NC):
        for e in range(2):
            start(name + str(e), src.at[:, e, pl.ds(c0, n)], dst.at[:, pl.ds(c0, n), pl.ds(8 * e, 8), :])
        cps[name] = Both(cps[name + "0"], cps[name + "1"])

    CH = P * NC
    HALO = 8 * NC

    def start_s(a):
        cols = pl.ds(a * P, P)
        start("s%d" % a, ssmk_hbm.at[:, cols], skbuf.at[:, cols])

    def start_kv(a):
        if a == 0:
            kbuf[0, pl.ds(0, HALO + 8), :] = jnp.zeros((HALO + 8, 128), BF16)
            start("k0", k_hbm.at[pl.ds(0, CH), :], kbuf.at[0, pl.ds(HALO, CH), :])
        else:
            start("k%d" % a, k_hbm.at[pl.ds(a * CH - HALO, CH + HALO), :], kbuf.at[a, pl.ds(0, CH + HALO), :])
        start("v%d" % a, v_hbm.at[pl.ds(a * CH, CH), :], vbuf.at[a, pl.ds(0, CH), :])

    for n in "s0 x0 s1 k0 k1 s2 k2 s3 k3".split():
        if n[0] == "s":
            start_s(int(n[1]))
        elif n[0] == "k":
            start_kv(int(n[1]))
        else:
            start("d", ssmd_hbm, dbuf)
            start("shift", shift_hbm, shiftbuf)
            start("c", c_hbm, cbuf)
    QA = TS + LEAD
    XA = 128
    QB = 2 * TS + LEAD
    W1A = 2

    def start_q(name, r0, n):
        start(name, q_hbm.at[pl.ds(r0, n), :], qbuf.at[pl.ds(r0, n), :])

    start_q("qa", 0, QA)
    start_w("wmoda", wmod_hbm, wmodbuf, 0, 3 * NC)
    start_w("wmodb", wmod_hbm, wmodbuf, 3 * NC, 2 * NC)
    start_q("qx", QA, XA)
    start_w("w1a", w1_hbm, w1buf, 0, W1A)
    start_w("w1b", w1_hbm, w1buf, W1A, NC - W1A)
    start_q("qb", QA + XA, QB - QA - XA)
    start_w("w2", w2_hbm, w2buf)
    start_w("w3", w3t_hbm, w3buf)
    start_w("w4", w4_hbm, w4buf)
    start_w("wmodg", wmod_hbm, wmodbuf, 5 * NC, NC)
    start_q("q1", QB, S - QB)

    kw = kbuf.bitcast(U32)
    vw = vbuf.bitcast(U32)
    zbuf[...] = jnp.zeros(zbuf.shape, U32)
    for j in range(64):
        zsm[j] = 0
    for c in range(NC):
        ybuf[c, pl.ds(S, LEAD), :] = jnp.zeros((LEAD, 128), F32)
        hhbuf[c, pl.ds(0, 8), :] = jnp.zeros((8, 128), F32)
    qbuf[pl.ds(S, LEAD), :] = jnp.zeros((LEAD, D), BF16)

    def sample(pos):
        return (pos & ~15) + 2 * (pos & 7) + ((pos >> 3) & 1)

    def tables(p, carry):
        f2, off = _freq(jax.lax.broadcasted_iota(jnp.int32, (256, 128), 0))
        n = R * sample(jax.lax.broadcasted_iota(jnp.int32, (256, 128), 1)) + p
        fwdbuf[p] = _cos(f2 * n + off, 1.0).astype(BF16)
        return carry

    jax.lax.fori_loop(0, R, tables, 0)

    def unit_g(kt, r):
        f2, off = _freq(jax.lax.broadcasted_iota(jnp.int32, (16, 128), 1) + 128 * kt)
        j0 = f2 * (R * (jax.lax.broadcasted_iota(jnp.int32, (16, 128), 0) + 16 * r)) + off
        for p in range(R):
            invbuf[kt, p, pl.ds(16 * r, 16), :] = _cos(j0 + p * f2, 1.0 / P).astype(BF16)
        return [invbuf.bitcast(U32)[kt, p, pl.ds(8 * r, 8), :] for p in range(R)]

    i0 = jax.lax.broadcasted_iota(jnp.int32, (128, 128), 0)
    i1 = jax.lax.broadcasted_iota(jnp.int32, (128, 128), 1)
    permbuf[...] = jnp.where(i1 == R * sample(i0 & 31) + (i0 >> 5), 1.0, 0.0).astype(BF16)

    def fill_coef():
        cv = cbuf[...].astype(F32)
        modbuf[6] = jnp.broadcast_to(cv * jax.nn.sigmoid(cv), (8, D))
        coef = shiftbuf[...].astype(F32)
        dval = dbuf[...].astype(F32)
        for c in range(NC):
            for j in range(4):
                coefbuf[c, j] = jnp.broadcast_to(coef[j:j + 1, c * 128:(c + 1) * 128], (8, 128))
            coefbuf[c, 4] = jnp.broadcast_to(dval[c:c + 1, :], (8, 128))

    xs = (xs0, xs1, xs2, xs3, xs4)
    wsbufs = dict(w1=w1s, w2=w2s, w3=w3s, w4=w4s, w3t=w3ts)
    def split_ri(t):
        t = t.reshape(16, 2, 8, 128)
        return t[:, 0], t[:, 1]

    def get_never():
        return zbuf[pl.ds(0, 8), :] != 0

    def packed(x, slot, r0):
        n = x.shape[1]
        stg[slot, :, pl.ds(r0, n), :] = x.astype(BF16)
        return [stg.bitcast(U32)[slot, p, pl.ds(r0 // 2, n // 2), :] for p in range(R)]

    UG = 8

    def unit_u(a, c, g0, UG):
        c0, c1, c2, c3 = (coefbuf[c, pl.ds(j, 1)][None] for j in range(4))
        rows = lambda ref, r: ref[a, pl.ds((r // 4) * 4 * NC + 4 * c + r % 4, 8 * UG, stride=4 * NC), :]
        kk = jnp.stack([rows(kw, 4 + 32 * g0 + d) for d in range(-2, 4)]).reshape(6, UG, 8, 128)
        vv = jnp.stack([rows(vw, 32 * g0 + d) for d in range(4)]).reshape(4, UG, 8, 128)
        lo, hi = _lo(kk), _hi(kk)
        k0, k1, k2 = lo[2:], hi[1:5], lo[1:5]
        even = ((k0 * c0 + k1 * c1) + (k2 * c2 + hi[:4] * c3)) * _lo(vv)
        odd = ((hi[2:] * c0 + k0 * c1) + (k1 * c2 + k2 * c3)) * _hi(vv)
        kv = jnp.stack([even, odd], axis=1).reshape(2, R, UG, 8, 128)
        return packed(jnp.stack([kv[0], kv[1]], axis=2).reshape(R, 16 * UG, 128), NC + c, 16 * g0)

    def unit_i(a, c, t0, UG, z, after=None):
        x_c = xs[c].at[pl.ds(z, NA)]
        ts = pl.ds(t0, UG)
        yr = yi = None
        for j in range(a + 1):
            ur, ui = x_c[j, :, ts, 0], x_c[j, :, ts, 1]
            kr, ki = x_c[a - j, :, ts, 2], x_c[a - j, :, ts, 3]
            pr = ur * kr - ui * ki
            pi = ur * ki + ui * kr
            yr = pr if yr is None else yr + pr
            yi = pi if yi is None else yi + pi
        sr, si, dr, di = yr[:2] + yr[2:], yi[:2] + yi[2:], yr[:2] - yr[2:], yi[:2] - yi[2:]
        (sr0, sr1), (si0, si1), (dr0, dr1), (di0, di1) = ((x[0], x[1]) for x in (sr, si, dr, di))
        wr = jnp.stack([sr0 + sr1, dr0 - di1, sr0 - sr1, dr0 + di1])
        wi = jnp.stack([si0 + si1, di0 + dr1, si0 - si1, di0 - dr1])
        if after is not None:
            never = jnp.broadcast_to(zbuf[pl.ds(0, 8), :], wr.shape) != 0
            wr = jax.lax.select(never, jnp.broadcast_to(after, wr.shape), wr)
        return packed(jnp.stack([wr, wi], axis=2).reshape(R, 16 * UG, 128), c, 16 * t0)

    def segment(spec, z, maxutil=1.0, mod_fn=None):
        order = [(n[0], int(n[1]), int(n[2])) for n in spec.split()]
        plan = _plan_tokens(order, maxutil) if maxutil > 0 else {}
        never = get_never()
        units, groups, res = {}, {}, {}

        paced = {k_ for s_, ks in plan.items() if len(s_) == 2 for k_ in ks}

        def width(name):
            n = 8 if name[0] == "u" else 16
            return UG if all(name + (j,) in paced for j in range(n)) else 1

        def group(key):
            kind, a, c, j = key
            ug = width(key[:3])
            key = (kind, a, c, j - j % ug)
            if key not in groups:
                if kind == "u":
                    groups[key] = unit_u(a, c, key[3], ug)
                else:
                    fresh = ("u", a, c) in order or ("k", a, c) in order
                    groups[key] = unit_i(a, c, key[3], ug, z if fresh else 0,
                                         res[plan[key]]() if kind == "c" else None)
            return groups[key]

        def unit(key):
            if key not in units:
                if key[0] == "g":
                    units[key] = unit_g(key[1], key[3])
                else:
                    r = 8 * (key[3] % width(key[:3]))
                    units[key] = [v[r:r + 8] for v in group(key)]
            return units[key]

        def lhs(name, p, full, r0=0):
            out, last = [], 0
            for r in range(full.shape[0] // 8):
                keys = plan.get((name, r0 + r), ())
                if keys:
                    if 8 * r > last:
                        out.append(full[last:8 * r])
                    v = full[8 * r:8 * r + 8]
                    for key in keys:
                        v = jax.lax.select(never, unit(key)[p], v)
                    out.append(v)
                    last = 8 * r + 8
            if last < full.shape[0]:
                out.append(full[last:] if last else full)
            return out[0] if len(out) == 1 else jnp.concatenate(out, axis=0)

        def dft(name, rhs):
            tr, ti = [], []
            for p in range(R):
                f = lhs(name, p, fwdbuf.bitcast(U32)[p])
                r_, i_ = split_ri(_dot(_unpack(f), rhs[p]))
                if p == 0:
                    res.update({(name, r): (lambda r=r, v=r_: v[r]) for r in range(16)})
                tr.append(r_)
                ti.append(i_)
            return _bfly(tr, ti)

        st = {}
        for name in order:
            kind, a, c = name
            x_c = xs[c]
            if kind == "g":
                for r in range(8):
                    unit(name + (r,))
            elif kind == "c":
                for t in range(16):
                    group(name + (t,))
            elif kind == "m":
                toks = {}
                for r in range(_DUR["m"]):
                    for n_, key in enumerate(plan.get((name, r), ())):
                        toks.setdefault(2 * r + n_ % 2, []).extend(unit(key))
                mod_fn(a, toks)
            elif kind == "t":
                trs = []
                for b in range(R):
                    pm = lhs(name, b, permbuf.bitcast(U32)[...])
                    trs.append(_dot_nt(_unpack(pm), skbuf[pl.ds(c * 128, 128), pl.ds(a * P + b * 128, 128)]))
                res.update({(name, r): (lambda r=r, v=trs[0]: v[16 * r:16 * r + 8]) for r in range(8)})
                g_ = 128 // R
                st[a, c] = [jnp.concatenate([trs[b][p * g_:(p + 1) * g_] for b in range(R)], axis=0).astype(BF16)
                            for p in range(R)]
            elif kind == "u":
                rhs = [_unpack(jnp.concatenate([group(name + (g,))[p] for g in range(0, 8, width(name))], axis=0)) for p in range(R)]
                xr, xi = dft(name, rhs)
                for q in range(R):
                    x_c[a, q, :, 0] = xr[q]
                    x_c[a, q, :, 1] = xi[q]
            elif kind == "k":
                xr, xi = dft(name, st[a, c])
                for q in range(R):
                    if a == 0:
                        x_c[a, q, :, 2] = xr[q] + coefbuf[c, 4]
                        x_c[a, q, :, 3] = xi[q]
                    else:
                        pr, pi = kraw[c, (a - 1) % 2, q, :, 0], kraw[c, (a - 1) % 2, q, :, 1]
                        x_c[a, q, pl.ds(0, 8), 2] = xr[q][:8] - pi[:8]
                        x_c[a, q, pl.ds(0, 8), 3] = xi[q][:8] + pr[:8]
                        x_c[a, q, pl.ds(8, 8), 2] = xr[q][8:] + pi[8:]
                        x_c[a, q, pl.ds(8, 8), 3] = xi[q][8:] - pr[8:]
                    if a + 1 < NA:
                        kraw[c, a % 2, q, :, 0] = xr[q]
                        kraw[c, a % 2, q, :, 1] = xi[q]
            else:
                for p in range(R):
                    cols = [lhs(name, 2 * (p % 2) + kt,
                                invbuf.bitcast(U32)[kt, p], 8 * (p // 2))
                            for kt in range(2)]
                    g = _unpack(jnp.concatenate(cols, axis=1))
                    if kind == "j":
                        wp = _unpack(stg.bitcast(U32)[c, p])
                    else:
                        wp = _unpack(jnp.concatenate([group(name + (t,))[p] for t in range(0, 16, width(name))], axis=0))
                    yp = _dot(g, wp)
                    if p % 2 == 0:
                        res.update({(name, 4 * p + r): (lambda r=r, v=yp: v[16 * r:16 * r + 8]) for r in range(8)})
                    ybuf[c, pl.ds(a * P + p, 128, stride=R), :] = yp

    one = jnp.minimum(pl.program_id(0) + 1, 1)

    def once(fn):
        def body(z, carry):
            fn(z)
            return carry
        jax.lax.fori_loop(0, one, body, 0)

    default = ("t00 t01 t02 k00 t03 k01 t04 k02 k03 k04 g00|"
               "t10 t11 t12 k10 k11 k12 g10|"
               "t13 t14 k13 u00 k14 u01 u02 u03 i00 u04 i01 c02 c03|"
               "j02 j03 u10 i04 u11 u12 u13 i10 u14 i11 c12 c13|"
               "t20 t21 j12 t22 j13 t23 t24 k20 u20 k21 u21 k22 i14 k23 u22 k24 u23 i20 u24 i21 c22|"
               "t30 t31 j22 t32 t33 t34 k30 u30 k31 u31 k32 i23 k33 u32 k34 i24 u33 i30 u34 i31 c32|"
               "m00 j32 m10 i33 m20 i34")
    specs = default.split("|")
    G5B = specs[-1]
    segs = list(zip("s0 d shift c|s1|k0 v0|k1 v1|s2 k2 v2|s3 k3 v3".split("|"), specs[:-1]))
    MU = 1.5
    for i, (waits, spec) in enumerate(segs):
        with jax.named_scope("g%d" % i):
            for n in waits.split():
                cps[n].wait()
            if i == 0:
                fill_coef()
            once(lambda z: segment(spec, z, MU))

    def mod_cols(lo, n, toks=None):
        m = _dot(modbuf[6], weights(wmodbuf, lo * NC, (lo + n) * NC, toks=toks))
        return [m[:, j * D:(j + 1) * D] for j in range(n)]

    def mul_mod(x, j, cols=None):
        m = modbuf[j] if cols is None else modbuf[j, :, cols]
        return (x.reshape(-1, 8, x.shape[-1]) * m[None]).reshape(x.shape)

    def add_mod(x, j):
        return (x.reshape(-1, 8, x.shape[-1]) + modbuf[j][None]).reshape(x.shape)

    def slabs(ref, r0, n):
        return jnp.concatenate([ref[c, pl.ds(r0, n), :] for c in range(NC)], axis=1)

    def put(ref, rows, x):
        for c in range(NC):
            ref[c, rows, :] = x[:, c * 128:(c + 1) * 128]

    def window(base, n):
        rows = pl.ds(base, n)
        return dict(q=qbuf.at[rows, :], y=ybuf.at[:, rows, :], x2=x2buf.at[rows, :], h=hbuf.at[:, rows, :],
                    hh=hhbuf.at[:, pl.ds(base, n + 8), :],
                    o=obuf.at[pl.ds(base, n - LEAD), :])

    def weights(ref, c0=0, c1=NC, r0=0, r1=None, toks=None, raw=False, z=None):
        r1 = 16 * ref.shape[0] if r1 is None else r1
        view = ref.bitcast(U32)
        if z is not None:
            view = view.at[pl.ds(z, ref.shape[0])]
        never = get_never() if toks else None
        rt = -(-(r1 - r0) // 128)
        cols = []
        for j in range(c0, c1):
            wu = view[pl.ds(r0 // 16, (r1 - r0) // 16), j].reshape((r1 - r0) // 2, 128)
            if toks:
                parts, last = [], 0
                for i in range(rt):
                    for n_, t in enumerate(toks.get((j - c0) * rt + i, ())):
                        r = 64 * i + 8 * n_
                        if r > last:
                            parts.append(wu[last:r])
                        parts.append(jax.lax.select(never, t, wu[r:r + 8]))
                        last = r + 8
                parts.append(wu[last:])
                wu = jnp.concatenate(parts, axis=0)
            cols.append(wu)
        wu = jnp.concatenate(cols, axis=1)
        return wu if raw else _unpack(wu)

    def keep(dst, v):
        h = v.shape[0] // 2
        for c in range(v.shape[1] // 128):
            for r in (0, h):
                dst[c, pl.ds(r, h), :] = v[r:r + h, 128 * c:128 * (c + 1)].astype(BF16)

    def fetch(src_):
        u = src_.bitcast(U32)
        return jnp.concatenate([u[c] for c in range(u.shape[0])], axis=1)

    def wblocks(name, j, z=None):
        if name == "w3":
            blk = lambda kh, nh: weights(w3buf, 2 * kh, 2 * kh + 2, 128 * (j + 6 * nh), 128 * (j + 6 * nh + 1), raw=True, z=z)
        elif name == "w4":
            def blk(kh, nh):
                c = j + 2 * nh
                parts = [weights(w4buf, c, c + 1, 768 * kh, 768 * (kh + 1), raw=True, z=z),
                         weights(w4buf, c, c + 1, 1536 + FT * kh, 1536 + FT * (kh + 1), raw=True, z=z),
                         jnp.zeros(((128 - FT) // 2, 128), U32)]
                return jnp.concatenate(parts, axis=0)
        elif name == "w3t":
            blk = lambda kh, nh: weights(w3buf, 2 * kh, 2 * kh + 2, 1536 + FT * nh, 1536 + FT * (nh + 1), raw=True, z=z)
        else:
            ref = w1buf if name == "w1" else w2buf
            blk = lambda kh, nh: weights(ref, j + 2 * nh, j + 2 * nh + 1, 256 * kh, 256 * (kh + 1), raw=True, z=z)
        return blk

    def wsum(name, j, k):
        blk = wblocks(name, j, zsm[k])
        p, q, sign = _SUMS_B[k]
        return psum(blk(p // 2, p % 2), blk(q // 2, q % 2), sign)

    pending = []

    def attach(wv):
        if not pending:
            return wv
        never = get_never()
        rows = [wv[8 * i:8 * i + 8, :128] for i in range(8)]
        for i, t in enumerate(pending):
            rows[i % 8] = jax.lax.select(never, pltpu.bitcast(t, U32), rows[i % 8])
        pending.clear()
        first = jnp.concatenate(rows + ([wv[64:, :128]] if wv.shape[0] > 64 else []), axis=0)
        return first if wv.shape[1] == 128 else jnp.concatenate([first, wv[:, 128:]], axis=1)

    def sprods(name, j, lhs, k0=0, k1=7, prep=False):
        blk, buf = wblocks(name, j), wsbufs[name]
        out = []
        for ia, ib in _STRASSEN[k0:k1]:
            if prep and ib < 5:
                wv = wsum(name, j, ib)
                keep(buf.at[ib, j], wv)
                wv = wv.astype(BF16)
            else:
                wv = _unpack(attach(blk(ib - 5, ib - 5) if ib >= 5 else fetch(buf.at[ib, j])))
            if name == "w3t":
                out.append(_dot_nt(wv, lhs(ia)))
            else:
                out.append((_dot_nt if name == "w3" else _dot)(lhs(ia), wv))
        return out

    def spair(name, j, lhs, prep=False):
        return _combine(*sprods(name, j, lhs, prep=prep))

    def dd_rest(name, t, b):
        ref = w1buf if name == "w1" else w2buf
        m = t.shape[0]
        xb = jnp.concatenate([t, b], axis=0)
        last = _dot(xb, weights(ref, 4, 5))
        rem = _dot(xb[:, 512:], weights(ref, 0, 4, r0=512))
        return t, b, rem[:m], rem[m:], last[:m], last[m:]

    def dd_main(name, parts, prep=False):
        t, b, rt, rb, lt, lb = (jnp.concatenate(v, axis=0) for v in zip(*parts))
        ops = _sums_a(t[:, :256], t[:, 256:512], b[:, :256], b[:, 256:512]) + [t[:, :256], b[:, 256:512]]
        top, bot = [None] * 4, [None] * 4
        for j in range(2):
            top[j], top[j + 2], bot[j], bot[j + 2] = spair(name, j, lambda i: ops[i], prep)
        return (jnp.concatenate([jnp.concatenate(top, axis=1) + rt, lt], axis=1),
                jnp.concatenate([jnp.concatenate(bot, axis=1) + rb, lb], axis=1))

    def stage_a0(w, r0, n):
        rows = pl.ds(r0, n)
        x = w["q"][rows, :].astype(F32)
        x2 = x + add_mod(mul_mod(_ln(x), 1), 0) * slabs(w["y"], r0, n)
        w["x2"][rows, :] = x2
        return _ln(x2)

    def stage_a1(w, r0, n, n2=None, f32=False):
        if n2 is None:
            n2 = stage_a0(w, r0, n)
        h = add_mod(mul_mod(n2, 4), 3)
        put(w["h"], pl.ds(r0, n), h)
        n3 = _ln(h, 4 * EPS)
        return n3 if f32 else n3.astype(BF16)

    def stage_a2(w, n3, r0, n, last_valid=None, fine=0, c0=0, c1=NC, prep=False):
        hh = _gelu2(_unrows2(*dd_main("w1", n3, prep)) if isinstance(n3, list) else _dot_fine(n3, weights(w1buf, c0, c1), fine))
        for c in range(c0, c1):
            blk = hh[:, (c - c0) * 128:(c - c0 + 1) * 128]
            w["hh"][c, pl.ds(r0 + 8, n - LEAD), :] = blk[:n - LEAD]
            tail = blk[n - LEAD:]
            if last_valid is not None:
                tail = jnp.where(last_valid, tail, 0.0)
            w["hh"][c, pl.ds(r0 + 8 + n - LEAD, LEAD), :] = tail

    def stage_b1a(w, r0, n, prep=False):
        lane = jax.lax.broadcasted_iota(jnp.int32, (n, 128), 1)
        sh = lambda c, d: w["hh"][c, pl.ds(r0 + 8 + d, n), :]
        g = jnp.concatenate([sh(0, -1),
                             jnp.where(lane < 32, sh(1, -1), sh(1, 1)),
                             jnp.where(lane < 64, sh(2, 1), sh(2, -2)),
                             jnp.where(lane < 96, sh(3, -2), sh(3, 2)),
                             sh(4, 2)], axis=1)
        x1 = slabs(w["h"], r0, n) + _unrows2(*dd_main("w2", [dd_rest("w2", *_rows2(g))], prep))
        put(w["h"], pl.ds(r0, n), x1)
        return x1

    def stage_b1b(w, x1, r0, n):
        t, b = _rows2(_ln(x1, 4 * EPS))
        ops = _sums_a(t[:, :256], t[:, 256:512], b[:, :256], b[:, 256:512]) + [t[:, :256], b[:, 256:512]]
        ops.append(jnp.concatenate([t[:, 512:], b[:, 512:]], axis=1))
        for i, v in enumerate(ops):
            keep(xobuf.at[i, :, pl.ds(r0 // 2, n // 2), :], v)

    def out_copy(r0, n):
        rows = pl.ds(r0, n)
        return pltpu.make_async_copy(obuf.at[rows, :], out_hbm.at[rows, :], sem_out.at[0])


    def opaque(ref, i):
        ref = ref.bitcast(U32)
        return ref.at[:, :, pl.ds(pl.multiple_of(zsm[i] * 32, 32), ref.shape[2]), :]

    def emit(h3, j, left, right):
        m = left.shape[0] // 2
        g = [left[:m], right[:m], left[m:], right[m:]]
        for k, v in enumerate(_sums_a(*g) + g):
            h3[j, k, pl.ds(0, m), :] = v.astype(BF16)

    def w3_operands(r0, n):
        u, rows = xobuf.bitcast(U32), pl.ds(r0 // 4, n // 4)
        xr = _unpack(jnp.concatenate([u[7, 0, rows, :], u[7, 1, rows, :]], axis=0))
        return xr, lambda i: _unpack(jnp.concatenate([u[i, 0, rows, :], u[i, 1, rows, :]], axis=1))

    def stage_b2h(w, h3, r0, n, prep=False):
        xr, ops = w3_operands(r0, n)
        m = n // 2
        rem = _dot_nt(weights(w3buf, 4, 5, r0=1536), xr)
        c11, c12, c21, c22 = spair("w3t", 0, ops, prep)
        pad = jnp.zeros((128 - FT, m), F32)
        g11, g12, g21, g22 = (jnp.concatenate([_gelu2(c + r), pad], axis=0).T for c, r in (
            (c11, rem[:FT, :m]), (c12, rem[FT:, :m]), (c21, rem[:FT, m:]), (c22, rem[FT:, m:])))
        emit(h3, 6, jnp.concatenate([g11, g21], axis=0), jnp.concatenate([g12, g22], axis=0))

    def stage_b2a(w, h3, r0, n, lo=0, hi=6, prep=False):
        xr, ops = w3_operands(r0, n)
        for j in range(lo, hi):
            r1, r2 = (_dot_nt(xr, weights(w3buf, 4, 5, 128 * t, 128 * (t + 1))) for t in (j, j + 6))
            c11, c12, c21, c22 = spair("w3", j, ops, prep)
            emit(h3, j, _gelu2(jnp.concatenate([c11, c21], axis=0) + r1), _gelu2(jnp.concatenate([c12, c22], axis=0) + r2))

    def finish(w, h2, r0, n, c):
        nc = h2.shape[1] // 128
        rows, cols = pl.ds(r0, n), pl.ds(c * 128, nc * 128)
        x1 = jnp.concatenate([w["h"][c + i, rows, :] for i in range(nc)], axis=1)
        w["o"][rows, cols] = (w["x2"][rows, cols] + mul_mod(x1 + h2, 5, cols)).astype(BF16)

    def b2_done(w, done, r0, n):
        if len(done[0]) == len(done[1]) == 7:
            c11, c12, c21, c22 = _combine(*[jnp.concatenate([done[0][k], done[1][k]], axis=1) for k in range(7)])
            finish(w, _unrows2(c11, c21), r0, n, 0)
            finish(w, _unrows2(c12, c22), r0, n, 2)

    def stage_b2b(w, h3, r0, n, j, k0=0, k1=7, done=None, prep=False, sub=0, marks=()):
        hv = opaque(h3, j)
        blk = lambda k: jnp.concatenate([hv[p, k, pl.ds(sub // 4, n // 4), :] for p in range(7)], axis=1)
        r0 += sub
        if j < 2:
            for k in range(k0, k1):
                if k not in NEST:
                    done[j][k] = sprods("w4", j, lambda i: _unpack(blk(8 if i == 6 else i)), k, k + 1, prep)[0]
                    b2_done(w, done, r0, n)
            return
        wb = wblocks("w4", 4)
        lhs = jnp.concatenate([jnp.concatenate([blk(5), blk(6)], axis=1),
                               jnp.concatenate([blk(7), blk(8)], axis=1)], axis=0)
        if marks:
            lo_, hi_ = 0, 52
            never, at = get_never(), {}
            for i, mk in enumerate(marks):
                s_ = lo_ + (hi_ - lo_) * i // len(marks)
                at[4 * (s_ // 16), s_ % 16] = mk
            cols = []
            for kt in range(14):
                col = lhs[:, 128 * kt:128 * (kt + 1)]
                if any(k_[0] == kt for k_ in at):
                    col = jnp.concatenate([jax.lax.select(never, at[kt, r], col[8 * r:8 * r + 8]) if (kt, r) in at
                                           else col[8 * r:8 * r + 8] for r in range(16)], axis=0)
                cols.append(col)
            lhs = jnp.concatenate(cols, axis=1)
        h2 = _dot(_unpack(lhs), _unpack(jnp.concatenate([wb(0, 0), wb(1, 0)], axis=0)))
        finish(w, _unrows2(h2[:n // 2], h2[n // 2:]), r0, n, 4)


    def psum(x, y, sign):
        x, y = _unpack(x).astype(F32), _unpack(y).astype(F32)
        return x + y if sign > 0 else x - y

    def prep_w4(nchunk):
        rows = 384 // nchunk
        marks = []
        for ch in [nchunk] + list(range(nchunk)):
            tail = ch == nchunk
            raw = {}
            for kh in range(2):
                for e in range(1 if tail else 2):
                    r0 = 1536 + FT * kh if tail else 768 * kh + 384 * e + rows * ch
                    x = weights(w4buf, 0, 4, r0, r0 + (FT if tail else rows), raw=True)
                    raw[kh, e] = _unpack(x).astype(F32)
            blk = lambda i, e: raw[i // 2, e][:, 256 * (i % 2):256 * (i % 2 + 1)]
            for k, (ia, ib) in enumerate(_STRASSEN):
                if k not in NEST or ib >= 5:
                    continue
                p_, q_, sg = _SUMS_B[ib]
                half = [blk(p_, e) + blk(q_, e) if sg > 0 else blk(p_, e) - blk(q_, e) for e in range(1 if tail else 2)]
                quad = lambda i: half[i // 2][:, 128 * (i % 2):128 * (i % 2 + 1)]
                first = NEST.index(k)
                if tail:
                    for j in range(2):
                        w4q[first, 7, pl.ds(128 * j, FT), :] = quad(j).astype(BF16)
                        w4q[first, 7, pl.ds(128 * j + FT, 128 - FT), :] = jnp.zeros((128 - FT, 128), BF16)
                    continue
                for jb, v in enumerate(_sums_b(*[quad(i) for i in range(4)]) + [quad(0), quad(3)]):
                    w4q[first, jb, pl.ds(rows * ch, rows), :] = v.astype(BF16)
            if not tail:
                marks.append(w4q.bitcast(U32).at[pl.ds(zsm[32 + ch], NQ)][first, 0, pl.ds(0, 8), :])
        return marks

    def stage_b2n(w, h3, r0, n, k, done, prep=False):
        ia, ib = _STRASSEN[k]
        ka, q, slot = (8 if ia == 6 else ia), n // 8, NEST.index(k)

        def lblk(i, z):
            hv = opaque(h3, z)
            return jnp.concatenate([hv[g + 3 * (i % 2), ka, pl.ds((i // 2) * q, q), :] for g in range(3)], axis=1)

        def raw(j, lo, hi, z=None):
            return wblocks("w4", j, z)(ib - 5, ib - 5)[lo:hi]

        quad = lambda i, z=None: raw(i % 2, 192 * (i // 2), 192 * (i // 2 + 1), z)
        if ib >= 5:
            wt = [raw(j, 384, 448) for j in range(2)]
        else:
            wq = w4q.bitcast(U32)
            wq = wq.at[pl.ds(zsm[6], NQ)] if prep else wq
            wt = [wq[slot, 7, pl.ds(64 * j, 64), :] for j in range(2)]
        tail = _dot(_unpack(opaque(h3, 5)[6, ka, pl.ds(0, 2 * q), :]), _unpack(jnp.concatenate(wt, axis=1)))
        ms = []
        for ja, jb in _STRASSEN:
            if ja >= 5:
                lv = _unpack(lblk(3 * (ja - 5), 5))
            else:
                p_, q_, sg = _SUMS_A[ja]
                lv = psum(lblk(p_, ja), lblk(q_, ja), sg)
            z = zsm[8 + 7 * slot + jb] if prep and ib >= 5 else None
            if ib < 5:
                wv = _unpack(wq[slot, jb])
            elif jb >= 5:
                wv = _unpack(quad(3 * (jb - 5), z))
            elif prep:
                p_, q_, sg = _SUMS_B[jb]
                wv = psum(quad(p_, z), quad(q_, z), sg)
                keep(w4n.at[slot, pl.ds(jb, 1)], wv)
                wv = wv.astype(BF16)
            else:
                wv = _unpack(w4n.bitcast(U32)[slot, jb])
            ms.append(_dot(lv, wv))
        c11, c12, c21, c22 = _combine(*ms)
        done[0][k] = jnp.concatenate([c11, c21], axis=0) + tail[:, :128]
        done[1][k] = jnp.concatenate([c12, c22], axis=0) + tail[:, 128:]
        b2_done(w, done, r0, n)

    w = window(0, 2 * TS + LEAD)
    H = TS // 2
    with jax.named_scope("t0a"):
        cps["qa"].wait()
        cps["wmoda"].wait()

        mv = {}

        def mod_fn(j, toks):
            mv[j] = mod_cols(j, 1, toks)[0]
            if len(mv) == 3:
                modbuf[0] = mv[2] * mv[0]
                modbuf[1] = mv[2] * (1.0 + mv[1])

        segment(G5B, 0, MU, mod_fn=mod_fn)
        put(w["h"], pl.ds(0, QA), stage_a0(w, 0, QA))
    with jax.named_scope("t0b"):
        cps["wmodb"].wait()
        sb, cb = mod_cols(3, 2)
        modbuf[3] = 2.0 * sb
        modbuf[4] = 2.0 + 2.0 * cb
        n3 = stage_a1(w, 0, QA, n2=slabs(w["h"], 0, QA))
    XB = TS - XA
    with jax.named_scope("t1a"):
        cps["w1a"].wait()
        cps["qx"].wait()
        put(w["h"], pl.ds(QA, XA), stage_a0(w, QA, XA))
        stage_a2(w, n3, 0, QA, c1=W1A, fine=80)
    with jax.named_scope("t1b"):
        cps["w1b"].wait()
        n3a = stage_a1(w, QA, XA, n2=slabs(w["h"], QA, XA), f32=True)
        stage_a2(w, n3, 0, QA, c0=W1A)
        stage_a2(w, [dd_rest("w1", *_rows2(n3a))], QA, XA, prep=True)
    with jax.named_scope("t2"):
        cps["qb"].wait()
        cps["w2"].wait()
        n3b = stage_a1(w, QA + XA, XB, f32=True)
        stage_b1b(w, stage_b1a(w, 0, TS, prep=True), 0, TS)
        stage_a2(w, [dd_rest("w1", *_rows2(n3b))], QA + XA, XB)
        stage_b1b(w, stage_b1a(w, TS, XA), TS, XA)
        stage_b1a(w, TS + XA, XB)
    with jax.named_scope("t3"):
        cps["w3"].wait()
        stage_b1b(w, slabs(w["h"], TS + XA, XB), TS + XA, XB)
        stage_b2h(w, hba, 0, TS, prep=True)
        stage_b2a(w, hba, 0, TS, prep=True)
        stage_b2h(w, hbb, TS, TS)
        stage_b2a(w, hbb, TS, TS)
    with jax.named_scope("t4"):
        cps["w4"].wait()
        cps["wmodg"].wait()
        done = {0: {}, 1: {}}
        for op in "m4 P m0 4:0:2:3 m2 8:0 m1 8:1 m3 8:3 4:1:2:3 8:6 8:4 8:5".split():
            op, *rng = op.split(":")
            rng = [int(x) for x in rng]
            if op[0] == "m":
                c = int(op[1])
                modbuf[5, :, pl.ds(c * 128, 128)] = 0.5 * _dot(modbuf[6], weights(wmodbuf, 5 * NC + c, 5 * NC + c + 1))
            elif op[0] == "8":
                stage_b2n(w, hba, 0, TS, *rng, done, prep=True)
            elif op[0] == "P":
                stage_b2b(w, hba, 0, TS, 2, marks=prep_w4(24))
            else:
                stage_b2b(w, hba, 0, TS, *rng, done=done, prep=True)
        out_copy(0, TS).start()
        cps["q1"].wait()

    CBS = (128, 128)
    PART = {"a": (TS, TS), "c": (TS, H), "d": (TS + H, H)}
    BODY = "4:2 4:0:2:3 4:1:2:3 8:3 8:0 r0 r1 1a 8:1 2c nc 2d nd 8:6 8:5 8:4 3a:0:2 ha 3a:2:6"

    def step(s, carry):
        r0 = pl.multiple_of(s * TS, TS)
        w = window(r0, 2 * TS + LEAD)
        x1, rest, done = {}, {}, {0: {}, 1: {}}
        for op in BODY.split():
            op, *rng = op.split(":")
            rng = [int(x) for x in rng]
            if op[0] == "3":
                stage_b2a(w, hbb, TS, TS, *rng)
            elif op[0] == "h":
                stage_b2h(w, hbb, TS, TS)
            elif op[0] == "4":
                stage_b2b(w, hbb, 0, TS, *rng, done=done)
            elif op[0] == "8":
                stage_b2n(w, hbb, 0, TS, *rng, done)
            elif op[0] == "2":
                x1[op[1]] = stage_b1a(w, *PART[op[1]])
            elif op[0] == "n":
                stage_b1b(w, x1[op[1]], *PART[op[1]])
            elif op[0] == "r":
                j = int(op[1])
                rest[j] = dd_rest("w1", *_rows2(stage_a1(w, TS + LEAD + sum(CBS[:j]), CBS[j], f32=True)))
            else:
                ra, n = PART[op[1]]
                parts = [rest[j] for j in range(len(CBS)) if ra - TS <= sum(CBS[:j]) < ra - TS + n]
                stage_a2(w, parts, ra + LEAD, n, last_valid=(s < NT - 2) if ra + n == 2 * TS else None)
        out_copy(r0, TS).start()
        return carry

    with jax.named_scope("p2main"):
        jax.lax.fori_loop(1, NT - 1, step, 0)
    with jax.named_scope("p2epi"):
        w = window(S - 2 * TS, 2 * TS + LEAD)
        rows = pl.ds(S - TS, TS)
        pending.append(hhbuf[0, pl.ds(S, 8), :])
        def flush(rows, cols):
            pltpu.make_async_copy(obuf.at[rows, cols], out_hbm.at[rows, cols], sem_out.at[0]).start()

        done = {0: {}, 1: {}}
        for j in range(2):
            stage_b2b(w, hbb, TS, TS, j, done=done)
        for k in NEST:
            stage_b2n(w, hbb, TS, TS, k, done)
        flush(rows, pl.ds(0, 512))
        sub = 0
        for n in (128, 64, 64):
            stage_b2b(w, hbb, TS, n, 2, sub=sub)
            flush(pl.ds(S - TS + sub, n), pl.ds(512, 128))
            sub += n
        pltpu.make_async_copy(obuf, out_hbm, sem_out.at[0]).wait()


@jax.jit
def pallas_adaLN_cond__ssm_conv_h3__mixer_s_mlp__prompt_kernel(
    A_q: jax.Array,
    A_k: jax.Array,
    A_v: jax.Array,
    A_shift_k: jax.Array,
    A_ssm_k: jax.Array,
    A_ssm_D: jax.Array,
    B_x: jax.Array,
    B_w1: jax.Array,
    B_w2: jax.Array,
    B_w3: jax.Array,
    B_w4: jax.Array,
    c: jax.Array,
    w_mod: jax.Array,
):
    del B_x

    def tiles(x):
        return x.reshape(S // 8, 8, NC, 128).transpose(0, 2, 1, 3).reshape(S * NC, 128)

    def pairs(x):
        r, n = x.shape
        return x.reshape(r // 16, 2, 8, n // 128, 128).transpose(0, 1, 3, 2, 4)

    args = (
        A_q.reshape(S, D), tiles(A_k), tiles(A_v),
        A_shift_k.T, A_ssm_k, A_ssm_D.reshape(NC, 128),
        pairs(B_w1), pairs(B_w2), pairs(B_w3.T), pairs(B_w4), c, pairs(w_mod),
    )
    scratch = [
        pltpu.VMEM((NA, P * NC + 128, 128), BF16),
        pltpu.VMEM((NA, P * NC + 64, 128), BF16),
        pltpu.VMEM((D, S), BF16),
        pltpu.VMEM((R, 256, 128), BF16),
        pltpu.VMEM((2, R, 128, 128), BF16),
        pltpu.VMEM((128, 128), BF16),
        pltpu.VMEM((D // 16, 6 * NC, 16, 128), BF16),
        pltpu.VMEM((D // 16, NC, 16, 128), BF16),
        pltpu.VMEM((D // 16, NC, 16, 128), BF16),
        pltpu.VMEM((FF // 16, NC, 16, 128), BF16),
        pltpu.VMEM((FF // 16, NC, 16, 128), BF16),
        pltpu.VMEM((S + 64, D), BF16),
        *[pltpu.VMEM((NA, R, 16, 4, 8, 128), F32) for _ in range(NC)],
        pltpu.VMEM((NC, 2, R, 16, 2, 8, 128), F32),
        pltpu.VMEM((2 * NC, R, 256, 128), BF16),
        pltpu.VMEM((32, 128), U32),
        pltpu.VMEM((NC, 8, 8, 128), F32),
        pltpu.VMEM((NC, S + 32, 128), F32),
        pltpu.VMEM((8, 8, D), F32),
        pltpu.VMEM((S + 32, D), F32),
        pltpu.VMEM((NC, S + 32, 128), F32),
        pltpu.VMEM((NC, S + 32, 128), F32),
        pltpu.VMEM((8, 2, TS + 16, 128), BF16),
        pltpu.VMEM((5, 2, 1, 256, 128), BF16),
        pltpu.VMEM((5, 2, 1, 256, 128), BF16),
        pltpu.VMEM((5, 6, 2, 128, 128), BF16),
        pltpu.VMEM((5, 2, 2, FT, 128), BF16),
        pltpu.VMEM((5, 2, 1, 896, 128), BF16),
        pltpu.VMEM((8, 9, 144, 128), BF16),
        pltpu.VMEM((8, 9, 144, 128), BF16),
        pltpu.VMEM((2, 8, 384, 128), BF16),
        pltpu.VMEM((NQ, 8, 384, 128), BF16),
        pltpu.VMEM((S, D), BF16),
        pltpu.VMEM((4, D), BF16),
        pltpu.VMEM((NC, 128), BF16),
        pltpu.VMEM((1, D), BF16),
        pltpu.SMEM((64,), jnp.int32),
        pltpu.SemaphoreType.DMA((40,)),
        pltpu.SemaphoreType.DMA((1,)),
    ]
    out = pl.pallas_call(
        _kernel,
        out_shape=jax.ShapeDtypeStruct((S, D), BF16),
        in_specs=[pl.BlockSpec(memory_space=pl.ANY)] * len(args),
        out_specs=pl.BlockSpec(memory_space=pl.ANY),
        scratch_shapes=scratch,
        grid=(1,),
        compiler_params=pltpu.CompilerParams(vmem_limit_bytes=108 * 1024 * 1024, disable_semaphore_checks=True,
                                             disable_bounds_checks=True),
        name="adaln_h3_mixer",
    )(*args)
    return out.reshape(1, S, D)
```

```python
import numpy as np
import jax
import jax.numpy as jnp
import jax.experimental.pallas as pl
import jax.experimental.pallas.tpu as pltpu

F32 = jnp.float32
BF16 = jnp.bfloat16
U32 = jnp.uint32

S = 2048
D = 640
FF = 1728
NC = D // 128
R = 4
P = 128 * R
NA = S // P
TS = 256
NT = S // TS
LEAD = 16
EPS = 1e-5
N3 = (1, 3, 4, 2)
NEST = (1, 4, 0, 2, 3, 5)
NQ = len(NEST)
FT = (FF - 1536) // 2


def _freq(row):
    t, part, s = row >> 4, (row >> 3) & 1, row & 7
    return 32 * (t & 7) + 4 * s + 2 * (t >> 3) + 1, P * part


def _cos(j, scale):
    jf = (j & (4 * P - 1)).astype(F32)
    u = 2.0 * np.pi / (4 * P)
    x = jnp.abs(jf * u - np.pi) - 0.5 * np.pi
    x2 = x * x
    poly = scale / 362880.0 - x2 * (scale / 39916800.0)
    for coef in (-1.0 / 5040.0, 1.0 / 120.0, -1.0 / 6.0, 1.0):
        poly = poly * x2 + coef * scale
    return poly * x


_DUR = {"t": 8, "u": 16, "k": 16, "i": 16, "m": 12, "g": 0, "c": 0, "j": 16}
_POST = {"t": 8.0, "u": 16.0, "k": 24.0, "i": 4.0, "j": 4.0, "m": 18.0}


def _plan_tokens(order, maxutil):
    lag, cap, pre, margin = 8, 62, 4, 3
    start, slots = {}, []
    for n in order:
        start[n] = len(slots)
        slots += [(n, r) for r in range(_DUR[n[0]])]
    nslot = len(slots) + lag
    free = [cap - (_POST[slots[i - lag][0][0]] if i >= lag else 0.0) for i in range(-pre, nslot)]
    units = []
    for n in order:
        kind, a, c = n
        if kind == "u":
            units += [(n + (g,), 94.0, start[n], -pre) for g in range(8)]
        elif kind == "g":
            units += [(n + (g,), 150.0, start[n], -pre) for g in range(8)]
        elif kind in "ic":
            src_ = [start[m] for m in (("u", a, c), ("k", a, c)) if m in start]
            for t in range(16):
                rel = max(max(src_) + 16, max(src_) + t + lag + 3) if src_ else -pre
                units.append((n + (t,), 32.0 * a + 48.0, nslot if kind == 'c' else start[n], rel))

    def simulate(util):
        left = [u[1] for u in units]
        done = [None] * len(units)
        for i in range(-pre, nslot):
            budget = util * free[i + pre]
            for j, u in enumerate(units):
                if budget <= 0.0:
                    break
                if done[j] is None and u[3] <= i:
                    use = min(budget, left[j])
                    left[j] -= use
                    budget -= use
                    if left[j] <= 1e-9:
                        done[j] = i + 1
        ok = all(u[2] < 8 or (d is not None and d <= max(u[2] - (1 if u[0][0] in 'cg' else margin), u[3] + 1))
                 for d, u in zip(done, units))
        return done, ok

    lo_, hi_ = 0.05, maxutil
    for _ in range(12):
        mid = 0.5 * (lo_ + hi_)
        if simulate(mid)[1]:
            hi_ = mid
        else:
            lo_ = mid
    done, _ = simulate(hi_)
    plan = {}
    for u, d in zip(units, done):
        if u[0][0] == "c":
            plan[u[0]] = slots[max((nslot - 1 if d is None else min(d, nslot - 1)) - lag, 0)]
        elif d is not None and 0 <= d < u[2]:
            plan.setdefault(slots[d], []).append(u[0])
    return plan


def _unpack(w):
    return pltpu.bitcast(w, BF16)


def _dot(a, b):
    return jnp.dot(a.astype(BF16), b, preferred_element_type=F32)


def _dot_nt(a, b):
    return jax.lax.dot_general(a.astype(BF16), b, (((1,), (1,)), ((), ())), preferred_element_type=F32)


def _dot_fine(x, w, chunk):
    if not chunk:
        return _dot(x, w)
    n = w.shape[1]
    head = _dot(x, w[:, :n - 128])
    last = jnp.concatenate([_dot(x[r:r + chunk], w[:, n - 128:]) for r in range(0, x.shape[0], chunk)], axis=0)
    return jnp.concatenate([head, last], axis=1)


def _rows2(x):
    n, c = x.shape
    x = x.reshape(n // 32, 2, 16, c)
    return x[:, 0].reshape(n // 2, c), x[:, 1].reshape(n // 2, c)


def _unrows2(top, bot):
    n, c = top.shape
    return jnp.stack([top.reshape(n // 16, 16, c), bot.reshape(n // 16, 16, c)], axis=1).reshape(2 * n, c)


def _sums_a(a11, a12, a21, a22):
    return [a11 + a22, a21 + a22, a11 + a12, a21 - a11, a12 - a22]


def _sums_b(b11, b12, b21, b22):
    return [b11 + b22, b12 - b22, b21 - b11, b11 + b12, b21 + b22]


_STRASSEN = ((0, 0), (1, 5), (5, 1), (6, 2), (2, 6), (3, 3), (4, 4))


_SUMS_A = ((0, 3, 1), (2, 3, 1), (0, 1, 1), (2, 0, -1), (1, 3, -1))
_SUMS_B = ((0, 3, 1), (1, 3, -1), (2, 0, -1), (0, 1, 1), (2, 3, 1))


def _combine(m1, m2, m3, m4, m5, m6, m7):
    return (m1 + m4) + (m7 - m5), m3 + m5, m2 + m4, (m1 - m2) + (m3 + m6)


def _lo(w):
    return pltpu.bitcast(w << 16, F32)


def _hi(w):
    return pltpu.bitcast(w & jnp.uint32(0xFFFF0000), F32)


def _ln(x, eps=EPS):
    m = jnp.sum(x, axis=-1, keepdims=True) * (1.0 / D)
    xc = x - m
    v = jnp.sum(xc * xc, axis=-1, keepdims=True) * (1.0 / D)
    return xc * jnp.exp(-0.5 * jnp.log(v + eps))


def _gelu2(x):
    c0 = 0.7978845608028654
    c1 = c0 * 0.044715
    return x + x * jnp.tanh(x * (c0 + c1 * (x * x)))


def _bfly(tr, ti):
    s02r, s02i = tr[0] + tr[2], ti[0] + ti[2]
    d02r, d02i = tr[0] - tr[2], ti[0] - ti[2]
    s13r, s13i = tr[1] + tr[3], ti[1] + ti[3]
    d13r, d13i = tr[1] - tr[3], ti[1] - ti[3]
    x0r, x0i = s02r + s13r, s02i + s13i
    x2r, x2i = s02r - s13r, s02i - s13i
    return [x0r, d02r + d13i, x2r, d02r - d13i], [x0i, d02i - d13r, x2i, d02i + d13r]


def _kernel(q_hbm, k_hbm, v_hbm, shift_hbm, ssmk_hbm, ssmd_hbm, w1_hbm, w2_hbm, w3t_hbm, w4_hbm,
            c_hbm, wmod_hbm,
            out_hbm,
            kbuf, vbuf, skbuf, fwdbuf, invbuf, permbuf,
            wmodbuf, w1buf, w2buf, w3buf, w4buf, qbuf,
            xs0, xs1, xs2, xs3, xs4, kraw, stg, zbuf, coefbuf, ybuf, modbuf, x2buf, hbuf, hhbuf, xobuf,
             w1s, w2s, w3s, w3ts, w4s, hba, hbb, w4n, w4q, w3n, xibuf, obuf, shiftbuf, dbuf, cbuf,
            zsm, sem_in, sem_out):
    cps = {}
    n_sem = [0]

    def start(name, src, dst):
        cp = pltpu.make_async_copy(src, dst, sem_in.at[n_sem[0]])
        n_sem[0] += 1
        cp.start()
        cps[name] = cp

    class Both:
        def __init__(self, a, b):
            self.cps = (a, b)

        def wait(self):
            for cp in self.cps:
                cp.wait()

    def start_w(name, src, dst, c0=0, n=NC):
        for e in range(2):
            start(name + str(e), src.at[:, e, pl.ds(c0, n)], dst.at[:, pl.ds(c0, n), pl.ds(8 * e, 8), :])
        cps[name] = Both(cps[name + "0"], cps[name + "1"])

    CH = P * NC
    HALO = 8 * NC

    def start_s(a):
        cols = pl.ds(a * P, P)
        start("s%d" % a, ssmk_hbm.at[:, cols], skbuf.at[:, cols])

    def start_kv(a):
        if a == 0:
            kbuf[0, pl.ds(0, HALO + 8), :] = jnp.zeros((HALO + 8, 128), BF16)
            start("k0", k_hbm.at[pl.ds(0, CH), :], kbuf.at[0, pl.ds(HALO, CH), :])
        else:
            start("k%d" % a, k_hbm.at[pl.ds(a * CH - HALO, CH + HALO), :], kbuf.at[a, pl.ds(0, CH + HALO), :])
        start("v%d" % a, v_hbm.at[pl.ds(a * CH, CH), :], vbuf.at[a, pl.ds(0, CH), :])

    for n in "s0 x0 s1 k0 k1 s2 k2 s3 k3".split():
        if n[0] == "s":
            start_s(int(n[1]))
        elif n[0] == "k":
            start_kv(int(n[1]))
        else:
            start("d", ssmd_hbm, dbuf)
            start("shift", shift_hbm, shiftbuf)
            start("c", c_hbm, cbuf)
    QA = TS + LEAD
    XA = 128
    QB = 2 * TS + LEAD
    W1A = 2

    def start_q(name, r0, n):
        start(name, q_hbm.at[pl.ds(r0, n), :], qbuf.at[pl.ds(r0, n), :])

    start_q("qa", 0, QA)
    start_w("wmoda", wmod_hbm, wmodbuf, 0, 3 * NC)
    start_w("wmodb", wmod_hbm, wmodbuf, 3 * NC, 2 * NC)
    start_q("qx", QA, XA)
    start_w("w1a", w1_hbm, w1buf, 0, W1A)
    start_w("w1b", w1_hbm, w1buf, W1A, NC - W1A)
    start_q("qb", QA + XA, QB - QA - XA)
    start_w("w2", w2_hbm, w2buf)
    start_w("w3", w3t_hbm, w3buf)
    start_w("w4", w4_hbm, w4buf)
    start_w("wmodg", wmod_hbm, wmodbuf, 5 * NC, NC)
    start_q("q1", QB, S - QB)

    kw = kbuf.bitcast(U32)
    vw = vbuf.bitcast(U32)
    zbuf[...] = jnp.zeros(zbuf.shape, U32)
    for j in range(64):
        zsm[j] = 0
    for c in range(NC):
        ybuf[c, pl.ds(S, LEAD), :] = jnp.zeros((LEAD, 128), F32)
        hhbuf[c, pl.ds(0, 8), :] = jnp.zeros((8, 128), F32)
    qbuf[pl.ds(S, LEAD), :] = jnp.zeros((LEAD, D), BF16)

    def sample(pos):
        return (pos & ~15) + 2 * (pos & 7) + ((pos >> 3) & 1)

    def tables(p, carry):
        f2, off = _freq(jax.lax.broadcasted_iota(jnp.int32, (256, 128), 0))
        n = R * sample(jax.lax.broadcasted_iota(jnp.int32, (256, 128), 1)) + p
        fwdbuf[p] = _cos(f2 * n + off, 1.0).astype(BF16)
        return carry

    jax.lax.fori_loop(0, R, tables, 0)

    def unit_g(kt, r):
        f2, off = _freq(jax.lax.broadcasted_iota(jnp.int32, (16, 128), 1) + 128 * kt)
        j0 = f2 * (R * (jax.lax.broadcasted_iota(jnp.int32, (16, 128), 0) + 16 * r)) + off
        for p in range(R):
            invbuf[kt, p, pl.ds(16 * r, 16), :] = _cos(j0 + p * f2, 1.0 / P).astype(BF16)
        return [invbuf.bitcast(U32)[kt, p, pl.ds(8 * r, 8), :] for p in range(R)]

    i0 = jax.lax.broadcasted_iota(jnp.int32, (128, 128), 0)
    i1 = jax.lax.broadcasted_iota(jnp.int32, (128, 128), 1)
    permbuf[...] = jnp.where(i1 == R * sample(i0 & 31) + (i0 >> 5), 1.0, 0.0).astype(BF16)

    def fill_coef():
        cv = cbuf[...].astype(F32)
        modbuf[6] = jnp.broadcast_to(cv * jax.nn.sigmoid(cv), (8, D))
        coef = shiftbuf[...].astype(F32)
        dval = dbuf[...].astype(F32)
        for c in range(NC):
            for j in range(4):
                coefbuf[c, j] = jnp.broadcast_to(coef[j:j + 1, c * 128:(c + 1) * 128], (8, 128))
            coefbuf[c, 4] = jnp.broadcast_to(dval[c:c + 1, :], (8, 128))

    xs = (xs0, xs1, xs2, xs3, xs4)
    wsbufs = dict(w1=w1s, w2=w2s, w3=w3s, w4=w4s, w3t=w3ts)
    def split_ri(t):
        t = t.reshape(16, 2, 8, 128)
        return t[:, 0], t[:, 1]

    def get_never():
        return zbuf[pl.ds(0, 8), :] != 0

    def packed(x, slot, r0):
        n = x.shape[1]
        stg[slot, :, pl.ds(r0, n), :] = x.astype(BF16)
        return [stg.bitcast(U32)[slot, p, pl.ds(r0 // 2, n // 2), :] for p in range(R)]

    UG = 8

    def unit_u(a, c, g0, UG):
        c0, c1, c2, c3 = (coefbuf[c, pl.ds(j, 1)][None] for j in range(4))
        rows = lambda ref, r: ref[a, pl.ds((r // 4) * 4 * NC + 4 * c + r % 4, 8 * UG, stride=4 * NC), :]
        kk = jnp.stack([rows(kw, 4 + 32 * g0 + d) for d in range(-2, 4)]).reshape(6, UG, 8, 128)
        vv = jnp.stack([rows(vw, 32 * g0 + d) for d in range(4)]).reshape(4, UG, 8, 128)
        lo, hi = _lo(kk), _hi(kk)
        k0, k1, k2 = lo[2:], hi[1:5], lo[1:5]
        even = ((k0 * c0 + k1 * c1) + (k2 * c2 + hi[:4] * c3)) * _lo(vv)
        odd = ((hi[2:] * c0 + k0 * c1) + (k1 * c2 + k2 * c3)) * _hi(vv)
        kv = jnp.stack([even, odd], axis=1).reshape(2, R, UG, 8, 128)
        return packed(jnp.stack([kv[0], kv[1]], axis=2).reshape(R, 16 * UG, 128), NC + c, 16 * g0)

    def unit_i(a, c, t0, UG, z, after=None):
        x_c = xs[c].at[pl.ds(z, NA)]
        ts = pl.ds(t0, UG)
        yr = yi = None
        for j in range(a + 1):
            ur, ui = x_c[j, :, ts, 0], x_c[j, :, ts, 1]
            kr, ki = x_c[a - j, :, ts, 2], x_c[a - j, :, ts, 3]
            pr = ur * kr - ui * ki
            pi = ur * ki + ui * kr
            yr = pr if yr is None else yr + pr
            yi = pi if yi is None else yi + pi
        sr, si, dr, di = yr[:2] + yr[2:], yi[:2] + yi[2:], yr[:2] - yr[2:], yi[:2] - yi[2:]
        (sr0, sr1), (si0, si1), (dr0, dr1), (di0, di1) = ((x[0], x[1]) for x in (sr, si, dr, di))
        wr = jnp.stack([sr0 + sr1, dr0 - di1, sr0 - sr1, dr0 + di1])
        wi = jnp.stack([si0 + si1, di0 + dr1, si0 - si1, di0 - dr1])
        if after is not None:
            never = jnp.broadcast_to(zbuf[pl.ds(0, 8), :], wr.shape) != 0
            wr = jax.lax.select(never, jnp.broadcast_to(after, wr.shape), wr)
        return packed(jnp.stack([wr, wi], axis=2).reshape(R, 16 * UG, 128), c, 16 * t0)

    def segment(spec, z, maxutil=1.0, mod_fn=None):
        order = [(n[0], int(n[1]), int(n[2])) for n in spec.split()]
        plan = _plan_tokens(order, maxutil) if maxutil > 0 else {}
        never = get_never()
        units, groups, res = {}, {}, {}

        paced = {k_ for s_, ks in plan.items() if len(s_) == 2 for k_ in ks}

        def width(name):
            n = 8 if name[0] == "u" else 16
            return UG if all(name + (j,) in paced for j in range(n)) else 1

        def group(key):
            kind, a, c, j = key
            ug = width(key[:3])
            key = (kind, a, c, j - j % ug)
            if key not in groups:
                if kind == "u":
                    groups[key] = unit_u(a, c, key[3], ug)
                else:
                    fresh = ("u", a, c) in order or ("k", a, c) in order
                    groups[key] = unit_i(a, c, key[3], ug, z if fresh else 0,
                                         res[plan[key]]() if kind == "c" else None)
            return groups[key]

        def unit(key):
            if key not in units:
                if key[0] == "g":
                    units[key] = unit_g(key[1], key[3])
                else:
                    r = 8 * (key[3] % width(key[:3]))
                    units[key] = [v[r:r + 8] for v in group(key)]
            return units[key]

        def lhs(name, p, full, r0=0):
            out, last = [], 0
            for r in range(full.shape[0] // 8):
                keys = plan.get((name, r0 + r), ())
                if keys:
                    if 8 * r > last:
                        out.append(full[last:8 * r])
                    v = full[8 * r:8 * r + 8]
                    for key in keys:
                        v = jax.lax.select(never, unit(key)[p], v)
                    out.append(v)
                    last = 8 * r + 8
            if last < full.shape[0]:
                out.append(full[last:] if last else full)
            return out[0] if len(out) == 1 else jnp.concatenate(out, axis=0)

        def dft(name, rhs):
            tr, ti = [], []
            for p in range(R):
                f = lhs(name, p, fwdbuf.bitcast(U32)[p])
                r_, i_ = split_ri(_dot(_unpack(f), rhs[p]))
                if p == 0:
                    res.update({(name, r): (lambda r=r, v=r_: v[r]) for r in range(16)})
                tr.append(r_)
                ti.append(i_)
            return _bfly(tr, ti)

        st = {}
        for name in order:
            kind, a, c = name
            x_c = xs[c]
            if kind == "g":
                for r in range(8):
                    unit(name + (r,))
            elif kind == "c":
                for t in range(16):
                    group(name + (t,))
            elif kind == "m":
                toks = {}
                for r in range(_DUR["m"]):
                    for n_, key in enumerate(plan.get((name, r), ())):
                        toks.setdefault(2 * r + n_ % 2, []).extend(unit(key))
                mod_fn(a, toks)
            elif kind == "t":
                trs = []
                for b in range(R):
                    pm = lhs(name, b, permbuf.bitcast(U32)[...])
                    trs.append(_dot_nt(_unpack(pm), skbuf[pl.ds(c * 128, 128), pl.ds(a * P + b * 128, 128)]))
                res.update({(name, r): (lambda r=r, v=trs[0]: v[16 * r:16 * r + 8]) for r in range(8)})
                g_ = 128 // R
                st[a, c] = [jnp.concatenate([trs[b][p * g_:(p + 1) * g_] for b in range(R)], axis=0).astype(BF16)
                            for p in range(R)]
            elif kind == "u":
                rhs = [_unpack(jnp.concatenate([group(name + (g,))[p] for g in range(0, 8, width(name))], axis=0)) for p in range(R)]
                xr, xi = dft(name, rhs)
                for q in range(R):
                    x_c[a, q, :, 0] = xr[q]
                    x_c[a, q, :, 1] = xi[q]
            elif kind == "k":
                xr, xi = dft(name, st[a, c])
                for q in range(R):
                    if a == 0:
                        x_c[a, q, :, 2] = xr[q] + coefbuf[c, 4]
                        x_c[a, q, :, 3] = xi[q]
                    else:
                        pr, pi = kraw[c, (a - 1) % 2, q, :, 0], kraw[c, (a - 1) % 2, q, :, 1]
                        x_c[a, q, pl.ds(0, 8), 2] = xr[q][:8] - pi[:8]
                        x_c[a, q, pl.ds(0, 8), 3] = xi[q][:8] + pr[:8]
                        x_c[a, q, pl.ds(8, 8), 2] = xr[q][8:] + pi[8:]
                        x_c[a, q, pl.ds(8, 8), 3] = xi[q][8:] - pr[8:]
                    if a + 1 < NA:
                        kraw[c, a % 2, q, :, 0] = xr[q]
                        kraw[c, a % 2, q, :, 1] = xi[q]
            else:
                for p in range(R):
                    cols = [lhs(name, 2 * (p % 2) + kt,
                                invbuf.bitcast(U32)[kt, p], 8 * (p // 2))
                            for kt in range(2)]
                    g = _unpack(jnp.concatenate(cols, axis=1))
                    if kind == "j":
                        wp = _unpack(stg.bitcast(U32)[c, p])
                    else:
                        wp = _unpack(jnp.concatenate([group(name + (t,))[p] for t in range(0, 16, width(name))], axis=0))
                    yp = _dot(g, wp)
                    if p % 2 == 0:
                        res.update({(name, 4 * p + r): (lambda r=r, v=yp: v[16 * r:16 * r + 8]) for r in range(8)})
                    ybuf[c, pl.ds(a * P + p, 128, stride=R), :] = yp

    one = jnp.minimum(pl.program_id(0) + 1, 1)

    def once(fn):
        def body(z, carry):
            fn(z)
            return carry
        jax.lax.fori_loop(0, one, body, 0)

    default = ("t00 t01 t02 k00 t03 k01 t04 k02 k03 k04 g00|"
               "t10 t11 t12 k10 k11 k12 g10|"
               "t13 t14 k13 u00 k14 u01 u02 u03 i00 u04 i01 c02 c03|"
               "j02 j03 u10 i04 u11 u12 u13 i10 u14 i11 c12 c13|"
               "t20 t21 j12 t22 j13 t23 t24 k20 u20 k21 u21 k22 i14 k23 u22 k24 u23 i20 u24 i21 c22|"
               "t30 t31 j22 t32 t33 t34 k30 u30 k31 u31 k32 i23 k33 u32 k34 i24 u33 i30 u34 i31 c32|"
               "m00 j32 m10 i33 m20 i34")
    specs = default.split("|")
    G5B = specs[-1]
    segs = list(zip("s0 d shift c|s1|k0 v0|k1 v1|s2 k2 v2|s3 k3 v3".split("|"), specs[:-1]))
    MU = 1.5
    for i, (waits, spec) in enumerate(segs):
        with jax.named_scope("g%d" % i):
            for n in waits.split():
                cps[n].wait()
            if i == 0:
                fill_coef()
            once(lambda z: segment(spec, z, MU))

    def mod_cols(lo, n, toks=None):
        m = _dot(modbuf[6], weights(wmodbuf, lo * NC, (lo + n) * NC, toks=toks))
        return [m[:, j * D:(j + 1) * D] for j in range(n)]

    def mul_mod(x, j, cols=None):
        m = modbuf[j] if cols is None else modbuf[j, :, cols]
        return (x.reshape(-1, 8, x.shape[-1]) * m[None]).reshape(x.shape)

    def add_mod(x, j):
        return (x.reshape(-1, 8, x.shape[-1]) + modbuf[j][None]).reshape(x.shape)

    def slabs(ref, r0, n):
        return jnp.concatenate([ref[c, pl.ds(r0, n), :] for c in range(NC)], axis=1)

    def put(ref, rows, x):
        for c in range(NC):
            ref[c, rows, :] = x[:, c * 128:(c + 1) * 128]

    def window(base, n):
        rows = pl.ds(base, n)
        return dict(q=qbuf.at[rows, :], y=ybuf.at[:, rows, :], x2=x2buf.at[rows, :], h=hbuf.at[:, rows, :],
                    hh=hhbuf.at[:, pl.ds(base, n + 8), :],
                    o=obuf.at[pl.ds(base, n - LEAD), :])

    def weights(ref, c0=0, c1=NC, r0=0, r1=None, toks=None, raw=False, z=None):
        r1 = 16 * ref.shape[0] if r1 is None else r1
        view = ref.bitcast(U32)
        if z is not None:
            view = view.at[pl.ds(z, ref.shape[0])]
        never = get_never() if toks else None
        rt = -(-(r1 - r0) // 128)
        cols = []
        for j in range(c0, c1):
            wu = view[pl.ds(r0 // 16, (r1 - r0) // 16), j].reshape((r1 - r0) // 2, 128)
            if toks:
                parts, last = [], 0
                for i in range(rt):
                    for n_, t in enumerate(toks.get((j - c0) * rt + i, ())):
                        r = 64 * i + 8 * n_
                        if r > last:
                            parts.append(wu[last:r])
                        parts.append(jax.lax.select(never, t, wu[r:r + 8]))
                        last = r + 8
                parts.append(wu[last:])
                wu = jnp.concatenate(parts, axis=0)
            cols.append(wu)
        wu = jnp.concatenate(cols, axis=1)
        return wu if raw else _unpack(wu)

    def keep(dst, v):
        h = v.shape[0] // 2
        for c in range(v.shape[1] // 128):
            for r in (0, h):
                dst[c, pl.ds(r, h), :] = v[r:r + h, 128 * c:128 * (c + 1)].astype(BF16)

    def fetch(src_):
        u = src_.bitcast(U32)
        return jnp.concatenate([u[c] for c in range(u.shape[0])], axis=1)

    def wblocks(name, j, z=None):
        if name == "w3":
            blk = lambda kh, nh: weights(w3buf, 2 * kh, 2 * kh + 2, 128 * (j + 6 * nh), 128 * (j + 6 * nh + 1), raw=True, z=z)
        elif name == "w4":
            def blk(kh, nh):
                c = j + 2 * nh
                parts = [weights(w4buf, c, c + 1, 768 * kh, 768 * (kh + 1), raw=True, z=z),
                         weights(w4buf, c, c + 1, 1536 + FT * kh, 1536 + FT * (kh + 1), raw=True, z=z),
                         jnp.zeros(((128 - FT) // 2, 128), U32)]
                return jnp.concatenate(parts, axis=0)
        elif name == "w3t":
            blk = lambda kh, nh: weights(w3buf, 2 * kh, 2 * kh + 2, 1536 + FT * nh, 1536 + FT * (nh + 1), raw=True, z=z)
        else:
            ref = w1buf if name == "w1" else w2buf
            blk = lambda kh, nh: weights(ref, j + 2 * nh, j + 2 * nh + 1, 256 * kh, 256 * (kh + 1), raw=True, z=z)
        return blk

    def wsum(name, j, k):
        blk = wblocks(name, j, zsm[k])
        p, q, sign = _SUMS_B[k]
        return psum(blk(p // 2, p % 2), blk(q // 2, q % 2), sign)

    pending = []

    def attach(wv):
        if not pending:
            return wv
        never = get_never()
        rows = [wv[8 * i:8 * i + 8, :128] for i in range(8)]
        for i, t in enumerate(pending):
            rows[i % 8] = jax.lax.select(never, pltpu.bitcast(t, U32), rows[i % 8])
        pending.clear()
        first = jnp.concatenate(rows + ([wv[64:, :128]] if wv.shape[0] > 64 else []), axis=0)
        return first if wv.shape[1] == 128 else jnp.concatenate([first, wv[:, 128:]], axis=1)

    def sprods(name, j, lhs, k0=0, k1=7, prep=False):
        blk, buf = wblocks(name, j), wsbufs[name]
        out = []
        for ia, ib in _STRASSEN[k0:k1]:
            if prep and ib < 5:
                wv = wsum(name, j, ib)
                keep(buf.at[ib, j], wv)
                wv = wv.astype(BF16)
            else:
                wv = _unpack(attach(blk(ib - 5, ib - 5) if ib >= 5 else fetch(buf.at[ib, j])))
            if name == "w3t":
                out.append(_dot_nt(wv, lhs(ia)))
            else:
                out.append((_dot_nt if name == "w3" else _dot)(lhs(ia), wv))
        return out

    def spair(name, j, lhs, prep=False):
        return _combine(*sprods(name, j, lhs, prep=prep))

    def dd_rest(name, t, b):
        ref = w1buf if name == "w1" else w2buf
        m = t.shape[0]
        xb = jnp.concatenate([t, b], axis=0)
        last = _dot(xb, weights(ref, 4, 5))
        rem = _dot(xb[:, 512:], weights(ref, 0, 4, r0=512))
        return t, b, rem[:m], rem[m:], last[:m], last[m:]

    def dd_main(name, parts, prep=False):
        t, b, rt, rb, lt, lb = (jnp.concatenate(v, axis=0) for v in zip(*parts))
        ops = _sums_a(t[:, :256], t[:, 256:512], b[:, :256], b[:, 256:512]) + [t[:, :256], b[:, 256:512]]
        top, bot = [None] * 4, [None] * 4
        for j in range(2):
            top[j], top[j + 2], bot[j], bot[j + 2] = spair(name, j, lambda i: ops[i], prep)
        return (jnp.concatenate([jnp.concatenate(top, axis=1) + rt, lt], axis=1),
                jnp.concatenate([jnp.concatenate(bot, axis=1) + rb, lb], axis=1))

    def stage_a0(w, r0, n):
        rows = pl.ds(r0, n)
        x = w["q"][rows, :].astype(F32)
        x2 = x + add_mod(mul_mod(_ln(x), 1), 0) * slabs(w["y"], r0, n)
        w["x2"][rows, :] = x2
        return _ln(x2)

    def stage_a1(w, r0, n, n2=None, f32=False):
        if n2 is None:
            n2 = stage_a0(w, r0, n)
        h = add_mod(mul_mod(n2, 4), 3)
        put(w["h"], pl.ds(r0, n), h)
        n3 = _ln(h, 4 * EPS)
        return n3 if f32 else n3.astype(BF16)

    def stage_a2(w, n3, r0, n, last_valid=None, fine=0, c0=0, c1=NC, prep=False):
        hh = _gelu2(_unrows2(*dd_main("w1", n3, prep)) if isinstance(n3, list) else _dot_fine(n3, weights(w1buf, c0, c1), fine))
        for c in range(c0, c1):
            blk = hh[:, (c - c0) * 128:(c - c0 + 1) * 128]
            w["hh"][c, pl.ds(r0 + 8, n - LEAD), :] = blk[:n - LEAD]
            tail = blk[n - LEAD:]
            if last_valid is not None:
                tail = jnp.where(last_valid, tail, 0.0)
            w["hh"][c, pl.ds(r0 + 8 + n - LEAD, LEAD), :] = tail

    def stage_b1a(w, r0, n, prep=False):
        lane = jax.lax.broadcasted_iota(jnp.int32, (n, 128), 1)
        sh = lambda c, d: w["hh"][c, pl.ds(r0 + 8 + d, n), :]
        g = jnp.concatenate([sh(0, -1),
                             jnp.where(lane < 32, sh(1, -1), sh(1, 1)),
                             jnp.where(lane < 64, sh(2, 1), sh(2, -2)),
                             jnp.where(lane < 96, sh(3, -2), sh(3, 2)),
                             sh(4, 2)], axis=1)
        x1 = slabs(w["h"], r0, n) + _unrows2(*dd_main("w2", [dd_rest("w2", *_rows2(g))], prep))
        put(w["h"], pl.ds(r0, n), x1)
        return x1

    def stage_b1b(w, x1, r0, n, deep=True):
        t, b = _rows2(_ln(x1, 4 * EPS))
        ops = _sums_a(t[:, :256], t[:, 256:512], b[:, :256], b[:, 256:512]) + [t[:, :256], b[:, 256:512]]
        ops.append(jnp.concatenate([t[:, 512:], b[:, 512:]], axis=1))
        for i, v in enumerate(ops):
            keep(xobuf.at[i, :, pl.ds(r0 // 2, n // 2), :], v)
        if deep:
            for s_, k in enumerate(N3):
                u, v = _rows2(ops[_STRASSEN[k][0]])
                for i, x in enumerate(_sums_a(u[:, :128], u[:, 128:], v[:, :128], v[:, 128:])):
                    xibuf[s_, i, pl.ds((r0 - TS) // 4, n // 4), :] = x.astype(BF16)
        return [ops[4][i:i + 8, :128] for i in range(0, n // 2, 8)]

    def out_copy(r0, n):
        rows = pl.ds(r0, n)
        return pltpu.make_async_copy(obuf.at[rows, :], out_hbm.at[rows, :], sem_out.at[0])


    def opaque(ref, i):
        ref = ref.bitcast(U32)
        return ref.at[:, :, pl.ds(pl.multiple_of(zsm[i] * 32, 32), ref.shape[2]), :]

    def emit(h3, j, left, right):
        m = left.shape[0] // 2
        g = [left[:m], right[:m], left[m:], right[m:]]
        for k, v in enumerate(_sums_a(*g) + g):
            h3[j, k, pl.ds(0, m), :] = v.astype(BF16)

    def w3_operands(r0, n):
        u, rows = xobuf.bitcast(U32), pl.ds(r0 // 4, n // 4)
        xr = _unpack(jnp.concatenate([u[7, 0, rows, :], u[7, 1, rows, :]], axis=0))
        return xr, lambda i: _unpack(jnp.concatenate([u[i, 0, rows, :], u[i, 1, rows, :]], axis=1))

    def stage_b2h(w, h3, r0, n, prep=False):
        xr, ops = w3_operands(r0, n)
        m = n // 2
        rem = _dot_nt(weights(w3buf, 4, 5, r0=1536), xr)
        c11, c12, c21, c22 = spair("w3t", 0, ops, prep)
        pad = jnp.zeros((128 - FT, m), F32)
        g11, g12, g21, g22 = (jnp.concatenate([_gelu2(c + r), pad], axis=0).T for c, r in (
            (c11, rem[:FT, :m]), (c12, rem[FT:, :m]), (c21, rem[:FT, m:]), (c22, rem[FT:, m:])))
        emit(h3, 6, jnp.concatenate([g11, g21], axis=0), jnp.concatenate([g12, g22], axis=0))

    def stage_b2a(w, h3, r0, n, lo=0, hi=6, prep=False):
        xr, ops = w3_operands(r0, n)
        for j in range(lo, hi):
            r1, r2 = (_dot_nt(xr, weights(w3buf, 4, 5, 128 * t, 128 * (t + 1))) for t in (j, j + 6))
            c11, c12, c21, c22 = spair("w3", j, ops, prep)
            emit(h3, j, _gelu2(jnp.concatenate([c11, c21], axis=0) + r1), _gelu2(jnp.concatenate([c12, c22], axis=0) + r2))

    def stage_b2z(w, h3, g, prep=False):
        xr, ops = w3_operands(TS, TS)
        ms, rem = {0: {}, 1: {}}, {}
        ZO = 0

        def nested(k):
            ib, slot = _STRASSEN[k][1], N3.index(k)

            def quad(i, z=None):
                j, cols = g + 3 * (i % 2), slice(128 * (i // 2), 128 * (i // 2 + 1))
                if ib >= 5:
                    return wblocks("w3", j, z)(ib - 5, ib - 5)[:, cols]
                u = w3s.bitcast(U32)
                return (u if z is None else u.at[pl.ds(z, 5)])[ib, j, i // 2]

            prods = []
            for ja, jb in _STRASSEN:
                if jb >= 5:
                    wv = _unpack(quad(3 * (jb - 5)))
                elif prep:
                    p_, q_, sg = _SUMS_B[jb]
                    wv = psum(quad(p_, zsm[jb]), quad(q_, zsm[jb]), sg)
                    keep(w3n.at[g, slot, pl.ds(jb, 1)], wv)
                    wv = wv.astype(BF16)
                else:
                    wv = _unpack(w3n.bitcast(U32)[g, slot, jb])
                if ja < 5:
                    lv = xibuf.bitcast(U32)[slot, ja, pl.ds(0, TS // 8), :]
                else:
                    e = ja - 5
                    lv = xobuf.bitcast(U32)[_STRASSEN[k][0], e, pl.ds(TS // 4, TS // 4), :]
                    lv = lv.reshape(TS // 64, 2, 8, 128)[:, e].reshape(TS // 8, 128)
                prods.append(_dot_nt(_unpack(lv), wv))
            c11, c12, c21, c22 = _combine(*prods)
            ms[0][k], ms[1][k] = _unrows2(c11, c21), _unrows2(c12, c22)

        def remf(t):
            rem[t] = _dot_nt(xr, weights(w3buf, 4, 5, 128 * t, 128 * (t + 1)))

        early = [g, g + 6, g + 3, g + 9][:ZO]
        for i, k in enumerate(N3):
            nested(k)
            if i < len(early):
                remf(early[i])
        for e in range(2):
            j = g + 3 * e
            for t in (j, j + 6):
                if t not in rem:
                    remf(t)
            for k in range(7):
                if k not in N3:
                    ms[e][k] = sprods("w3", j, ops, k, k + 1)[0]
            c11, c12, c21, c22 = _combine(*[ms[e][k] for k in range(7)])
            emit(h3, j, _gelu2(jnp.concatenate([c11, c21], axis=0) + rem[j]),
                 _gelu2(jnp.concatenate([c12, c22], axis=0) + rem[j + 6]))

    def finish(w, h2, r0, n, c):
        nc = h2.shape[1] // 128
        rows, cols = pl.ds(r0, n), pl.ds(c * 128, nc * 128)
        x1 = jnp.concatenate([w["h"][c + i, rows, :] for i in range(nc)], axis=1)
        w["o"][rows, cols] = (w["x2"][rows, cols] + mul_mod(x1 + h2, 5, cols)).astype(BF16)

    def b2_done(w, done, r0, n):
        if len(done[0]) == len(done[1]) == 7:
            c11, c12, c21, c22 = _combine(*[jnp.concatenate([done[0][k], done[1][k]], axis=1) for k in range(7)])
            finish(w, _unrows2(c11, c21), r0, n, 0)
            finish(w, _unrows2(c12, c22), r0, n, 2)

    def stage_b2b(w, h3, r0, n, j, k0=0, k1=7, done=None, prep=False, sub=0, marks=()):
        hv = opaque(h3, j)
        blk = lambda k: jnp.concatenate([hv[p, k, pl.ds(sub // 4, n // 4), :] for p in range(7)], axis=1)
        r0 += sub
        if j < 2:
            for k in range(k0, k1):
                if k not in NEST:
                    done[j][k] = sprods("w4", j, lambda i: _unpack(blk(8 if i == 6 else i)), k, k + 1, prep)[0]
                    b2_done(w, done, r0, n)
            return
        wb = wblocks("w4", 4)
        lhs = jnp.concatenate([jnp.concatenate([blk(5), blk(6)], axis=1),
                               jnp.concatenate([blk(7), blk(8)], axis=1)], axis=0)
        if marks:
            lo_, hi_ = 0, 52
            never, at = get_never(), {}
            for i, mk in enumerate(marks):
                s_ = lo_ + (hi_ - lo_) * i // len(marks)
                at[4 * (s_ // 16), s_ % 16] = mk
            cols = []
            for kt in range(14):
                col = lhs[:, 128 * kt:128 * (kt + 1)]
                if any(k_[0] == kt for k_ in at):
                    col = jnp.concatenate([jax.lax.select(never, at[kt, r], col[8 * r:8 * r + 8]) if (kt, r) in at
                                           else col[8 * r:8 * r + 8] for r in range(16)], axis=0)
                cols.append(col)
            lhs = jnp.concatenate(cols, axis=1)
        h2 = _dot(_unpack(lhs), _unpack(jnp.concatenate([wb(0, 0), wb(1, 0)], axis=0)))
        finish(w, _unrows2(h2[:n // 2], h2[n // 2:]), r0, n, 4)


    def psum(x, y, sign):
        x, y = _unpack(x).astype(F32), _unpack(y).astype(F32)
        return x + y if sign > 0 else x - y

    def prep_w4(nchunk):
        rows = 384 // nchunk
        marks = []
        for ch in [nchunk] + list(range(nchunk)):
            tail = ch == nchunk
            raw = {}
            for kh in range(2):
                for e in range(1 if tail else 2):
                    r0 = 1536 + FT * kh if tail else 768 * kh + 384 * e + rows * ch
                    x = weights(w4buf, 0, 4, r0, r0 + (FT if tail else rows), raw=True)
                    raw[kh, e] = _unpack(x).astype(F32)
            blk = lambda i, e: raw[i // 2, e][:, 256 * (i % 2):256 * (i % 2 + 1)]
            for k, (ia, ib) in enumerate(_STRASSEN):
                if k not in NEST or ib >= 5:
                    continue
                p_, q_, sg = _SUMS_B[ib]
                half = [blk(p_, e) + blk(q_, e) if sg > 0 else blk(p_, e) - blk(q_, e) for e in range(1 if tail else 2)]
                quad = lambda i: half[i // 2][:, 128 * (i % 2):128 * (i % 2 + 1)]
                first = NEST.index(k)
                if tail:
                    for j in range(2):
                        w4q[first, 7, pl.ds(128 * j, FT), :] = quad(j).astype(BF16)
                        w4q[first, 7, pl.ds(128 * j + FT, 128 - FT), :] = jnp.zeros((128 - FT, 128), BF16)
                    continue
                for jb, v in enumerate(_sums_b(*[quad(i) for i in range(4)]) + [quad(0), quad(3)]):
                    w4q[first, jb, pl.ds(rows * ch, rows), :] = v.astype(BF16)
            if not tail:
                marks.append(w4q.bitcast(U32).at[pl.ds(zsm[32 + ch], NQ)][first, 0, pl.ds(0, 8), :])
        return marks

    def stage_b2n(w, h3, r0, n, k, done, prep=False):
        ia, ib = _STRASSEN[k]
        ka, q, slot = (8 if ia == 6 else ia), n // 8, NEST.index(k)

        def lblk(i, z):
            hv = opaque(h3, z)
            return jnp.concatenate([hv[g + 3 * (i % 2), ka, pl.ds((i // 2) * q, q), :] for g in range(3)], axis=1)

        def raw(j, lo, hi, z=None):
            return wblocks("w4", j, z)(ib - 5, ib - 5)[lo:hi]

        quad = lambda i, z=None: raw(i % 2, 192 * (i // 2), 192 * (i // 2 + 1), z)
        if ib >= 5:
            wt = [raw(j, 384, 448) for j in range(2)]
        else:
            wq = w4q.bitcast(U32)
            wq = wq.at[pl.ds(zsm[6], NQ)] if prep else wq
            wt = [wq[slot, 7, pl.ds(64 * j, 64), :] for j in range(2)]
        tail = _dot(_unpack(opaque(h3, 5)[6, ka, pl.ds(0, 2 * q), :]), _unpack(jnp.concatenate(wt, axis=1)))
        ms = []
        for ja, jb in _STRASSEN:
            if ja >= 5:
                lv = _unpack(lblk(3 * (ja - 5), 5))
            else:
                p_, q_, sg = _SUMS_A[ja]
                lv = psum(lblk(p_, ja), lblk(q_, ja), sg)
            z = zsm[8 + 7 * slot + jb] if prep and ib >= 5 else None
            if ib < 5:
                wv = _unpack(attach(wq[slot, jb]))
            elif jb >= 5:
                wv = _unpack(quad(3 * (jb - 5), z))
            elif prep:
                p_, q_, sg = _SUMS_B[jb]
                wv = psum(quad(p_, z), quad(q_, z), sg)
                keep(w4n.at[slot, pl.ds(jb, 1)], wv)
                wv = wv.astype(BF16)
            else:
                wv = _unpack(attach(w4n.bitcast(U32)[slot, jb]))
            ms.append(_dot(lv, wv))
        c11, c12, c21, c22 = _combine(*ms)
        done[0][k] = jnp.concatenate([c11, c21], axis=0) + tail[:, :128]
        done[1][k] = jnp.concatenate([c12, c22], axis=0) + tail[:, 128:]
        b2_done(w, done, r0, n)

    w = window(0, 2 * TS + LEAD)
    H = TS // 2
    with jax.named_scope("t0a"):
        cps["qa"].wait()
        cps["wmoda"].wait()

        mv = {}

        def mod_fn(j, toks):
            mv[j] = mod_cols(j, 1, toks)[0]
            if len(mv) == 3:
                modbuf[0] = mv[2] * mv[0]
                modbuf[1] = mv[2] * (1.0 + mv[1])

        segment(G5B, 0, MU, mod_fn=mod_fn)
        put(w["h"], pl.ds(0, QA), stage_a0(w, 0, QA))
    with jax.named_scope("t0b"):
        cps["wmodb"].wait()
        sb, cb = mod_cols(3, 2)
        modbuf[3] = 2.0 * sb
        modbuf[4] = 2.0 + 2.0 * cb
        n3 = stage_a1(w, 0, QA, n2=slabs(w["h"], 0, QA))
    XB = TS - XA
    with jax.named_scope("t1a"):
        cps["w1a"].wait()
        cps["qx"].wait()
        put(w["h"], pl.ds(QA, XA), stage_a0(w, QA, XA))
        stage_a2(w, n3, 0, QA, c1=W1A, fine=80)
    with jax.named_scope("t1b"):
        cps["w1b"].wait()
        n3a = stage_a1(w, QA, XA, n2=slabs(w["h"], QA, XA), f32=True)
        stage_a2(w, n3, 0, QA, c0=W1A)
        stage_a2(w, [dd_rest("w1", *_rows2(n3a))], QA, XA, prep=True)
    with jax.named_scope("t2"):
        cps["qb"].wait()
        cps["w2"].wait()
        n3b = stage_a1(w, QA + XA, XB, f32=True)
        stage_b1b(w, stage_b1a(w, 0, TS, prep=True), 0, TS, deep=False)
        stage_a2(w, [dd_rest("w1", *_rows2(n3b))], QA + XA, XB)
        stage_b1b(w, stage_b1a(w, TS, XA), TS, XA)
        stage_b1a(w, TS + XA, XB)
    with jax.named_scope("t3"):
        cps["w3"].wait()
        stage_b1b(w, slabs(w["h"], TS + XA, XB), TS + XA, XB)
        stage_b2h(w, hba, 0, TS, prep=True)
        stage_b2a(w, hba, 0, TS, prep=True)
        stage_b2h(w, hbb, TS, TS)
        if N3:
            for g in range(3):
                stage_b2z(w, hbb, g, prep=True)
        else:
            stage_b2a(w, hbb, TS, TS)
    with jax.named_scope("t4"):
        cps["w4"].wait()
        cps["wmodg"].wait()
        done = {0: {}, 1: {}}
        for op in "m4 P m0 4:0:6:7 m2 8:0 m1 8:1 m3 8:3 4:1:6:7 8:2 8:4 8:5".split():
            op, *rng = op.split(":")
            rng = [int(x) for x in rng]
            if op[0] == "m":
                c = int(op[1])
                modbuf[5, :, pl.ds(c * 128, 128)] = 0.5 * _dot(modbuf[6], weights(wmodbuf, 5 * NC + c, 5 * NC + c + 1))
            elif op[0] == "8":
                stage_b2n(w, hba, 0, TS, *rng, done, prep=True)
            elif op[0] == "P":
                stage_b2b(w, hba, 0, TS, 2, marks=prep_w4(24))
            else:
                stage_b2b(w, hba, 0, TS, *rng, done=done, prep=True)
        out_copy(0, TS).start()
        cps["q1"].wait()

    CBS = (128, 128)
    PART = {"a": (TS, TS), "c": (TS, H), "d": (TS + H, H)}
    BODY = "4:0:6:7 4:1:6:7 4:2 8:1 8:5 r0 r1 1a 8:3 2c 2d Nc nd 8:0 8:4 8:2 z:0 ha z:1 z:2"

    def step(s, carry):
        r0 = pl.multiple_of(s * TS, TS)
        w = window(r0, 2 * TS + LEAD)
        x1, rest, done = {}, {}, {0: {}, 1: {}}
        for op in BODY.split():
            op, *rng = op.split(":")
            rng = [int(x) for x in rng]
            if op[0] == "3":
                stage_b2a(w, hbb, TS, TS, *rng)
            elif op[0] == "z":
                stage_b2z(w, hbb, *rng)
            elif op[0] == "N":
                pending.extend(stage_b1b(w, x1[op[1]], *PART[op[1]]))
            elif op[0] == "h":
                stage_b2h(w, hbb, TS, TS)
            elif op[0] == "4":
                stage_b2b(w, hbb, 0, TS, *rng, done=done)
            elif op[0] == "8":
                stage_b2n(w, hbb, 0, TS, *rng, done)
            elif op[0] == "2":
                x1[op[1]] = stage_b1a(w, *PART[op[1]])
            elif op[0] == "n":
                stage_b1b(w, x1[op[1]], *PART[op[1]])
            elif op[0] == "r":
                j = int(op[1])
                rest[j] = dd_rest("w1", *_rows2(stage_a1(w, TS + LEAD + sum(CBS[:j]), CBS[j], f32=True)))
            else:
                ra, n = PART[op[1]]
                parts = [rest[j] for j in range(len(CBS)) if ra - TS <= sum(CBS[:j]) < ra - TS + n]
                stage_a2(w, parts, ra + LEAD, n, last_valid=(s < NT - 2) if ra + n == 2 * TS else None)
        out_copy(r0, TS).start()
        return carry

    with jax.named_scope("p2main"):
        jax.lax.fori_loop(1, NT - 1, step, 0)
    with jax.named_scope("p2epi"):
        w = window(S - 2 * TS, 2 * TS + LEAD)
        rows = pl.ds(S - TS, TS)
        pending.append(hhbuf[0, pl.ds(S, 8), :])
        def flush(rows, cols):
            pltpu.make_async_copy(obuf.at[rows, cols], out_hbm.at[rows, cols], sem_out.at[0]).start()

        done = {0: {}, 1: {}}
        for j in range(2):
            stage_b2b(w, hbb, TS, TS, j, done=done)
        for k in NEST:
            stage_b2n(w, hbb, TS, TS, k, done)
        flush(rows, pl.ds(0, 512))
        sub = 0
        for n in (128, 64, 64):
            stage_b2b(w, hbb, TS, n, 2, sub=sub)
            flush(pl.ds(S - TS + sub, n), pl.ds(512, 128))
            sub += n
        pltpu.make_async_copy(obuf, out_hbm, sem_out.at[0]).wait()


@jax.jit
def pallas_adaLN_cond__ssm_conv_h3__mixer_s_mlp__prompt_kernel(
    A_q: jax.Array,
    A_k: jax.Array,
    A_v: jax.Array,
    A_shift_k: jax.Array,
    A_ssm_k: jax.Array,
    A_ssm_D: jax.Array,
    B_x: jax.Array,
    B_w1: jax.Array,
    B_w2: jax.Array,
    B_w3: jax.Array,
    B_w4: jax.Array,
    c: jax.Array,
    w_mod: jax.Array,
):
    del B_x

    def tiles(x):
        return x.reshape(S // 8, 8, NC, 128).transpose(0, 2, 1, 3).reshape(S * NC, 128)

    def pairs(x):
        r, n = x.shape
        return x.reshape(r // 16, 2, 8, n // 128, 128).transpose(0, 1, 3, 2, 4)

    args = (
        A_q.reshape(S, D), tiles(A_k), tiles(A_v),
        A_shift_k.T, A_ssm_k, A_ssm_D.reshape(NC, 128),
        pairs(B_w1), pairs(B_w2), pairs(B_w3.T), pairs(B_w4), c, pairs(w_mod),
    )
    scratch = [
        pltpu.VMEM((NA, P * NC + 128, 128), BF16),
        pltpu.VMEM((NA, P * NC + 64, 128), BF16),
        pltpu.VMEM((D, S), BF16),
        pltpu.VMEM((R, 256, 128), BF16),
        pltpu.VMEM((2, R, 128, 128), BF16),
        pltpu.VMEM((128, 128), BF16),
        pltpu.VMEM((D // 16, 6 * NC, 16, 128), BF16),
        pltpu.VMEM((D // 16, NC, 16, 128), BF16),
        pltpu.VMEM((D // 16, NC, 16, 128), BF16),
        pltpu.VMEM((FF // 16, NC, 16, 128), BF16),
        pltpu.VMEM((FF // 16, NC, 16, 128), BF16),
        pltpu.VMEM((S + 64, D), BF16),
        *[pltpu.VMEM((NA, R, 16, 4, 8, 128), F32) for _ in range(NC)],
        pltpu.VMEM((NC, 2, R, 16, 2, 8, 128), F32),
        pltpu.VMEM((2 * NC, R, 256, 128), BF16),
        pltpu.VMEM((32, 128), U32),
        pltpu.VMEM((NC, 8, 8, 128), F32),
        pltpu.VMEM((NC, S + 32, 128), F32),
        pltpu.VMEM((8, 8, D), F32),
        pltpu.VMEM((S + 32, D), F32),
        pltpu.VMEM((NC, S + 32, 128), F32),
        pltpu.VMEM((NC, S + 32, 128), F32),
        pltpu.VMEM((8, 2, TS + 16, 128), BF16),
        pltpu.VMEM((5, 2, 1, 256, 128), BF16),
        pltpu.VMEM((5, 2, 1, 256, 128), BF16),
        pltpu.VMEM((5, 6, 2, 128, 128), BF16),
        pltpu.VMEM((5, 2, 2, FT, 128), BF16),
        pltpu.VMEM((5, 2, 1, 896, 128), BF16),
        pltpu.VMEM((8, 9, 144, 128), BF16),
        pltpu.VMEM((8, 9, 144, 128), BF16),
        pltpu.VMEM((2, 8, 384, 128), BF16),
        pltpu.VMEM((NQ, 8, 384, 128), BF16),
        pltpu.VMEM((3, 7, 5, 128, 128), BF16),
        pltpu.VMEM((8, 5, 80, 128), BF16),
        pltpu.VMEM((S, D), BF16),
        pltpu.VMEM((4, D), BF16),
        pltpu.VMEM((NC, 128), BF16),
        pltpu.VMEM((1, D), BF16),
        pltpu.SMEM((64,), jnp.int32),
        pltpu.SemaphoreType.DMA((40,)),
        pltpu.SemaphoreType.DMA((1,)),
    ]
    out = pl.pallas_call(
        _kernel,
        out_shape=jax.ShapeDtypeStruct((S, D), BF16),
        in_specs=[pl.BlockSpec(memory_space=pl.ANY)] * len(args),
        out_specs=pl.BlockSpec(memory_space=pl.ANY),
        scratch_shapes=scratch,
        grid=(1,),
        compiler_params=pltpu.CompilerParams(vmem_limit_bytes=108 * 1024 * 1024, disable_semaphore_checks=True,
                                             disable_bounds_checks=True),
        name="adaln_h3_mixer",
    )(*args)
    return out.reshape(1, S, D)
```

```python
import numpy as np
import jax
import jax.numpy as jnp
import jax.experimental.pallas as pl
import jax.experimental.pallas.tpu as pltpu

F32 = jnp.float32
BF16 = jnp.bfloat16
U32 = jnp.uint32

S = 2048
D = 640
FF = 1728
NC = D // 128
R = 4
P = 128 * R
NA = S // P
TS = 256
NT = S // TS
LEAD = 16
EPS = 1e-5
N3 = (1, 3, 4, 2)
NEST = (1, 4, 0, 2, 3, 5)
NQ = len(NEST)
FT = (FF - 1536) // 2


def _freq(row):
    t, part, s = row >> 4, (row >> 3) & 1, row & 7
    return 32 * (t & 7) + 4 * s + 2 * (t >> 3) + 1, P * part


def _cos(j, scale):
    jf = (j & (4 * P - 1)).astype(F32)
    u = 2.0 * np.pi / (4 * P)
    x = jnp.abs(jf * u - np.pi) - 0.5 * np.pi
    x2 = x * x
    poly = scale / 362880.0 - x2 * (scale / 39916800.0)
    for coef in (-1.0 / 5040.0, 1.0 / 120.0, -1.0 / 6.0, 1.0):
        poly = poly * x2 + coef * scale
    return poly * x


_DUR = {"t": 8, "u": 16, "k": 16, "i": 16, "m": 12, "g": 0, "c": 0, "j": 16}
_POST = {"t": 8.0, "u": 16.0, "k": 24.0, "i": 4.0, "j": 4.0, "m": 18.0}


def _plan_tokens(order, maxutil):
    lag, cap, pre, margin = 8, 62, 4, 3
    start, slots = {}, []
    for n in order:
        start[n] = len(slots)
        slots += [(n, r) for r in range(_DUR[n[0]])]
    nslot = len(slots) + lag
    free = [cap - (_POST[slots[i - lag][0][0]] if i >= lag else 0.0) for i in range(-pre, nslot)]
    units = []
    for n in order:
        kind, a, c = n
        if kind == "u":
            units += [(n + (g,), 94.0, start[n], -pre) for g in range(8)]
        elif kind == "g":
            units += [(n + (g,), 150.0, start[n], -pre) for g in range(8)]
        elif kind in "ic":
            src_ = [start[m] for m in (("u", a, c), ("k", a, c)) if m in start]
            for t in range(16):
                rel = max(max(src_) + 16, max(src_) + t + lag + 3) if src_ else -pre
                units.append((n + (t,), 32.0 * a + 48.0, nslot if kind == 'c' else start[n], rel))

    def simulate(util):
        left = [u[1] for u in units]
        done = [None] * len(units)
        for i in range(-pre, nslot):
            budget = util * free[i + pre]
            for j, u in enumerate(units):
                if budget <= 0.0:
                    break
                if done[j] is None and u[3] <= i:
                    use = min(budget, left[j])
                    left[j] -= use
                    budget -= use
                    if left[j] <= 1e-9:
                        done[j] = i + 1
        ok = all(u[2] < 8 or (d is not None and d <= max(u[2] - (1 if u[0][0] in 'cg' else margin), u[3] + 1))
                 for d, u in zip(done, units))
        return done, ok

    lo_, hi_ = 0.05, maxutil
    for _ in range(12):
        mid = 0.5 * (lo_ + hi_)
        if simulate(mid)[1]:
            hi_ = mid
        else:
            lo_ = mid
    done, _ = simulate(hi_)
    plan = {}
    for u, d in zip(units, done):
        if u[0][0] == "c":
            plan[u[0]] = slots[max((nslot - 1 if d is None else min(d, nslot - 1)) - lag, 0)]
        elif d is not None and 0 <= d < u[2]:
            plan.setdefault(slots[d], []).append(u[0])
    return plan


def _unpack(w):
    return pltpu.bitcast(w, BF16)


def _dot(a, b):
    return jnp.dot(a.astype(BF16), b, preferred_element_type=F32)


def _dot_nt(a, b):
    return jax.lax.dot_general(a.astype(BF16), b, (((1,), (1,)), ((), ())), preferred_element_type=F32)


def _dot_fine(x, w, chunk):
    if not chunk:
        return _dot(x, w)
    n = w.shape[1]
    head = _dot(x, w[:, :n - 128])
    last = jnp.concatenate([_dot(x[r:r + chunk], w[:, n - 128:]) for r in range(0, x.shape[0], chunk)], axis=0)
    return jnp.concatenate([head, last], axis=1)


def _rows2(x):
    n, c = x.shape
    x = x.reshape(n // 32, 2, 16, c)
    return x[:, 0].reshape(n // 2, c), x[:, 1].reshape(n // 2, c)


def _unrows2(top, bot):
    n, c = top.shape
    return jnp.stack([top.reshape(n // 16, 16, c), bot.reshape(n // 16, 16, c)], axis=1).reshape(2 * n, c)


def _sums_a(a11, a12, a21, a22):
    return [a11 + a22, a21 + a22, a11 + a12, a21 - a11, a12 - a22]


def _sums_b(b11, b12, b21, b22):
    return [b11 + b22, b12 - b22, b21 - b11, b11 + b12, b21 + b22]


_STRASSEN = ((0, 0), (1, 5), (5, 1), (6, 2), (2, 6), (3, 3), (4, 4))


_SUMS_A = ((0, 3, 1), (2, 3, 1), (0, 1, 1), (2, 0, -1), (1, 3, -1))
_SUMS_B = ((0, 3, 1), (1, 3, -1), (2, 0, -1), (0, 1, 1), (2, 3, 1))


def _combine(m1, m2, m3, m4, m5, m6, m7):
    return (m1 + m4) + (m7 - m5), m3 + m5, m2 + m4, (m1 - m2) + (m3 + m6)


def _lo(w):
    return pltpu.bitcast(w << 16, F32)


def _hi(w):
    return pltpu.bitcast(w & jnp.uint32(0xFFFF0000), F32)


def _ln(x, eps=EPS):
    m = jnp.sum(x, axis=-1, keepdims=True) * (1.0 / D)
    xc = x - m
    v = jnp.sum(xc * xc, axis=-1, keepdims=True) * (1.0 / D)
    return xc * jnp.exp(-0.5 * jnp.log(v + eps))


def _gelu2(x):
    c0 = 0.7978845608028654
    c1 = c0 * 0.044715
    return x + x * jnp.tanh(x * (c0 + c1 * (x * x)))


def _bfly(tr, ti):
    s02r, s02i = tr[0] + tr[2], ti[0] + ti[2]
    d02r, d02i = tr[0] - tr[2], ti[0] - ti[2]
    s13r, s13i = tr[1] + tr[3], ti[1] + ti[3]
    d13r, d13i = tr[1] - tr[3], ti[1] - ti[3]
    x0r, x0i = s02r + s13r, s02i + s13i
    x2r, x2i = s02r - s13r, s02i - s13i
    return [x0r, d02r + d13i, x2r, d02r - d13i], [x0i, d02i - d13r, x2i, d02i + d13r]


def _kernel(q_hbm, k_hbm, v_hbm, shift_hbm, ssmk_hbm, ssmd_hbm, w1_hbm, w2_hbm, w3t_hbm, w4_hbm,
            c_hbm, wmod_hbm,
            out_hbm,
            kbuf, vbuf, skbuf, fwdbuf, invbuf, permbuf,
            wmodbuf, w1buf, w2buf, w3buf, w4buf, qbuf,
            xs0, xs1, xs2, xs3, xs4, kraw, stg, zbuf, coefbuf, ybuf, modbuf, x2buf, hbuf, hhbuf, xobuf,
             w1s, w2s, w3s, w3ts, w4s, hba, hbb, w4n, w4q, w3n, xibuf, obuf, shiftbuf, dbuf, cbuf,
            zsm, sem_in, sem_out):
    cps = {}
    n_sem = [0]

    def start(name, src, dst):
        cp = pltpu.make_async_copy(src, dst, sem_in.at[n_sem[0]])
        n_sem[0] += 1
        cp.start()
        cps[name] = cp

    class Both:
        def __init__(self, a, b):
            self.cps = (a, b)

        def wait(self):
            for cp in self.cps:
                cp.wait()

    def start_w(name, src, dst, c0=0, n=NC):
        for e in range(2):
            start(name + str(e), src.at[:, e, pl.ds(c0, n)], dst.at[:, pl.ds(c0, n), pl.ds(8 * e, 8), :])
        cps[name] = Both(cps[name + "0"], cps[name + "1"])

    CH = P * NC
    HALO = 8 * NC

    def start_s(a):
        cols = pl.ds(a * P, P)
        start("s%d" % a, ssmk_hbm.at[:, cols], skbuf.at[:, cols])

    def start_kv(a):
        if a == 0:
            kbuf[0, pl.ds(0, HALO + 8), :] = jnp.zeros((HALO + 8, 128), BF16)
            start("k0", k_hbm.at[pl.ds(0, CH), :], kbuf.at[0, pl.ds(HALO, CH), :])
        else:
            start("k%d" % a, k_hbm.at[pl.ds(a * CH - HALO, CH + HALO), :], kbuf.at[a, pl.ds(0, CH + HALO), :])
        start("v%d" % a, v_hbm.at[pl.ds(a * CH, CH), :], vbuf.at[a, pl.ds(0, CH), :])

    for n in "s0 x0 s1 k0 k1 s2 k2 s3 k3".split():
        if n[0] == "s":
            start_s(int(n[1]))
        elif n[0] == "k":
            start_kv(int(n[1]))
        else:
            start("d", ssmd_hbm, dbuf)
            start("shift", shift_hbm, shiftbuf)
            start("c", c_hbm, cbuf)
    QA = TS + LEAD
    XA = 128
    QB = 2 * TS + LEAD
    W1A = 2

    def start_q(name, r0, n):
        start(name, q_hbm.at[pl.ds(r0, n), :], qbuf.at[pl.ds(r0, n), :])

    start_q("qa", 0, QA)
    start_w("wmoda", wmod_hbm, wmodbuf, 0, 3 * NC)
    start_w("wmodb", wmod_hbm, wmodbuf, 3 * NC, 2 * NC)
    start_q("qx", QA, XA)
    start_w("w1a", w1_hbm, w1buf, 0, W1A)
    start_w("w1b", w1_hbm, w1buf, W1A, NC - W1A)
    start_q("qb", QA + XA, QB - QA - XA)
    start_w("w2", w2_hbm, w2buf)
    start_w("w3", w3t_hbm, w3buf)
    start_w("w4", w4_hbm, w4buf)
    start_w("wmodg", wmod_hbm, wmodbuf, 5 * NC, NC)
    start_q("q1", QB, S - QB)

    kw = kbuf.bitcast(U32)
    vw = vbuf.bitcast(U32)
    zbuf[...] = jnp.zeros(zbuf.shape, U32)
    for j in range(64):
        zsm[j] = 0
    for c in range(NC):
        ybuf[c, pl.ds(S, LEAD), :] = jnp.zeros((LEAD, 128), F32)
        hhbuf[c, pl.ds(0, 8), :] = jnp.zeros((8, 128), F32)
    qbuf[pl.ds(S, LEAD), :] = jnp.zeros((LEAD, D), BF16)

    def sample(pos):
        return (pos & ~15) + 2 * (pos & 7) + ((pos >> 3) & 1)

    def tables(p, carry):
        f2, off = _freq(jax.lax.broadcasted_iota(jnp.int32, (256, 128), 0))
        n = R * sample(jax.lax.broadcasted_iota(jnp.int32, (256, 128), 1)) + p
        fwdbuf[p] = _cos(f2 * n + off, 1.0).astype(BF16)
        return carry

    jax.lax.fori_loop(0, R, tables, 0)

    def unit_g(kt, r):
        f2, off = _freq(jax.lax.broadcasted_iota(jnp.int32, (16, 128), 1) + 128 * kt)
        j0 = f2 * (R * (jax.lax.broadcasted_iota(jnp.int32, (16, 128), 0) + 16 * r)) + off
        for p in range(R):
            invbuf[kt, p, pl.ds(16 * r, 16), :] = _cos(j0 + p * f2, 1.0 / P).astype(BF16)
        return [invbuf.bitcast(U32)[kt, p, pl.ds(8 * r, 8), :] for p in range(R)]

    i0 = jax.lax.broadcasted_iota(jnp.int32, (128, 128), 0)
    i1 = jax.lax.broadcasted_iota(jnp.int32, (128, 128), 1)
    permbuf[...] = jnp.where(i1 == R * sample(i0 & 31) + (i0 >> 5), 1.0, 0.0).astype(BF16)

    def fill_coef():
        cv = cbuf[...].astype(F32)
        modbuf[6] = jnp.broadcast_to(cv * jax.nn.sigmoid(cv), (8, D))
        coef = shiftbuf[...].astype(F32)
        dval = dbuf[...].astype(F32)
        for c in range(NC):
            for j in range(4):
                coefbuf[c, j] = jnp.broadcast_to(coef[j:j + 1, c * 128:(c + 1) * 128], (8, 128))
            coefbuf[c, 4] = jnp.broadcast_to(dval[c:c + 1, :], (8, 128))

    xs = (xs0, xs1, xs2, xs3, xs4)
    wsbufs = dict(w1=w1s, w2=w2s, w3=w3s, w4=w4s, w3t=w3ts)
    def split_ri(t):
        t = t.reshape(16, 2, 8, 128)
        return t[:, 0], t[:, 1]

    def get_never():
        return zbuf[pl.ds(0, 8), :] != 0

    def packed(x, slot, r0):
        n = x.shape[1]
        stg[slot, :, pl.ds(r0, n), :] = x.astype(BF16)
        return [stg.bitcast(U32)[slot, p, pl.ds(r0 // 2, n // 2), :] for p in range(R)]

    UG = 8

    def unit_u(a, c, g0, UG):
        c0, c1, c2, c3 = (coefbuf[c, pl.ds(j, 1)][None] for j in range(4))
        rows = lambda ref, r: ref[a, pl.ds((r // 4) * 4 * NC + 4 * c + r % 4, 8 * UG, stride=4 * NC), :]
        kk = jnp.stack([rows(kw, 4 + 32 * g0 + d) for d in range(-2, 4)]).reshape(6, UG, 8, 128)
        vv = jnp.stack([rows(vw, 32 * g0 + d) for d in range(4)]).reshape(4, UG, 8, 128)
        lo, hi = _lo(kk), _hi(kk)
        k0, k1, k2 = lo[2:], hi[1:5], lo[1:5]
        even = ((k0 * c0 + k1 * c1) + (k2 * c2 + hi[:4] * c3)) * _lo(vv)
        odd = ((hi[2:] * c0 + k0 * c1) + (k1 * c2 + k2 * c3)) * _hi(vv)
        kv = jnp.stack([even, odd], axis=1).reshape(2, R, UG, 8, 128)
        return packed(jnp.stack([kv[0], kv[1]], axis=2).reshape(R, 16 * UG, 128), NC + c, 16 * g0)

    def unit_i(a, c, t0, UG, z, after=None):
        x_c = xs[c].at[pl.ds(z, NA)]
        ts = pl.ds(t0, UG)
        yr = yi = None
        for j in range(a + 1):
            ur, ui = x_c[j, :, ts, 0], x_c[j, :, ts, 1]
            kr, ki = x_c[a - j, :, ts, 2], x_c[a - j, :, ts, 3]
            pr = ur * kr - ui * ki
            pi = ur * ki + ui * kr
            yr = pr if yr is None else yr + pr
            yi = pi if yi is None else yi + pi
        sr, si, dr, di = yr[:2] + yr[2:], yi[:2] + yi[2:], yr[:2] - yr[2:], yi[:2] - yi[2:]
        (sr0, sr1), (si0, si1), (dr0, dr1), (di0, di1) = ((x[0], x[1]) for x in (sr, si, dr, di))
        wr = jnp.stack([sr0 + sr1, dr0 - di1, sr0 - sr1, dr0 + di1])
        wi = jnp.stack([si0 + si1, di0 + dr1, si0 - si1, di0 - dr1])
        if after is not None:
            never = jnp.broadcast_to(zbuf[pl.ds(0, 8), :], wr.shape) != 0
            wr = jax.lax.select(never, jnp.broadcast_to(after, wr.shape), wr)
        return packed(jnp.stack([wr, wi], axis=2).reshape(R, 16 * UG, 128), c, 16 * t0)

    def segment(spec, z, maxutil=1.0, mod_fn=None):
        order = [(n[0], int(n[1]), int(n[2])) for n in spec.split()]
        plan = _plan_tokens(order, maxutil) if maxutil > 0 else {}
        never = get_never()
        units, groups, res = {}, {}, {}

        paced = {k_ for s_, ks in plan.items() if len(s_) == 2 for k_ in ks}

        def width(name):
            n = 8 if name[0] == "u" else 16
            return UG if all(name + (j,) in paced for j in range(n)) else 1

        def group(key):
            kind, a, c, j = key
            ug = width(key[:3])
            key = (kind, a, c, j - j % ug)
            if key not in groups:
                if kind == "u":
                    groups[key] = unit_u(a, c, key[3], ug)
                else:
                    fresh = ("u", a, c) in order or ("k", a, c) in order
                    groups[key] = unit_i(a, c, key[3], ug, z if fresh else 0,
                                         res[plan[key]]() if kind == "c" else None)
            return groups[key]

        def unit(key):
            if key not in units:
                if key[0] == "g":
                    units[key] = unit_g(key[1], key[3])
                else:
                    r = 8 * (key[3] % width(key[:3]))
                    units[key] = [v[r:r + 8] for v in group(key)]
            return units[key]

        def lhs(name, p, full, r0=0):
            out, last = [], 0
            for r in range(full.shape[0] // 8):
                keys = plan.get((name, r0 + r), ())
                if keys:
                    if 8 * r > last:
                        out.append(full[last:8 * r])
                    v = full[8 * r:8 * r + 8]
                    for key in keys:
                        v = jax.lax.select(never, unit(key)[p], v)
                    out.append(v)
                    last = 8 * r + 8
            if last < full.shape[0]:
                out.append(full[last:] if last else full)
            return out[0] if len(out) == 1 else jnp.concatenate(out, axis=0)

        def dft(name, rhs):
            tr, ti = [], []
            for p in range(R):
                f = lhs(name, p, fwdbuf.bitcast(U32)[p])
                r_, i_ = split_ri(_dot(_unpack(f), rhs[p]))
                if p == 0:
                    res.update({(name, r): (lambda r=r, v=r_: v[r]) for r in range(16)})
                tr.append(r_)
                ti.append(i_)
            return _bfly(tr, ti)

        st = {}
        for name in order:
            kind, a, c = name
            x_c = xs[c]
            if kind == "g":
                for r in range(8):
                    unit(name + (r,))
            elif kind == "c":
                for t in range(16):
                    group(name + (t,))
            elif kind == "m":
                toks = {}
                for r in range(_DUR["m"]):
                    for n_, key in enumerate(plan.get((name, r), ())):
                        toks.setdefault(2 * r + n_ % 2, []).extend(unit(key))
                mod_fn(a, toks)
            elif kind == "t":
                trs = []
                for b in range(R):
                    pm = lhs(name, b, permbuf.bitcast(U32)[...])
                    trs.append(_dot_nt(_unpack(pm), skbuf[pl.ds(c * 128, 128), pl.ds(a * P + b * 128, 128)]))
                res.update({(name, r): (lambda r=r, v=trs[0]: v[16 * r:16 * r + 8]) for r in range(8)})
                g_ = 128 // R
                st[a, c] = [jnp.concatenate([trs[b][p * g_:(p + 1) * g_] for b in range(R)], axis=0).astype(BF16)
                            for p in range(R)]
            elif kind == "u":
                rhs = [_unpack(jnp.concatenate([group(name + (g,))[p] for g in range(0, 8, width(name))], axis=0)) for p in range(R)]
                xr, xi = dft(name, rhs)
                for q in range(R):
                    x_c[a, q, :, 0] = xr[q]
                    x_c[a, q, :, 1] = xi[q]
            elif kind == "k":
                xr, xi = dft(name, st[a, c])
                for q in range(R):
                    if a == 0:
                        x_c[a, q, :, 2] = xr[q] + coefbuf[c, 4]
                        x_c[a, q, :, 3] = xi[q]
                    else:
                        pr, pi = kraw[c, (a - 1) % 2, q, :, 0], kraw[c, (a - 1) % 2, q, :, 1]
                        x_c[a, q, pl.ds(0, 8), 2] = xr[q][:8] - pi[:8]
                        x_c[a, q, pl.ds(0, 8), 3] = xi[q][:8] + pr[:8]
                        x_c[a, q, pl.ds(8, 8), 2] = xr[q][8:] + pi[8:]
                        x_c[a, q, pl.ds(8, 8), 3] = xi[q][8:] - pr[8:]
                    if a + 1 < NA:
                        kraw[c, a % 2, q, :, 0] = xr[q]
                        kraw[c, a % 2, q, :, 1] = xi[q]
            else:
                for p in range(R):
                    cols = [lhs(name, 2 * (p % 2) + kt,
                                invbuf.bitcast(U32)[kt, p], 8 * (p // 2))
                            for kt in range(2)]
                    g = _unpack(jnp.concatenate(cols, axis=1))
                    if kind == "j":
                        wp = _unpack(stg.bitcast(U32)[c, p])
                    else:
                        wp = _unpack(jnp.concatenate([group(name + (t,))[p] for t in range(0, 16, width(name))], axis=0))
                    yp = _dot(g, wp)
                    if p % 2 == 0:
                        res.update({(name, 4 * p + r): (lambda r=r, v=yp: v[16 * r:16 * r + 8]) for r in range(8)})
                    ybuf[c, pl.ds(a * P + p, 128, stride=R), :] = yp

    one = jnp.minimum(pl.program_id(0) + 1, 1)

    def once(fn):
        def body(z, carry):
            fn(z)
            return carry
        jax.lax.fori_loop(0, one, body, 0)

    default = ("t00 t01 t02 k00 t03 k01 t04 k02 k03 k04 g00|"
               "t10 t11 t12 k10 k11 k12 g10|"
               "t13 t14 k13 u00 k14 u01 u02 u03 i00 u04 i01 c02 c03|"
               "j02 j03 u10 i04 u11 u12 u13 i10 u14 i11 c12 c13|"
               "t20 t21 j12 t22 j13 t23 t24 k20 u20 k21 u21 k22 i14 k23 u22 k24 u23 i20 u24 i21 c22|"
               "t30 t31 j22 t32 t33 t34 k30 u30 k31 u31 k32 i23 k33 u32 k34 i24 u33 i30 u34 i31 c32|"
               "m00 j32 m10 i33 m20 i34")
    specs = default.split("|")
    G5B = specs[-1]
    segs = list(zip("s0 d shift c|s1|k0 v0|k1 v1|s2 k2 v2|s3 k3 v3".split("|"), specs[:-1]))
    MU = 1.5
    for i, (waits, spec) in enumerate(segs):
        with jax.named_scope("g%d" % i):
            for n in waits.split():
                cps[n].wait()
            if i == 0:
                fill_coef()
            once(lambda z: segment(spec, z, MU))

    def mod_cols(lo, n, toks=None):
        m = _dot(modbuf[6], weights(wmodbuf, lo * NC, (lo + n) * NC, toks=toks))
        return [m[:, j * D:(j + 1) * D] for j in range(n)]

    def mul_mod(x, j, cols=None):
        m = modbuf[j] if cols is None else modbuf[j, :, cols]
        return (x.reshape(-1, 8, x.shape[-1]) * m[None]).reshape(x.shape)

    def add_mod(x, j):
        return (x.reshape(-1, 8, x.shape[-1]) + modbuf[j][None]).reshape(x.shape)

    def slabs(ref, r0, n):
        return jnp.concatenate([ref[c, pl.ds(r0, n), :] for c in range(NC)], axis=1)

    def put(ref, rows, x):
        for c in range(NC):
            ref[c, rows, :] = x[:, c * 128:(c + 1) * 128]

    def window(base, n):
        rows = pl.ds(base, n)
        return dict(q=qbuf.at[rows, :], y=ybuf.at[:, rows, :], x2=x2buf.at[rows, :], h=hbuf.at[:, rows, :],
                    hh=hhbuf.at[:, pl.ds(base, n + 8), :],
                    o=obuf.at[pl.ds(base, n - LEAD), :])

    def weights(ref, c0=0, c1=NC, r0=0, r1=None, toks=None, raw=False, z=None):
        r1 = 16 * ref.shape[0] if r1 is None else r1
        view = ref.bitcast(U32)
        if z is not None:
            view = view.at[pl.ds(z, ref.shape[0])]
        never = get_never() if toks else None
        rt = -(-(r1 - r0) // 128)
        cols = []
        for j in range(c0, c1):
            wu = view[pl.ds(r0 // 16, (r1 - r0) // 16), j].reshape((r1 - r0) // 2, 128)
            if toks:
                parts, last = [], 0
                for i in range(rt):
                    for n_, t in enumerate(toks.get((j - c0) * rt + i, ())):
                        r = 64 * i + 8 * n_
                        if r > last:
                            parts.append(wu[last:r])
                        parts.append(jax.lax.select(never, t, wu[r:r + 8]))
                        last = r + 8
                parts.append(wu[last:])
                wu = jnp.concatenate(parts, axis=0)
            cols.append(wu)
        wu = jnp.concatenate(cols, axis=1)
        return wu if raw else _unpack(wu)

    def keep(dst, v):
        h = v.shape[0] // 2
        for c in range(v.shape[1] // 128):
            for r in (0, h):
                dst[c, pl.ds(r, h), :] = v[r:r + h, 128 * c:128 * (c + 1)].astype(BF16)

    def fetch(src_):
        u = src_.bitcast(U32)
        return jnp.concatenate([u[c] for c in range(u.shape[0])], axis=1)

    def wblocks(name, j, z=None):
        if name == "w3":
            blk = lambda kh, nh: weights(w3buf, 2 * kh, 2 * kh + 2, 128 * (j + 6 * nh), 128 * (j + 6 * nh + 1), raw=True, z=z)
        elif name == "w4":
            def blk(kh, nh):
                c = j + 2 * nh
                parts = [weights(w4buf, c, c + 1, 768 * kh, 768 * (kh + 1), raw=True, z=z),
                         weights(w4buf, c, c + 1, 1536 + FT * kh, 1536 + FT * (kh + 1), raw=True, z=z),
                         jnp.zeros(((128 - FT) // 2, 128), U32)]
                return jnp.concatenate(parts, axis=0)
        elif name == "w3t":
            blk = lambda kh, nh: weights(w3buf, 2 * kh, 2 * kh + 2, 1536 + FT * nh, 1536 + FT * (nh + 1), raw=True, z=z)
        else:
            ref = w1buf if name == "w1" else w2buf
            blk = lambda kh, nh: weights(ref, j + 2 * nh, j + 2 * nh + 1, 256 * kh, 256 * (kh + 1), raw=True, z=z)
        return blk

    def wsum(name, j, k):
        blk = wblocks(name, j, zsm[k])
        p, q, sign = _SUMS_B[k]
        return psum(blk(p // 2, p % 2), blk(q // 2, q % 2), sign)

    pending = []

    def attach(wv):
        if not pending:
            return wv
        never = get_never()
        rows = [wv[8 * i:8 * i + 8, :128] for i in range(8)]
        for i, t in enumerate(pending):
            rows[i % 8] = jax.lax.select(never, pltpu.bitcast(t, U32), rows[i % 8])
        pending.clear()
        first = jnp.concatenate(rows + ([wv[64:, :128]] if wv.shape[0] > 64 else []), axis=0)
        return first if wv.shape[1] == 128 else jnp.concatenate([first, wv[:, 128:]], axis=1)

    def sprods(name, j, lhs, k0=0, k1=7, prep=False):
        blk, buf = wblocks(name, j), wsbufs[name]
        out = []
        for ia, ib in _STRASSEN[k0:k1]:
            if prep and ib < 5:
                wv = wsum(name, j, ib)
                keep(buf.at[ib, j], wv)
                wv = wv.astype(BF16)
            else:
                wv = _unpack(attach(blk(ib - 5, ib - 5) if ib >= 5 else fetch(buf.at[ib, j])))
            if name == "w3t":
                out.append(_dot_nt(wv, lhs(ia)))
            else:
                out.append((_dot_nt if name == "w3" else _dot)(lhs(ia), wv))
        return out

    def spair(name, j, lhs, prep=False):
        return _combine(*sprods(name, j, lhs, prep=prep))

    def dd_rest(name, t, b):
        ref = w1buf if name == "w1" else w2buf
        m = t.shape[0]
        xb = jnp.concatenate([t, b], axis=0)
        last = _dot(xb, weights(ref, 4, 5))
        rem = _dot(xb[:, 512:], weights(ref, 0, 4, r0=512))
        return t, b, rem[:m], rem[m:], last[:m], last[m:]

    def dd_main(name, parts, prep=False):
        t, b, rt, rb, lt, lb = (jnp.concatenate(v, axis=0) for v in zip(*parts))
        ops = _sums_a(t[:, :256], t[:, 256:512], b[:, :256], b[:, 256:512]) + [t[:, :256], b[:, 256:512]]
        top, bot = [None] * 4, [None] * 4
        for j in range(2):
            top[j], top[j + 2], bot[j], bot[j + 2] = spair(name, j, lambda i: ops[i], prep)
        return (jnp.concatenate([jnp.concatenate(top, axis=1) + rt, lt], axis=1),
                jnp.concatenate([jnp.concatenate(bot, axis=1) + rb, lb], axis=1))

    def stage_a0(w, r0, n):
        rows = pl.ds(r0, n)
        x = w["q"][rows, :].astype(F32)
        x2 = x + add_mod(mul_mod(_ln(x), 1), 0) * slabs(w["y"], r0, n)
        w["x2"][rows, :] = x2
        return _ln(x2)

    def stage_a1(w, r0, n, n2=None, f32=False):
        if n2 is None:
            n2 = stage_a0(w, r0, n)
        h = add_mod(mul_mod(n2, 4), 3)
        put(w["h"], pl.ds(r0, n), h)
        n3 = _ln(h, 4 * EPS)
        return n3 if f32 else n3.astype(BF16)

    def stage_a2(w, n3, r0, n, last_valid=None, fine=0, c0=0, c1=NC, prep=False):
        hh = _gelu2(_unrows2(*dd_main("w1", n3, prep)) if isinstance(n3, list) else _dot_fine(n3, weights(w1buf, c0, c1), fine))
        for c in range(c0, c1):
            blk = hh[:, (c - c0) * 128:(c - c0 + 1) * 128]
            w["hh"][c, pl.ds(r0 + 8, n - LEAD), :] = blk[:n - LEAD]
            tail = blk[n - LEAD:]
            if last_valid is not None:
                tail = jnp.where(last_valid, tail, 0.0)
            w["hh"][c, pl.ds(r0 + 8 + n - LEAD, LEAD), :] = tail

    def stage_b1a(w, r0, n, prep=False):
        lane = jax.lax.broadcasted_iota(jnp.int32, (n, 128), 1)
        sh = lambda c, d: w["hh"][c, pl.ds(r0 + 8 + d, n), :]
        g = jnp.concatenate([sh(0, -1),
                             jnp.where(lane < 32, sh(1, -1), sh(1, 1)),
                             jnp.where(lane < 64, sh(2, 1), sh(2, -2)),
                             jnp.where(lane < 96, sh(3, -2), sh(3, 2)),
                             sh(4, 2)], axis=1)
        x1 = slabs(w["h"], r0, n) + _unrows2(*dd_main("w2", [dd_rest("w2", *_rows2(g))], prep))
        put(w["h"], pl.ds(r0, n), x1)
        return x1

    def stage_b1b(w, x1, r0, n, deep=True):
        t, b = _rows2(_ln(x1, 4 * EPS))
        ops = _sums_a(t[:, :256], t[:, 256:512], b[:, :256], b[:, 256:512]) + [t[:, :256], b[:, 256:512]]
        ops.append(jnp.concatenate([t[:, 512:], b[:, 512:]], axis=1))
        for i, v in enumerate(ops):
            keep(xobuf.at[i, :, pl.ds(r0 // 2, n // 2), :], v)
        if deep:
            for s_, k in enumerate(N3):
                u, v = _rows2(ops[_STRASSEN[k][0]])
                for i, x in enumerate(_sums_a(u[:, :128], u[:, 128:], v[:, :128], v[:, 128:])):
                    xibuf[s_, i, pl.ds((r0 - TS) // 4, n // 4), :] = x.astype(BF16)
        return [ops[4][i:i + 8, :128] for i in range(0, n // 2, 8)]

    def out_copy(r0, n):
        rows = pl.ds(r0, n)
        return pltpu.make_async_copy(obuf.at[rows, :], out_hbm.at[rows, :], sem_out.at[0])


    def opaque(ref, i):
        ref = ref.bitcast(U32)
        return ref.at[:, :, pl.ds(pl.multiple_of(zsm[i] * 32, 32), ref.shape[2]), :]

    def emit(h3, j, left, right):
        m = left.shape[0] // 2
        g = [left[:m], right[:m], left[m:], right[m:]]
        for k, v in enumerate(_sums_a(*g) + g):
            h3[j, k, pl.ds(0, m), :] = v.astype(BF16)

    def w3_operands(r0, n):
        u, rows = xobuf.bitcast(U32), pl.ds(r0 // 4, n // 4)
        xr = _unpack(jnp.concatenate([u[7, 0, rows, :], u[7, 1, rows, :]], axis=0))
        return xr, lambda i: _unpack(jnp.concatenate([u[i, 0, rows, :], u[i, 1, rows, :]], axis=1))

    def stage_b2h(w, h3, r0, n, prep=False):
        xr, ops = w3_operands(r0, n)
        m = n // 2
        rem = _dot_nt(weights(w3buf, 4, 5, r0=1536), xr)
        c11, c12, c21, c22 = spair("w3t", 0, ops, prep)
        pad = jnp.zeros((128 - FT, m), F32)
        g11, g12, g21, g22 = (jnp.concatenate([_gelu2(c + r), pad], axis=0).T for c, r in (
            (c11, rem[:FT, :m]), (c12, rem[FT:, :m]), (c21, rem[:FT, m:]), (c22, rem[FT:, m:])))
        emit(h3, 6, jnp.concatenate([g11, g21], axis=0), jnp.concatenate([g12, g22], axis=0))

    def stage_b2a(w, h3, r0, n, lo=0, hi=6, prep=False):
        xr, ops = w3_operands(r0, n)
        for j in range(lo, hi):
            r1, r2 = (_dot_nt(xr, weights(w3buf, 4, 5, 128 * t, 128 * (t + 1))) for t in (j, j + 6))
            c11, c12, c21, c22 = spair("w3", j, ops, prep)
            emit(h3, j, _gelu2(jnp.concatenate([c11, c21], axis=0) + r1), _gelu2(jnp.concatenate([c12, c22], axis=0) + r2))

    def stage_b2z(w, h3, g, prep=False):
        xr, ops = w3_operands(TS, TS)
        ms, rem = {0: {}, 1: {}}, {}
        ZO = 0

        def nested(k):
            ib, slot = _STRASSEN[k][1], N3.index(k)

            def quad(i, z=None):
                j, cols = g + 3 * (i % 2), slice(128 * (i // 2), 128 * (i // 2 + 1))
                if ib >= 5:
                    return wblocks("w3", j, z)(ib - 5, ib - 5)[:, cols]
                u = w3s.bitcast(U32)
                return (u if z is None else u.at[pl.ds(z, 5)])[ib, j, i // 2]

            prods = []
            for ja, jb in _STRASSEN:
                if jb >= 5:
                    wv = _unpack(quad(3 * (jb - 5)))
                elif prep:
                    p_, q_, sg = _SUMS_B[jb]
                    wv = psum(quad(p_, zsm[jb]), quad(q_, zsm[jb]), sg)
                    keep(w3n.at[g, slot, pl.ds(jb, 1)], wv)
                    wv = wv.astype(BF16)
                else:
                    wv = _unpack(w3n.bitcast(U32)[g, slot, jb])
                if ja < 5:
                    lv = xibuf.bitcast(U32)[slot, ja, pl.ds(0, TS // 8), :]
                else:
                    e = ja - 5
                    lv = xobuf.bitcast(U32)[_STRASSEN[k][0], e, pl.ds(TS // 4, TS // 4), :]
                    lv = lv.reshape(TS // 64, 2, 8, 128)[:, e].reshape(TS // 8, 128)
                prods.append(_dot_nt(_unpack(lv), wv))
            c11, c12, c21, c22 = _combine(*prods)
            ms[0][k], ms[1][k] = _unrows2(c11, c21), _unrows2(c12, c22)

        def remf(t):
            rem[t] = _dot_nt(xr, weights(w3buf, 4, 5, 128 * t, 128 * (t + 1)))

        early = [g, g + 6, g + 3, g + 9][:ZO]
        for i, k in enumerate(N3):
            nested(k)
            if i < len(early):
                remf(early[i])
        for e in range(2):
            j = g + 3 * e
            for t in (j, j + 6):
                if t not in rem:
                    remf(t)
            for k in range(7):
                if k not in N3:
                    ms[e][k] = sprods("w3", j, ops, k, k + 1)[0]
            c11, c12, c21, c22 = _combine(*[ms[e][k] for k in range(7)])
            emit(h3, j, _gelu2(jnp.concatenate([c11, c21], axis=0) + rem[j]),
                 _gelu2(jnp.concatenate([c12, c22], axis=0) + rem[j + 6]))

    def finish(w, h2, r0, n, c):
        nc = h2.shape[1] // 128
        rows, cols = pl.ds(r0, n), pl.ds(c * 128, nc * 128)
        x1 = jnp.concatenate([w["h"][c + i, rows, :] for i in range(nc)], axis=1)
        w["o"][rows, cols] = (w["x2"][rows, cols] + mul_mod(x1 + h2, 5, cols)).astype(BF16)

    def b2_done(w, done, r0, n):
        if len(done[0]) == len(done[1]) == 7:
            c11, c12, c21, c22 = _combine(*[jnp.concatenate([done[0][k], done[1][k]], axis=1) for k in range(7)])
            finish(w, _unrows2(c11, c21), r0, n, 0)
            finish(w, _unrows2(c12, c22), r0, n, 2)

    def stage_b2b(w, h3, r0, n, j, k0=0, k1=7, done=None, prep=False, sub=0, marks=()):
        hv = opaque(h3, j)
        blk = lambda k: jnp.concatenate([hv[p, k, pl.ds(sub // 4, n // 4), :] for p in range(7)], axis=1)
        r0 += sub
        if j < 2:
            for k in range(k0, k1):
                if k not in NEST:
                    done[j][k] = sprods("w4", j, lambda i: _unpack(blk(8 if i == 6 else i)), k, k + 1, prep)[0]
                    b2_done(w, done, r0, n)
            return
        wb = wblocks("w4", 4)
        lhs = jnp.concatenate([jnp.concatenate([blk(5), blk(6)], axis=1),
                               jnp.concatenate([blk(7), blk(8)], axis=1)], axis=0)
        if marks:
            lo_, hi_ = 0, 52
            never, at = get_never(), {}
            for i, mk in enumerate(marks):
                s_ = lo_ + (hi_ - lo_) * i // len(marks)
                at[4 * (s_ // 16), s_ % 16] = mk
            cols = []
            for kt in range(14):
                col = lhs[:, 128 * kt:128 * (kt + 1)]
                if any(k_[0] == kt for k_ in at):
                    col = jnp.concatenate([jax.lax.select(never, at[kt, r], col[8 * r:8 * r + 8]) if (kt, r) in at
                                           else col[8 * r:8 * r + 8] for r in range(16)], axis=0)
                cols.append(col)
            lhs = jnp.concatenate(cols, axis=1)
        h2 = _dot(_unpack(lhs), _unpack(jnp.concatenate([wb(0, 0), wb(1, 0)], axis=0)))
        finish(w, _unrows2(h2[:n // 2], h2[n // 2:]), r0, n, 4)


    def psum(x, y, sign):
        x, y = _unpack(x).astype(F32), _unpack(y).astype(F32)
        return x + y if sign > 0 else x - y

    def prep_w4(nchunk):
        rows = 384 // nchunk
        marks = []
        for ch in [nchunk] + list(range(nchunk)):
            tail = ch == nchunk
            raw = {}
            for kh in range(2):
                for e in range(1 if tail else 2):
                    r0 = 1536 + FT * kh if tail else 768 * kh + 384 * e + rows * ch
                    x = weights(w4buf, 0, 4, r0, r0 + (FT if tail else rows), raw=True)
                    raw[kh, e] = _unpack(x).astype(F32)
            blk = lambda i, e: raw[i // 2, e][:, 256 * (i % 2):256 * (i % 2 + 1)]
            for k, (ia, ib) in enumerate(_STRASSEN):
                if k not in NEST or ib >= 5:
                    continue
                p_, q_, sg = _SUMS_B[ib]
                half = [blk(p_, e) + blk(q_, e) if sg > 0 else blk(p_, e) - blk(q_, e) for e in range(1 if tail else 2)]
                quad = lambda i: half[i // 2][:, 128 * (i % 2):128 * (i % 2 + 1)]
                first = NEST.index(k)
                if tail:
                    for j in range(2):
                        w4q[first, 7, pl.ds(128 * j, FT), :] = quad(j).astype(BF16)
                        w4q[first, 7, pl.ds(128 * j + FT, 128 - FT), :] = jnp.zeros((128 - FT, 128), BF16)
                    continue
                for jb, v in enumerate(_sums_b(*[quad(i) for i in range(4)]) + [quad(0), quad(3)]):
                    w4q[first, jb, pl.ds(rows * ch, rows), :] = v.astype(BF16)
            if not tail:
                marks.append(w4q.bitcast(U32).at[pl.ds(zsm[32 + ch], NQ)][first, 0, pl.ds(0, 8), :])
        return marks

    def stage_b2n(w, h3, r0, n, k, done, prep=False):
        ia, ib = _STRASSEN[k]
        ka, q, slot = (8 if ia == 6 else ia), n // 8, NEST.index(k)

        def lblk(i, z):
            hv = opaque(h3, z)
            return jnp.concatenate([hv[g + 3 * (i % 2), ka, pl.ds((i // 2) * q, q), :] for g in range(3)], axis=1)

        def raw(j, lo, hi, z=None):
            return wblocks("w4", j, z)(ib - 5, ib - 5)[lo:hi]

        quad = lambda i, z=None: raw(i % 2, 192 * (i // 2), 192 * (i // 2 + 1), z)
        if ib >= 5:
            wt = [raw(j, 384, 448) for j in range(2)]
        else:
            wq = w4q.bitcast(U32)
            wq = wq.at[pl.ds(zsm[6], NQ)] if prep else wq
            wt = [wq[slot, 7, pl.ds(64 * j, 64), :] for j in range(2)]
        tail = _dot(_unpack(opaque(h3, 5)[6, ka, pl.ds(0, 2 * q), :]), _unpack(jnp.concatenate(wt, axis=1)))
        ms = []
        for ja, jb in _STRASSEN:
            if ja >= 5:
                lv = _unpack(lblk(3 * (ja - 5), 5))
            else:
                p_, q_, sg = _SUMS_A[ja]
                lv = psum(lblk(p_, ja), lblk(q_, ja), sg)
            z = zsm[8 + 7 * slot + jb] if prep and ib >= 5 else None
            if ib < 5:
                wv = _unpack(attach(wq[slot, jb]))
            elif jb >= 5:
                wv = _unpack(quad(3 * (jb - 5), z))
            elif prep:
                p_, q_, sg = _SUMS_B[jb]
                wv = psum(quad(p_, z), quad(q_, z), sg)
                keep(w4n.at[slot, pl.ds(jb, 1)], wv)
                wv = wv.astype(BF16)
            else:
                wv = _unpack(attach(w4n.bitcast(U32)[slot, jb]))
            ms.append(_dot(lv, wv))
        c11, c12, c21, c22 = _combine(*ms)
        done[0][k] = jnp.concatenate([c11, c21], axis=0) + tail[:, :128]
        done[1][k] = jnp.concatenate([c12, c22], axis=0) + tail[:, 128:]
        b2_done(w, done, r0, n)

    w = window(0, 2 * TS + LEAD)
    H = TS // 2
    with jax.named_scope("t0a"):
        cps["qa"].wait()
        cps["wmoda"].wait()

        mv = {}

        def mod_fn(j, toks):
            mv[j] = mod_cols(j, 1, toks)[0]
            if len(mv) == 3:
                modbuf[0] = mv[2] * mv[0]
                modbuf[1] = mv[2] * (1.0 + mv[1])

        segment(G5B, 0, MU, mod_fn=mod_fn)
        put(w["h"], pl.ds(0, QA), stage_a0(w, 0, QA))
    with jax.named_scope("t0b"):
        cps["wmodb"].wait()
        sb, cb = mod_cols(3, 2)
        modbuf[3] = 2.0 * sb
        modbuf[4] = 2.0 + 2.0 * cb
        n3 = stage_a1(w, 0, QA, n2=slabs(w["h"], 0, QA))
    XB = TS - XA
    with jax.named_scope("t1a"):
        cps["w1a"].wait()
        cps["qx"].wait()
        put(w["h"], pl.ds(QA, XA), stage_a0(w, QA, XA))
        stage_a2(w, n3, 0, QA, c1=W1A, fine=80)
    with jax.named_scope("t1b"):
        cps["w1b"].wait()
        n3a = stage_a1(w, QA, XA, n2=slabs(w["h"], QA, XA), f32=True)
        stage_a2(w, n3, 0, QA, c0=W1A)
        stage_a2(w, [dd_rest("w1", *_rows2(n3a))], QA, XA, prep=True)
    with jax.named_scope("t2"):
        cps["qb"].wait()
        cps["w2"].wait()
        n3b = stage_a1(w, QA + XA, XB, f32=True)
        stage_b1b(w, stage_b1a(w, 0, TS, prep=True), 0, TS, deep=False)
        stage_a2(w, [dd_rest("w1", *_rows2(n3b))], QA + XA, XB)
        stage_b1b(w, stage_b1a(w, TS, XA), TS, XA)
        stage_b1a(w, TS + XA, XB)
    with jax.named_scope("t3"):
        cps["w3"].wait()
        stage_b1b(w, slabs(w["h"], TS + XA, XB), TS + XA, XB)
        for op in "a0 h a1 a2 a3 a4 a5 H z0 z1 z2".split():
            if op[0] in "hH":
                stage_b2h(w, *((hba, 0) if op == "h" else (hbb, TS)), TS, prep=op == "h")
            elif op[0] == "a":
                stage_b2a(w, hba, 0, TS, int(op[1]), int(op[1]) + 1, prep=True)
            else:
                stage_b2z(w, hbb, int(op[1]), prep=True)
    with jax.named_scope("t4"):
        cps["w4"].wait()
        cps["wmodg"].wait()
        done = {0: {}, 1: {}}
        for op in "m4 P m0 4:0:6:7 m2 8:0 m1 8:1 m3 8:3 4:1:6:7 8:2 8:4 8:5".split():
            op, *rng = op.split(":")
            rng = [int(x) for x in rng]
            if op[0] == "m":
                c = int(op[1])
                modbuf[5, :, pl.ds(c * 128, 128)] = 0.5 * _dot(modbuf[6], weights(wmodbuf, 5 * NC + c, 5 * NC + c + 1))
            elif op[0] == "8":
                stage_b2n(w, hba, 0, TS, *rng, done, prep=True)
            elif op[0] == "P":
                stage_b2b(w, hba, 0, TS, 2, marks=prep_w4(24))
            else:
                stage_b2b(w, hba, 0, TS, *rng, done=done, prep=True)
        out_copy(0, TS).start()
        cps["q1"].wait()

    CBS = (128, 128)
    PART = {"a": (TS, TS), "c": (TS, H), "d": (TS + H, H)}
    BODY = "4:0:6:7 4:1:6:7 4:2 8:1 8:5 r0 r1 1a 8:3 2c 2d Nc nd 8:0 8:4 8:2 z:0 ha z:1 z:2"

    def step(s, carry):
        r0 = pl.multiple_of(s * TS, TS)
        w = window(r0, 2 * TS + LEAD)
        x1, rest, done = {}, {}, {0: {}, 1: {}}
        for op in BODY.split():
            op, *rng = op.split(":")
            rng = [int(x) for x in rng]
            if op[0] == "3":
                stage_b2a(w, hbb, TS, TS, *rng)
            elif op[0] == "z":
                stage_b2z(w, hbb, *rng)
            elif op[0] == "N":
                pending.extend(stage_b1b(w, x1[op[1]], *PART[op[1]]))
            elif op[0] == "h":
                stage_b2h(w, hbb, TS, TS)
            elif op[0] == "4":
                stage_b2b(w, hbb, 0, TS, *rng, done=done)
            elif op[0] == "8":
                stage_b2n(w, hbb, 0, TS, *rng, done)
            elif op[0] == "2":
                x1[op[1]] = stage_b1a(w, *PART[op[1]])
            elif op[0] == "n":
                stage_b1b(w, x1[op[1]], *PART[op[1]])
            elif op[0] == "r":
                j = int(op[1])
                rest[j] = dd_rest("w1", *_rows2(stage_a1(w, TS + LEAD + sum(CBS[:j]), CBS[j], f32=True)))
            else:
                ra, n = PART[op[1]]
                parts = [rest[j] for j in range(len(CBS)) if ra - TS <= sum(CBS[:j]) < ra - TS + n]
                stage_a2(w, parts, ra + LEAD, n, last_valid=(s < NT - 2) if ra + n == 2 * TS else None)
        out_copy(r0, TS).start()
        return carry

    with jax.named_scope("p2main"):
        jax.lax.fori_loop(1, NT - 1, step, 0)
    with jax.named_scope("p2epi"):
        w = window(S - 2 * TS, 2 * TS + LEAD)
        rows = pl.ds(S - TS, TS)
        pending.append(hhbuf[0, pl.ds(S, 8), :])
        def flush(rows, cols):
            pltpu.make_async_copy(obuf.at[rows, cols], out_hbm.at[rows, cols], sem_out.at[0]).start()

        done = {0: {}, 1: {}}
        for op in "p0 1 3 2 4 0 5 p1".split():
            if op[0] == "p":
                stage_b2b(w, hbb, TS, TS, int(op[1]), done=done)
            else:
                stage_b2n(w, hbb, TS, TS, int(op), done)
        flush(rows, pl.ds(0, 512))
        sub = 0
        for n in (128, 64, 64):
            stage_b2b(w, hbb, TS, n, 2, sub=sub)
            flush(pl.ds(S - TS + sub, n), pl.ds(512, 128))
            sub += n
        pltpu.make_async_copy(obuf, out_hbm, sem_out.at[0]).wait()


@jax.jit
def pallas_adaLN_cond__ssm_conv_h3__mixer_s_mlp__prompt_kernel(
    A_q: jax.Array,
    A_k: jax.Array,
    A_v: jax.Array,
    A_shift_k: jax.Array,
    A_ssm_k: jax.Array,
    A_ssm_D: jax.Array,
    B_x: jax.Array,
    B_w1: jax.Array,
    B_w2: jax.Array,
    B_w3: jax.Array,
    B_w4: jax.Array,
    c: jax.Array,
    w_mod: jax.Array,
):
    del B_x

    def tiles(x):
        return x.reshape(S // 8, 8, NC, 128).transpose(0, 2, 1, 3).reshape(S * NC, 128)

    def pairs(x):
        r, n = x.shape
        return x.reshape(r // 16, 2, 8, n // 128, 128).transpose(0, 1, 3, 2, 4)

    args = (
        A_q.reshape(S, D), tiles(A_k), tiles(A_v),
        A_shift_k.T, A_ssm_k, A_ssm_D.reshape(NC, 128),
        pairs(B_w1), pairs(B_w2), pairs(B_w3.T), pairs(B_w4), c, pairs(w_mod),
    )
    scratch = [
        pltpu.VMEM((NA, P * NC + 128, 128), BF16),
        pltpu.VMEM((NA, P * NC + 64, 128), BF16),
        pltpu.VMEM((D, S), BF16),
        pltpu.VMEM((R, 256, 128), BF16),
        pltpu.VMEM((2, R, 128, 128), BF16),
        pltpu.VMEM((128, 128), BF16),
        pltpu.VMEM((D // 16, 6 * NC, 16, 128), BF16),
        pltpu.VMEM((D // 16, NC, 16, 128), BF16),
        pltpu.VMEM((D // 16, NC, 16, 128), BF16),
        pltpu.VMEM((FF // 16, NC, 16, 128), BF16),
        pltpu.VMEM((FF // 16, NC, 16, 128), BF16),
        pltpu.VMEM((S + 64, D), BF16),
        *[pltpu.VMEM((NA, R, 16, 4, 8, 128), F32) for _ in range(NC)],
        pltpu.VMEM((NC, 2, R, 16, 2, 8, 128), F32),
        pltpu.VMEM((2 * NC, R, 256, 128), BF16),
        pltpu.VMEM((32, 128), U32),
        pltpu.VMEM((NC, 8, 8, 128), F32),
        pltpu.VMEM((NC, S + 32, 128), F32),
        pltpu.VMEM((8, 8, D), F32),
        pltpu.VMEM((S + 32, D), F32),
        pltpu.VMEM((NC, S + 32, 128), F32),
        pltpu.VMEM((NC, S + 32, 128), F32),
        pltpu.VMEM((8, 2, TS + 16, 128), BF16),
        pltpu.VMEM((5, 2, 1, 256, 128), BF16),
        pltpu.VMEM((5, 2, 1, 256, 128), BF16),
        pltpu.VMEM((5, 6, 2, 128, 128), BF16),
        pltpu.VMEM((5, 2, 2, FT, 128), BF16),
        pltpu.VMEM((5, 2, 1, 896, 128), BF16),
        pltpu.VMEM((8, 9, 144, 128), BF16),
        pltpu.VMEM((8, 9, 144, 128), BF16),
        pltpu.VMEM((2, 8, 384, 128), BF16),
        pltpu.VMEM((NQ, 8, 384, 128), BF16),
        pltpu.VMEM((3, 7, 5, 128, 128), BF16),
        pltpu.VMEM((8, 5, 80, 128), BF16),
        pltpu.VMEM((S, D), BF16),
        pltpu.VMEM((4, D), BF16),
        pltpu.VMEM((NC, 128), BF16),
        pltpu.VMEM((1, D), BF16),
        pltpu.SMEM((64,), jnp.int32),
        pltpu.SemaphoreType.DMA((40,)),
        pltpu.SemaphoreType.DMA((1,)),
    ]
    out = pl.pallas_call(
        _kernel,
        out_shape=jax.ShapeDtypeStruct((S, D), BF16),
        in_specs=[pl.BlockSpec(memory_space=pl.ANY)] * len(args),
        out_specs=pl.BlockSpec(memory_space=pl.ANY),
        scratch_shapes=scratch,
        grid=(1,),
        compiler_params=pltpu.CompilerParams(vmem_limit_bytes=108 * 1024 * 1024, disable_semaphore_checks=True,
                                             disable_bounds_checks=True),
        name="adaln_h3_mixer",
    )(*args)
    return out.reshape(1, S, D)
```

```python
import numpy as np
import jax
import jax.numpy as jnp
import jax.experimental.pallas as pl
import jax.experimental.pallas.tpu as pltpu

F32 = jnp.float32
BF16 = jnp.bfloat16
U32 = jnp.uint32

S = 2048
D = 640
FF = 1728
NC = D // 128
R = 4
P = 128 * R
NA = S // P
TS = 256
NT = S // TS
LEAD = 16
EPS = 1e-5
N3 = (1, 3, 4, 2)
NEST = (1, 4, 0, 2, 3, 5)
NQ = len(NEST)
FT = (FF - 1536) // 2


def _freq(row):
    t, part, s = row >> 4, (row >> 3) & 1, row & 7
    return 32 * (t & 7) + 4 * s + 2 * (t >> 3) + 1, P * part


def _cos(j, scale):
    jf = (j & (4 * P - 1)).astype(F32)
    u = 2.0 * np.pi / (4 * P)
    x = jnp.abs(jf * u - np.pi) - 0.5 * np.pi
    x2 = x * x
    poly = scale / 362880.0 - x2 * (scale / 39916800.0)
    for coef in (-1.0 / 5040.0, 1.0 / 120.0, -1.0 / 6.0, 1.0):
        poly = poly * x2 + coef * scale
    return poly * x


_DUR = {"t": 8, "u": 16, "k": 16, "i": 16, "m": 12, "g": 0, "c": 0, "j": 16}
_POST = {"t": 8.0, "u": 16.0, "k": 24.0, "i": 4.0, "j": 4.0, "m": 18.0}


def _plan_tokens(order, maxutil):
    lag, cap, pre, margin = 8, 62, 4, 3
    start, slots = {}, []
    for n in order:
        start[n] = len(slots)
        slots += [(n, r) for r in range(_DUR[n[0]])]
    nslot = len(slots) + lag
    free = [cap - (_POST[slots[i - lag][0][0]] if i >= lag else 0.0) for i in range(-pre, nslot)]
    units = []
    for n in order:
        kind, a, c = n
        if kind == "u":
            units += [(n + (g,), 94.0, start[n], -pre) for g in range(8)]
        elif kind == "g":
            units += [(n + (g,), 150.0, start[n], -pre) for g in range(8)]
        elif kind in "ic":
            src_ = [start[m] for m in (("u", a, c), ("k", a, c)) if m in start]
            for t in range(16):
                rel = max(max(src_) + 16, max(src_) + t + lag + 3) if src_ else -pre
                units.append((n + (t,), 32.0 * a + 48.0, nslot if kind == 'c' else start[n], rel))

    def simulate(util):
        left = [u[1] for u in units]
        done = [None] * len(units)
        for i in range(-pre, nslot):
            budget = util * free[i + pre]
            for j, u in enumerate(units):
                if budget <= 0.0:
                    break
                if done[j] is None and u[3] <= i:
                    use = min(budget, left[j])
                    left[j] -= use
                    budget -= use
                    if left[j] <= 1e-9:
                        done[j] = i + 1
        ok = all(u[2] < 8 or (d is not None and d <= max(u[2] - (1 if u[0][0] in 'cg' else margin), u[3] + 1))
                 for d, u in zip(done, units))
        return done, ok

    lo_, hi_ = 0.05, maxutil
    for _ in range(12):
        mid = 0.5 * (lo_ + hi_)
        if simulate(mid)[1]:
            hi_ = mid
        else:
            lo_ = mid
    done, _ = simulate(hi_)
    plan = {}
    for u, d in zip(units, done):
        if u[0][0] == "c":
            plan[u[0]] = slots[max((nslot - 1 if d is None else min(d, nslot - 1)) - lag, 0)]
        elif d is not None and 0 <= d < u[2]:
            plan.setdefault(slots[d], []).append(u[0])
    return plan


def _unpack(w):
    return pltpu.bitcast(w, BF16)


def _dot(a, b):
    return jnp.dot(a.astype(BF16), b, preferred_element_type=F32)


def _dot_nt(a, b):
    return jax.lax.dot_general(a.astype(BF16), b, (((1,), (1,)), ((), ())), preferred_element_type=F32)


def _dot_fine(x, w, chunk):
    if not chunk:
        return _dot(x, w)
    n = w.shape[1]
    head = _dot(x, w[:, :n - 128])
    last = jnp.concatenate([_dot(x[r:r + chunk], w[:, n - 128:]) for r in range(0, x.shape[0], chunk)], axis=0)
    return jnp.concatenate([head, last], axis=1)


def _rows2(x):
    n, c = x.shape
    x = x.reshape(n // 32, 2, 16, c)
    return x[:, 0].reshape(n // 2, c), x[:, 1].reshape(n // 2, c)


def _unrows2(top, bot):
    n, c = top.shape
    return jnp.stack([top.reshape(n // 16, 16, c), bot.reshape(n // 16, 16, c)], axis=1).reshape(2 * n, c)


def _sums_a(a11, a12, a21, a22):
    return [a11 + a22, a21 + a22, a11 + a12, a21 - a11, a12 - a22]


def _sums_b(b11, b12, b21, b22):
    return [b11 + b22, b12 - b22, b21 - b11, b11 + b12, b21 + b22]


_STRASSEN = ((0, 0), (1, 5), (5, 1), (6, 2), (2, 6), (3, 3), (4, 4))


_SUMS_A = ((0, 3, 1), (2, 3, 1), (0, 1, 1), (2, 0, -1), (1, 3, -1))
_SUMS_B = ((0, 3, 1), (1, 3, -1), (2, 0, -1), (0, 1, 1), (2, 3, 1))


def _combine(m1, m2, m3, m4, m5, m6, m7):
    return (m1 + m4) + (m7 - m5), m3 + m5, m2 + m4, (m1 - m2) + (m3 + m6)


def _lo(w):
    return pltpu.bitcast(w << 16, F32)


def _hi(w):
    return pltpu.bitcast(w & jnp.uint32(0xFFFF0000), F32)


def _ln(x, eps=EPS):
    m = jnp.sum(x, axis=-1, keepdims=True) * (1.0 / D)
    xc = x - m
    v = jnp.sum(xc * xc, axis=-1, keepdims=True) * (1.0 / D)
    return xc * jnp.exp(-0.5 * jnp.log(v + eps))


def _gelu2(x):
    c0 = 0.7978845608028654
    c1 = c0 * 0.044715
    return x + x * jnp.tanh(x * (c0 + c1 * (x * x)))


def _bfly(tr, ti):
    s02r, s02i = tr[0] + tr[2], ti[0] + ti[2]
    d02r, d02i = tr[0] - tr[2], ti[0] - ti[2]
    s13r, s13i = tr[1] + tr[3], ti[1] + ti[3]
    d13r, d13i = tr[1] - tr[3], ti[1] - ti[3]
    x0r, x0i = s02r + s13r, s02i + s13i
    x2r, x2i = s02r - s13r, s02i - s13i
    return [x0r, d02r + d13i, x2r, d02r - d13i], [x0i, d02i - d13r, x2i, d02i + d13r]


def _kernel(q_hbm, k_hbm, v_hbm, shift_hbm, ssmk_hbm, ssmd_hbm, w1_hbm, w2_hbm, w3t_hbm, w4_hbm,
            c_hbm, wmod_hbm,
            out_hbm,
            kbuf, vbuf, skbuf, fwdbuf, invbuf, permbuf,
            wmodbuf, w1buf, w2buf, w3buf, w4buf, qbuf,
            xs0, xs1, xs2, xs3, xs4, kraw, stg, zbuf, coefbuf, ybuf, modbuf, x2buf, hbuf, hhbuf, xobuf,
             w1s, w2s, w3s, w3ts, w4s, hba, hbb, w4n, w4q, w3n, xibuf, obuf, shiftbuf, dbuf, cbuf,
            zsm, sem_in, sem_out):
    cps = {}
    n_sem = [0]

    def start(name, src, dst):
        cp = pltpu.make_async_copy(src, dst, sem_in.at[n_sem[0]])
        n_sem[0] += 1
        cp.start()
        cps[name] = cp

    class Both:
        def __init__(self, a, b):
            self.cps = (a, b)

        def wait(self):
            for cp in self.cps:
                cp.wait()

    def start_w(name, src, dst, c0=0, n=NC):
        for e in range(2):
            start(name + str(e), src.at[:, e, pl.ds(c0, n)], dst.at[:, pl.ds(c0, n), pl.ds(8 * e, 8), :])
        cps[name] = Both(cps[name + "0"], cps[name + "1"])

    CH = P * NC
    HALO = 8 * NC

    def start_s(a):
        cols = pl.ds(a * P, P)
        start("s%d" % a, ssmk_hbm.at[:, cols], skbuf.at[:, cols])

    def start_kv(a):
        if a == 0:
            kbuf[0, pl.ds(0, HALO + 8), :] = jnp.zeros((HALO + 8, 128), BF16)
            start("k0", k_hbm.at[pl.ds(0, CH), :], kbuf.at[0, pl.ds(HALO, CH), :])
        else:
            start("k%d" % a, k_hbm.at[pl.ds(a * CH - HALO, CH + HALO), :], kbuf.at[a, pl.ds(0, CH + HALO), :])
        start("v%d" % a, v_hbm.at[pl.ds(a * CH, CH), :], vbuf.at[a, pl.ds(0, CH), :])

    for n in "s0 x0 s1 k0 k1 s2 k2 s3 k3".split():
        if n[0] == "s":
            start_s(int(n[1]))
        elif n[0] == "k":
            start_kv(int(n[1]))
        else:
            start("d", ssmd_hbm, dbuf)
            start("shift", shift_hbm, shiftbuf)
            start("c", c_hbm, cbuf)
    QA = TS + LEAD
    XA = 128
    QB = 2 * TS + LEAD
    W1A = 2

    def start_q(name, r0, n):
        start(name, q_hbm.at[pl.ds(r0, n), :], qbuf.at[pl.ds(r0, n), :])

    start_q("qa", 0, QA)
    start_w("wmoda", wmod_hbm, wmodbuf, 0, 3 * NC)
    start_w("wmodb", wmod_hbm, wmodbuf, 3 * NC, 2 * NC)
    start_q("qx", QA, XA)
    start_w("w1a", w1_hbm, w1buf, 0, W1A)
    start_w("w1b", w1_hbm, w1buf, W1A, NC - W1A)
    start_q("qb", QA + XA, QB - QA - XA)
    start_w("w2", w2_hbm, w2buf)
    start_w("w3", w3t_hbm, w3buf)
    start_w("w4", w4_hbm, w4buf)
    start_w("wmodg", wmod_hbm, wmodbuf, 5 * NC, NC)
    start_q("q1", QB, S - QB)

    kw = kbuf.bitcast(U32)
    vw = vbuf.bitcast(U32)
    zbuf[...] = jnp.zeros(zbuf.shape, U32)
    for j in range(64):
        zsm[j] = 0
    for c in range(NC):
        ybuf[c, pl.ds(S, LEAD), :] = jnp.zeros((LEAD, 128), F32)
        hhbuf[c, pl.ds(0, 8), :] = jnp.zeros((8, 128), F32)
    qbuf[pl.ds(S, LEAD), :] = jnp.zeros((LEAD, D), BF16)

    def sample(pos):
        return (pos & ~15) + 2 * (pos & 7) + ((pos >> 3) & 1)

    def tables(p, carry):
        f2, off = _freq(jax.lax.broadcasted_iota(jnp.int32, (256, 128), 0))
        n = R * sample(jax.lax.broadcasted_iota(jnp.int32, (256, 128), 1)) + p
        fwdbuf[p] = _cos(f2 * n + off, 1.0).astype(BF16)
        return carry

    jax.lax.fori_loop(0, R, tables, 0)

    def unit_g(kt, r):
        f2, off = _freq(jax.lax.broadcasted_iota(jnp.int32, (16, 128), 1) + 128 * kt)
        j0 = f2 * (R * (jax.lax.broadcasted_iota(jnp.int32, (16, 128), 0) + 16 * r)) + off
        for p in range(R):
            invbuf[kt, p, pl.ds(16 * r, 16), :] = _cos(j0 + p * f2, 1.0 / P).astype(BF16)
        return [invbuf.bitcast(U32)[kt, p, pl.ds(8 * r, 8), :] for p in range(R)]

    i0 = jax.lax.broadcasted_iota(jnp.int32, (128, 128), 0)
    i1 = jax.lax.broadcasted_iota(jnp.int32, (128, 128), 1)
    permbuf[...] = jnp.where(i1 == R * sample(i0 & 31) + (i0 >> 5), 1.0, 0.0).astype(BF16)

    def fill_coef():
        cv = cbuf[...].astype(F32)
        modbuf[6] = jnp.broadcast_to(cv * jax.nn.sigmoid(cv), (8, D))
        coef = shiftbuf[...].astype(F32)
        dval = dbuf[...].astype(F32)
        for c in range(NC):
            for j in range(4):
                coefbuf[c, j] = jnp.broadcast_to(coef[j:j + 1, c * 128:(c + 1) * 128], (8, 128))
            coefbuf[c, 4] = jnp.broadcast_to(dval[c:c + 1, :], (8, 128))

    xs = (xs0, xs1, xs2, xs3, xs4)
    wsbufs = dict(w1=w1s, w2=w2s, w3=w3s, w4=w4s, w3t=w3ts)
    def split_ri(t):
        t = t.reshape(16, 2, 8, 128)
        return t[:, 0], t[:, 1]

    def get_never():
        return zbuf[pl.ds(0, 8), :] != 0

    def packed(x, slot, r0):
        n = x.shape[1]
        stg[slot, :, pl.ds(r0, n), :] = x.astype(BF16)
        return [stg.bitcast(U32)[slot, p, pl.ds(r0 // 2, n // 2), :] for p in range(R)]

    UG = 8

    def unit_u(a, c, g0, UG):
        c0, c1, c2, c3 = (coefbuf[c, pl.ds(j, 1)][None] for j in range(4))
        rows = lambda ref, r: ref[a, pl.ds((r // 4) * 4 * NC + 4 * c + r % 4, 8 * UG, stride=4 * NC), :]
        kk = jnp.stack([rows(kw, 4 + 32 * g0 + d) for d in range(-2, 4)]).reshape(6, UG, 8, 128)
        vv = jnp.stack([rows(vw, 32 * g0 + d) for d in range(4)]).reshape(4, UG, 8, 128)
        lo, hi = _lo(kk), _hi(kk)
        k0, k1, k2 = lo[2:], hi[1:5], lo[1:5]
        even = ((k0 * c0 + k1 * c1) + (k2 * c2 + hi[:4] * c3)) * _lo(vv)
        odd = ((hi[2:] * c0 + k0 * c1) + (k1 * c2 + k2 * c3)) * _hi(vv)
        kv = jnp.stack([even, odd], axis=1).reshape(2, R, UG, 8, 128)
        return packed(jnp.stack([kv[0], kv[1]], axis=2).reshape(R, 16 * UG, 128), NC + c, 16 * g0)

    def unit_i(a, c, t0, UG, z, after=None):
        x_c = xs[c].at[pl.ds(z, NA)]
        ts = pl.ds(t0, UG)
        yr = yi = None
        for j in range(a + 1):
            ur, ui = x_c[j, :, ts, 0], x_c[j, :, ts, 1]
            kr, ki = x_c[a - j, :, ts, 2], x_c[a - j, :, ts, 3]
            pr = ur * kr - ui * ki
            pi = ur * ki + ui * kr
            yr = pr if yr is None else yr + pr
            yi = pi if yi is None else yi + pi
        sr, si, dr, di = yr[:2] + yr[2:], yi[:2] + yi[2:], yr[:2] - yr[2:], yi[:2] - yi[2:]
        (sr0, sr1), (si0, si1), (dr0, dr1), (di0, di1) = ((x[0], x[1]) for x in (sr, si, dr, di))
        wr = jnp.stack([sr0 + sr1, dr0 - di1, sr0 - sr1, dr0 + di1])
        wi = jnp.stack([si0 + si1, di0 + dr1, si0 - si1, di0 - dr1])
        if after is not None:
            never = jnp.broadcast_to(zbuf[pl.ds(0, 8), :], wr.shape) != 0
            wr = jax.lax.select(never, jnp.broadcast_to(after, wr.shape), wr)
        return packed(jnp.stack([wr, wi], axis=2).reshape(R, 16 * UG, 128), c, 16 * t0)

    def segment(spec, z, maxutil=1.0, mod_fn=None):
        order = [(n[0], int(n[1]), int(n[2])) for n in spec.split()]
        plan = _plan_tokens(order, maxutil) if maxutil > 0 else {}
        never = get_never()
        units, groups, res = {}, {}, {}

        paced = {k_ for s_, ks in plan.items() if len(s_) == 2 for k_ in ks}

        def width(name):
            n = 8 if name[0] == "u" else 16
            return UG if all(name + (j,) in paced for j in range(n)) else 1

        def group(key):
            kind, a, c, j = key
            ug = width(key[:3])
            key = (kind, a, c, j - j % ug)
            if key not in groups:
                if kind == "u":
                    groups[key] = unit_u(a, c, key[3], ug)
                else:
                    fresh = ("u", a, c) in order or ("k", a, c) in order
                    groups[key] = unit_i(a, c, key[3], ug, z if fresh else 0,
                                         res[plan[key]]() if kind == "c" else None)
            return groups[key]

        def unit(key):
            if key not in units:
                if key[0] == "g":
                    units[key] = unit_g(key[1], key[3])
                else:
                    r = 8 * (key[3] % width(key[:3]))
                    units[key] = [v[r:r + 8] for v in group(key)]
            return units[key]

        def lhs(name, p, full, r0=0):
            out, last = [], 0
            for r in range(full.shape[0] // 8):
                keys = plan.get((name, r0 + r), ())
                if keys:
                    if 8 * r > last:
                        out.append(full[last:8 * r])
                    v = full[8 * r:8 * r + 8]
                    for key in keys:
                        v = jax.lax.select(never, unit(key)[p], v)
                    out.append(v)
                    last = 8 * r + 8
            if last < full.shape[0]:
                out.append(full[last:] if last else full)
            return out[0] if len(out) == 1 else jnp.concatenate(out, axis=0)

        def dft(name, rhs):
            tr, ti = [], []
            for p in range(R):
                f = lhs(name, p, fwdbuf.bitcast(U32)[p])
                r_, i_ = split_ri(_dot(_unpack(f), rhs[p]))
                if p == 0:
                    res.update({(name, r): (lambda r=r, v=r_: v[r]) for r in range(16)})
                tr.append(r_)
                ti.append(i_)
            return _bfly(tr, ti)

        st = {}
        for name in order:
            kind, a, c = name
            x_c = xs[c]
            if kind == "g":
                for r in range(8):
                    unit(name + (r,))
            elif kind == "c":
                for t in range(16):
                    group(name + (t,))
            elif kind == "m":
                toks = {}
                for r in range(_DUR["m"]):
                    for n_, key in enumerate(plan.get((name, r), ())):
                        toks.setdefault(2 * r + n_ % 2, []).extend(unit(key))
                mod_fn(a, toks)
            elif kind == "t":
                trs = []
                for b in range(R):
                    pm = lhs(name, b, permbuf.bitcast(U32)[...])
                    trs.append(_dot_nt(_unpack(pm), skbuf[pl.ds(c * 128, 128), pl.ds(a * P + b * 128, 128)]))
                res.update({(name, r): (lambda r=r, v=trs[0]: v[16 * r:16 * r + 8]) for r in range(8)})
                g_ = 128 // R
                st[a, c] = [jnp.concatenate([trs[b][p * g_:(p + 1) * g_] for b in range(R)], axis=0).astype(BF16)
                            for p in range(R)]
            elif kind == "u":
                rhs = [_unpack(jnp.concatenate([group(name + (g,))[p] for g in range(0, 8, width(name))], axis=0)) for p in range(R)]
                xr, xi = dft(name, rhs)
                for q in range(R):
                    x_c[a, q, :, 0] = xr[q]
                    x_c[a, q, :, 1] = xi[q]
            elif kind == "k":
                xr, xi = dft(name, st[a, c])
                for q in range(R):
                    if a == 0:
                        x_c[a, q, :, 2] = xr[q] + coefbuf[c, 4]
                        x_c[a, q, :, 3] = xi[q]
                    else:
                        pr, pi = kraw[c, (a - 1) % 2, q, :, 0], kraw[c, (a - 1) % 2, q, :, 1]
                        x_c[a, q, pl.ds(0, 8), 2] = xr[q][:8] - pi[:8]
                        x_c[a, q, pl.ds(0, 8), 3] = xi[q][:8] + pr[:8]
                        x_c[a, q, pl.ds(8, 8), 2] = xr[q][8:] + pi[8:]
                        x_c[a, q, pl.ds(8, 8), 3] = xi[q][8:] - pr[8:]
                    if a + 1 < NA:
                        kraw[c, a % 2, q, :, 0] = xr[q]
                        kraw[c, a % 2, q, :, 1] = xi[q]
            else:
                for p in range(R):
                    cols = [lhs(name, 2 * (p % 2) + kt,
                                invbuf.bitcast(U32)[kt, p], 8 * (p // 2))
                            for kt in range(2)]
                    g = _unpack(jnp.concatenate(cols, axis=1))
                    if kind == "j":
                        wp = _unpack(stg.bitcast(U32)[c, p])
                    else:
                        wp = _unpack(jnp.concatenate([group(name + (t,))[p] for t in range(0, 16, width(name))], axis=0))
                    yp = _dot(g, wp)
                    if p % 2 == 0:
                        res.update({(name, 4 * p + r): (lambda r=r, v=yp: v[16 * r:16 * r + 8]) for r in range(8)})
                    ybuf[c, pl.ds(a * P + p, 128, stride=R), :] = yp

    one = jnp.minimum(pl.program_id(0) + 1, 1)

    def once(fn):
        def body(z, carry):
            fn(z)
            return carry
        jax.lax.fori_loop(0, one, body, 0)

    default = ("t00 t01 t02 k00 t03 k01 t04 k02 k03 k04 g00|"
               "t10 t11 t12 k10 k11 k12 g10|"
               "t13 t14 k13 u00 k14 u01 u02 u03 i00 u04 i01 c02 c03|"
               "j02 j03 u10 i04 u11 u12 u13 i10 u14 i11 c12 c13|"
               "t20 t21 j12 t22 j13 t23 t24 k20 u20 k21 u21 k22 i14 k23 u22 k24 u23 i20 u24 i21 c22|"
               "t30 t31 j22 t32 t33 t34 k30 u30 k31 u31 k32 i23 k33 u32 k34 i24 u33 i30 u34 i31 c32|"
               "m00 j32 m10 i33 m20 i34")
    specs = default.split("|")
    G5B = specs[-1]
    segs = list(zip("s0 d shift c|s1|k0 v0|k1 v1|s2 k2 v2|s3 k3 v3".split("|"), specs[:-1]))
    MU = 1.5
    for i, (waits, spec) in enumerate(segs):
        with jax.named_scope("g%d" % i):
            for n in waits.split():
                cps[n].wait()
            if i == 0:
                fill_coef()
            once(lambda z: segment(spec, z, MU))

    def mod_cols(lo, n, toks=None):
        m = _dot(modbuf[6], weights(wmodbuf, lo * NC, (lo + n) * NC, toks=toks))
        return [m[:, j * D:(j + 1) * D] for j in range(n)]

    def mul_mod(x, j, cols=None):
        m = modbuf[j] if cols is None else modbuf[j, :, cols]
        return (x.reshape(-1, 8, x.shape[-1]) * m[None]).reshape(x.shape)

    def add_mod(x, j):
        return (x.reshape(-1, 8, x.shape[-1]) + modbuf[j][None]).reshape(x.shape)

    def slabs(ref, r0, n):
        return jnp.concatenate([ref[c, pl.ds(r0, n), :] for c in range(NC)], axis=1)

    def put(ref, rows, x):
        for c in range(NC):
            ref[c, rows, :] = x[:, c * 128:(c + 1) * 128]

    def window(base, n):
        rows = pl.ds(base, n)
        return dict(q=qbuf.at[rows, :], y=ybuf.at[:, rows, :], x2=x2buf.at[rows, :], h=hbuf.at[:, rows, :],
                    hh=hhbuf.at[:, pl.ds(base, n + 8), :],
                    o=obuf.at[pl.ds(base, n - LEAD), :])

    def weights(ref, c0=0, c1=NC, r0=0, r1=None, toks=None, raw=False, z=None):
        r1 = 16 * ref.shape[0] if r1 is None else r1
        view = ref.bitcast(U32)
        if z is not None:
            view = view.at[pl.ds(z, ref.shape[0])]
        never = get_never() if toks else None
        rt = -(-(r1 - r0) // 128)
        cols = []
        for j in range(c0, c1):
            wu = view[pl.ds(r0 // 16, (r1 - r0) // 16), j].reshape((r1 - r0) // 2, 128)
            if toks:
                parts, last = [], 0
                for i in range(rt):
                    for n_, t in enumerate(toks.get((j - c0) * rt + i, ())):
                        r = 64 * i + 8 * n_
                        if r > last:
                            parts.append(wu[last:r])
                        parts.append(jax.lax.select(never, t, wu[r:r + 8]))
                        last = r + 8
                parts.append(wu[last:])
                wu = jnp.concatenate(parts, axis=0)
            cols.append(wu)
        wu = jnp.concatenate(cols, axis=1)
        return wu if raw else _unpack(wu)

    def keep(dst, v):
        h = v.shape[0] // 2
        for c in range(v.shape[1] // 128):
            for r in (0, h):
                dst[c, pl.ds(r, h), :] = v[r:r + h, 128 * c:128 * (c + 1)].astype(BF16)

    def fetch(src_):
        u = src_.bitcast(U32)
        return jnp.concatenate([u[c] for c in range(u.shape[0])], axis=1)

    def wblocks(name, j, z=None):
        if name == "w3":
            blk = lambda kh, nh: weights(w3buf, 2 * kh, 2 * kh + 2, 128 * (j + 6 * nh), 128 * (j + 6 * nh + 1), raw=True, z=z)
        elif name == "w4":
            def blk(kh, nh):
                c = j + 2 * nh
                parts = [weights(w4buf, c, c + 1, 768 * kh, 768 * (kh + 1), raw=True, z=z),
                         weights(w4buf, c, c + 1, 1536 + FT * kh, 1536 + FT * (kh + 1), raw=True, z=z),
                         jnp.zeros(((128 - FT) // 2, 128), U32)]
                return jnp.concatenate(parts, axis=0)
        elif name == "w3t":
            blk = lambda kh, nh: weights(w3buf, 2 * kh, 2 * kh + 2, 1536 + FT * nh, 1536 + FT * (nh + 1), raw=True, z=z)
        else:
            ref = w1buf if name == "w1" else w2buf
            blk = lambda kh, nh: weights(ref, j + 2 * nh, j + 2 * nh + 1, 256 * kh, 256 * (kh + 1), raw=True, z=z)
        return blk

    def wsum(name, j, k):
        blk = wblocks(name, j, zsm[k])
        p, q, sign = _SUMS_B[k]
        return psum(blk(p // 2, p % 2), blk(q // 2, q % 2), sign)

    pending = []

    def attach(wv):
        if not pending:
            return wv
        never = get_never()
        rows = [wv[8 * i:8 * i + 8, :128] for i in range(8)]
        for i, t in enumerate(pending):
            rows[i % 8] = jax.lax.select(never, pltpu.bitcast(t, U32), rows[i % 8])
        pending.clear()
        first = jnp.concatenate(rows + ([wv[64:, :128]] if wv.shape[0] > 64 else []), axis=0)
        return first if wv.shape[1] == 128 else jnp.concatenate([first, wv[:, 128:]], axis=1)

    def sprods(name, j, lhs, k0=0, k1=7, prep=False):
        blk, buf = wblocks(name, j), wsbufs[name]
        out = []
        for ia, ib in _STRASSEN[k0:k1]:
            if prep and ib < 5:
                wv = wsum(name, j, ib)
                keep(buf.at[ib, j], wv)
                wv = wv.astype(BF16)
            else:
                wv = _unpack(attach(blk(ib - 5, ib - 5) if ib >= 5 else fetch(buf.at[ib, j])))
            if name == "w3t":
                out.append(_dot_nt(wv, lhs(ia)))
            else:
                out.append((_dot_nt if name == "w3" else _dot)(lhs(ia), wv))
        return out

    def spair(name, j, lhs, prep=False):
        return _combine(*sprods(name, j, lhs, prep=prep))

    def dd_rest(name, t, b):
        ref = w1buf if name == "w1" else w2buf
        m = t.shape[0]
        xb = jnp.concatenate([t, b], axis=0)
        last = _dot(xb, weights(ref, 4, 5))
        rem = _dot(xb[:, 512:], weights(ref, 0, 4, r0=512))
        return t, b, rem[:m], rem[m:], last[:m], last[m:]

    def dd_main(name, parts, prep=False):
        t, b, rt, rb, lt, lb = (jnp.concatenate(v, axis=0) for v in zip(*parts))
        ops = _sums_a(t[:, :256], t[:, 256:512], b[:, :256], b[:, 256:512]) + [t[:, :256], b[:, 256:512]]
        top, bot = [None] * 4, [None] * 4
        for j in range(2):
            top[j], top[j + 2], bot[j], bot[j + 2] = spair(name, j, lambda i: ops[i], prep)
        return (jnp.concatenate([jnp.concatenate(top, axis=1) + rt, lt], axis=1),
                jnp.concatenate([jnp.concatenate(bot, axis=1) + rb, lb], axis=1))

    def stage_a0(w, r0, n):
        rows = pl.ds(r0, n)
        x = w["q"][rows, :].astype(F32)
        x2 = x + add_mod(mul_mod(_ln(x), 1), 0) * slabs(w["y"], r0, n)
        w["x2"][rows, :] = x2
        return _ln(x2)

    def stage_a1(w, r0, n, n2=None, f32=False):
        if n2 is None:
            n2 = stage_a0(w, r0, n)
        h = add_mod(mul_mod(n2, 4), 3)
        put(w["h"], pl.ds(r0, n), h)
        n3 = _ln(h, 4 * EPS)
        return n3 if f32 else n3.astype(BF16)

    def stage_a2(w, n3, r0, n, last_valid=None, fine=0, c0=0, c1=NC, prep=False):
        hh = _gelu2(_unrows2(*dd_main("w1", n3, prep)) if isinstance(n3, list) else _dot_fine(n3, weights(w1buf, c0, c1), fine))
        for c in range(c0, c1):
            blk = hh[:, (c - c0) * 128:(c - c0 + 1) * 128]
            w["hh"][c, pl.ds(r0 + 8, n - LEAD), :] = blk[:n - LEAD]
            tail = blk[n - LEAD:]
            if last_valid is not None:
                tail = jnp.where(last_valid, tail, 0.0)
            w["hh"][c, pl.ds(r0 + 8 + n - LEAD, LEAD), :] = tail

    def stage_b1a(w, r0, n, prep=False):
        lane = jax.lax.broadcasted_iota(jnp.int32, (n, 128), 1)
        sh = lambda c, d: w["hh"][c, pl.ds(r0 + 8 + d, n), :]
        g = jnp.concatenate([sh(0, -1),
                             jnp.where(lane < 32, sh(1, -1), sh(1, 1)),
                             jnp.where(lane < 64, sh(2, 1), sh(2, -2)),
                             jnp.where(lane < 96, sh(3, -2), sh(3, 2)),
                             sh(4, 2)], axis=1)
        x1 = slabs(w["h"], r0, n) + _unrows2(*dd_main("w2", [dd_rest("w2", *_rows2(g))], prep))
        put(w["h"], pl.ds(r0, n), x1)
        return x1

    def stage_b1b(w, x1, r0, n, deep=True):
        t, b = _rows2(_ln(x1, 4 * EPS))
        ops = _sums_a(t[:, :256], t[:, 256:512], b[:, :256], b[:, 256:512]) + [t[:, :256], b[:, 256:512]]
        ops.append(jnp.concatenate([t[:, 512:], b[:, 512:]], axis=1))
        for i, v in enumerate(ops):
            keep(xobuf.at[i, :, pl.ds(r0 // 2, n // 2), :], v)
        if deep:
            for s_, k in enumerate(N3):
                u, v = _rows2(ops[_STRASSEN[k][0]])
                for i, x in enumerate(_sums_a(u[:, :128], u[:, 128:], v[:, :128], v[:, 128:])):
                    xibuf[s_, i, pl.ds((r0 - TS) // 4, n // 4), :] = x.astype(BF16)
        return [ops[4][i:i + 8, :128] for i in range(0, n // 2, 8)]

    def out_copy(r0, n):
        rows = pl.ds(r0, n)
        return pltpu.make_async_copy(obuf.at[rows, :], out_hbm.at[rows, :], sem_out.at[0])

    def opaque(ref, i):
        ref = ref.bitcast(U32)
        return ref.at[:, :, pl.ds(pl.multiple_of(zsm[i] * 32, 32), ref.shape[2]), :]

    def emit(h3, j, left, right):
        m = left.shape[0] // 2
        g = [left[:m], right[:m], left[m:], right[m:]]
        for k, v in enumerate(_sums_a(*g) + g):
            h3[j, k, pl.ds(0, m), :] = v.astype(BF16)

    def w3_operands(r0, n):
        u, rows = xobuf.bitcast(U32), pl.ds(r0 // 4, n // 4)
        xr = _unpack(jnp.concatenate([u[7, 0, rows, :], u[7, 1, rows, :]], axis=0))
        return xr, lambda i: _unpack(jnp.concatenate([u[i, 0, rows, :], u[i, 1, rows, :]], axis=1))

    def stage_b2h(w, h3, r0, n, prep=False):
        xr, ops = w3_operands(r0, n)
        m = n // 2
        rem = _dot_nt(weights(w3buf, 4, 5, r0=1536), xr)
        c11, c12, c21, c22 = spair("w3t", 0, ops, prep)
        pad = jnp.zeros((128 - FT, m), F32)
        g11, g12, g21, g22 = (jnp.concatenate([_gelu2(c + r), pad], axis=0).T for c, r in (
            (c11, rem[:FT, :m]), (c12, rem[FT:, :m]), (c21, rem[:FT, m:]), (c22, rem[FT:, m:])))
        emit(h3, 6, jnp.concatenate([g11, g21], axis=0), jnp.concatenate([g12, g22], axis=0))

    def stage_b2a(w, h3, r0, n, lo=0, hi=6, prep=False):
        xr, ops = w3_operands(r0, n)
        for j in range(lo, hi):
            r1, r2 = (_dot_nt(xr, weights(w3buf, 4, 5, 128 * t, 128 * (t + 1))) for t in (j, j + 6))
            c11, c12, c21, c22 = spair("w3", j, ops, prep)
            emit(h3, j, _gelu2(jnp.concatenate([c11, c21], axis=0) + r1), _gelu2(jnp.concatenate([c12, c22], axis=0) + r2))

    def stage_b2z(w, h3, g, prep=False):
        xr, ops = w3_operands(TS, TS)
        ms = {0: {}, 1: {}}

        def nested(k):
            ib, slot = _STRASSEN[k][1], N3.index(k)

            def quad(i, z=None):
                j, cols = g + 3 * (i % 2), slice(128 * (i // 2), 128 * (i // 2 + 1))
                if ib >= 5:
                    return wblocks("w3", j, z)(ib - 5, ib - 5)[:, cols]
                u = w3s.bitcast(U32)
                return (u if z is None else u.at[pl.ds(z, 5)])[ib, j, i // 2]

            prods = []
            for ja, jb in _STRASSEN:
                if jb >= 5:
                    wv = _unpack(quad(3 * (jb - 5)))
                elif prep:
                    p_, q_, sg = _SUMS_B[jb]
                    wv = psum(quad(p_, zsm[jb]), quad(q_, zsm[jb]), sg)
                    keep(w3n.at[g, slot, pl.ds(jb, 1)], wv)
                    wv = wv.astype(BF16)
                else:
                    wv = _unpack(w3n.bitcast(U32)[g, slot, jb])
                if ja < 5:
                    lv = xibuf.bitcast(U32)[slot, ja, pl.ds(0, TS // 8), :]
                else:
                    e = ja - 5
                    lv = xobuf.bitcast(U32)[_STRASSEN[k][0], e, pl.ds(TS // 4, TS // 4), :]
                    lv = lv.reshape(TS // 64, 2, 8, 128)[:, e].reshape(TS // 8, 128)
                prods.append(_dot_nt(_unpack(lv), wv))
            c11, c12, c21, c22 = _combine(*prods)
            ms[0][k], ms[1][k] = _unrows2(c11, c21), _unrows2(c12, c22)

        for k in N3:
            nested(k)
        for e in range(2):
            j = g + 3 * e
            r1, r2 = (_dot_nt(xr, weights(w3buf, 4, 5, 128 * t, 128 * (t + 1))) for t in (j, j + 6))
            for k in range(7):
                if k not in N3:
                    ms[e][k] = sprods("w3", j, ops, k, k + 1)[0]
            c11, c12, c21, c22 = _combine(*[ms[e][k] for k in range(7)])
            emit(h3, j, _gelu2(jnp.concatenate([c11, c21], axis=0) + r1),
                 _gelu2(jnp.concatenate([c12, c22], axis=0) + r2))

    def finish(w, h2, r0, n, c):
        nc = h2.shape[1] // 128
        rows, cols = pl.ds(r0, n), pl.ds(c * 128, nc * 128)
        x1 = jnp.concatenate([w["h"][c + i, rows, :] for i in range(nc)], axis=1)
        w["o"][rows, cols] = (w["x2"][rows, cols] + mul_mod(x1 + h2, 5, cols)).astype(BF16)

    def b2_done(w, done, r0, n):
        if len(done[0]) == len(done[1]) == 7:
            c11, c12, c21, c22 = _combine(*[jnp.concatenate([done[0][k], done[1][k]], axis=1) for k in range(7)])
            finish(w, _unrows2(c11, c21), r0, n, 0)
            finish(w, _unrows2(c12, c22), r0, n, 2)

    def stage_b2b(w, h3, r0, n, j, k0=0, k1=7, done=None, prep=False, sub=0, marks=()):
        hv = opaque(h3, j)
        blk = lambda k: jnp.concatenate([hv[p, k, pl.ds(sub // 4, n // 4), :] for p in range(7)], axis=1)
        r0 += sub
        if j < 2:
            for k in range(k0, k1):
                if k not in NEST:
                    done[j][k] = sprods("w4", j, lambda i: _unpack(blk(8 if i == 6 else i)), k, k + 1, prep)[0]
                    b2_done(w, done, r0, n)
            return
        wb = wblocks("w4", 4)
        lhs = jnp.concatenate([jnp.concatenate([blk(5), blk(6)], axis=1),
                               jnp.concatenate([blk(7), blk(8)], axis=1)], axis=0)
        if marks:
            lo_, hi_ = 0, 52
            never, at = get_never(), {}
            for i, mk in enumerate(marks):
                s_ = lo_ + (hi_ - lo_) * i // len(marks)
                at[4 * (s_ // 16), s_ % 16] = mk
            cols = []
            for kt in range(14):
                col = lhs[:, 128 * kt:128 * (kt + 1)]
                if any(k_[0] == kt for k_ in at):
                    col = jnp.concatenate([jax.lax.select(never, at[kt, r], col[8 * r:8 * r + 8]) if (kt, r) in at
                                           else col[8 * r:8 * r + 8] for r in range(16)], axis=0)
                cols.append(col)
            lhs = jnp.concatenate(cols, axis=1)
        h2 = _dot(_unpack(lhs), _unpack(jnp.concatenate([wb(0, 0), wb(1, 0)], axis=0)))
        finish(w, _unrows2(h2[:n // 2], h2[n // 2:]), r0, n, 4)

    def psum(x, y, sign):
        x, y = _unpack(x).astype(F32), _unpack(y).astype(F32)
        return x + y if sign > 0 else x - y

    def prep_w4(nchunk):
        rows = 384 // nchunk
        marks = []
        for ch in [nchunk] + list(range(nchunk)):
            tail = ch == nchunk
            raw = {}
            for kh in range(2):
                for e in range(1 if tail else 2):
                    r0 = 1536 + FT * kh if tail else 768 * kh + 384 * e + rows * ch
                    x = weights(w4buf, 0, 4, r0, r0 + (FT if tail else rows), raw=True)
                    raw[kh, e] = _unpack(x).astype(F32)
            blk = lambda i, e: raw[i // 2, e][:, 256 * (i % 2):256 * (i % 2 + 1)]
            for k, (ia, ib) in enumerate(_STRASSEN):
                if k not in NEST or ib >= 5:
                    continue
                p_, q_, sg = _SUMS_B[ib]
                half = [blk(p_, e) + blk(q_, e) if sg > 0 else blk(p_, e) - blk(q_, e) for e in range(1 if tail else 2)]
                quad = lambda i: half[i // 2][:, 128 * (i % 2):128 * (i % 2 + 1)]
                first = NEST.index(k)
                if tail:
                    for j in range(2):
                        w4q[first, 7, pl.ds(128 * j, FT), :] = quad(j).astype(BF16)
                        w4q[first, 7, pl.ds(128 * j + FT, 128 - FT), :] = jnp.zeros((128 - FT, 128), BF16)
                    continue
                for jb, v in enumerate(_sums_b(*[quad(i) for i in range(4)]) + [quad(0), quad(3)]):
                    w4q[first, jb, pl.ds(rows * ch, rows), :] = v.astype(BF16)
            if not tail:
                marks.append(w4q.bitcast(U32).at[pl.ds(zsm[32 + ch], NQ)][first, 0, pl.ds(0, 8), :])
        return marks

    def stage_b2n(w, h3, r0, n, k, done, prep=False):
        ia, ib = _STRASSEN[k]
        ka, q, slot = (8 if ia == 6 else ia), n // 8, NEST.index(k)

        def lblk(i, z):
            hv = opaque(h3, z)
            return jnp.concatenate([hv[g + 3 * (i % 2), ka, pl.ds((i // 2) * q, q), :] for g in range(3)], axis=1)

        def raw(j, lo, hi, z=None):
            return wblocks("w4", j, z)(ib - 5, ib - 5)[lo:hi]

        quad = lambda i, z=None: raw(i % 2, 192 * (i // 2), 192 * (i // 2 + 1), z)
        if ib >= 5:
            wt = [raw(j, 384, 448) for j in range(2)]
        else:
            wq = w4q.bitcast(U32)
            wq = wq.at[pl.ds(zsm[6], NQ)] if prep else wq
            wt = [wq[slot, 7, pl.ds(64 * j, 64), :] for j in range(2)]
        tail = _dot(_unpack(opaque(h3, 5)[6, ka, pl.ds(0, 2 * q), :]), _unpack(jnp.concatenate(wt, axis=1)))
        ms = []
        for ja, jb in _STRASSEN:
            if ja >= 5:
                lv = _unpack(lblk(3 * (ja - 5), 5))
            else:
                p_, q_, sg = _SUMS_A[ja]
                lv = psum(lblk(p_, ja), lblk(q_, ja), sg)
            z = zsm[8 + 7 * slot + jb] if prep and ib >= 5 else None
            if ib < 5:
                wv = _unpack(attach(wq[slot, jb]))
            elif jb >= 5:
                wv = _unpack(quad(3 * (jb - 5), z))
            elif prep:
                p_, q_, sg = _SUMS_B[jb]
                wv = psum(quad(p_, z), quad(q_, z), sg)
                keep(w4n.at[slot, pl.ds(jb, 1)], wv)
                wv = wv.astype(BF16)
            else:
                wv = _unpack(attach(w4n.bitcast(U32)[slot, jb]))
            ms.append(_dot(lv, wv))
        c11, c12, c21, c22 = _combine(*ms)
        done[0][k] = jnp.concatenate([c11, c21], axis=0) + tail[:, :128]
        done[1][k] = jnp.concatenate([c12, c22], axis=0) + tail[:, 128:]
        b2_done(w, done, r0, n)

    w = window(0, 2 * TS + LEAD)
    H = TS // 2
    with jax.named_scope("t0a"):
        cps["qa"].wait()
        cps["wmoda"].wait()

        mv = {}

        def mod_fn(j, toks):
            mv[j] = mod_cols(j, 1, toks)[0]
            if len(mv) == 3:
                modbuf[0] = mv[2] * mv[0]
                modbuf[1] = mv[2] * (1.0 + mv[1])

        segment(G5B, 0, MU, mod_fn=mod_fn)
        put(w["h"], pl.ds(0, QA), stage_a0(w, 0, QA))
    with jax.named_scope("t0b"):
        cps["wmodb"].wait()
        sb, cb = mod_cols(3, 2)
        modbuf[3] = 2.0 * sb
        modbuf[4] = 2.0 + 2.0 * cb
        n3 = stage_a1(w, 0, QA, n2=slabs(w["h"], 0, QA))
    XB = TS - XA
    with jax.named_scope("t1a"):
        cps["w1a"].wait()
        cps["qx"].wait()
        put(w["h"], pl.ds(QA, XA), stage_a0(w, QA, XA))
        stage_a2(w, n3, 0, QA, c1=W1A, fine=80)
    with jax.named_scope("t1b"):
        cps["w1b"].wait()
        n3a = stage_a1(w, QA, XA, n2=slabs(w["h"], QA, XA), f32=True)
        stage_a2(w, n3, 0, QA, c0=W1A)
        stage_a2(w, [dd_rest("w1", *_rows2(n3a))], QA, XA, prep=True)
    with jax.named_scope("t2"):
        cps["qb"].wait()
        cps["w2"].wait()
        n3b = stage_a1(w, QA + XA, XB, f32=True)
        stage_b1b(w, stage_b1a(w, 0, TS, prep=True), 0, TS, deep=False)
        stage_a2(w, [dd_rest("w1", *_rows2(n3b))], QA + XA, XB)
        stage_b1b(w, stage_b1a(w, TS, XA), TS, XA)
        stage_b1a(w, TS + XA, XB)
    with jax.named_scope("t3"):
        cps["w3"].wait()
        stage_b1b(w, slabs(w["h"], TS + XA, XB), TS + XA, XB)
        for op in "a0 h a1 a2 a3 a4 a5 H z0 z1 z2".split():
            if op[0] in "hH":
                stage_b2h(w, *((hba, 0) if op == "h" else (hbb, TS)), TS, prep=op == "h")
            elif op[0] == "a":
                stage_b2a(w, hba, 0, TS, int(op[1]), int(op[1]) + 1, prep=True)
            else:
                stage_b2z(w, hbb, int(op[1]), prep=True)
    with jax.named_scope("t4"):
        cps["w4"].wait()
        cps["wmodg"].wait()
        done = {0: {}, 1: {}}
        for op in "m4 P m0 4:0:6:7 m2 8:0 m1 8:1 m3 8:3 4:1:6:7 8:2 8:4 8:5".split():
            op, *rng = op.split(":")
            rng = [int(x) for x in rng]
            if op[0] == "m":
                c = int(op[1])
                modbuf[5, :, pl.ds(c * 128, 128)] = 0.5 * _dot(modbuf[6], weights(wmodbuf, 5 * NC + c, 5 * NC + c + 1))
            elif op[0] == "8":
                stage_b2n(w, hba, 0, TS, *rng, done, prep=True)
            elif op[0] == "P":
                stage_b2b(w, hba, 0, TS, 2, marks=prep_w4(24))
            else:
                stage_b2b(w, hba, 0, TS, *rng, done=done, prep=True)
        out_copy(0, TS).start()
        cps["q1"].wait()

    CBS = (128, 128)
    PART = {"a": (TS, TS), "c": (TS, H), "d": (TS + H, H)}
    BODY = "4:0:6:7 4:1:6:7 4:2 8:1 8:5 r0 r1 1a 8:3 2c 2d Nc nd 8:0 8:4 8:2 z:0 ha z:1 z:2"

    def step(s, carry):
        r0 = pl.multiple_of(s * TS, TS)
        w = window(r0, 2 * TS + LEAD)
        x1, rest, done = {}, {}, {0: {}, 1: {}}
        for op in BODY.split():
            op, *rng = op.split(":")
            rng = [int(x) for x in rng]
            if op[0] == "z":
                stage_b2z(w, hbb, *rng)
            elif op[0] == "N":
                pending.extend(stage_b1b(w, x1[op[1]], *PART[op[1]]))
            elif op[0] == "h":
                stage_b2h(w, hbb, TS, TS)
            elif op[0] == "4":
                stage_b2b(w, hbb, 0, TS, *rng, done=done)
            elif op[0] == "8":
                stage_b2n(w, hbb, 0, TS, *rng, done)
            elif op[0] == "2":
                x1[op[1]] = stage_b1a(w, *PART[op[1]])
            elif op[0] == "n":
                stage_b1b(w, x1[op[1]], *PART[op[1]])
            elif op[0] == "r":
                j = int(op[1])
                rest[j] = dd_rest("w1", *_rows2(stage_a1(w, TS + LEAD + sum(CBS[:j]), CBS[j], f32=True)))
            else:
                ra, n = PART[op[1]]
                parts = [rest[j] for j in range(len(CBS)) if ra - TS <= sum(CBS[:j]) < ra - TS + n]
                stage_a2(w, parts, ra + LEAD, n, last_valid=(s < NT - 2) if ra + n == 2 * TS else None)
        out_copy(r0, TS).start()
        return carry

    with jax.named_scope("p2main"):
        jax.lax.fori_loop(1, NT - 1, step, 0)
    with jax.named_scope("p2epi"):
        w = window(S - 2 * TS, 2 * TS + LEAD)
        rows = pl.ds(S - TS, TS)
        pending.append(hhbuf[0, pl.ds(S, 8), :])

        def flush(rows, cols):
            pltpu.make_async_copy(obuf.at[rows, cols], out_hbm.at[rows, cols], sem_out.at[0]).start()

        done = {0: {}, 1: {}}
        for op in "p0 1 3 2 4 0 5 p1".split():
            if op[0] == "p":
                stage_b2b(w, hbb, TS, TS, int(op[1]), done=done)
            else:
                stage_b2n(w, hbb, TS, TS, int(op), done)
        flush(rows, pl.ds(0, 512))
        sub = 0
        for n in (128, 64, 64):
            stage_b2b(w, hbb, TS, n, 2, sub=sub)
            flush(pl.ds(S - TS + sub, n), pl.ds(512, 128))
            sub += n
        pltpu.make_async_copy(obuf, out_hbm, sem_out.at[0]).wait()


@jax.jit
def pallas_adaLN_cond__ssm_conv_h3__mixer_s_mlp__prompt_kernel(
    A_q: jax.Array,
    A_k: jax.Array,
    A_v: jax.Array,
    A_shift_k: jax.Array,
    A_ssm_k: jax.Array,
    A_ssm_D: jax.Array,
    B_x: jax.Array,
    B_w1: jax.Array,
    B_w2: jax.Array,
    B_w3: jax.Array,
    B_w4: jax.Array,
    c: jax.Array,
    w_mod: jax.Array,
):
    del B_x

    def tiles(x):
        return x.reshape(S // 8, 8, NC, 128).transpose(0, 2, 1, 3).reshape(S * NC, 128)

    def pairs(x):
        r, n = x.shape
        return x.reshape(r // 16, 2, 8, n // 128, 128).transpose(0, 1, 3, 2, 4)

    args = (
        A_q.reshape(S, D), tiles(A_k), tiles(A_v),
        A_shift_k.T, A_ssm_k, A_ssm_D.reshape(NC, 128),
        pairs(B_w1), pairs(B_w2), pairs(B_w3.T), pairs(B_w4), c, pairs(w_mod),
    )
    scratch = [
        pltpu.VMEM((NA, P * NC + 128, 128), BF16),
        pltpu.VMEM((NA, P * NC + 64, 128), BF16),
        pltpu.VMEM((D, S), BF16),
        pltpu.VMEM((R, 256, 128), BF16),
        pltpu.VMEM((2, R, 128, 128), BF16),
        pltpu.VMEM((128, 128), BF16),
        pltpu.VMEM((D // 16, 6 * NC, 16, 128), BF16),
        pltpu.VMEM((D // 16, NC, 16, 128), BF16),
        pltpu.VMEM((D // 16, NC, 16, 128), BF16),
        pltpu.VMEM((FF // 16, NC, 16, 128), BF16),
        pltpu.VMEM((FF // 16, NC, 16, 128), BF16),
        pltpu.VMEM((S + 64, D), BF16),
        *[pltpu.VMEM((NA, R, 16, 4, 8, 128), F32) for _ in range(NC)],
        pltpu.VMEM((NC, 2, R, 16, 2, 8, 128), F32),
        pltpu.VMEM((2 * NC, R, 256, 128), BF16),
        pltpu.VMEM((32, 128), U32),
        pltpu.VMEM((NC, 8, 8, 128), F32),
        pltpu.VMEM((NC, S + 32, 128), F32),
        pltpu.VMEM((8, 8, D), F32),
        pltpu.VMEM((S + 32, D), F32),
        pltpu.VMEM((NC, S + 32, 128), F32),
        pltpu.VMEM((NC, S + 32, 128), F32),
        pltpu.VMEM((8, 2, TS + 16, 128), BF16),
        pltpu.VMEM((5, 2, 1, 256, 128), BF16),
        pltpu.VMEM((5, 2, 1, 256, 128), BF16),
        pltpu.VMEM((5, 6, 2, 128, 128), BF16),
        pltpu.VMEM((5, 2, 2, FT, 128), BF16),
        pltpu.VMEM((5, 2, 1, 896, 128), BF16),
        pltpu.VMEM((8, 9, 144, 128), BF16),
        pltpu.VMEM((8, 9, 144, 128), BF16),
        pltpu.VMEM((2, 8, 384, 128), BF16),
        pltpu.VMEM((NQ, 8, 384, 128), BF16),
        pltpu.VMEM((3, len(N3), 5, 128, 128), BF16),
        pltpu.VMEM((8, 5, 80, 128), BF16),
        pltpu.VMEM((S, D), BF16),
        pltpu.VMEM((4, D), BF16),
        pltpu.VMEM((NC, 128), BF16),
        pltpu.VMEM((1, D), BF16),
        pltpu.SMEM((64,), jnp.int32),
        pltpu.SemaphoreType.DMA((40,)),
        pltpu.SemaphoreType.DMA((1,)),
    ]
    out = pl.pallas_call(
        _kernel,
        out_shape=jax.ShapeDtypeStruct((S, D), BF16),
        in_specs=[pl.BlockSpec(memory_space=pl.ANY)] * len(args),
        out_specs=pl.BlockSpec(memory_space=pl.ANY),
        scratch_shapes=scratch,
        grid=(1,),
        compiler_params=pltpu.CompilerParams(vmem_limit_bytes=108 * 1024 * 1024, disable_semaphore_checks=True,
                                             disable_bounds_checks=True),
        name="adaln_h3_mixer",
    )(*args)
    return out.reshape(1, S, D)
```
